```python
import jax
import jax.numpy as jnp

def _softmax(x, axis=-1):
    return jax.nn.softmax(x, axis=axis)

def _gelu(x):
    return jax.nn.gelu(x, approximate=True)

def _silu(x):
    return jax.nn.silu(x)

def _sigmoid(x):
    return jax.nn.sigmoid(x)

def _layernorm(x, axis=-1, eps=1e-05):
    m = jnp.mean(x, axis=axis, keepdims=True)
    v = jnp.var(x, axis=axis, keepdims=True)
    return (x - m) / jnp.sqrt(v + eps)

def _scatter_add(tgt, idx, src, axis=0):
    return tgt.at[idx].add(src)

def _segment_sum(src, seg, n):
    return jax.ops.segment_sum(src, seg, n)

class _Rng:

    def __init__(self, key):
        self._k = key

    def _next(self):
        self._k, sub = jax.random.split(self._k)
        return sub

    def normal(self, shape):
        return jax.random.normal(self._next(), shape, dtype=jnp.bfloat16)

    def randint(self, lo, hi, shape):
        return jax.random.randint(self._next(), shape, lo, hi, dtype=jnp.int32)

    def uniform(self, shape, lo=0.0, hi=1.0):
        return jax.random.uniform(self._next(), shape, jnp.bfloat16, lo, hi)

    def permutation(self, n):
        return jax.random.permutation(self._next(), n)
kernel_name = 'adaLN_cond__mha_block_cached__moe_arch_mod__prompt'

def setup_inputs():
    _rng = _Rng(jax.random.key(int.from_bytes(__import__("os").urandom(4), "little")))
    _w = lambda a: (lambda t: t.astype(jnp.bfloat16) if jnp.issubdtype(t.dtype, jnp.floating) else t)(jnp.asarray(a))

    def _A_setup():
        B, Sq, D = (1, 2048, 1024)
        H, Sk, Dh = (32, 2048, 128)
        return {'x': _w((lambda *s: _rng.normal(s) * 0.05)(B, Sq, D)), 'k_cache': _w((lambda *s: _rng.normal(s) * 0.05)(B, H, Sk, Dh)), 'v_cache': _w((lambda *s: _rng.normal(s) * 0.05)(B, H, Sk, Dh)), 'wq': _w((lambda *s: _rng.normal(s) * 0.05)(D, H * Dh) * D ** (-0.5)), 'wo': _w((lambda *s: _rng.normal(s) * 0.05)(H * Dh, D) * (H * Dh) ** (-0.5))}
    _A_in = _A_setup()

    def _B_setup():
        B, S, D, F, C = (1, 2048, 1024, 3584, 2)
        return {'x': _w((lambda *s: _rng.normal(s) * 0.05)(B, S, D)), 'w_r': _w((lambda *s: _rng.normal(s) * 0.05)(D)), 'w_gate': _w((lambda *s: _rng.normal(s) * 0.05)(D, F)), 'w_up': _w((lambda *s: _rng.normal(s) * 0.05)(D, F)), 'w_down': _w((lambda *s: _rng.normal(s) * 0.05)(F, D))}
    _B_in = _B_setup()
    return {'A_x': _A_in['x'], 'A_k_cache': _A_in['k_cache'], 'A_v_cache': _A_in['v_cache'], 'A_wq': _A_in['wq'], 'A_wo': _A_in['wo'], 'B_x': _B_in['x'], 'B_w_r': _B_in['w_r'], 'B_w_gate': _B_in['w_gate'], 'B_w_up': _B_in['w_up'], 'B_w_down': _B_in['w_down'], 'c': _w((lambda *s: _rng.normal(s) * 0.05)(1, 1024)), 'w_mod': _w((lambda *s: _rng.normal(s) * 0.05)(1024, 6 * 1024) * 1024 ** (-0.5))}

def reference(A_x, A_k_cache, A_v_cache, A_wq, A_wo, B_x, B_w_r, B_w_gate, B_w_up, B_w_down, c, w_mod):

    def _A_ref(x, k_cache, v_cache, wq, wo):
        B, Sq, D = x.shape
        H, Dh = (32, 128)
        q = (lambda x, *d: x.transpose(*d))((x @ wq).reshape(B, Sq, H, Dh), 0, 2, 1, 3)
        scores = jnp.einsum('bhqd,bhkd->bhqk', q, k_cache) * Dh ** (-0.5)
        p = _softmax(scores, axis=-1)
        o = jnp.einsum('bhqk,bhkd->bhqd', p, v_cache)
        return (lambda x, *d: x.transpose(*d))(o, 0, 2, 1, 3).reshape(B, Sq, H * Dh) @ wo

    def _B_ref(x, w_r, w_gate, w_up, w_down):
        B, S, D = x.shape
        C = 2
        r = x @ w_r
        idx = jnp.argsort(-r, axis=-1)[:, :C]
        idx_e = jnp.repeat(idx.reshape(B, C, 1), D, axis=2)
        x_sel = jnp.take_along_axis(x, idx_e, axis=1)
        g = _silu(x_sel @ w_gate)
        u = x_sel @ w_up
        y = g * u @ w_down
        r_sel = _sigmoid(jnp.take_along_axis(r, idx, axis=1))
        y = y * r_sel.reshape(B, C, 1)
        b_off = (jnp.arange(B) * S).reshape(B, 1)
        flat_idx = (idx + b_off).reshape(B * C)
        zero = (x * 0.0).reshape(B * S, D)
        upd = _scatter_add(zero, flat_idx, y.reshape(B * C, D), axis=0)
        return x + upd.reshape(B, S, D)
    x = A_x
    mod = (_silu(c) @ w_mod).reshape(c.shape[0], 6, 1, -1)
    sa, ca, ga, sb, cb, gb = (mod[:, 0].copy(), mod[:, 1].copy(), mod[:, 2].copy(), mod[:, 3].copy(), mod[:, 4].copy(), mod[:, 5].copy())
    h = _layernorm(x, axis=-1) * (1 + ca) + sa
    x = x + ga * _A_ref(h, A_k_cache, A_v_cache, A_wq, A_wo)
    h = _layernorm(x, axis=-1) * (1 + cb) + sb
    x = x + gb * _B_ref(h, B_w_r, B_w_gate, B_w_up, B_w_down)
    return x
```

```python
import jax
import jax.numpy as jnp
from jax import lax
import jax.experimental.pallas as pl
import jax.experimental.pallas.tpu as pltpu

F32 = jnp.float32
BF16 = jnp.bfloat16

S = 2048
DM = 1024
H = 32
DH = 128
FF = 3584
BQ = 512
TQ = 256
NH = 4
NQ = S // BQ
NG = H // NH
NSTEP = NQ * NG
LNR = BQ // NG
KG = 512
EPS = 1e-5
QSCALE = DH ** -0.5 * 1.4426950408889634
NT = (((1,), (1,)), ((), ()))
FIX = 16

SEM_C, SEM_WR, SEM_X0, SEM_X1, SEM_X2, SEM_X3 = 0, 1, 2, 3, 4, 5
SEM_MOD0 = 6
SEM_MODR = SEM_MOD0 + 4
SEM_H0 = SEM_MODR + 1
SEM_WO0 = SEM_H0 + 3 * NH
SEM_G = SEM_WO0 + 1
SEM_FFN = SEM_G + 4 * (NG - 1)
SEM_OUT = SEM_FFN + 3
SEM_FIX = SEM_OUT + NQ
NSEM = SEM_FIX + 2


def _rows8(v, rows):
    return jnp.tile(v, (rows // 8, 1))


def _normalize(x):
    mean = jnp.sum(x, axis=-1, keepdims=True) * (1.0 / DM)
    xc = x - mean
    var = jnp.sum(xc * xc, axis=-1, keepdims=True) * (1.0 / DM)
    return xc * lax.rsqrt(var + EPS)


def _kernel(x_hbm, k_hbm, v_hbm, wq_hbm, wo_hbm, wr_hbm, wg_hbm, wu_hbm, wd_hbm, c_hbm, wm_hbm,
            out_hbm,
            xbuf, kbuf, vbuf, wqbuf, wobuf, wrbuf, wgbuf, wubuf, wdbuf, cbuf, wmbuf,
            hn, acc, h2buf, obuf, mod, wr32, top, sem):
    cp = pltpu.make_async_copy

    c_cp = cp(c_hbm, cbuf, sem.at[SEM_C])
    wr_cp = cp(wr_hbm, wrbuf, sem.at[SEM_WR])
    x_rng = ((0, TQ), (TQ, BQ), (BQ, 2 * BQ), (2 * BQ, S))
    x_cp = [cp(x_hbm.at[a:b], xbuf.at[a:b], sem.at[SEM_X0 + n]) for n, (a, b) in enumerate(x_rng)]
    mod_cp = [cp(wm_hbm.at[:, n * 512:(n + 1) * 512], wmbuf.at[:, n * 512:(n + 1) * 512],
                 sem.at[SEM_MOD0 + n]) for n in range(4)]
    modr_cp = cp(wm_hbm.at[:, 2 * DM:], wmbuf.at[:, 2 * DM:], sem.at[SEM_MODR])
    wq0_cp = [cp(wq_hbm.at[:, h * DH:(h + 1) * DH], wqbuf.at[0, :, h * DH:(h + 1) * DH],
                 sem.at[SEM_H0 + 3 * h]) for h in range(NH)]
    k0_cp = [cp(k_hbm.at[h], kbuf.at[h], sem.at[SEM_H0 + 3 * h + 1]) for h in range(NH)]
    v0_cp = [cp(v_hbm.at[h], vbuf.at[h], sem.at[SEM_H0 + 3 * h + 2]) for h in range(NH)]
    wo0_cp = cp(wo_hbm.at[0], wobuf.at[0], sem.at[SEM_WO0])

    def group_cps(g):
        s0 = SEM_G + 4 * (g - 1)
        if isinstance(g, int):
            cols = slice(g * NH * DH, (g + 1) * NH * DH)
        else:
            cols = pl.ds(pl.multiple_of(g * (NH * DH), NH * DH), NH * DH)
        heads = pl.ds(g * NH, NH)
        return [cp(wq_hbm.at[:, cols], wqbuf.at[g], sem.at[s0]),
                cp(k_hbm.at[heads], kbuf.at[heads], sem.at[s0 + 1]),
                cp(v_hbm.at[heads], vbuf.at[heads], sem.at[s0 + 2]),
                cp(wo_hbm.at[g], wobuf.at[g], sem.at[s0 + 3])]

    ffn_cp = [cp(wg_hbm, wgbuf, sem.at[SEM_FFN]), cp(wu_hbm, wubuf, sem.at[SEM_FFN + 1]),
              cp(wd_hbm, wdbuf, sem.at[SEM_FFN + 2])]

    def out_cp(j):
        if isinstance(j, int):
            rows = slice(j * BQ, (j + 1) * BQ)
        else:
            rows = pl.ds(pl.multiple_of(j * BQ, BQ), BQ)
        return cp(obuf.at[rows], out_hbm.at[rows], sem.at[SEM_OUT + j])

    c_cp.start()
    x_cp[0].start()
    for d in mod_cp:
        d.start()
    wq0_cp[0].start()
    k0_cp[0].start()
    x_cp[1].start()
    v0_cp[0].start()
    for h in range(1, NH):
        wq0_cp[h].start()
        k0_cp[h].start()
        v0_cp[h].start()
    wo0_cp.start()
    x_cp[2].start()
    wr_cp.start()
    for g in range(1, NG):
        for d in group_cps(g):
            d.start()
    modr_cp.start()
    x_cp[3].start()
    for d in ffn_cp:
        d.start()

    acc[1] = jnp.zeros((BQ, DM), F32)
    mod[:, 2 * DM:] = jnp.zeros((8, 4 * DM), F32)
    top[0] = jnp.full((8, 128), -jnp.inf, F32)
    top[1] = jnp.zeros((8, 128), F32)
    top[2] = jnp.full((8, 128), -jnp.inf, F32)
    top[3] = jnp.zeros((8, 128), F32)

    def silu_c():
        cf = cbuf[...].astype(F32)
        sc = cf * jax.nn.sigmoid(cf)
        return jnp.broadcast_to(sc, (16, DM)).astype(BF16)

    def mod_cols(sc, lo, hi):
        mod[:, lo:hi] = jnp.dot(sc, wmbuf[:, lo:hi], preferred_element_type=F32)[:8]

    def ln1_apply(n, rows):
        return (n * (1.0 + _rows8(mod[:, DM:2 * DM], rows)) + _rows8(mod[:, 0:DM], rows)).astype(BF16)

    def ln2(a, row0, rows, valid):
        rs = pl.ds(row0, rows)
        x1 = xbuf[rs, :].astype(F32) + _rows8(mod[:, 2 * DM:3 * DM], rows) * a
        h2 = (_normalize(x1) * (1.0 + _rows8(mod[:, 4 * DM:5 * DM], rows))
              + _rows8(mod[:, 3 * DM:4 * DM], rows))
        h2buf[rs, :] = h2
        obuf[rs, :] = (x1 + _rows8(mod[:, 5 * DM:6 * DM], rows) * h2).astype(BF16)
        r = jnp.sum(h2 * _rows8(wr32[...], rows), axis=-1, keepdims=True)
        r = jnp.broadcast_to(r, (rows, 128))
        if valid is not None:
            r = jnp.where(valid, r, -jnp.inf)
        m1, i1, m2, i2 = top[0], top[1], top[2], top[3]
        base = (lax.broadcasted_iota(jnp.int32, (8, 128), 0) + row0).astype(F32)
        for u in range(rows // 8):
            ru = r[u * 8:(u + 1) * 8]
            iu = base + float(u * 8)
            gt1 = ru > m1
            gt2 = ru > m2
            m2 = jnp.where(gt1, m1, jnp.where(gt2, ru, m2))
            i2 = jnp.where(gt1, i1, jnp.where(gt2, iu, i2))
            m1 = jnp.where(gt1, ru, m1)
            i1 = jnp.where(gt1, iu, i1)
        top[0], top[1], top[2], top[3] = m1, i1, m2, i2

    def qproj(i, g, c, h):
        q = jnp.dot(hn[i, c * TQ:(c + 1) * TQ, :], wqbuf[g, :, h * DH:(h + 1) * DH],
                    preferred_element_type=F32)
        return (q * QSCALE).astype(BF16)

    def qk(q, g, h):
        return lax.dot_general(q, kbuf[g * NH + h], NT, preferred_element_type=F32)

    def pv(s, g, h):
        m = jnp.max(s, axis=-1, keepdims=True)
        lsum = None
        parts = []
        for j in range(S // KG):
            ps = [jnp.exp2(s[:, j * KG + u * 128:j * KG + (u + 1) * 128] - m) for u in range(KG // 128)]
            t = (ps[0] + ps[1]) + (ps[2] + ps[3])
            lsum = t if lsum is None else lsum + t
            ps[-1] = jnp.minimum(ps[-1], lsum)
            parts += ps
        p = jnp.concatenate(parts, axis=-1).astype(BF16)
        return jnp.dot(p, vbuf[g * NH + h], preferred_element_type=F32), lsum

    def normcat(res):
        gate = jnp.minimum(res[-1][0], 0.0)
        outs = []
        for o, lsum in res:
            l = jnp.sum(jnp.maximum(lsum, gate), axis=-1, keepdims=True)
            r = pl.reciprocal(l, approx=True)
            r = r * (2.0 - l * r)
            outs.append(o * r)
        return jnp.concatenate(outs, axis=-1).astype(BF16)

    def woproj(slot, g, first, c, oc, lo, hi):
        y = jnp.dot(oc, wobuf[g, :, lo:hi], preferred_element_type=F32)
        rows = slice(c * TQ, (c + 1) * TQ)
        if first is True:
            acc[slot, rows, lo:hi] = y
        elif first is False:
            acc[slot, rows, lo:hi] = acc[slot, rows, lo:hi] + y
        else:
            acc[slot, rows, lo:hi] = jnp.where(first, 0.0, acc[slot, rows, lo:hi]) + y

    def ln1_chunk(i, g):
        row0 = jnp.minimum((i + 1) * BQ + g * LNR, S - LNR)
        row0 = pl.multiple_of(row0, LNR)
        n = _normalize(xbuf[pl.ds(row0, LNR), :].astype(F32))
        hn[i + 1, pl.ds(pl.multiple_of(g * LNR, LNR), LNR), :] = ln1_apply(n, LNR)

    def ln2_chunk(i, g):
        row0 = pl.multiple_of(jnp.maximum(i - 1, 0) * BQ + g * LNR, LNR)
        a = acc[(i + 1) % 2, pl.ds(pl.multiple_of(g * LNR, LNR), LNR), :]
        ln2(a, row0, LNR, i > 0)

    WA, WB = 256, 512

    def attention_step(i, g, slot, first):
        chains = [(c, h) for c in range(2) for h in range(NH)]
        q = qproj(i, g, 0, 0)
        res = ([], [])
        o0 = None
        for n, (c, h) in enumerate(chains):
            s = qk(q, g, h)
            if n + 1 < len(chains):
                q = qproj(i, g, *chains[n + 1])
            if (c, h) == (1, 0):
                o0 = normcat(res[0])
                woproj(slot, g, first, 0, o0, 0, WA)
            if (c, h) == (1, NH - 1):
                woproj(slot, g, first, 0, o0, WA, WB)
            res[c].append(pv(s, g, h))
        o1 = normcat(res[1])
        woproj(slot, g, first, 0, o0, WB, DM)
        woproj(slot, g, first, 1, o1, 0, DM)

    c_cp.wait()
    x_cp[0].wait()
    sc = silu_c()
    n0 = _normalize(xbuf[0:TQ, :].astype(F32))
    acc[0, 0:TQ, :] = n0
    for n in range(4):
        mod_cp[n].wait()
        mod_cols(sc, n * 512, (n + 1) * 512)
    hn[0, 0:TQ, :] = ln1_apply(acc[0, 0:TQ, :], TQ)

    wq0_cp[0].wait()
    k0_cp[0].wait()
    x_cp[1].wait()
    v0_cp[0].wait()
    hn[0, TQ:BQ, :] = ln1_apply(_normalize(xbuf[TQ:BQ, :].astype(F32)), TQ)
    chains0 = [(c, h) for h in range(NH) for c in range(2)]
    q = qproj(0, 0, 0, 0)
    res = ([], [])
    o0 = None
    for n, (c, h) in enumerate(chains0):
        s = qk(q, 0, h)
        if n + 1 < len(chains0):
            c2, h2_ = chains0[n + 1]
            if c2 == 0:
                wq0_cp[h2_].wait()
                k0_cp[h2_].wait()
                v0_cp[h2_].wait()
                if h2_ == NH - 1:
                    wo0_cp.wait()
                    x_cp[2].wait()
                    wr_cp.wait()
            q = qproj(0, 0, c2, h2_)
        else:
            o0 = normcat(res[0])
            woproj(0, 0, True, 0, o0, 0, WB)
        res[c].append(pv(s, 0, h))
    o1 = normcat(res[1])
    woproj(0, 0, True, 0, o0, WB, DM)
    woproj(0, 0, True, 1, o1, 0, DM)
    hn[1, 0:LNR, :] = ln1_apply(_normalize(xbuf[BQ:BQ + LNR, :].astype(F32)), LNR)
    wr32[...] = jnp.broadcast_to(wrbuf[...].astype(F32).reshape(1, DM), (8, DM))

    def step(t, carry):
        i = t // NG
        g = t % NG

        @pl.when(t < NG)
        def _():
            for d in group_cps(g):
                d.wait()

        @pl.when(t == NG)
        def _():
            modr_cp.wait()
            x_cp[3].wait()
            mod_cols(silu_c(), 2 * DM, 6 * DM)

        @pl.when(jnp.logical_and(g == 0, i >= 2))
        def _():
            out_cp(i - 2).start()

        ln2_chunk(i, g)
        attention_step(i, g, i % 2, g == 0)
        ln1_chunk(i, g)
        return carry

    lax.fori_loop(1, NSTEP, step, 0)

    out_cp(NQ - 2).start()
    last = (NQ - 1) % 2
    for u in range(BQ // LNR):
        ln2(acc[last, u * LNR:(u + 1) * LNR, :], (NQ - 1) * BQ + u * LNR, LNR, None)
    out_cp(NQ - 1).start()

    m1, i1, m2, i2 = top[0], top[1], top[2], top[3]
    big = float(S)
    v1 = jnp.max(m1, axis=0, keepdims=True)
    j1 = jnp.min(jnp.where(m1 == v1, i1, big), axis=0, keepdims=True)
    taken = i1 == j1
    m1b = jnp.where(taken, m2, m1)
    i1b = jnp.where(taken, i2, i1)
    v2 = jnp.max(m1b, axis=0, keepdims=True)
    j2 = jnp.min(jnp.where(m1b == v2, i1b, big), axis=0, keepdims=True)
    idx1 = jnp.clip(j1[0, 0].astype(jnp.int32), 0, S - 1)
    idx2 = jnp.clip(j2[0, 0].astype(jnp.int32), 0, S - 1)

    for d in ffn_cp:
        d.wait()
    row = lax.broadcasted_iota(jnp.int32, (16, DM), 0)
    xs = jnp.where(row == 0, h2buf[pl.ds(idx1, 1), :], h2buf[pl.ds(idx2, 1), :]).astype(BF16)
    gt = jnp.dot(xs, wgbuf[...], preferred_element_type=F32)
    up = jnp.dot(xs, wubuf[...], preferred_element_type=F32)
    act = (gt * jax.nn.sigmoid(gt) * up).astype(BF16)
    y = jnp.dot(act, wdbuf[...], preferred_element_type=F32)
    gb = mod[0:1, 5 * DM:6 * DM]
    y1 = y[0:1, :] * jax.nn.sigmoid(v1[:, 0:1]) * gb
    y2 = y[1:2, :] * jax.nn.sigmoid(v2[:, 0:1]) * gb

    for j in range(NQ):
        out_cp(j).wait()

    base1 = pl.multiple_of((idx1 // FIX) * FIX, FIX)
    base2 = pl.multiple_of((idx2 // FIX) * FIX, FIX)

    def fix(base, idx, yy):
        rs = pl.ds(base, FIX)
        upd = jnp.where(row + base == idx, yy, 0.0)
        obuf[rs, :] = (obuf[rs, :].astype(F32) + upd).astype(BF16)

    fix(base1, idx1, y1)
    fix(base2, idx2, y2)
    fix1 = cp(obuf.at[pl.ds(base1, FIX)], out_hbm.at[pl.ds(base1, FIX)], sem.at[SEM_FIX])
    fix2 = cp(obuf.at[pl.ds(base2, FIX)], out_hbm.at[pl.ds(base2, FIX)], sem.at[SEM_FIX + 1])
    fix1.start()

    @pl.when(base1 != base2)
    def _():
        fix2.start()
        fix2.wait()

    fix1.wait()


@jax.jit
def pallas_adaLN_cond__mha_block_cached__moe_arch_mod__prompt_kernel(
    A_x: jax.Array,
    A_k_cache: jax.Array,
    A_v_cache: jax.Array,
    A_wq: jax.Array,
    A_wo: jax.Array,
    B_x: jax.Array,
    B_w_r: jax.Array,
    B_w_gate: jax.Array,
    B_w_up: jax.Array,
    B_w_down: jax.Array,
    c: jax.Array,
    w_mod: jax.Array,
):
    del B_x
    x = A_x.reshape(S, DM)
    k = A_k_cache.reshape(H, S, DH)
    v = A_v_cache.reshape(H, S, DH)
    wo = A_wo.reshape(NG, NH * DH, DM)
    any_spec = pl.BlockSpec(memory_space=pl.ANY)
    out = pl.pallas_call(
        _kernel,
        in_specs=[any_spec] * 11,
        out_specs=any_spec,
        out_shape=jax.ShapeDtypeStruct((S, DM), BF16),
        scratch_shapes=[
            pltpu.VMEM((S, DM), BF16),
            pltpu.VMEM((H, S, DH), BF16),
            pltpu.VMEM((H, S, DH), BF16),
            pltpu.VMEM((NG, DM, NH * DH), BF16),
            pltpu.VMEM((NG, NH * DH, DM), BF16),
            pltpu.VMEM((DM,), BF16),
            pltpu.VMEM((DM, FF), BF16),
            pltpu.VMEM((DM, FF), BF16),
            pltpu.VMEM((FF, DM), BF16),
            pltpu.VMEM((1, DM), BF16),
            pltpu.VMEM((DM, 6 * DM), BF16),
            pltpu.VMEM((NQ + 1, BQ, DM), BF16),
            pltpu.VMEM((2, BQ, DM), F32),
            pltpu.VMEM((S, DM), F32),
            pltpu.VMEM((S, DM), BF16),
            pltpu.VMEM((8, 6 * DM), F32),
            pltpu.VMEM((8, DM), F32),
            pltpu.VMEM((4, 8, 128), F32),
            pltpu.SemaphoreType.DMA((NSEM,)),
        ],
        compiler_params=pltpu.CompilerParams(vmem_limit_bytes=124 * 1024 * 1024),
        name="adaln_mha_moe",
    )(x, k, v, A_wq, wo, B_w_r, B_w_gate, B_w_up, B_w_down, c, w_mod)
    return out.reshape(1, S, DM)
```

```python
import jax
import jax.numpy as jnp
from jax import lax
import jax.experimental.pallas as pl
import jax.experimental.pallas.tpu as pltpu

F32 = jnp.float32
BF16 = jnp.bfloat16

S = 2048
DM = 1024
H = 32
DH = 128
FF = 3584
BQ = 512
TQ = 256
NH = 4
NQ = S // BQ
NG = H // NH
NSTEP = NQ * NG
LNR = BQ // NG
NP2 = 4
KG = 512
EPS = 1e-5
QSCALE = DH ** -0.5 * 1.4426950408889634
NT = (((1,), (1,)), ((), ()))
FIX = 16
PAD = 128

SEM_CX = 0
SEM_MOD0 = 1
SEM_A = SEM_MOD0 + 4
SEM_H0 = SEM_A + 3
SEM_G = SEM_H0 + NH - 1
SEM_MODR = SEM_G + NG - 1
SEM_FFN = SEM_MODR + 1
SEM_OUT = SEM_FFN + 1
SEM_FIX = SEM_OUT + 1
NSEM = SEM_FIX + 1


def _rows8(v, rows):
    return jnp.tile(v, (rows // 8, 1))


def _normalize(x):
    mean = jnp.sum(x, axis=-1, keepdims=True) * (1.0 / DM)
    xc = x - mean
    var = jnp.sum(xc * xc, axis=-1, keepdims=True) * (1.0 / DM)
    return xc * lax.rsqrt(var + EPS)


def _kernel(x_hbm, k_hbm, v_hbm, wq_hbm, wo_hbm, wr_hbm, wg_hbm, wu_hbm, wd_hbm, c_hbm, wm_hbm,
            out_hbm,
            xbuf, kbuf, vbuf, wqbuf, wobuf, wrbuf, wgbuf, wubuf, wdbuf, cbuf, wmbuf,
            hn, acc, h2buf, obuf, mod, wr32, top, flag, sem):
    cp = pltpu.make_async_copy

    sem_last = SEM_H0 + NH - 2
    c_cp = cp(c_hbm, cbuf, sem.at[SEM_CX])
    wr_cp = cp(wr_hbm, wrbuf, sem.at[sem_last])
    x_rng = ((0, BQ, SEM_CX), (BQ, 2 * BQ, sem_last), (2 * BQ, S, SEM_MODR))
    x_cp = [cp(x_hbm.at[a:b], xbuf.at[a:b], sem.at[n]) for a, b, n in x_rng]
    mod_cp = [cp(wm_hbm.at[:, n * 512:(n + 1) * 512], wmbuf.at[:, n * 512:(n + 1) * 512],
                 sem.at[SEM_MOD0 + n]) for n in range(4)]
    modr_cp = cp(wm_hbm.at[:, 2 * DM:], wmbuf.at[:, 2 * DM:6 * DM], sem.at[SEM_MODR])

    def head0_cps(h):
        sq, sk, sv = (SEM_A, SEM_A + 1, SEM_A + 2) if h == 0 else (SEM_H0 + h - 1,) * 3
        return [cp(wq_hbm.at[:, h * DH:(h + 1) * DH], wqbuf.at[0, :, h * DH:(h + 1) * DH], sem.at[sq]),
                cp(k_hbm.at[h], kbuf.at[h], sem.at[sk]),
                cp(v_hbm.at[h], vbuf.at[h], sem.at[sv])]

    wo0_cp = cp(wo_hbm.at[0], wobuf.at[0], sem.at[sem_last])

    def group_cps(g):
        sg = sem.at[SEM_G + g - 1]
        if isinstance(g, int):
            cols = slice(g * NH * DH, (g + 1) * NH * DH)
        else:
            cols = pl.ds(pl.multiple_of(g * (NH * DH), NH * DH), NH * DH)
        heads = pl.ds(g * NH, NH)
        return [cp(wq_hbm.at[:, cols], wqbuf.at[g], sg),
                cp(k_hbm.at[heads], kbuf.at[heads], sg),
                cp(v_hbm.at[heads], vbuf.at[heads], sg),
                cp(wo_hbm.at[g], wobuf.at[g], sg)]

    ffn_cp = [cp(wg_hbm, wgbuf, sem.at[SEM_FFN]), cp(wu_hbm, wubuf, sem.at[SEM_FFN]),
              cp(wd_hbm, wdbuf.at[:, 0:DM], sem.at[SEM_FFN])]

    def out_cp(j):
        if isinstance(j, int):
            rows = slice(j * BQ, (j + 1) * BQ)
        else:
            rows = pl.ds(pl.multiple_of(j * BQ, BQ), BQ)
        return cp(obuf.at[rows], out_hbm.at[rows], sem.at[SEM_OUT])

    c_cp.start()
    x_cp[0].start()
    for d in mod_cp:
        d.start()
    for h in range(NH):
        for d in head0_cps(h):
            d.start()
    wo0_cp.start()
    x_cp[1].start()
    wr_cp.start()
    for g in range(1, NG):
        for d in group_cps(g):
            d.start()
    modr_cp.start()
    x_cp[2].start()
    for d in ffn_cp:
        d.start()

    flag[0] = 0
    acc[1, :, 0:DM] = jnp.zeros((BQ, DM), F32)
    mod[:, 2 * DM:] = jnp.zeros((8, 4 * DM), F32)
    top[0] = jnp.full((8, 128), -jnp.inf, F32)
    top[1] = jnp.zeros((8, 128), F32)
    top[2] = jnp.full((8, 128), -jnp.inf, F32)
    top[3] = jnp.zeros((8, 128), F32)

    def silu_c():
        cf = cbuf[...].astype(F32)
        sc = cf * jax.nn.sigmoid(cf)
        return jnp.broadcast_to(sc, (16, DM)).astype(BF16)

    def mod_cols(sc, lo, hi):
        mod[:, lo:hi] = jnp.dot(sc, wmbuf[:, lo:hi], preferred_element_type=F32)[:8]

    def tie(val, dep):
        if dep is None:
            return val
        n = dep.shape[0]
        head = jnp.where(flag[0] != 0, dep, val[:n])
        return head if n == val.shape[0] else jnp.concatenate([head, val[n:]], axis=0)

    def ln1_apply(n, rows):
        return n * (1.0 + _rows8(mod[:, DM:2 * DM], rows)) + _rows8(mod[:, 0:DM], rows)

    def load_top():
        return top[0], top[1], top[2], top[3]

    def store_top(st):
        top[0], top[1], top[2], top[3] = st

    def ln2(a, row0, rows, valid, st):
        rs = pl.ds(row0, rows)
        x1 = xbuf[rs, :].astype(F32) + _rows8(mod[:, 2 * DM:3 * DM], rows) * a
        h2 = (_normalize(x1) * (1.0 + _rows8(mod[:, 4 * DM:5 * DM], rows))
              + _rows8(mod[:, 3 * DM:4 * DM], rows))
        h2buf[rs, :] = h2
        obuf[rs, :] = (x1 + _rows8(mod[:, 5 * DM:6 * DM], rows) * h2).astype(BF16)
        r = jnp.sum(h2 * _rows8(wr32[...], rows), axis=-1, keepdims=True)
        r = jnp.broadcast_to(r, (rows, 128))
        if valid is not None:
            r = jnp.where(valid, r, -jnp.inf)
        m1, i1, m2, i2 = st
        base = (lax.broadcasted_iota(jnp.int32, (8, 128), 0) + row0).astype(F32)
        for u in range(rows // 8):
            ru = r[u * 8:(u + 1) * 8]
            iu = base + float(u * 8)
            gt1 = ru > m1
            gt2 = ru > m2
            m2 = jnp.where(gt1, m1, jnp.where(gt2, ru, m2))
            i2 = jnp.where(gt1, i1, jnp.where(gt2, iu, i2))
            m1 = jnp.where(gt1, ru, m1)
            i1 = jnp.where(gt1, iu, i1)
        return m1, i1, m2, i2

    def qproj(i, g, c, h):
        q = jnp.dot(hn[i, c * TQ:(c + 1) * TQ, :], wqbuf[g, :, h * DH:(h + 1) * DH],
                    preferred_element_type=F32)
        return (q * QSCALE).astype(BF16)

    def qk(q, g, h):
        return lax.dot_general(q, kbuf[g * NH + h], NT, preferred_element_type=F32)

    def pv(s, g, h, dep=None):
        m = jnp.max(s, axis=-1, keepdims=True)
        lsum = None
        parts = []
        for j in range(S // KG):
            ss = [s[:, j * KG + u * 128:j * KG + (u + 1) * 128] for u in range(KG // 128)]
            if j == 0:
                ss[0] = tie(ss[0], dep)
            ps = [jnp.exp2(z - m) for z in ss]
            t = (ps[0] + ps[1]) + (ps[2] + ps[3])
            lsum = t if lsum is None else lsum + t
            ps[-1] = jnp.minimum(ps[-1], lsum)
            parts += ps
        p = jnp.concatenate(parts, axis=-1).astype(BF16)
        return jnp.dot(p, vbuf[g * NH + h], preferred_element_type=F32), lsum

    def normalize_heads(res):
        gate = jnp.minimum(res[-1][0], 0.0)
        outs = []
        for o, lsum in res:
            l = jnp.sum(jnp.maximum(lsum, gate), axis=-1, keepdims=True)
            r = pl.reciprocal(l, approx=True)
            r = r * (2.0 - l * r)
            outs.append(o * r)
        return outs

    def woproj(slot, g, first, c, outs, lo, hi, dep=None, r0=0, r1=TQ):
        parts = [o[r0:r1] for o in outs]
        oc = jnp.concatenate([tie(parts[0], dep)] + parts[1:], axis=-1).astype(BF16)
        y = jnp.dot(oc, wobuf[g, :, lo:hi], preferred_element_type=F32)
        rows = slice(c * TQ + r0, c * TQ + r1)
        if first is True:
            acc[slot, rows, lo:hi] = y
        elif first is False:
            acc[slot, rows, lo:hi] = acc[slot, rows, lo:hi] + y
        else:
            acc[slot, rows, lo:hi] = jnp.where(first, 0.0, acc[slot, rows, lo:hi]) + y

    def ln1_chunk(i, g):
        if isinstance(i, int) and isinstance(g, int):
            row0, off = (i + 1) * BQ + g * LNR, g * LNR
        else:
            row0 = pl.multiple_of(jnp.minimum((i + 1) * BQ + g * LNR, S - LNR), LNR)
            off = pl.multiple_of(g * LNR, LNR)
        hv = ln1_apply(_normalize(xbuf[pl.ds(row0, LNR), :].astype(F32)), LNR)
        hn[i + 1, pl.ds(off, LNR), :] = hv.astype(BF16)
        return hv[:, 0:128]

    def ln2_chunks(i, g, st):
        deps = []
        pr = LNR // NP2
        for u in range(NP2):
            off = g * LNR + u * pr
            if isinstance(i, int) and isinstance(g, int):
                row0, valid = (i - 1) * BQ + off, None
            else:
                row0 = pl.multiple_of(jnp.maximum(i - 1, 0) * BQ + off, pr)
                off = pl.multiple_of(off, pr)
                valid = i > 0
            st = ln2(acc[(i + 1) % 2, pl.ds(off, pr), 0:DM], row0, pr, valid, st)
            deps.append(st[3])
        return deps, st

    WA, WB, WC = 256, 512, 768
    chains = [(c, h) for c in range(2) for h in range(NH)]

    def attention_step(i, g, slot, first):
        deps, st = ln2_chunks(i, g, load_top())
        store_top(st)
        pv_dep = {(0, h): deps[h * NP2 // NH] for h in range(0, NH, NH // NP2)}
        q = qproj(i, g, 0, 0)
        res = ([], [])
        o0 = None
        for n, (c, h) in enumerate(chains):
            s = qk(q, g, h)
            if n + 1 < len(chains):
                q = qproj(i, g, *chains[n + 1])
            if (c, h) == (1, 0):
                o0 = normalize_heads(res[0])
                woproj(slot, g, first, 0, o0, 0, WA)
            if (c, h) == (1, NH - 1):
                woproj(slot, g, first, 0, o0, WA, WB)
            res[c].append(pv(s, g, h, pv_dep.get((c, h))))
        o1 = normalize_heads(res[1])
        woproj(slot, g, first, 0, o0, WB, DM)
        woproj(slot, g, first, 1, o1, 0, WC)
        woproj(slot, g, first, 1, o1, WC, DM, ln1_chunk(i, g))

    c_cp.wait()
    x_cp[0].wait()
    sc = silu_c()
    acc[0, :, 0:DM] = _normalize(xbuf[0:BQ, :].astype(F32))
    for n in range(4):
        mod_cp[n].wait()
        mod_cols(sc, n * 512, (n + 1) * 512)
    hn[0] = ln1_apply(acc[0, :, 0:DM], BQ).astype(BF16)

    wq_cp, k_cp, v_cp = head0_cps(0)
    wq_cp.wait()
    qa = qproj(0, 0, 0, 0)
    qb = qproj(0, 0, 1, 0)
    k_cp.wait()
    sa = qk(qa, 0, 0)
    s = qk(qb, 0, 0)
    v_cp.wait()
    res = ([pv(sa, 0, 0)], [])
    for h in range(NH):
        if h + 1 < NH:
            for d in head0_cps(h + 1):
                d.wait()
            if h + 2 == NH:
                wo0_cp.wait()
                x_cp[1].wait()
                wr_cp.wait()
            q = qproj(0, 0, 0, h + 1)
            res[1].append(pv(s, 0, h))
            s = qk(q, 0, h + 1)
            q = qproj(0, 0, 1, h + 1)
            res[0].append(pv(s, 0, h + 1))
            s = qk(q, 0, h + 1)
        else:
            o0 = normalize_heads(res[0])
            woproj(0, 0, True, 0, o0, 0, WB)
            res[1].append(pv(s, 0, h))
    o1 = normalize_heads(res[1])
    woproj(0, 0, True, 0, o0, WB, DM)
    woproj(0, 0, True, 1, o1, 0, WC)
    woproj(0, 0, True, 1, o1, WC, DM, ln1_chunk(0, 0))
    wr32[...] = jnp.broadcast_to(wrbuf[...].astype(F32).reshape(1, DM), (8, DM))

    def step(t, carry):
        i = t // NG
        g = t % NG

        @pl.when(t < NG)
        def _():
            for d in group_cps(g):
                d.wait()

        @pl.when(t == NG)
        def _():
            modr_cp.wait()
            x_cp[2].wait()
            mod_cols(silu_c(), 2 * DM, 6 * DM)

        attention_step(i, g, i % 2, g == 0)

        @pl.when(jnp.logical_and(g == NG - 1, i >= 1))
        def _():
            out_cp(i - 1).start()

        return carry

    lax.fori_loop(1, NSTEP, step, 0)

    for d in ffn_cp:
        d.wait()
    last = (NQ - 1) % 2
    st = load_top()
    for u in range(BQ // LNR):
        st = ln2(acc[last, u * LNR:(u + 1) * LNR, 0:DM], (NQ - 1) * BQ + u * LNR, LNR, None, st)
    out_cp(NQ - 1).start()

    m1, i1, m2, i2 = st
    big = float(S)
    v1 = jnp.max(m1, axis=0, keepdims=True)
    j1 = jnp.min(jnp.where(m1 == v1, i1, big), axis=0, keepdims=True)
    taken = i1 == j1
    m1b = jnp.where(taken, m2, m1)
    i1b = jnp.where(taken, i2, i1)
    v2 = jnp.max(m1b, axis=0, keepdims=True)
    j2 = jnp.min(jnp.where(m1b == v2, i1b, big), axis=0, keepdims=True)
    idx1 = jnp.clip(j1[0, 0].astype(jnp.int32), 0, S - 1)
    idx2 = jnp.clip(j2[0, 0].astype(jnp.int32), 0, S - 1)

    row = lax.broadcasted_iota(jnp.int32, (16, DM), 0)
    xs = jnp.where(row == 0, h2buf[pl.ds(idx1, 1), :], h2buf[pl.ds(idx2, 1), :]).astype(BF16)
    gt = jnp.dot(xs, wgbuf[...], preferred_element_type=F32)
    up = jnp.dot(xs, wubuf[...], preferred_element_type=F32)
    act = (gt * jax.nn.sigmoid(gt) * up).astype(BF16)
    y = jnp.dot(act, wdbuf[:, 0:DM], preferred_element_type=F32)
    gb = mod[0:1, 5 * DM:6 * DM]
    y1 = y[0:1, :] * jax.nn.sigmoid(v1[:, 0:1]) * gb
    y2 = y[1:2, :] * jax.nn.sigmoid(v2[:, 0:1]) * gb

    for j in range(NQ):
        out_cp(j).wait()

    base1 = pl.multiple_of((idx1 // FIX) * FIX, FIX)
    base2 = pl.multiple_of((idx2 // FIX) * FIX, FIX)

    def fix(base, idx, yy):
        rs = pl.ds(base, FIX)
        upd = jnp.where(row + base == idx, yy, 0.0)
        obuf[rs, :] = (obuf[rs, :].astype(F32) + upd).astype(BF16)

    fix(base1, idx1, y1)
    fix(base2, idx2, y2)
    fix1 = cp(obuf.at[pl.ds(base1, FIX)], out_hbm.at[pl.ds(base1, FIX)], sem.at[SEM_FIX])
    fix2 = cp(obuf.at[pl.ds(base2, FIX)], out_hbm.at[pl.ds(base2, FIX)], sem.at[SEM_FIX])
    fix1.start()

    @pl.when(base1 != base2)
    def _():
        fix2.start()
        fix2.wait()

    fix1.wait()


@jax.jit
def pallas_adaLN_cond__mha_block_cached__moe_arch_mod__prompt_kernel(
    A_x: jax.Array,
    A_k_cache: jax.Array,
    A_v_cache: jax.Array,
    A_wq: jax.Array,
    A_wo: jax.Array,
    B_x: jax.Array,
    B_w_r: jax.Array,
    B_w_gate: jax.Array,
    B_w_up: jax.Array,
    B_w_down: jax.Array,
    c: jax.Array,
    w_mod: jax.Array,
):
    del B_x
    x = A_x.reshape(S, DM)
    k = A_k_cache.reshape(H, S, DH)
    v = A_v_cache.reshape(H, S, DH)
    wo = A_wo.reshape(NG, NH * DH, DM)
    any_spec = pl.BlockSpec(memory_space=pl.ANY)
    out = pl.pallas_call(
        _kernel,
        in_specs=[any_spec] * 11,
        out_specs=any_spec,
        out_shape=jax.ShapeDtypeStruct((S, DM), BF16),
        scratch_shapes=[
            pltpu.VMEM((S, DM), BF16),
            pltpu.VMEM((H, S, DH), BF16),
            pltpu.VMEM((H, S, DH), BF16),
            pltpu.VMEM((NG, DM, NH * DH), BF16),
            pltpu.VMEM((NG, NH * DH, DM), BF16),
            pltpu.VMEM((DM,), BF16),
            pltpu.VMEM((DM, FF), BF16),
            pltpu.VMEM((DM, FF), BF16),
            pltpu.VMEM((FF, DM + PAD), BF16),
            pltpu.VMEM((1, DM), BF16),
            pltpu.VMEM((DM, 6 * DM + PAD), BF16),
            pltpu.VMEM((NQ + 1, BQ, DM), BF16),
            pltpu.VMEM((2, BQ, DM + PAD), F32),
            pltpu.VMEM((S, DM), F32),
            pltpu.VMEM((S, DM), BF16),
            pltpu.VMEM((8, 6 * DM), F32),
            pltpu.VMEM((8, DM), F32),
            pltpu.VMEM((4, 8, 128), F32),
            pltpu.SMEM((1,), jnp.int32),
            pltpu.SemaphoreType.DMA((NSEM,)),
        ],
        compiler_params=pltpu.CompilerParams(vmem_limit_bytes=124 * 1024 * 1024),
        name="adaln_mha_moe",
    )(x, k, v, A_wq, wo, B_w_r, B_w_gate, B_w_up, B_w_down, c, w_mod)
    return out.reshape(1, S, DM)
```

```python
import jax
import jax.numpy as jnp
from jax import lax
import jax.experimental.pallas as pl
import jax.experimental.pallas.tpu as pltpu

F32 = jnp.float32
BF16 = jnp.bfloat16

S = 2048
DM = 1024
H = 32
DH = 128
FF = 3584
BQ = 512
TQ = 256
NH = 4
NQ = S // BQ
NG = H // NH
NSTEP = NQ * NG
LNR = BQ // NG
LN1_AT = (1, 3)
NP1 = len(LN1_AT)
WA, WB = 256, 512
NP2 = 4
KG = 512
EPS = 1e-5
QSCALE = DH ** -0.5 * 1.4426950408889634
NT = (((1,), (1,)), ((), ()))
FIX = 16
PAD = 128

SEM_CX = 0
SEM_MOD0 = 1
SEM_A = SEM_MOD0 + 4
SEM_H0 = SEM_A + 3
SEM_G = SEM_H0 + NH - 1
SEM_MODR = SEM_G + NG - 1
SEM_FFN = SEM_MODR + 1
SEM_OUT = SEM_FFN + 1
SEM_FIX = SEM_OUT + 1
NSEM = SEM_FIX + 1


def _rows8(v, rows):
    return jnp.tile(v, (rows // 8, 1))


def _normalize(x):
    mean = jnp.sum(x, axis=-1, keepdims=True) * (1.0 / DM)
    xc = x - mean
    var = jnp.sum(xc * xc, axis=-1, keepdims=True) * (1.0 / DM)
    return xc * lax.rsqrt(var + EPS)


def _kernel(x_hbm, k_hbm, v_hbm, wq_hbm, wo_hbm, wr_hbm, wg_hbm, wu_hbm, wd_hbm, c_hbm, wm_hbm,
            out_hbm,
            xbuf, kbuf, vbuf, wqbuf, wobuf, wrbuf, wgbuf, wubuf, wdbuf, cbuf, wmbuf,
            hn, acc, h2buf, obuf, mod, wr32, top, flag, sem):
    cp = pltpu.make_async_copy

    sem_last = SEM_H0 + NH - 2
    c_cp = cp(c_hbm, cbuf, sem.at[SEM_CX])
    wr_cp = cp(wr_hbm, wrbuf, sem.at[sem_last])
    x_rng = ((0, BQ, SEM_CX), (BQ, 2 * BQ, sem_last), (2 * BQ, S, SEM_MODR))
    x_cp = [cp(x_hbm.at[a:b], xbuf.at[a:b], sem.at[n]) for a, b, n in x_rng]
    mod_cp = [cp(wm_hbm.at[:, n * 512:(n + 1) * 512], wmbuf.at[:, n * 512:(n + 1) * 512],
                 sem.at[SEM_MOD0 + n]) for n in range(4)]
    modr_cp = cp(wm_hbm.at[:, 2 * DM:], wmbuf.at[:, 2 * DM:6 * DM], sem.at[SEM_MODR])

    def head0_cps(h):
        sq, sk, sv = (SEM_A, SEM_A + 1, SEM_A + 2) if h == 0 else (SEM_H0 + h - 1,) * 3
        return [cp(wq_hbm.at[:, h * DH:(h + 1) * DH], wqbuf.at[0, :, h * DH:(h + 1) * DH], sem.at[sq]),
                cp(k_hbm.at[h], kbuf.at[h], sem.at[sk]),
                cp(v_hbm.at[h], vbuf.at[h], sem.at[sv])]

    wo0_cp = cp(wo_hbm.at[0], wobuf.at[0], sem.at[sem_last])

    def group_cps(g):
        sg = sem.at[SEM_G + g - 1]
        if isinstance(g, int):
            cols = slice(g * NH * DH, (g + 1) * NH * DH)
        else:
            cols = pl.ds(pl.multiple_of(g * (NH * DH), NH * DH), NH * DH)
        heads = pl.ds(g * NH, NH)
        return [cp(wq_hbm.at[:, cols], wqbuf.at[g], sg),
                cp(k_hbm.at[heads], kbuf.at[heads], sg),
                cp(v_hbm.at[heads], vbuf.at[heads], sg),
                cp(wo_hbm.at[g], wobuf.at[g], sg)]

    ffn_cp = [cp(wg_hbm, wgbuf, sem.at[SEM_FFN]), cp(wu_hbm, wubuf, sem.at[SEM_FFN]),
              cp(wd_hbm, wdbuf.at[:, 0:DM], sem.at[SEM_FFN])]

    def out_cp(j):
        if isinstance(j, int):
            rows = slice(j * BQ, (j + 1) * BQ)
        else:
            rows = pl.ds(pl.multiple_of(j * BQ, BQ), BQ)
        return cp(obuf.at[rows], out_hbm.at[rows], sem.at[SEM_OUT])

    c_cp.start()
    x_cp[0].start()
    for d in mod_cp:
        d.start()
    for h in range(NH):
        for d in head0_cps(h):
            d.start()
    wo0_cp.start()
    x_cp[1].start()
    wr_cp.start()
    for g in range(1, NG):
        for d in group_cps(g):
            d.start()
    modr_cp.start()
    x_cp[2].start()
    for d in ffn_cp:
        d.start()

    flag[0] = 0
    acc[1, :, 0:DM] = jnp.zeros((BQ, DM), F32)
    mod[:, 2 * DM:] = jnp.zeros((8, 4 * DM), F32)
    top[0] = jnp.full((8, 128), -jnp.inf, F32)
    top[1] = jnp.zeros((8, 128), F32)
    top[2] = jnp.full((8, 128), -jnp.inf, F32)
    top[3] = jnp.zeros((8, 128), F32)

    def silu_c():
        cf = cbuf[...].astype(F32)
        sc = cf * jax.nn.sigmoid(cf)
        return jnp.broadcast_to(sc, (16, DM)).astype(BF16)

    def mod_cols(sc, lo, hi):
        mod[:, lo:hi] = jnp.dot(sc, wmbuf[:, lo:hi], preferred_element_type=F32)[:8]

    def tie(val, dep):
        if dep is None:
            return val
        n = dep.shape[0]
        head = jnp.where(flag[0] != 0, dep, val[:n])
        return head if n == val.shape[0] else jnp.concatenate([head, val[n:]], axis=0)

    def ln1_apply(n, rows):
        return n * (1.0 + _rows8(mod[:, DM:2 * DM], rows)) + _rows8(mod[:, 0:DM], rows)

    def load_top():
        return top[0], top[1], top[2], top[3]

    def store_top(st):
        top[0], top[1], top[2], top[3] = st

    def ln2(a, row0, rows, valid, st):
        rs = pl.ds(row0, rows)
        x1 = xbuf[rs, :].astype(F32) + _rows8(mod[:, 2 * DM:3 * DM], rows) * a
        h2 = (_normalize(x1) * (1.0 + _rows8(mod[:, 4 * DM:5 * DM], rows))
              + _rows8(mod[:, 3 * DM:4 * DM], rows))
        h2buf[rs, :] = h2
        obuf[rs, :] = (x1 + _rows8(mod[:, 5 * DM:6 * DM], rows) * h2).astype(BF16)
        r = jnp.sum(h2 * _rows8(wr32[...], rows), axis=-1, keepdims=True)
        r = jnp.broadcast_to(r, (rows, 128))
        if valid is not None:
            r = jnp.where(valid, r, -jnp.inf)
        m1, i1, m2, i2 = st
        base = (lax.broadcasted_iota(jnp.int32, (8, 128), 0) + row0).astype(F32)
        for u in range(rows // 8):
            ru = r[u * 8:(u + 1) * 8]
            iu = base + float(u * 8)
            gt1 = ru > m1
            gt2 = ru > m2
            m2 = jnp.where(gt1, m1, jnp.where(gt2, ru, m2))
            i2 = jnp.where(gt1, i1, jnp.where(gt2, iu, i2))
            m1 = jnp.where(gt1, ru, m1)
            i1 = jnp.where(gt1, iu, i1)
        return m1, i1, m2, i2

    def qproj(i, g, c, h):
        q = jnp.dot(hn[i, c * TQ:(c + 1) * TQ, :], wqbuf[g, :, h * DH:(h + 1) * DH],
                    preferred_element_type=F32)
        return (q * QSCALE).astype(BF16)

    def qk(q, g, h):
        return lax.dot_general(q, kbuf[g * NH + h], NT, preferred_element_type=F32)

    def pv(s, g, h, dep=None):
        m = jnp.max(s, axis=-1, keepdims=True)
        lsum = None
        parts = []
        for j in range(S // KG):
            ss = [s[:, j * KG + u * 128:j * KG + (u + 1) * 128] for u in range(KG // 128)]
            if j == 0:
                ss[0] = tie(ss[0], dep)
            ps = [jnp.exp2(z - m) for z in ss]
            t = (ps[0] + ps[1]) + (ps[2] + ps[3])
            lsum = t if lsum is None else lsum + t
            ps[-1] = jnp.minimum(ps[-1], lsum)
            parts += ps
        p = jnp.concatenate(parts, axis=-1).astype(BF16)
        return jnp.dot(p, vbuf[g * NH + h], preferred_element_type=F32), lsum

    def normalize_heads(res):
        gate = jnp.minimum(res[-1][0], 0.0)
        outs = []
        for o, lsum in res:
            l = jnp.sum(jnp.maximum(lsum, gate), axis=-1, keepdims=True)
            r = pl.reciprocal(l, approx=True)
            r = r * (2.0 - l * r)
            outs.append(o * r)
        return outs

    def woproj(slot, g, first, c, outs, lo, hi, dep=None, r0=0, r1=TQ):
        parts = [o[r0:r1] for o in outs]
        oc = jnp.concatenate([tie(parts[0], dep)] + parts[1:], axis=-1).astype(BF16)
        y = jnp.dot(oc, wobuf[g, :, lo:hi], preferred_element_type=F32)
        rows = slice(c * TQ + r0, c * TQ + r1)
        if first is True:
            acc[slot, rows, lo:hi] = y
        elif first is False:
            acc[slot, rows, lo:hi] = acc[slot, rows, lo:hi] + y
        else:
            acc[slot, rows, lo:hi] = jnp.where(first, 0.0, acc[slot, rows, lo:hi]) + y
        return y

    def ln1_piece(i, g, u, gate):
        pr = LNR // NP1
        if isinstance(i, int) and isinstance(g, int):
            row0, off = (i + 1) * BQ + g * LNR + u * pr, g * LNR + u * pr
        else:
            row0 = pl.multiple_of(jnp.minimum((i + 1) * BQ + g * LNR, S - LNR) + u * pr, pr)
            off = pl.multiple_of(g * LNR + u * pr, pr)
        xv = xbuf[pl.ds(row0, pr), :].astype(F32)
        xv = jnp.concatenate([tie(xv[:, 0:128], gate[0:pr, 0:128]), xv[:, 128:]], axis=-1)
        hv = ln1_apply(_normalize(xv), pr)
        hn[i + 1, pl.ds(off, pr), :] = hv.astype(BF16)
        return hv[:, 0:128]

    def wo_tail(i, g, slot, first, o0, o1):
        w = 256
        pieces = [(0, o0, lo) for lo in range(WB, DM, w)] + [(1, o1, lo) for lo in range(0, DM, w)]
        deps = {}
        for n, (c, o, lo) in enumerate(pieces):
            y = woproj(slot, g, first, c, o, lo, lo + w, deps.get(n))
            if n in LN1_AT:
                deps[n + 2] = ln1_piece(i, g, LN1_AT.index(n), y)

    def ln2_chunks(i, g, st):
        deps = []
        pr = LNR // NP2
        for u in range(NP2):
            off = g * LNR + u * pr
            if isinstance(i, int) and isinstance(g, int):
                row0, valid = (i - 1) * BQ + off, None
            else:
                row0 = pl.multiple_of(jnp.maximum(i - 1, 0) * BQ + off, pr)
                off = pl.multiple_of(off, pr)
                valid = i > 0
            st = ln2(acc[(i + 1) & 1, pl.ds(off, pr), 0:DM], row0, pr, valid, st)
            deps.append(st[3])
        return deps, st

    chains = [(c, h) for c in range(2) for h in range(NH)]

    def attention_step(i, g, slot, first):
        deps, st = ln2_chunks(i, g, load_top())
        store_top(st)
        pv_dep = {(0, h): deps[h * NP2 // NH] for h in range(0, NH, NH // NP2)}
        q = qproj(i, g, 0, 0)
        res = ([], [])
        o0 = None
        for n, (c, h) in enumerate(chains):
            s = qk(q, g, h)
            if n + 1 < len(chains):
                q = qproj(i, g, *chains[n + 1])
            if (c, h) == (1, 0):
                o0 = normalize_heads(res[0])
                woproj(slot, g, first, 0, o0, 0, WA)
            if (c, h) == (1, NH - 1):
                woproj(slot, g, first, 0, o0, WA, WB)
            res[c].append(pv(s, g, h, pv_dep.get((c, h))))
        o1 = normalize_heads(res[1])
        wo_tail(i, g, slot, first, o0, o1)

    c_cp.wait()
    x_cp[0].wait()
    sc = silu_c()
    acc[0, :, 0:DM] = _normalize(xbuf[0:BQ, :].astype(F32))
    for n in range(4):
        mod_cp[n].wait()
        mod_cols(sc, n * 512, (n + 1) * 512)
    hn[0] = ln1_apply(acc[0, :, 0:DM], BQ).astype(BF16)

    wq_cp, k_cp, v_cp = head0_cps(0)
    wq_cp.wait()
    qa = qproj(0, 0, 0, 0)
    qb = qproj(0, 0, 1, 0)
    k_cp.wait()
    sa = qk(qa, 0, 0)
    s = qk(qb, 0, 0)
    v_cp.wait()
    res = ([pv(sa, 0, 0)], [])
    for h in range(NH):
        if h + 1 < NH:
            for d in head0_cps(h + 1):
                d.wait()
            if h + 2 == NH:
                wo0_cp.wait()
                x_cp[1].wait()
                wr_cp.wait()
            q = qproj(0, 0, 0, h + 1)
            res[1].append(pv(s, 0, h))
            s = qk(q, 0, h + 1)
            q = qproj(0, 0, 1, h + 1)
            res[0].append(pv(s, 0, h + 1))
            s = qk(q, 0, h + 1)
        else:
            o0 = normalize_heads(res[0])
            woproj(0, 0, True, 0, o0, 0, WB)
            res[1].append(pv(s, 0, h))
    wo_tail(0, 0, 0, True, o0, normalize_heads(res[1]))
    wr32[...] = jnp.broadcast_to(wrbuf[...].astype(F32).reshape(1, DM), (8, DM))

    def step(t, carry):
        i = lax.shift_right_logical(t, NG.bit_length() - 1)
        g = t & (NG - 1)

        @pl.when(jnp.logical_or(t < NG, g == 0))
        def _():
            @pl.when(t < NG)
            def _():
                for d in group_cps(g):
                    d.wait()

            @pl.when(t == NG)
            def _():
                modr_cp.wait()
                x_cp[2].wait()
                mod_cols(silu_c(), 2 * DM, 6 * DM)

            @pl.when(t >= 2 * NG)
            def _():
                out_cp(i - 2).start()

        attention_step(i, g, i & 1, g == 0)
        return carry

    lax.fori_loop(1, NSTEP, step, 0)

    out_cp(NQ - 2).start()
    for d in ffn_cp:
        d.wait()
    last = (NQ - 1) % 2
    st = load_top()
    for u in range(BQ // LNR):
        st = ln2(acc[last, u * LNR:(u + 1) * LNR, 0:DM], (NQ - 1) * BQ + u * LNR, LNR, None, st)
    out_cp(NQ - 1).start()

    m1, i1, m2, i2 = st
    big = float(S)
    v1 = jnp.max(m1, axis=0, keepdims=True)
    j1 = jnp.min(jnp.where(m1 == v1, i1, big), axis=0, keepdims=True)
    taken = i1 == j1
    m1b = jnp.where(taken, m2, m1)
    i1b = jnp.where(taken, i2, i1)
    v2 = jnp.max(m1b, axis=0, keepdims=True)
    j2 = jnp.min(jnp.where(m1b == v2, i1b, big), axis=0, keepdims=True)
    idx1 = jnp.clip(j1[0, 0].astype(jnp.int32), 0, S - 1)
    idx2 = jnp.clip(j2[0, 0].astype(jnp.int32), 0, S - 1)

    row = lax.broadcasted_iota(jnp.int32, (16, DM), 0)
    xs = jnp.where(row == 0, h2buf[pl.ds(idx1, 1), :], h2buf[pl.ds(idx2, 1), :]).astype(BF16)
    gt = jnp.dot(xs, wgbuf[...], preferred_element_type=F32)
    up = jnp.dot(xs, wubuf[...], preferred_element_type=F32)
    act = (gt * jax.nn.sigmoid(gt) * up).astype(BF16)
    y = jnp.dot(act, wdbuf[:, 0:DM], preferred_element_type=F32)
    gb = mod[0:1, 5 * DM:6 * DM]
    y1 = y[0:1, :] * jax.nn.sigmoid(v1[:, 0:1]) * gb
    y2 = y[1:2, :] * jax.nn.sigmoid(v2[:, 0:1]) * gb

    for j in range(NQ):
        out_cp(j).wait()

    base1 = pl.multiple_of((idx1 // FIX) * FIX, FIX)
    base2 = pl.multiple_of((idx2 // FIX) * FIX, FIX)

    def fix(base, idx, yy):
        rs = pl.ds(base, FIX)
        upd = jnp.where(row + base == idx, yy, 0.0)
        obuf[rs, :] = (obuf[rs, :].astype(F32) + upd).astype(BF16)

    fix(base1, idx1, y1)
    fix(base2, idx2, y2)
    fix1 = cp(obuf.at[pl.ds(base1, FIX)], out_hbm.at[pl.ds(base1, FIX)], sem.at[SEM_FIX])
    fix2 = cp(obuf.at[pl.ds(base2, FIX)], out_hbm.at[pl.ds(base2, FIX)], sem.at[SEM_FIX])
    fix1.start()

    @pl.when(base1 != base2)
    def _():
        fix2.start()
        fix2.wait()

    fix1.wait()


@jax.jit
def pallas_adaLN_cond__mha_block_cached__moe_arch_mod__prompt_kernel(
    A_x: jax.Array,
    A_k_cache: jax.Array,
    A_v_cache: jax.Array,
    A_wq: jax.Array,
    A_wo: jax.Array,
    B_x: jax.Array,
    B_w_r: jax.Array,
    B_w_gate: jax.Array,
    B_w_up: jax.Array,
    B_w_down: jax.Array,
    c: jax.Array,
    w_mod: jax.Array,
):
    del B_x
    x = A_x.reshape(S, DM)
    k = A_k_cache.reshape(H, S, DH)
    v = A_v_cache.reshape(H, S, DH)
    wo = A_wo.reshape(NG, NH * DH, DM)
    any_spec = pl.BlockSpec(memory_space=pl.ANY)
    out = pl.pallas_call(
        _kernel,
        in_specs=[any_spec] * 11,
        out_specs=any_spec,
        out_shape=jax.ShapeDtypeStruct((S, DM), BF16),
        scratch_shapes=[
            pltpu.VMEM((S, DM), BF16),
            pltpu.VMEM((H, S, DH), BF16),
            pltpu.VMEM((H, S, DH), BF16),
            pltpu.VMEM((NG, DM, NH * DH), BF16),
            pltpu.VMEM((NG, NH * DH, DM), BF16),
            pltpu.VMEM((DM,), BF16),
            pltpu.VMEM((DM, FF), BF16),
            pltpu.VMEM((DM, FF), BF16),
            pltpu.VMEM((FF, DM + PAD), BF16),
            pltpu.VMEM((1, DM), BF16),
            pltpu.VMEM((DM, 6 * DM + PAD), BF16),
            pltpu.VMEM((NQ + 1, BQ, DM), BF16),
            pltpu.VMEM((2, BQ, DM + PAD), F32),
            pltpu.VMEM((S, DM), F32),
            pltpu.VMEM((S, DM), BF16),
            pltpu.VMEM((8, 6 * DM), F32),
            pltpu.VMEM((8, DM), F32),
            pltpu.VMEM((4, 8, 128), F32),
            pltpu.SMEM((1,), jnp.int32),
            pltpu.SemaphoreType.DMA((NSEM,)),
        ],
        compiler_params=pltpu.CompilerParams(vmem_limit_bytes=124 * 1024 * 1024),
        name="adaln_mha_moe",
    )(x, k, v, A_wq, wo, B_w_r, B_w_gate, B_w_up, B_w_down, c, w_mod)
    return out.reshape(1, S, DM)
```

```python
import jax
import jax.numpy as jnp
from jax import lax
import jax.experimental.pallas as pl
import jax.experimental.pallas.tpu as pltpu

F32 = jnp.float32
BF16 = jnp.bfloat16

S = 2048
DM = 1024
H = 32
DH = 128
FF = 3584
BQ = 512
TQ = 256
NH = 4
NQ = S // BQ
NG = H // NH
NSTEP = NQ * NG
LNR = BQ // NG
LN1_AT = (0, 1, 2, 3)
NP1 = len(LN1_AT)
WA, WB = 256, 512
NP2 = 4
KG = 512
EPS = 1e-5
QSCALE = DH ** -0.5 * 1.4426950408889634
NT = (((1,), (1,)), ((), ()))
FIX = 16
PAD = 128

SEM_CX = 0
SEM_MOD0 = 1
SEM_A = SEM_MOD0 + 4
SEM_H0 = SEM_A + 3
SEM_G = SEM_H0 + NH - 1
SEM_MODR = SEM_G + NG - 1
SEM_FFN = SEM_MODR + 1
SEM_OUT = SEM_FFN + 1
SEM_FIX = SEM_OUT + 1
NSEM = SEM_FIX + 1


def _rows8(v, rows):
    return jnp.tile(v, (rows // 8, 1))


def _normalize(x):
    mean = jnp.sum(x, axis=-1, keepdims=True) * (1.0 / DM)
    xc = x - mean
    var = jnp.sum(xc * xc, axis=-1, keepdims=True) * (1.0 / DM)
    return xc * lax.rsqrt(var + EPS)


def _kernel(x_hbm, k_hbm, v_hbm, wq_hbm, wo_hbm, wr_hbm, wg_hbm, wu_hbm, wd_hbm, c_hbm, wm_hbm,
            out_hbm,
            xbuf, kbuf, vbuf, wqbuf, wobuf, wrbuf, wgbuf, wubuf, wdbuf, cbuf, wmbuf,
            hn, hnext, acc, h2buf, obuf, mod, wr32, top, flag, sem):
    cp = pltpu.make_async_copy

    sem_last = SEM_H0 + NH - 2
    c_cp = cp(c_hbm, cbuf, sem.at[SEM_CX])
    wr_cp = cp(wr_hbm, wrbuf, sem.at[sem_last])
    x_rng = ((0, BQ, SEM_CX), (BQ, 2 * BQ, sem_last), (2 * BQ, S, SEM_MODR))
    x_cp = [cp(x_hbm.at[a:b], xbuf.at[a:b], sem.at[n]) for a, b, n in x_rng]
    mod_cp = [cp(wm_hbm.at[:, n * 512:(n + 1) * 512], wmbuf.at[:, n * 512:(n + 1) * 512],
                 sem.at[SEM_MOD0 + n]) for n in range(4)]
    modr_cp = cp(wm_hbm.at[:, 2 * DM:], wmbuf.at[:, 2 * DM:6 * DM], sem.at[SEM_MODR])

    def head0_cps(h):
        sq, sk, sv = (SEM_A, SEM_A + 1, SEM_A + 2) if h == 0 else (SEM_H0 + h - 1,) * 3
        return [cp(wq_hbm.at[:, h * DH:(h + 1) * DH], wqbuf.at[0, :, h * DH:(h + 1) * DH], sem.at[sq]),
                cp(k_hbm.at[h], kbuf.at[h], sem.at[sk]),
                cp(v_hbm.at[h], vbuf.at[h], sem.at[sv])]

    wo0_cp = cp(wo_hbm.at[0], wobuf.at[0], sem.at[sem_last])

    def group_cps(g):
        sg = sem.at[SEM_G + g - 1]
        if isinstance(g, int):
            cols = slice(g * NH * DH, (g + 1) * NH * DH)
        else:
            cols = pl.ds(pl.multiple_of(g * (NH * DH), NH * DH), NH * DH)
        heads = pl.ds(g * NH, NH)
        return [cp(wq_hbm.at[:, cols], wqbuf.at[g], sg),
                cp(k_hbm.at[heads], kbuf.at[heads], sg),
                cp(v_hbm.at[heads], vbuf.at[heads], sg),
                cp(wo_hbm.at[g], wobuf.at[g], sg)]

    ffn_cp = [cp(wg_hbm, wgbuf, sem.at[SEM_FFN]), cp(wu_hbm, wubuf, sem.at[SEM_FFN]),
              cp(wd_hbm, wdbuf.at[:, 0:DM], sem.at[SEM_FFN])]

    def out_cp(j):
        if isinstance(j, int):
            rows = slice(j * BQ, (j + 1) * BQ)
        else:
            rows = pl.ds(pl.multiple_of(j * BQ, BQ), BQ)
        return cp(obuf.at[rows], out_hbm.at[rows], sem.at[SEM_OUT])

    c_cp.start()
    x_cp[0].start()
    for d in mod_cp:
        d.start()
    for h in range(NH):
        for d in head0_cps(h):
            d.start()
    wo0_cp.start()
    x_cp[1].start()
    wr_cp.start()
    for g in range(1, NG):
        for d in group_cps(g):
            d.start()
    modr_cp.start()
    x_cp[2].start()
    for d in ffn_cp:
        d.start()

    flag[0] = 0
    acc[1, :, 0:DM] = jnp.zeros((BQ, DM), F32)
    mod[:, 2 * DM:] = jnp.zeros((8, 4 * DM), F32)
    top[0] = jnp.full((8, 128), -jnp.inf, F32)
    top[1] = jnp.zeros((8, 128), F32)
    top[2] = jnp.full((8, 128), -jnp.inf, F32)
    top[3] = jnp.zeros((8, 128), F32)

    def silu_c():
        cf = cbuf[...].astype(F32)
        sc = cf * jax.nn.sigmoid(cf)
        return jnp.broadcast_to(sc, (16, DM)).astype(BF16)

    def mod_cols(sc, lo, hi):
        mod[:, lo:hi] = jnp.dot(sc, wmbuf[:, lo:hi], preferred_element_type=F32)[:8]

    def tie(val, dep):
        if dep is None:
            return val
        n = dep.shape[0]
        head = jnp.where(flag[0] != 0, dep, val[:n])
        return head if n == val.shape[0] else jnp.concatenate([head, val[n:]], axis=0)

    def ln1_apply(n, rows):
        return n * (1.0 + _rows8(mod[:, DM:2 * DM], rows)) + _rows8(mod[:, 0:DM], rows)

    def load_top():
        return top[0], top[1], top[2], top[3]

    def store_top(st):
        top[0], top[1], top[2], top[3] = st

    def ln2(a, row0, rows, valid, st):
        rs = pl.ds(row0, rows)
        x1 = xbuf[rs, :].astype(F32) + _rows8(mod[:, 2 * DM:3 * DM], rows) * a
        h2 = (_normalize(x1) * (1.0 + _rows8(mod[:, 4 * DM:5 * DM], rows))
              + _rows8(mod[:, 3 * DM:4 * DM], rows))
        h2buf[rs, :] = h2
        obuf[rs, :] = (x1 + _rows8(mod[:, 5 * DM:6 * DM], rows) * h2).astype(BF16)
        r = jnp.sum(h2 * _rows8(wr32[...], rows), axis=-1, keepdims=True)
        r = jnp.broadcast_to(r, (rows, 128))
        if valid is not None:
            r = jnp.where(valid, r, -jnp.inf)
        m1, i1, m2, i2 = st
        base = (lax.broadcasted_iota(jnp.int32, (8, 128), 0) + row0).astype(F32)
        for u in range(rows // 8):
            ru = r[u * 8:(u + 1) * 8]
            iu = base + float(u * 8)
            gt1 = ru > m1
            gt2 = ru > m2
            m2 = jnp.where(gt1, m1, jnp.where(gt2, ru, m2))
            i2 = jnp.where(gt1, i1, jnp.where(gt2, iu, i2))
            m1 = jnp.where(gt1, ru, m1)
            i1 = jnp.where(gt1, iu, i1)
        return m1, i1, m2, i2

    def qproj(g, c, h):
        q = jnp.dot(hn[c * TQ:(c + 1) * TQ, :], wqbuf[g, :, h * DH:(h + 1) * DH],
                    preferred_element_type=F32)
        return (q * QSCALE).astype(BF16)

    def qk(q, g, h):
        return lax.dot_general(q, kbuf[g * NH + h], NT, preferred_element_type=F32)

    def pv(s, g, h, dep=None):
        m = jnp.max(s, axis=-1, keepdims=True)
        lsum = None
        parts = []
        for j in range(S // KG):
            ss = [s[:, j * KG + u * 128:j * KG + (u + 1) * 128] for u in range(KG // 128)]
            if j == 0:
                ss[0] = tie(ss[0], dep)
            ps = [jnp.exp2(z - m) for z in ss]
            t = (ps[0] + ps[1]) + (ps[2] + ps[3])
            lsum = t if lsum is None else lsum + t
            ps[-1] = jnp.minimum(ps[-1], lsum)
            parts += ps
        p = jnp.concatenate(parts, axis=-1).astype(BF16)
        return jnp.dot(p, vbuf[g * NH + h], preferred_element_type=F32), lsum

    def normalize_heads(res):
        gate = jnp.minimum(res[-1][0], 0.0)
        outs = []
        for o, lsum in res:
            l = jnp.sum(jnp.maximum(lsum, gate), axis=-1, keepdims=True)
            r = pl.reciprocal(l, approx=True)
            r = r * (2.0 - l * r)
            outs.append(o * r)
        return outs

    def woproj(slot, g, first, c, outs, lo, hi, dep=None, r0=0, r1=TQ):
        parts = [o[r0:r1] for o in outs]
        oc = jnp.concatenate([tie(parts[0], dep)] + parts[1:], axis=-1).astype(BF16)
        y = jnp.dot(oc, wobuf[g, :, lo:hi], preferred_element_type=F32)
        rows = slice(c * TQ + r0, c * TQ + r1)
        if first is True:
            acc[slot, rows, lo:hi] = y
        elif first is False:
            acc[slot, rows, lo:hi] = acc[slot, rows, lo:hi] + y
        else:
            acc[slot, rows, lo:hi] = jnp.where(first, 0.0, acc[slot, rows, lo:hi]) + y
        return y

    def ln1_piece(i, g, u, gate):
        pr = LNR // NP1
        if isinstance(i, int) and isinstance(g, int):
            row0, off = (i + 1) * BQ + g * LNR + u * pr, g * LNR + u * pr
        else:
            row0 = pl.multiple_of(jnp.minimum((i + 1) * BQ + g * LNR, S - LNR) + u * pr, pr)
            off = pl.multiple_of(g * LNR + u * pr, pr)
        xv = xbuf[pl.ds(row0, pr), :].astype(F32)
        xv = jnp.concatenate([tie(xv[:, 0:128], gate[0:pr, 0:128]), xv[:, 128:]], axis=-1)
        hv = ln1_apply(_normalize(xv), pr)
        hnext[pl.ds(off, pr), :] = hv.astype(BF16)
        return hv[:, 0:128]

    def wo_tail(i, g, slot, first, o0, o1):
        w = 256
        pieces = [(0, o0, lo) for lo in range(WB, DM, w)] + [(1, o1, lo) for lo in range(0, DM, w)]
        deps = {}
        for n, (c, o, lo) in enumerate(pieces):
            y = woproj(slot, g, first, c, o, lo, lo + w, deps.get(n))
            if n in LN1_AT:
                deps[n + 2] = ln1_piece(i, g, LN1_AT.index(n), y)

    def ln2_chunks(i, g, st):
        deps = []
        pr = LNR // NP2
        for u in range(NP2):
            off = g * LNR + u * pr
            if isinstance(i, int) and isinstance(g, int):
                row0, valid = (i - 1) * BQ + off, None
            else:
                row0 = pl.multiple_of(jnp.maximum(i - 1, 0) * BQ + off, pr)
                off = pl.multiple_of(off, pr)
                valid = i > 0
            st = ln2(acc[(i + 1) & 1, pl.ds(off, pr), 0:DM], row0, pr, valid, st)
            deps.append(st[3])
        return deps, st

    chains = [(c, h) for c in range(2) for h in range(NH)]

    def attention_step(i, g, slot, first):
        deps, st = ln2_chunks(i, g, load_top())
        store_top(st)
        pv_dep = {(0, h): deps[h * NP2 // NH] for h in range(0, NH, NH // NP2)}
        q = qproj(g, 0, 0)
        res = ([], [])
        o0 = None
        for n, (c, h) in enumerate(chains):
            s = qk(q, g, h)
            if n + 1 < len(chains):
                q = qproj(g, *chains[n + 1])
            if (c, h) == (1, 0):
                o0 = normalize_heads(res[0])
                woproj(slot, g, first, 0, o0, 0, WA)
            if (c, h) == (1, NH - 1):
                woproj(slot, g, first, 0, o0, WA, WB)
            res[c].append(pv(s, g, h, pv_dep.get((c, h))))
        o1 = normalize_heads(res[1])
        wo_tail(i, g, slot, first, o0, o1)

    c_cp.wait()
    x_cp[0].wait()
    sc = silu_c()
    acc[0, :, 0:DM] = _normalize(xbuf[0:BQ, :].astype(F32))
    for n in range(4):
        mod_cp[n].wait()
        mod_cols(sc, n * 512, (n + 1) * 512)
    hn[...] = ln1_apply(acc[0, :, 0:DM], BQ).astype(BF16)

    wq_cp, k_cp, v_cp = head0_cps(0)
    wq_cp.wait()
    qa = qproj(0, 0, 0)
    qb = qproj(0, 1, 0)
    k_cp.wait()
    sa = qk(qa, 0, 0)
    s = qk(qb, 0, 0)
    v_cp.wait()
    res = ([pv(sa, 0, 0)], [])
    for h in range(NH):
        if h + 1 < NH:
            for d in head0_cps(h + 1):
                d.wait()
            if h + 2 == NH:
                wo0_cp.wait()
                x_cp[1].wait()
                wr_cp.wait()
            q = qproj(0, 0, h + 1)
            res[1].append(pv(s, 0, h))
            s = qk(q, 0, h + 1)
            q = qproj(0, 1, h + 1)
            res[0].append(pv(s, 0, h + 1))
            s = qk(q, 0, h + 1)
        else:
            o0 = normalize_heads(res[0])
            woproj(0, 0, True, 0, o0, 0, WB)
            res[1].append(pv(s, 0, h))
    wo_tail(0, 0, 0, True, o0, normalize_heads(res[1]))
    wr32[...] = jnp.broadcast_to(wrbuf[...].astype(F32).reshape(1, DM), (8, DM))

    def step(t, carry):
        i = lax.shift_right_logical(t, NG.bit_length() - 1)
        g = t & (NG - 1)

        @pl.when(jnp.logical_or(t < NG, g == 0))
        def _():
            @pl.when(t < NG)
            def _():
                for d in group_cps(g):
                    d.wait()

            @pl.when(t == NG)
            def _():
                modr_cp.wait()
                x_cp[2].wait()
                mod_cols(silu_c(), 2 * DM, 6 * DM)

            @pl.when(t >= 2 * NG)
            def _():
                out_cp(i - 2).start()

            @pl.when(g == 0)
            def _():
                hn[...] = hnext[...]

        attention_step(i, g, i & 1, g == 0)
        return carry

    lax.fori_loop(1, NSTEP, step, 0)

    out_cp(NQ - 2).start()
    for d in ffn_cp:
        d.wait()
    last = (NQ - 1) % 2
    st = load_top()
    for u in range(BQ // LNR):
        st = ln2(acc[last, u * LNR:(u + 1) * LNR, 0:DM], (NQ - 1) * BQ + u * LNR, LNR, None, st)
    out_cp(NQ - 1).start()

    m1, i1, m2, i2 = st
    big = float(S)
    v1 = jnp.max(m1, axis=0, keepdims=True)
    j1 = jnp.min(jnp.where(m1 == v1, i1, big), axis=0, keepdims=True)
    taken = i1 == j1
    m1b = jnp.where(taken, m2, m1)
    i1b = jnp.where(taken, i2, i1)
    v2 = jnp.max(m1b, axis=0, keepdims=True)
    j2 = jnp.min(jnp.where(m1b == v2, i1b, big), axis=0, keepdims=True)
    idx1 = jnp.clip(j1[0, 0].astype(jnp.int32), 0, S - 1)
    idx2 = jnp.clip(j2[0, 0].astype(jnp.int32), 0, S - 1)

    row = lax.broadcasted_iota(jnp.int32, (16, DM), 0)
    xs = jnp.where(row == 0, h2buf[pl.ds(idx1, 1), :], h2buf[pl.ds(idx2, 1), :]).astype(BF16)
    gt = jnp.dot(xs, wgbuf[...], preferred_element_type=F32)
    up = jnp.dot(xs, wubuf[...], preferred_element_type=F32)
    act = (gt * jax.nn.sigmoid(gt) * up).astype(BF16)
    y = jnp.dot(act, wdbuf[:, 0:DM], preferred_element_type=F32)
    gb = mod[0:1, 5 * DM:6 * DM]
    y1 = y[0:1, :] * jax.nn.sigmoid(v1[:, 0:1]) * gb
    y2 = y[1:2, :] * jax.nn.sigmoid(v2[:, 0:1]) * gb

    for j in range(NQ):
        out_cp(j).wait()

    base1 = pl.multiple_of((idx1 // FIX) * FIX, FIX)
    base2 = pl.multiple_of((idx2 // FIX) * FIX, FIX)

    def fix(base, idx, yy):
        rs = pl.ds(base, FIX)
        upd = jnp.where(row + base == idx, yy, 0.0)
        obuf[rs, :] = (obuf[rs, :].astype(F32) + upd).astype(BF16)

    fix(base1, idx1, y1)
    fix(base2, idx2, y2)
    fix1 = cp(obuf.at[pl.ds(base1, FIX)], out_hbm.at[pl.ds(base1, FIX)], sem.at[SEM_FIX])
    fix2 = cp(obuf.at[pl.ds(base2, FIX)], out_hbm.at[pl.ds(base2, FIX)], sem.at[SEM_FIX])
    fix1.start()

    @pl.when(base1 != base2)
    def _():
        fix2.start()
        fix2.wait()

    fix1.wait()


@jax.jit
def pallas_adaLN_cond__mha_block_cached__moe_arch_mod__prompt_kernel(
    A_x: jax.Array,
    A_k_cache: jax.Array,
    A_v_cache: jax.Array,
    A_wq: jax.Array,
    A_wo: jax.Array,
    B_x: jax.Array,
    B_w_r: jax.Array,
    B_w_gate: jax.Array,
    B_w_up: jax.Array,
    B_w_down: jax.Array,
    c: jax.Array,
    w_mod: jax.Array,
):
    del B_x
    x = A_x.reshape(S, DM)
    k = A_k_cache.reshape(H, S, DH)
    v = A_v_cache.reshape(H, S, DH)
    wo = A_wo.reshape(NG, NH * DH, DM)
    any_spec = pl.BlockSpec(memory_space=pl.ANY)
    out = pl.pallas_call(
        _kernel,
        in_specs=[any_spec] * 11,
        out_specs=any_spec,
        out_shape=jax.ShapeDtypeStruct((S, DM), BF16),
        scratch_shapes=[
            pltpu.VMEM((S, DM), BF16),
            pltpu.VMEM((H, S, DH), BF16),
            pltpu.VMEM((H, S, DH), BF16),
            pltpu.VMEM((NG, DM, NH * DH), BF16),
            pltpu.VMEM((NG, NH * DH, DM), BF16),
            pltpu.VMEM((DM,), BF16),
            pltpu.VMEM((DM, FF), BF16),
            pltpu.VMEM((DM, FF), BF16),
            pltpu.VMEM((FF, DM + PAD), BF16),
            pltpu.VMEM((1, DM), BF16),
            pltpu.VMEM((DM, 6 * DM + PAD), BF16),
            pltpu.VMEM((BQ, DM), BF16),
            pltpu.VMEM((BQ, DM), BF16),
            pltpu.VMEM((2, BQ, DM + PAD), F32),
            pltpu.VMEM((S, DM), F32),
            pltpu.VMEM((S, DM), BF16),
            pltpu.VMEM((8, 6 * DM), F32),
            pltpu.VMEM((8, DM), F32),
            pltpu.VMEM((4, 8, 128), F32),
            pltpu.SMEM((1,), jnp.int32),
            pltpu.SemaphoreType.DMA((NSEM,)),
        ],
        compiler_params=pltpu.CompilerParams(vmem_limit_bytes=124 * 1024 * 1024),
        name="adaln_mha_moe",
    )(x, k, v, A_wq, wo, B_w_r, B_w_gate, B_w_up, B_w_down, c, w_mod)
    return out.reshape(1, S, DM)
```

```python
import jax
import jax.numpy as jnp
from jax import lax
import jax.experimental.pallas as pl
import jax.experimental.pallas.tpu as pltpu

F32 = jnp.float32
BF16 = jnp.bfloat16

S = 2048
DM = 1024
H = 32
DH = 128
FF = 3584
BQ = 512
TQ = 256
NH = 4
NQ = S // BQ
NG = H // NH
NSTEP = NQ * NG
LNR = BQ // NG
LN1_AT = (0, 1, 2, 3)
NP1 = len(LN1_AT)
WA, WB = 256, 512
NP2 = 4
KG = 512
EPS = 1e-5
QSCALE = DH ** -0.5 * 1.4426950408889634
NT = (((1,), (1,)), ((), ()))
FIX = 16
PAD = 128

SEM_CX = 0
MODC = (0, 512, 896, 1024)
SEM_MOD0 = 1
SEM_A = SEM_MOD0 + len(MODC) - 1
SEM_H0 = SEM_A + 3
SEM_G = SEM_H0 + NH - 1
SEM_MODR = SEM_G + NG - 1
SEM_FFN = SEM_MODR + 1
SEM_OUT = SEM_FFN + 1
SEM_FIX = SEM_OUT + 1
NSEM = SEM_FIX + 1


def _rows8(v, rows):
    return jnp.tile(v, (rows // 8, 1))


def _normalize(x):
    mean = jnp.sum(x, axis=-1, keepdims=True) * (1.0 / DM)
    xc = x - mean
    var = jnp.sum(xc * xc, axis=-1, keepdims=True) * (1.0 / DM)
    return xc * lax.rsqrt(var + EPS)


def _kernel(x_hbm, k_hbm, v_hbm, wq_hbm, wo_hbm, wr_hbm, wg_hbm, wu_hbm, wd_hbm, c_hbm, wm_hbm,
            out_hbm,
            xbuf, kbuf, vbuf, wqbuf, wobuf, wrbuf, wgbuf, wubuf, wdbuf, cbuf, wmbuf,
            hn, hnext, acc, h2buf, obuf, mod, wr32, top, flag, sem):
    cp = pltpu.make_async_copy

    sem_last = SEM_H0 + NH - 2
    c_cp = cp(c_hbm, cbuf, sem.at[SEM_CX])
    wr_cp = cp(wr_hbm, wrbuf, sem.at[sem_last])
    x_rng = ((0, BQ, SEM_CX), (BQ, BQ + 2 * LNR, sem_last), (2 * BQ, S, SEM_MODR),
             (BQ + 2 * LNR, 2 * BQ, SEM_G + 1))
    x_cp = [cp(x_hbm.at[a:b], xbuf.at[a:b], sem.at[n]) for a, b, n in x_rng]
    mod_cp = [[cp(wm_hbm.at[:, o + MODC[n]:o + MODC[n + 1]], wmbuf.at[:, o + MODC[n]:o + MODC[n + 1]],
                  sem.at[SEM_MOD0 + n]) for o in (0, DM)] for n in range(len(MODC) - 1)]
    modr_cp = cp(wm_hbm.at[:, 2 * DM:], wmbuf.at[:, 2 * DM:6 * DM], sem.at[SEM_MODR])

    def head0_cps(h):
        sq, sk, sv = (SEM_A, SEM_A + 1, SEM_A + 2) if h == 0 else (SEM_H0 + h - 1,) * 3
        return [cp(wq_hbm.at[:, h * DH:(h + 1) * DH], wqbuf.at[0, :, h * DH:(h + 1) * DH], sem.at[sq]),
                cp(k_hbm.at[h], kbuf.at[h], sem.at[sk]),
                cp(v_hbm.at[h], vbuf.at[h], sem.at[sv])]

    wo0_cp = cp(wo_hbm.at[0], wobuf.at[0], sem.at[sem_last])

    def group_cps(g):
        sg = sem.at[SEM_G + g - 1]
        if isinstance(g, int):
            cols = slice(g * NH * DH, (g + 1) * NH * DH)
        else:
            cols = pl.ds(pl.multiple_of(g * (NH * DH), NH * DH), NH * DH)
        heads = pl.ds(g * NH, NH)
        return [cp(wq_hbm.at[:, cols], wqbuf.at[g], sg),
                cp(k_hbm.at[heads], kbuf.at[heads], sg),
                cp(v_hbm.at[heads], vbuf.at[heads], sg),
                cp(wo_hbm.at[g], wobuf.at[g], sg)]

    ffn_cp = [cp(wg_hbm, wgbuf, sem.at[SEM_FFN]), cp(wu_hbm, wubuf, sem.at[SEM_FFN]),
              cp(wd_hbm, wdbuf.at[:, 0:DM], sem.at[SEM_FFN])]

    def out_cp(j):
        if isinstance(j, int):
            rows = slice(j * BQ, (j + 1) * BQ)
        else:
            rows = pl.ds(pl.multiple_of(j * BQ, BQ), BQ)
        return cp(obuf.at[rows], out_hbm.at[rows], sem.at[SEM_OUT])

    c_cp.start()
    x_cp[0].start()
    for ds in mod_cp:
        for d in ds:
            d.start()
    for h in range(NH):
        for d in head0_cps(h):
            d.start()
    wo0_cp.start()
    x_cp[1].start()
    wr_cp.start()
    for g in range(1, NG):
        for d in group_cps(g):
            d.start()
        if g == 2:
            x_cp[3].start()
    modr_cp.start()
    x_cp[2].start()
    for d in ffn_cp:
        d.start()

    flag[0] = 0
    acc[1, :, 0:DM] = jnp.zeros((BQ, DM), F32)
    mod[:, 2 * DM:] = jnp.zeros((8, 4 * DM), F32)
    top[0] = jnp.full((8, 128), -jnp.inf, F32)
    top[1] = jnp.zeros((8, 128), F32)
    top[2] = jnp.full((8, 128), -jnp.inf, F32)
    top[3] = jnp.zeros((8, 128), F32)

    def silu_c():
        cf = cbuf[...].astype(F32)
        sc = cf * jax.nn.sigmoid(cf)
        return jnp.broadcast_to(sc, (16, DM)).astype(BF16)

    def mod_cols(sc, lo, hi):
        mod[:, lo:hi] = jnp.dot(sc, wmbuf[:, lo:hi], preferred_element_type=F32)[:8]

    def tie(val, dep):
        if dep is None:
            return val
        n = dep.shape[0]
        head = jnp.where(flag[0] != 0, dep, val[:n])
        return head if n == val.shape[0] else jnp.concatenate([head, val[n:]], axis=0)

    def ln1_apply(n, rows, lo=0, hi=DM):
        return n * (1.0 + _rows8(mod[:, DM + lo:DM + hi], rows)) + _rows8(mod[:, lo:hi], rows)

    def load_top():
        return top[0], top[1], top[2], top[3]

    def store_top(st):
        top[0], top[1], top[2], top[3] = st

    def ln2(a, row0, rows, valid, st):
        rs = pl.ds(row0, rows)
        x1 = xbuf[rs, :].astype(F32) + _rows8(mod[:, 2 * DM:3 * DM], rows) * a
        h2 = (_normalize(x1) * (1.0 + _rows8(mod[:, 4 * DM:5 * DM], rows))
              + _rows8(mod[:, 3 * DM:4 * DM], rows))
        h2buf[rs, :] = h2
        obuf[rs, :] = (x1 + _rows8(mod[:, 5 * DM:6 * DM], rows) * h2).astype(BF16)
        r = jnp.sum(h2 * _rows8(wr32[...], rows), axis=-1, keepdims=True)
        r = jnp.broadcast_to(r, (rows, 128))
        if valid is not None:
            r = jnp.where(valid, r, -jnp.inf)
        m1, i1, m2, i2 = st
        base = (lax.broadcasted_iota(jnp.int32, (8, 128), 0) + row0).astype(F32)
        for u in range(rows // 8):
            ru = r[u * 8:(u + 1) * 8]
            iu = base + float(u * 8)
            gt1 = ru > m1
            gt2 = ru > m2
            m2 = jnp.where(gt1, m1, jnp.where(gt2, ru, m2))
            i2 = jnp.where(gt1, i1, jnp.where(gt2, iu, i2))
            m1 = jnp.where(gt1, ru, m1)
            i1 = jnp.where(gt1, iu, i1)
        return m1, i1, m2, i2

    def qproj(g, c, h):
        q = jnp.dot(hn[c * TQ:(c + 1) * TQ, :], wqbuf[g, :, h * DH:(h + 1) * DH],
                    preferred_element_type=F32)
        return (q * QSCALE).astype(BF16)

    def qk(q, g, h):
        return lax.dot_general(q, kbuf[g * NH + h], NT, preferred_element_type=F32)

    def pv(s, g, h, dep=None, m=None):
        if m is None:
            m = jnp.max(s, axis=-1, keepdims=True)
        lsum = None
        parts = []
        for j in range(S // KG):
            ss = [s[:, j * KG + u * 128:j * KG + (u + 1) * 128] for u in range(KG // 128)]
            if j == 0:
                ss[0] = tie(ss[0], dep)
            ps = [jnp.exp2(z - m) for z in ss]
            t = (ps[0] + ps[1]) + (ps[2] + ps[3])
            lsum = t if lsum is None else lsum + t
            ps[-1] = jnp.minimum(ps[-1], lsum)
            parts += ps
        p = jnp.concatenate(parts, axis=-1).astype(BF16)
        return jnp.dot(p, vbuf[g * NH + h], preferred_element_type=F32), lsum

    def normalize_heads(res):
        gate = jnp.minimum(res[-1][0], 0.0)
        outs = []
        for o, lsum in res:
            l = jnp.sum(jnp.maximum(lsum, gate), axis=-1, keepdims=True)
            r = pl.reciprocal(l, approx=True)
            r = r * (2.0 - l * r)
            outs.append(o * r)
        return outs

    def woproj(slot, g, first, c, outs, lo, hi, dep=None, r0=0, r1=TQ):
        parts = [o[r0:r1] for o in outs]
        oc = jnp.concatenate([tie(parts[0], dep)] + parts[1:], axis=-1).astype(BF16)
        y = jnp.dot(oc, wobuf[g, :, lo:hi], preferred_element_type=F32)
        rows = slice(c * TQ + r0, c * TQ + r1)
        if first is True:
            acc[slot, rows, lo:hi] = y
        elif first is False:
            acc[slot, rows, lo:hi] = acc[slot, rows, lo:hi] + y
        else:
            acc[slot, rows, lo:hi] = jnp.where(first, 0.0, acc[slot, rows, lo:hi]) + y
        return y

    def ln1_piece(i, g, u, gate):
        pr = LNR // NP1
        if isinstance(i, int) and isinstance(g, int):
            row0, off = (i + 1) * BQ + g * LNR + u * pr, g * LNR + u * pr
        else:
            row0 = pl.multiple_of(jnp.minimum((i + 1) * BQ + g * LNR, S - LNR) + u * pr, pr)
            off = pl.multiple_of(g * LNR + u * pr, pr)
        xv = xbuf[pl.ds(row0, pr), :].astype(F32)
        xv = jnp.concatenate([tie(xv[:, 0:128], gate[0:pr, 0:128]), xv[:, 128:]], axis=-1)
        hv = ln1_apply(_normalize(xv), pr)
        hnext[pl.ds(off, pr), :] = hv.astype(BF16)
        return hv[:, 0:128]

    def wo_tail(i, g, slot, first, o0, o1):
        w = 256
        pieces = [(0, o0, lo) for lo in range(WB, DM, w)] + [(1, o1, lo) for lo in range(0, DM, w)]
        deps = {}
        for n, (c, o, lo) in enumerate(pieces):
            y = woproj(slot, g, first, c, o, lo, lo + w, deps.get(n))
            if n in LN1_AT:
                deps[n + 2] = ln1_piece(i, g, LN1_AT.index(n), y)

    def ln2_chunks(i, g, st):
        deps = []
        pr = LNR // NP2
        for u in range(NP2):
            off = g * LNR + u * pr
            if isinstance(i, int) and isinstance(g, int):
                row0, valid = (i - 1) * BQ + off, None
            else:
                row0 = pl.multiple_of(jnp.maximum(i - 1, 0) * BQ + off, pr)
                off = pl.multiple_of(off, pr)
                valid = i > 0
            st = ln2(acc[(i + 1) & 1, pl.ds(off, pr), 0:DM], row0, pr, valid, st)
            deps.append(st[3])
        return deps, st

    chains = [(c, h) for c in range(2) for h in range(NH)]

    def attention_step(i, g, slot, first):
        deps, st = ln2_chunks(i, g, load_top())
        store_top(st)
        pv_dep = {(0, h): deps[h * NP2 // NH] for h in range(0, NH, NH // NP2)}
        q = qproj(g, 0, 0)
        res = ([], [])
        o0 = None
        for n, (c, h) in enumerate(chains):
            s = qk(q, g, h)
            if n + 1 < len(chains):
                q = qproj(g, *chains[n + 1])
            if (c, h) == (1, 0):
                o0 = normalize_heads(res[0])
                woproj(slot, g, first, 0, o0, 0, WA)
            if (c, h) == (1, NH - 1):
                woproj(slot, g, first, 0, o0, WA, WB)
            res[c].append(pv(s, g, h, pv_dep.get((c, h))))
        o1 = normalize_heads(res[1])
        wo_tail(i, g, slot, first, o0, o1)

    c_cp.wait()
    x_cp[0].wait()
    sc = silu_c()
    acc[0, :, 0:DM] = _normalize(xbuf[0:BQ, :].astype(F32))
    for n in range(len(MODC) - 1):
        lo, hi = MODC[n], MODC[n + 1]
        for d in mod_cp[n]:
            d.wait()
        mod_cols(sc, lo, hi)
        mod_cols(sc, DM + lo, DM + hi)
        hn[:, lo:hi] = ln1_apply(acc[0, :, lo:hi], BQ, lo, hi).astype(BF16)

    wq_cp, k_cp, v_cp = head0_cps(0)
    wq_cp.wait()
    qa = qproj(0, 0, 0)
    qb = qproj(0, 1, 0)
    k_cp.wait()
    sa = qk(qa, 0, 0)
    s = qk(qb, 0, 0)
    ma = jnp.max(sa, axis=-1, keepdims=True)
    v_cp.wait()
    res = ([pv(sa, 0, 0, None, ma)], [pv(s, 0, 0)])
    for h in range(1, NH):
        for d in head0_cps(h):
            d.wait()
        if h + 1 == NH:
            wo0_cp.wait()
            x_cp[1].wait()
            wr_cp.wait()
        q = qproj(0, 0, h)
        if h > 1:
            res[1].append(pv(s, 0, h - 1))
        s = qk(q, 0, h)
        q = qproj(0, 1, h)
        res[0].append(pv(s, 0, h))
        s = qk(q, 0, h)
    o0 = normalize_heads(res[0])
    woproj(0, 0, True, 0, o0, 0, WB)
    res[1].append(pv(s, 0, NH - 1))
    wo_tail(0, 0, 0, True, o0, normalize_heads(res[1]))
    wr32[...] = jnp.broadcast_to(wrbuf[...].astype(F32).reshape(1, DM), (8, DM))

    def step(t, carry):
        i = lax.shift_right_logical(t, NG.bit_length() - 1)
        g = t & (NG - 1)

        @pl.when(jnp.logical_or(t < NG, g == 0))
        def _():
            @pl.when(t < NG)
            def _():
                for d in group_cps(g):
                    d.wait()

            @pl.when(t == 2)
            def _():
                x_cp[3].wait()

            @pl.when(t == NG)
            def _():
                modr_cp.wait()
                x_cp[2].wait()
                mod_cols(silu_c(), 2 * DM, 6 * DM)

            @pl.when(t >= 2 * NG)
            def _():
                out_cp(i - 2).start()

            @pl.when(g == 0)
            def _():
                hn[...] = hnext[...]

        attention_step(i, g, i & 1, g == 0)
        return carry

    lax.fori_loop(1, NSTEP, step, 0)

    out_cp(NQ - 2).start()
    for d in ffn_cp:
        d.wait()
    last = (NQ - 1) % 2
    st = load_top()
    for u in range(BQ // LNR):
        st = ln2(acc[last, u * LNR:(u + 1) * LNR, 0:DM], (NQ - 1) * BQ + u * LNR, LNR, None, st)
    out_cp(NQ - 1).start()

    m1, i1, m2, i2 = st
    big = float(S)
    v1 = jnp.max(m1, axis=0, keepdims=True)
    j1 = jnp.min(jnp.where(m1 == v1, i1, big), axis=0, keepdims=True)
    taken = i1 == j1
    m1b = jnp.where(taken, m2, m1)
    i1b = jnp.where(taken, i2, i1)
    v2 = jnp.max(m1b, axis=0, keepdims=True)
    j2 = jnp.min(jnp.where(m1b == v2, i1b, big), axis=0, keepdims=True)
    idx1 = jnp.clip(j1[0, 0].astype(jnp.int32), 0, S - 1)
    idx2 = jnp.clip(j2[0, 0].astype(jnp.int32), 0, S - 1)

    row = lax.broadcasted_iota(jnp.int32, (16, DM), 0)
    xs = jnp.where(row == 0, h2buf[pl.ds(idx1, 1), :], h2buf[pl.ds(idx2, 1), :]).astype(BF16)
    gt = jnp.dot(xs, wgbuf[...], preferred_element_type=F32)
    up = jnp.dot(xs, wubuf[...], preferred_element_type=F32)
    act = (gt * jax.nn.sigmoid(gt) * up).astype(BF16)
    y = jnp.dot(act, wdbuf[:, 0:DM], preferred_element_type=F32)
    gb = mod[0:1, 5 * DM:6 * DM]
    y1 = y[0:1, :] * jax.nn.sigmoid(v1[:, 0:1]) * gb
    y2 = y[1:2, :] * jax.nn.sigmoid(v2[:, 0:1]) * gb

    for j in range(NQ):
        out_cp(j).wait()

    base1 = pl.multiple_of((idx1 // FIX) * FIX, FIX)
    base2 = pl.multiple_of((idx2 // FIX) * FIX, FIX)

    def fix(base, idx, yy):
        rs = pl.ds(base, FIX)
        upd = jnp.where(row + base == idx, yy, 0.0)
        obuf[rs, :] = (obuf[rs, :].astype(F32) + upd).astype(BF16)

    fix(base1, idx1, y1)
    fix(base2, idx2, y2)
    fix1 = cp(obuf.at[pl.ds(base1, FIX)], out_hbm.at[pl.ds(base1, FIX)], sem.at[SEM_FIX])
    fix2 = cp(obuf.at[pl.ds(base2, FIX)], out_hbm.at[pl.ds(base2, FIX)], sem.at[SEM_FIX])
    fix1.start()

    @pl.when(base1 != base2)
    def _():
        fix2.start()
        fix2.wait()

    fix1.wait()


@jax.jit
def pallas_adaLN_cond__mha_block_cached__moe_arch_mod__prompt_kernel(
    A_x: jax.Array,
    A_k_cache: jax.Array,
    A_v_cache: jax.Array,
    A_wq: jax.Array,
    A_wo: jax.Array,
    B_x: jax.Array,
    B_w_r: jax.Array,
    B_w_gate: jax.Array,
    B_w_up: jax.Array,
    B_w_down: jax.Array,
    c: jax.Array,
    w_mod: jax.Array,
):
    del B_x
    x = A_x.reshape(S, DM)
    k = A_k_cache.reshape(H, S, DH)
    v = A_v_cache.reshape(H, S, DH)
    wo = A_wo.reshape(NG, NH * DH, DM)
    any_spec = pl.BlockSpec(memory_space=pl.ANY)
    out = pl.pallas_call(
        _kernel,
        in_specs=[any_spec] * 11,
        out_specs=any_spec,
        out_shape=jax.ShapeDtypeStruct((S, DM), BF16),
        scratch_shapes=[
            pltpu.VMEM((S, DM), BF16),
            pltpu.VMEM((H, S, DH), BF16),
            pltpu.VMEM((H, S, DH), BF16),
            pltpu.VMEM((NG, DM, NH * DH), BF16),
            pltpu.VMEM((NG, NH * DH, DM), BF16),
            pltpu.VMEM((DM,), BF16),
            pltpu.VMEM((DM, FF), BF16),
            pltpu.VMEM((DM, FF), BF16),
            pltpu.VMEM((FF, DM + PAD), BF16),
            pltpu.VMEM((1, DM), BF16),
            pltpu.VMEM((DM, 6 * DM + PAD), BF16),
            pltpu.VMEM((BQ, DM), BF16),
            pltpu.VMEM((BQ, DM), BF16),
            pltpu.VMEM((2, BQ, DM + PAD), F32),
            pltpu.VMEM((S, DM), F32),
            pltpu.VMEM((S, DM), BF16),
            pltpu.VMEM((8, 6 * DM), F32),
            pltpu.VMEM((8, DM), F32),
            pltpu.VMEM((4, 8, 128), F32),
            pltpu.SMEM((1,), jnp.int32),
            pltpu.SemaphoreType.DMA((NSEM,)),
        ],
        compiler_params=pltpu.CompilerParams(vmem_limit_bytes=124 * 1024 * 1024),
        name="adaln_mha_moe",
    )(x, k, v, A_wq, wo, B_w_r, B_w_gate, B_w_up, B_w_down, c, w_mod)
    return out.reshape(1, S, DM)
```

```python
import jax
import jax.numpy as jnp
from jax import lax
import jax.experimental.pallas as pl
import jax.experimental.pallas.tpu as pltpu

F32 = jnp.float32
BF16 = jnp.bfloat16

S = 2048
DM = 1024
H = 32
DH = 128
FF = 3584
BQ = 512
TQ = 256
NH = 4
NQ = S // BQ
NG = H // NH
NSTEP = NQ * NG
LAST0 = S - BQ
LNR = BQ // NG
LN1_AT = (0, 1, 2, 3)
NP1 = len(LN1_AT)
WA, WB = 256, 512
NP2 = 4
NFC = 14
NOUT = 8
LRW = 16
ORW = 16
KG = 512
EPS = 1e-5
QSCALE = DH ** -0.5 * 1.4426950408889634
NT = (((1,), (1,)), ((), ()))
FIX = 16
PAD = 128

SEM_CX = 0
MODC = (0, 512, 896, 1024)
SEM_MOD0 = 1
SEM_A = SEM_MOD0 + len(MODC) - 1
SEM_H0 = SEM_A + 3
SEM_G = SEM_H0 + NH - 1
SEM_MODR = SEM_G + NG - 1
SEM_FFN = SEM_MODR + 1
SEM_OUT = SEM_FFN + 1
SEM_FIX = SEM_OUT + 1
NSEM = SEM_FIX + 1


def _rows8(v, rows):
    return jnp.tile(v, (rows // 8, 1))


def _normalize(x):
    mean = jnp.sum(x, axis=-1, keepdims=True) * (1.0 / DM)
    xc = x - mean
    var = jnp.sum(xc * xc, axis=-1, keepdims=True) * (1.0 / DM)
    return xc * lax.rsqrt(var + EPS)


def _kernel(x_hbm, k_hbm, v_hbm, wq_hbm, wo_hbm, wr_hbm, wg_hbm, wu_hbm, wd_hbm, c_hbm, wm_hbm,
            out_hbm,
            xbuf, kbuf, vbuf, wqbuf, wobuf, wrbuf, wgbuf, wubuf, wdbuf, cbuf, wmbuf,
            hn, hnext, acc, nbuf, stat, obuf, mod, vec, top, flag, sem):
    cp = pltpu.make_async_copy

    sem_last = SEM_H0 + NH - 2
    c_cp = cp(c_hbm, cbuf, sem.at[SEM_CX])
    wr_cp = cp(wr_hbm, wrbuf, sem.at[SEM_MODR])
    x_rng = ((0, BQ, SEM_CX), (BQ, BQ + 2 * LNR, sem_last), (2 * BQ, S, SEM_MODR),
             (BQ + 2 * LNR, 2 * BQ, SEM_G + 1))
    x_cp = [cp(x_hbm.at[a:b], xbuf.at[a:b], sem.at[n]) for a, b, n in x_rng]
    mod_cp = [[cp(wm_hbm.at[:, o + MODC[n]:o + MODC[n + 1]], wmbuf.at[:, o + MODC[n]:o + MODC[n + 1]],
                  sem.at[SEM_MOD0 + n]) for o in (0, DM)] for n in range(len(MODC) - 1)]
    modr_cp = cp(wm_hbm.at[:, 2 * DM:], wmbuf.at[:, 2 * DM:6 * DM], sem.at[SEM_MODR])

    def head0_cps(h):
        sq, sk, sv = (SEM_A, SEM_A + 1, SEM_A + 2) if h == 0 else (SEM_H0 + h - 1,) * 3
        return [cp(wq_hbm.at[:, h * DH:(h + 1) * DH], wqbuf.at[0, :, h * DH:(h + 1) * DH], sem.at[sq]),
                cp(k_hbm.at[h], kbuf.at[h], sem.at[sk]),
                cp(v_hbm.at[h], vbuf.at[h], sem.at[sv])]

    wo0_cp = cp(wo_hbm.at[0], wobuf.at[0], sem.at[sem_last])

    def group_cps(g):
        sg = sem.at[SEM_G + g - 1]
        if isinstance(g, int):
            cols = slice(g * NH * DH, (g + 1) * NH * DH)
        else:
            cols = pl.ds(pl.multiple_of(g * (NH * DH), NH * DH), NH * DH)
        heads = pl.ds(g * NH, NH)
        return [cp(wq_hbm.at[:, cols], wqbuf.at[g], sg),
                cp(k_hbm.at[heads], kbuf.at[heads], sg),
                cp(v_hbm.at[heads], vbuf.at[heads], sg),
                cp(wo_hbm.at[g], wobuf.at[g], sg)]

    ffn_cp = [cp(wg_hbm, wgbuf, sem.at[SEM_FFN]), cp(wu_hbm, wubuf, sem.at[SEM_FFN]),
              cp(wd_hbm, wdbuf.at[:, 0:DM], sem.at[SEM_FFN])]

    def out_cp(j):
        if isinstance(j, int):
            rows = slice(j * BQ, (j + 1) * BQ)
        else:
            rows = pl.ds(pl.multiple_of(j * BQ, BQ), BQ)
        return cp(obuf.at[rows], out_hbm.at[rows], sem.at[SEM_OUT])

    c_cp.start()
    x_cp[0].start()
    for ds in mod_cp:
        for d in ds:
            d.start()
    for h in range(NH):
        for d in head0_cps(h):
            d.start()
    wo0_cp.start()
    x_cp[1].start()
    wr_cp.start()
    for g in range(1, NG):
        for d in group_cps(g):
            d.start()
        if g == 2:
            x_cp[3].start()
    modr_cp.start()
    x_cp[2].start()
    for d in ffn_cp:
        d.start()

    flag[0] = 0
    acc[1, :, 0:DM] = jnp.zeros((BQ, DM), F32)
    mod[:, 2 * DM:] = jnp.zeros((8, 4 * DM), F32)
    vec[...] = jnp.zeros((4, 8, DM), F32)
    top[0] = jnp.full((8, 128), -jnp.inf, F32)
    top[1] = jnp.zeros((8, 128), F32)
    top[2] = jnp.full((8, 128), -jnp.inf, F32)
    top[3] = jnp.zeros((8, 128), F32)

    def silu_c():
        cf = cbuf[...].astype(F32)
        sc = cf * jax.nn.sigmoid(cf)
        return jnp.broadcast_to(sc, (16, DM)).astype(BF16)

    def mod_cols(sc, lo, hi):
        mod[:, lo:hi] = jnp.dot(sc, wmbuf[:, lo:hi], preferred_element_type=F32)[:8]

    def tie(val, dep):
        if dep is None:
            return val
        n = dep.shape[0]
        head = jnp.where(flag[0] != 0, dep, val[:n])
        return head if n == val.shape[0] else jnp.concatenate([head, val[n:]], axis=0)

    def ln1_apply(n, rows, lo=0, hi=DM):
        return n * (1.0 + _rows8(mod[:, DM + lo:DM + hi], rows)) + _rows8(mod[:, lo:hi], rows)

    def load_top():
        return top[0], top[1], top[2], top[3]

    def store_top(st):
        top[0], top[1], top[2], top[3] = st

    def fold_vectors():
        sb, cb1, gb = mod[:, 3 * DM:4 * DM], 1.0 + mod[:, 4 * DM:5 * DM], mod[:, 5 * DM:6 * DM]
        wr = jnp.broadcast_to(wrbuf[...].astype(F32).reshape(1, DM), (8, DM))
        vec[0] = gb * cb1
        vec[1] = gb * sb
        vec[2] = cb1 * wr
        vec[3] = jnp.broadcast_to(jnp.sum(sb * wr, axis=-1, keepdims=True), (8, DM))

    def ln2_out(x1, n, row0, rows):
        out = x1 + n * _rows8(vec[0], rows) + _rows8(vec[1], rows)
        obuf[pl.ds(row0, rows), :] = out.astype(BF16)
        return out

    def ln2(a, row0, rows, valid, st, finish=True):
        rs = pl.ds(row0, rows)
        x1 = xbuf[rs, :].astype(F32) + _rows8(mod[:, 2 * DM:3 * DM], rows) * a
        mean = jnp.sum(x1, axis=-1, keepdims=True) * (1.0 / DM)
        xc = x1 - mean
        var = jnp.sum(xc * xc, axis=-1, keepdims=True) * (1.0 / DM)
        rstd = lax.rsqrt(var + EPS)
        if finish:
            n = xc * rstd
            nbuf[rs, :] = n
            ln2_out(x1, n, row0, rows)
        else:
            nbuf[rs, :] = x1
            stat[0, pl.ds(row0 - LAST0, rows), :] = jnp.broadcast_to(mean, (rows, 128))
            stat[1, pl.ds(row0 - LAST0, rows), :] = jnp.broadcast_to(rstd, (rows, 128))
        r = jnp.sum(xc * _rows8(vec[2], rows), axis=-1, keepdims=True) * rstd
        r = r + _rows8(vec[3, :, 0:128], rows)
        if valid is not None:
            r = jnp.where(valid, r, -jnp.inf)
        m1, i1, m2, i2 = st
        base = (lax.broadcasted_iota(jnp.int32, (8, 128), 0) + row0).astype(F32)
        for u in range(rows // 8):
            ru = r[u * 8:(u + 1) * 8]
            iu = base + float(u * 8)
            gt1 = ru > m1
            gt2 = ru > m2
            m2 = jnp.where(gt1, m1, jnp.where(gt2, ru, m2))
            i2 = jnp.where(gt1, i1, jnp.where(gt2, iu, i2))
            m1 = jnp.where(gt1, ru, m1)
            i1 = jnp.where(gt1, iu, i1)
        return m1, i1, m2, i2

    def qproj(g, c, h):
        q = jnp.dot(hn[c * TQ:(c + 1) * TQ, :], wqbuf[g, :, h * DH:(h + 1) * DH],
                    preferred_element_type=F32)
        return (q * QSCALE).astype(BF16)

    def qk(q, g, h):
        return lax.dot_general(q, kbuf[g * NH + h], NT, preferred_element_type=F32)

    def pv(s, g, h, dep=None, m=None):
        if m is None:
            m = jnp.max(s, axis=-1, keepdims=True)
        lsum = None
        parts = []
        for j in range(S // KG):
            ss = [s[:, j * KG + u * 128:j * KG + (u + 1) * 128] for u in range(KG // 128)]
            if j == 0:
                ss[0] = tie(ss[0], dep)
            ps = [jnp.exp2(z - m) for z in ss]
            t = (ps[0] + ps[1]) + (ps[2] + ps[3])
            lsum = t if lsum is None else lsum + t
            ps[-1] = jnp.minimum(ps[-1], lsum)
            parts += ps
        p = jnp.concatenate(parts, axis=-1).astype(BF16)
        return jnp.dot(p, vbuf[g * NH + h], preferred_element_type=F32), lsum

    def normalize_heads(res):
        gate = jnp.minimum(res[-1][0], 0.0)
        outs = []
        for o, lsum in res:
            l = jnp.sum(jnp.maximum(lsum, gate), axis=-1, keepdims=True)
            r = pl.reciprocal(l, approx=True)
            r = r * (2.0 - l * r)
            outs.append(o * r)
        return outs

    def woproj(slot, g, first, c, outs, lo, hi, dep=None, r0=0, r1=TQ):
        parts = [o[r0:r1] for o in outs]
        oc = jnp.concatenate([tie(parts[0], dep)] + parts[1:], axis=-1).astype(BF16)
        y = jnp.dot(oc, wobuf[g, :, lo:hi], preferred_element_type=F32)
        rows = slice(c * TQ + r0, c * TQ + r1)
        if first is True:
            acc[slot, rows, lo:hi] = y
        elif first is False:
            acc[slot, rows, lo:hi] = acc[slot, rows, lo:hi] + y
        else:
            acc[slot, rows, lo:hi] = jnp.where(first, 0.0, acc[slot, rows, lo:hi]) + y
        return y

    def ln1_piece(i, g, u, gate):
        pr = LNR // NP1
        if isinstance(i, int) and isinstance(g, int):
            row0, off = (i + 1) * BQ + g * LNR + u * pr, g * LNR + u * pr
        else:
            row0 = pl.multiple_of(jnp.minimum((i + 1) * BQ + g * LNR, S - LNR) + u * pr, pr)
            off = pl.multiple_of(g * LNR + u * pr, pr)
        xv = xbuf[pl.ds(row0, pr), :].astype(F32)
        xv = jnp.concatenate([tie(xv[:, 0:128], gate[0:pr, 0:128]), xv[:, 128:]], axis=-1)
        hv = ln1_apply(_normalize(xv), pr)
        hnext[pl.ds(off, pr), :] = hv.astype(BF16)
        return hv[:, 0:128]

    def wo_tail(i, g, slot, first, o0, o1):
        w = 256
        pieces = [(0, o0, lo) for lo in range(WB, DM, w)] + [(1, o1, lo) for lo in range(0, DM, w)]
        deps = {}
        for n, (c, o, lo) in enumerate(pieces):
            y = woproj(slot, g, first, c, o, lo, lo + w, deps.get(n))
            if n in LN1_AT:
                deps[n + 2] = ln1_piece(i, g, LN1_AT.index(n), y)

    def ln2_chunks(i, g):
        st = load_top()
        deps = []
        for u in range(LNR // LRW):
            off = pl.multiple_of(g * LNR + u * LRW, LRW)
            row0 = pl.multiple_of(jnp.maximum(i - 1, 0) * BQ + off, LRW)
            st = ln2(acc[(i + 1) & 1, pl.ds(off, LRW), 0:DM], row0, LRW, i > 0, st)
            if ((u + 1) * LRW) % (LNR // NP2) == 0:
                deps.append(st[3])
        store_top(st)
        return deps

    chains = [(c, h) for c in range(2) for h in range(NH)]

    def attention_step(i, g, slot, first):
        pv_dep = {(0, u): d for u, d in enumerate(ln2_chunks(i, g))}
        q = qproj(g, 0, 0)
        res = ([], [])
        o0 = None
        for n, (c, h) in enumerate(chains):
            s = qk(q, g, h)
            if n + 1 < len(chains):
                q = qproj(g, *chains[n + 1])
            if (c, h) == (1, 0):
                o0 = normalize_heads(res[0])
                woproj(slot, g, first, 0, o0, 0, WA)
            if (c, h) == (1, NH - 1):
                woproj(slot, g, first, 0, o0, WA, WB)
            res[c].append(pv(s, g, h, pv_dep.get((c, h))))
        o1 = normalize_heads(res[1])
        wo_tail(i, g, slot, first, o0, o1)

    c_cp.wait()
    x_cp[0].wait()
    sc = silu_c()
    acc[0, :, 0:DM] = _normalize(xbuf[0:BQ, :].astype(F32))
    for n in range(len(MODC) - 1):
        lo, hi = MODC[n], MODC[n + 1]
        for d in mod_cp[n]:
            d.wait()
        mod_cols(sc, lo, hi)
        mod_cols(sc, DM + lo, DM + hi)
        hn[:, lo:hi] = ln1_apply(acc[0, :, lo:hi], BQ, lo, hi).astype(BF16)

    wq_cp, k_cp, v_cp = head0_cps(0)
    wq_cp.wait()
    qa = qproj(0, 0, 0)
    qb = qproj(0, 1, 0)
    k_cp.wait()
    sa = qk(qa, 0, 0)
    s = qk(qb, 0, 0)
    ma = jnp.max(sa, axis=-1, keepdims=True)
    v_cp.wait()
    res = ([pv(sa, 0, 0, None, ma)], [pv(s, 0, 0)])
    for h in range(1, NH):
        for d in head0_cps(h):
            d.wait()
        if h + 1 == NH:
            wo0_cp.wait()
            x_cp[1].wait()
        q = qproj(0, 0, h)
        if h > 1:
            res[1].append(pv(s, 0, h - 1))
        s = qk(q, 0, h)
        q = qproj(0, 1, h)
        res[0].append(pv(s, 0, h))
        s = qk(q, 0, h)
    o0 = normalize_heads(res[0])
    woproj(0, 0, True, 0, o0, 0, WB)
    res[1].append(pv(s, 0, NH - 1))
    wo_tail(0, 0, 0, True, o0, normalize_heads(res[1]))

    def step(t, carry):
        i = lax.shift_right_logical(t, NG.bit_length() - 1)
        g = t & (NG - 1)

        @pl.when(jnp.logical_or(t < NG, g == 0))
        def _():
            @pl.when(t < NG)
            def _():
                for d in group_cps(g):
                    d.wait()

            @pl.when(t == 2)
            def _():
                x_cp[3].wait()

            @pl.when(t == NG)
            def _():
                modr_cp.wait()
                x_cp[2].wait()
                wr_cp.wait()
                mod_cols(silu_c(), 2 * DM, 6 * DM)
                fold_vectors()

            @pl.when(t >= 2 * NG)
            def _():
                out_cp(i - 2).start()

            @pl.when(g == 0)
            def _():
                hn[...] = hnext[...]

        attention_step(i, g, i & 1, g == 0)
        return carry

    lax.fori_loop(1, NSTEP, step, 0)

    out_cp(NQ - 2).start()
    for d in ffn_cp:
        d.wait()
    last = (NQ - 1) % 2
    st = load_top()
    for u in range(BQ // LNR):
        st = ln2(acc[last, u * LNR:(u + 1) * LNR, 0:DM], LAST0 + u * LNR, LNR, None, st, False)

    m1, i1, m2, i2 = st
    big = float(S)
    v1 = jnp.max(m1, axis=0, keepdims=True)
    j1 = jnp.min(jnp.where(m1 == v1, i1, big), axis=0, keepdims=True)
    taken = i1 == j1
    m1b = jnp.where(taken, m2, m1)
    i1b = jnp.where(taken, i2, i1)
    v2 = jnp.max(m1b, axis=0, keepdims=True)
    j2 = jnp.min(jnp.where(m1b == v2, i1b, big), axis=0, keepdims=True)
    idx1 = jnp.clip(j1[0, 0].astype(jnp.int32), 0, S - 1)
    idx2 = jnp.clip(j2[0, 0].astype(jnp.int32), 0, S - 1)

    row = lax.broadcasted_iota(jnp.int32, (16, DM), 0)
    def routed_row(idx):
        late = idx >= LAST0
        k = jnp.maximum(idx - LAST0, 0)
        mean = jnp.where(late, stat[0, pl.ds(k, 1), :], 0.0)
        rstd = jnp.where(late, stat[1, pl.ds(k, 1), :], 1.0)
        return (nbuf[pl.ds(idx, 1), :] - jnp.tile(mean, (1, DM // 128))) * jnp.tile(rstd, (1, DM // 128))

    xs = (jnp.where(row == 0, routed_row(idx1), routed_row(idx2))
          * (1.0 + _rows8(mod[:, 4 * DM:5 * DM], 16)) + _rows8(mod[:, 3 * DM:4 * DM], 16))

    FC = FF // NFC
    acts = []
    deps = {}
    for n in range(NFC):
        cols = slice(n * FC, (n + 1) * FC)
        xb = jnp.concatenate([tie(xs[:, 0:128], deps.get(n)), xs[:, 128:]], axis=-1).astype(BF16)
        gt = jnp.dot(xb, wgbuf[:, cols], preferred_element_type=F32)
        up = jnp.dot(xb, wubuf[:, cols], preferred_element_type=F32)
        acts.append((gt * jax.nn.sigmoid(gt) * up).astype(BF16))
        if n < NOUT:
            dep = None
            for u in range(BQ // NOUT // ORW):
                r0 = n * (BQ // NOUT) + u * ORW
                x1 = nbuf[LAST0 + r0:LAST0 + r0 + ORW, :]
                mean = tie(stat[0, r0:r0 + ORW, :], gt[0:ORW, 0:128])
                nv = ((x1 - jnp.tile(mean, (1, DM // 128)))
                      * jnp.tile(stat[1, r0:r0 + ORW, :], (1, DM // 128)))
                o = ln2_out(x1, nv, LAST0 + r0, ORW)[:, DM - 128:]
                dep = o if dep is None else jnp.maximum(dep, o)
            deps[n + 2] = dep
            if n + 1 == NOUT:
                out_cp(NQ - 1).start()
    y = jnp.dot(jnp.concatenate(acts, axis=-1), wdbuf[:, 0:DM], preferred_element_type=F32)
    gb = mod[0:1, 5 * DM:6 * DM]
    y1 = y[0:1, :] * jax.nn.sigmoid(v1[:, 0:1]) * gb
    y2 = y[1:2, :] * jax.nn.sigmoid(v2[:, 0:1]) * gb

    for j in range(NQ):
        out_cp(j).wait()

    base1 = pl.multiple_of((idx1 // FIX) * FIX, FIX)
    base2 = pl.multiple_of((idx2 // FIX) * FIX, FIX)

    def fix(base, idx, yy):
        rs = pl.ds(base, FIX)
        upd = jnp.where(row + base == idx, yy, 0.0)
        obuf[rs, :] = (obuf[rs, :].astype(F32) + upd).astype(BF16)

    fix(base1, idx1, y1)
    fix(base2, idx2, y2)
    fix1 = cp(obuf.at[pl.ds(base1, FIX)], out_hbm.at[pl.ds(base1, FIX)], sem.at[SEM_FIX])
    fix2 = cp(obuf.at[pl.ds(base2, FIX)], out_hbm.at[pl.ds(base2, FIX)], sem.at[SEM_FIX])
    fix1.start()

    @pl.when(base1 != base2)
    def _():
        fix2.start()
        fix2.wait()

    fix1.wait()


@jax.jit
def pallas_adaLN_cond__mha_block_cached__moe_arch_mod__prompt_kernel(
    A_x: jax.Array,
    A_k_cache: jax.Array,
    A_v_cache: jax.Array,
    A_wq: jax.Array,
    A_wo: jax.Array,
    B_x: jax.Array,
    B_w_r: jax.Array,
    B_w_gate: jax.Array,
    B_w_up: jax.Array,
    B_w_down: jax.Array,
    c: jax.Array,
    w_mod: jax.Array,
):
    del B_x
    x = A_x.reshape(S, DM)
    k = A_k_cache.reshape(H, S, DH)
    v = A_v_cache.reshape(H, S, DH)
    wo = A_wo.reshape(NG, NH * DH, DM)
    any_spec = pl.BlockSpec(memory_space=pl.ANY)
    out = pl.pallas_call(
        _kernel,
        in_specs=[any_spec] * 11,
        out_specs=any_spec,
        out_shape=jax.ShapeDtypeStruct((S, DM), BF16),
        scratch_shapes=[
            pltpu.VMEM((S, DM), BF16),
            pltpu.VMEM((H, S, DH), BF16),
            pltpu.VMEM((H, S, DH), BF16),
            pltpu.VMEM((NG, DM, NH * DH), BF16),
            pltpu.VMEM((NG, NH * DH, DM), BF16),
            pltpu.VMEM((DM,), BF16),
            pltpu.VMEM((DM, FF), BF16),
            pltpu.VMEM((DM, FF), BF16),
            pltpu.VMEM((FF, DM + PAD), BF16),
            pltpu.VMEM((1, DM), BF16),
            pltpu.VMEM((DM, 6 * DM + PAD), BF16),
            pltpu.VMEM((BQ, DM), BF16),
            pltpu.VMEM((BQ, DM), BF16),
            pltpu.VMEM((2, BQ, DM + PAD), F32),
            pltpu.VMEM((S, DM), F32),
            pltpu.VMEM((2, BQ, 128), F32),
            pltpu.VMEM((S, DM), BF16),
            pltpu.VMEM((8, 6 * DM), F32),
            pltpu.VMEM((4, 8, DM), F32),
            pltpu.VMEM((4, 8, 128), F32),
            pltpu.SMEM((1,), jnp.int32),
            pltpu.SemaphoreType.DMA((NSEM,)),
        ],
        compiler_params=pltpu.CompilerParams(vmem_limit_bytes=124 * 1024 * 1024),
        name="adaln_mha_moe",
    )(x, k, v, A_wq, wo, B_w_r, B_w_gate, B_w_up, B_w_down, c, w_mod)
    return out.reshape(1, S, DM)
```

```python
import jax
import jax.numpy as jnp
from jax import lax
import jax.experimental.pallas as pl
import jax.experimental.pallas.tpu as pltpu

F32 = jnp.float32
BF16 = jnp.bfloat16

S = 2048
DM = 1024
H = 32
DH = 128
FF = 3584
BQ = 512
TQ = 256
NH = 4
NQ = S // BQ
NG = H // NH
NSTEP = NQ * NG
LAST0 = S - BQ
LNR = BQ // NG
LN1_AT = (0, 1, 2, 3)
NP1 = len(LN1_AT)
WA, WB = 256, 512
NP2 = 4
NFC = 14
NOUT = 8
LRW = 16
ORW = 16
KG = 512
EPS = 1e-5
QSCALE = DH ** -0.5 * 1.4426950408889634
NT = (((1,), (1,)), ((), ()))
FIX = 16
PAD = 128

SEM_CX = 0
MODC = (0, 512, 896, 1024)
SEM_MOD0 = 1
SEM_A = SEM_MOD0 + len(MODC) - 1
SEM_H0 = SEM_A + 3
GWAIT = (1, 2, 3, 5)
SEM_G = SEM_H0 + NH - 1
SEM_REST = SEM_G + len(GWAIT)
NSEM = SEM_REST + 1
SEM_OUT = SEM_CX
SEM_FIX = SEM_MOD0


def _rows8(v, rows):
    return jnp.tile(v, (rows // 8, 1))


def _normalize(x):
    mean = jnp.sum(x, axis=-1, keepdims=True) * (1.0 / DM)
    xc = x - mean
    var = jnp.sum(xc * xc, axis=-1, keepdims=True) * (1.0 / DM)
    return xc * lax.rsqrt(var + EPS)


def _kernel(x_hbm, k_hbm, v_hbm, wq_hbm, wo_hbm, wr_hbm, wg_hbm, wu_hbm, wd_hbm, c_hbm, wm_hbm,
            out_hbm,
            xbuf, kbuf, vbuf, wqbuf, wobuf, wrbuf, wgbuf, wubuf, wdbuf, cbuf, wmbuf,
            hn, hnext, acc, nbuf, stat, obuf, fixbuf, mod, vec, top, flag, sem):
    cp = pltpu.make_async_copy

    sem_last = SEM_H0 + NH - 2
    c_cp = cp(c_hbm, cbuf, sem.at[SEM_CX])
    wr_cp = cp(wr_hbm, wrbuf, sem.at[SEM_REST])
    x_rng = ((0, BQ, SEM_CX), (BQ, BQ + 2 * LNR, sem_last), (2 * BQ, S, SEM_REST),
             (BQ + 2 * LNR, 2 * BQ, SEM_G + 1))
    x_cp = [cp(x_hbm.at[a:b], xbuf.at[a:b], sem.at[n]) for a, b, n in x_rng]
    mod_cp = [[cp(wm_hbm.at[:, o + MODC[n]:o + MODC[n + 1]], wmbuf.at[:, o + MODC[n]:o + MODC[n + 1]],
                  sem.at[SEM_MOD0 + n]) for o in (0, DM)] for n in range(len(MODC) - 1)]
    modr_cp = cp(wm_hbm.at[:, 2 * DM:], wmbuf.at[:, 2 * DM:6 * DM], sem.at[SEM_REST])

    def head0_cps(h):
        sq, sk, sv = (SEM_A, SEM_A + 1, SEM_A + 2) if h == 0 else (SEM_H0 + h - 1,) * 3
        return [cp(wq_hbm.at[:, h * DH:(h + 1) * DH], wqbuf.at[0, :, h * DH:(h + 1) * DH], sem.at[sq]),
                cp(k_hbm.at[h], kbuf.at[h], sem.at[sk]),
                cp(v_hbm.at[h], vbuf.at[h], sem.at[sv])]

    wo0_cp = cp(wo_hbm.at[0], wobuf.at[0], sem.at[sem_last])

    def group_cps(g):
        sg = sem.at[SEM_G + max(n for n, t in enumerate(GWAIT) if t <= g)]
        heads = slice(g * NH, (g + 1) * NH)
        return [cp(wq_hbm.at[:, g * NH * DH:(g + 1) * NH * DH], wqbuf.at[g], sg),
                cp(k_hbm.at[heads], kbuf.at[heads], sg),
                cp(v_hbm.at[heads], vbuf.at[heads], sg),
                cp(wo_hbm.at[g], wobuf.at[g], sg)]

    ffn_cp = [cp(wg_hbm, wgbuf, sem.at[SEM_REST]), cp(wu_hbm, wubuf, sem.at[SEM_REST]),
              cp(wd_hbm, wdbuf.at[:, 0:DM], sem.at[SEM_REST])]

    def out_cp(j):
        if isinstance(j, int):
            rows = slice(j * BQ, (j + 1) * BQ)
        else:
            rows = pl.ds(pl.multiple_of(j * BQ, BQ), BQ)
        return cp(obuf.at[rows], out_hbm.at[rows], sem.at[SEM_OUT])

    c_cp.start()
    x_cp[0].start()
    for ds in mod_cp:
        for d in ds:
            d.start()
    for h in range(NH):
        for d in head0_cps(h):
            d.start()
    wo0_cp.start()
    x_cp[1].start()
    wr_cp.start()
    for g in range(1, NG):
        for d in group_cps(g):
            d.start()
        if g == 2:
            x_cp[3].start()
    modr_cp.start()
    x_cp[2].start()
    for d in ffn_cp:
        d.start()

    flag[0] = 0
    acc[1, :, 0:DM] = jnp.zeros((BQ, DM), F32)
    mod[:, 2 * DM:] = jnp.zeros((8, 4 * DM), F32)
    vec[...] = jnp.zeros((4, 8, DM), F32)
    top[0] = jnp.full((8, 128), -jnp.inf, F32)
    top[1] = jnp.zeros((8, 128), F32)
    top[2] = jnp.full((8, 128), -jnp.inf, F32)
    top[3] = jnp.zeros((8, 128), F32)

    def silu_c():
        cf = cbuf[...].astype(F32)
        sc = cf * jax.nn.sigmoid(cf)
        return jnp.broadcast_to(sc, (16, DM)).astype(BF16)

    def mod_cols(sc, lo, hi):
        mod[:, lo:hi] = jnp.dot(sc, wmbuf[:, lo:hi], preferred_element_type=F32)[:8]

    def tie(val, dep):
        if dep is None:
            return val
        n = dep.shape[0]
        head = jnp.where(flag[0] != 0, dep, val[:n])
        return head if n == val.shape[0] else jnp.concatenate([head, val[n:]], axis=0)

    def ln1_apply(n, rows, lo=0, hi=DM):
        return n * (1.0 + _rows8(mod[:, DM + lo:DM + hi], rows)) + _rows8(mod[:, lo:hi], rows)

    def load_top():
        return top[0], top[1], top[2], top[3]

    def store_top(st):
        top[0], top[1], top[2], top[3] = st

    def fold_vectors():
        sb, cb1, gb = mod[:, 3 * DM:4 * DM], 1.0 + mod[:, 4 * DM:5 * DM], mod[:, 5 * DM:6 * DM]
        wr = jnp.broadcast_to(wrbuf[...].astype(F32).reshape(1, DM), (8, DM))
        vec[0] = gb * cb1
        vec[1] = gb * sb
        vec[2] = cb1 * wr
        vec[3] = jnp.broadcast_to(jnp.sum(sb * wr, axis=-1, keepdims=True), (8, DM))

    def ln2_out(x1, n, row0, rows):
        out = x1 + n * _rows8(vec[0], rows) + _rows8(vec[1], rows)
        obuf[pl.ds(row0, rows), :] = out.astype(BF16)
        return out

    def ln2(a, row0, rows, valid, st, finish=True):
        rs = pl.ds(row0, rows)
        x1 = xbuf[rs, :].astype(F32) + _rows8(mod[:, 2 * DM:3 * DM], rows) * a
        mean = jnp.sum(x1, axis=-1, keepdims=True) * (1.0 / DM)
        xc = x1 - mean
        var = jnp.sum(xc * xc, axis=-1, keepdims=True) * (1.0 / DM)
        rstd = lax.rsqrt(var + EPS)
        if finish:
            n = xc * rstd
            nbuf[rs, :] = n
            ln2_out(x1, n, row0, rows)
        else:
            nbuf[rs, :] = x1
            stat[0, pl.ds(row0 - LAST0, rows), :] = jnp.broadcast_to(mean, (rows, 128))
            stat[1, pl.ds(row0 - LAST0, rows), :] = jnp.broadcast_to(rstd, (rows, 128))
        r = jnp.sum(xc * _rows8(vec[2], rows), axis=-1, keepdims=True) * rstd
        r = r + _rows8(vec[3, :, 0:128], rows)
        if valid is not None:
            r = jnp.where(valid, r, -jnp.inf)
        m1, i1, m2, i2 = st
        base = (lax.broadcasted_iota(jnp.int32, (8, 128), 0) + row0).astype(F32)
        for u in range(rows // 8):
            ru = r[u * 8:(u + 1) * 8]
            iu = base + float(u * 8)
            gt1 = ru > m1
            gt2 = ru > m2
            m2 = jnp.where(gt1, m1, jnp.where(gt2, ru, m2))
            i2 = jnp.where(gt1, i1, jnp.where(gt2, iu, i2))
            m1 = jnp.where(gt1, ru, m1)
            i1 = jnp.where(gt1, iu, i1)
        return m1, i1, m2, i2

    def qproj(g, c, h):
        q = jnp.dot(hn[c * TQ:(c + 1) * TQ, :], wqbuf[g, :, h * DH:(h + 1) * DH],
                    preferred_element_type=F32)
        return (q * QSCALE).astype(BF16)

    def qk(q, g, h):
        return lax.dot_general(q, kbuf[g * NH + h], NT, preferred_element_type=F32)

    def pv(s, g, h, dep=None, m=None):
        if m is None:
            m = jnp.max(s, axis=-1, keepdims=True)
        lsum = None
        parts = []
        for j in range(S // KG):
            ss = [s[:, j * KG + u * 128:j * KG + (u + 1) * 128] for u in range(KG // 128)]
            if j == 0:
                ss[0] = tie(ss[0], dep)
            ps = [jnp.exp2(z - m) for z in ss]
            t = (ps[0] + ps[1]) + (ps[2] + ps[3])
            lsum = t if lsum is None else lsum + t
            ps[-1] = jnp.minimum(ps[-1], lsum)
            parts += ps
        p = jnp.concatenate(parts, axis=-1).astype(BF16)
        return jnp.dot(p, vbuf[g * NH + h], preferred_element_type=F32), lsum

    def normalize_heads(res):
        gate = jnp.minimum(res[-1][0], 0.0)
        outs = []
        for o, lsum in res:
            l = jnp.sum(jnp.maximum(lsum, gate), axis=-1, keepdims=True)
            r = pl.reciprocal(l, approx=True)
            r = r * (2.0 - l * r)
            outs.append(o * r)
        return outs

    def woproj(slot, g, first, c, outs, lo, hi, dep=None, r0=0, r1=TQ):
        parts = [o[r0:r1] for o in outs]
        oc = jnp.concatenate([tie(parts[0], dep)] + parts[1:], axis=-1).astype(BF16)
        y = jnp.dot(oc, wobuf[g, :, lo:hi], preferred_element_type=F32)
        rows = slice(c * TQ + r0, c * TQ + r1)
        if first is True:
            acc[slot, rows, lo:hi] = y
        elif first is False:
            acc[slot, rows, lo:hi] = acc[slot, rows, lo:hi] + y
        else:
            acc[slot, rows, lo:hi] = jnp.where(first, 0.0, acc[slot, rows, lo:hi]) + y
        return y

    def ln1_piece(i, g, u, gate):
        pr = LNR // NP1
        if isinstance(i, int) and isinstance(g, int):
            row0, off = (i + 1) * BQ + g * LNR + u * pr, g * LNR + u * pr
        else:
            row0 = pl.multiple_of(jnp.minimum((i + 1) * BQ + g * LNR, S - LNR) + u * pr, pr)
            off = pl.multiple_of(g * LNR + u * pr, pr)
        xv = xbuf[pl.ds(row0, pr), :].astype(F32)
        xv = jnp.concatenate([tie(xv[:, 0:128], gate[0:pr, 0:128]), xv[:, 128:]], axis=-1)
        hv = ln1_apply(_normalize(xv), pr)
        hnext[pl.ds(off, pr), :] = hv.astype(BF16)
        return hv[:, 0:128]

    def wo_tail(i, g, slot, first, o0, o1):
        w = 256
        pieces = [(0, o0, lo) for lo in range(WB, DM, w)] + [(1, o1, lo) for lo in range(0, DM, w)]
        deps = {}
        for n, (c, o, lo) in enumerate(pieces):
            y = woproj(slot, g, first, c, o, lo, lo + w, deps.get(n))
            if n in LN1_AT:
                deps[n + 2] = ln1_piece(i, g, LN1_AT.index(n), y)

    def ln2_chunks(i, g):
        st = load_top()
        deps = []
        for u in range(LNR // LRW):
            off = pl.multiple_of(g * LNR + u * LRW, LRW)
            row0 = pl.multiple_of(jnp.maximum(i - 1, 0) * BQ + off, LRW)
            st = ln2(acc[(i + 1) & 1, pl.ds(off, LRW), 0:DM], row0, LRW, i > 0, st)
            if ((u + 1) * LRW) % (LNR // NP2) == 0:
                deps.append(st[3])
        store_top(st)
        return deps

    chains = [(c, h) for c in range(2) for h in range(NH)]

    def attention_step(i, g, slot, first):
        pv_dep = {(0, u): d for u, d in enumerate(ln2_chunks(i, g))}
        q = qproj(g, 0, 0)
        res = ([], [])
        o0 = None
        for n, (c, h) in enumerate(chains):
            s = qk(q, g, h)
            if n + 1 < len(chains):
                q = qproj(g, *chains[n + 1])
            if (c, h) == (1, 0):
                o0 = normalize_heads(res[0])
                woproj(slot, g, first, 0, o0, 0, WA)
            if (c, h) == (1, NH - 1):
                woproj(slot, g, first, 0, o0, WA, WB)
            res[c].append(pv(s, g, h, pv_dep.get((c, h))))
        o1 = normalize_heads(res[1])
        wo_tail(i, g, slot, first, o0, o1)

    c_cp.wait()
    x_cp[0].wait()
    sc = silu_c()
    acc[0, :, 0:DM] = _normalize(xbuf[0:BQ, :].astype(F32))
    for n in range(len(MODC) - 1):
        lo, hi = MODC[n], MODC[n + 1]
        for d in mod_cp[n]:
            d.wait()
        mod_cols(sc, lo, hi)
        mod_cols(sc, DM + lo, DM + hi)
        hn[:, lo:hi] = ln1_apply(acc[0, :, lo:hi], BQ, lo, hi).astype(BF16)

    wq_cp, k_cp, v_cp = head0_cps(0)
    wq_cp.wait()
    qa = qproj(0, 0, 0)
    qb = qproj(0, 1, 0)
    k_cp.wait()
    sa = qk(qa, 0, 0)
    s = qk(qb, 0, 0)
    ma = jnp.max(sa, axis=-1, keepdims=True)
    v_cp.wait()
    res = ([pv(sa, 0, 0, None, ma)], [pv(s, 0, 0)])
    for h in range(1, NH):
        for d in head0_cps(h):
            d.wait()
        if h + 1 == NH:
            wo0_cp.wait()
            x_cp[1].wait()
        q = qproj(0, 0, h)
        if h > 1:
            res[1].append(pv(s, 0, h - 1))
        s = qk(q, 0, h)
        q = qproj(0, 1, h)
        res[0].append(pv(s, 0, h))
        s = qk(q, 0, h)
    o0 = normalize_heads(res[0])
    woproj(0, 0, True, 0, o0, 0, WB)
    res[1].append(pv(s, 0, NH - 1))
    wo_tail(0, 0, 0, True, o0, normalize_heads(res[1]))

    def step(t, carry):
        i = lax.shift_right_logical(t, NG.bit_length() - 1)
        g = t & (NG - 1)

        @pl.when(jnp.logical_or(t <= GWAIT[-1], g == 0))
        def _():
            for t0, t1 in zip(GWAIT, GWAIT[1:] + (NG,)):
                @pl.when(t == t0)
                def _():
                    for gg in range(t0, t1):
                        for d in group_cps(gg):
                            d.wait()
                    if t0 == 2:
                        x_cp[3].wait()

            @pl.when(g == 0)
            def _():
                @pl.when(t == NG)
                def _():
                    for d in [modr_cp, x_cp[2], wr_cp] + ffn_cp:
                        d.wait()
                    hn[...] = hnext[...]
                    mod_cols(silu_c(), 2 * DM, 6 * DM)
                    fold_vectors()

                @pl.when(t > NG)
                def _():
                    out_cp(i - 2).start()
                    hn[...] = hnext[...]

        attention_step(i, g, i & 1, g == 0)
        return carry

    lax.fori_loop(1, NSTEP, step, 0)

    out_cp(NQ - 2).start()
    last = (NQ - 1) % 2
    st = load_top()
    for u in range(BQ // LNR):
        st = ln2(acc[last, u * LNR:(u + 1) * LNR, 0:DM], LAST0 + u * LNR, LNR, None, st, False)

    m1, i1, m2, i2 = st
    big = float(S)
    v1 = jnp.max(m1, axis=0, keepdims=True)
    j1 = jnp.min(jnp.where(m1 == v1, i1, big), axis=0, keepdims=True)
    taken = i1 == j1
    m1b = jnp.where(taken, m2, m1)
    i1b = jnp.where(taken, i2, i1)
    v2 = jnp.max(m1b, axis=0, keepdims=True)
    j2 = jnp.min(jnp.where(m1b == v2, i1b, big), axis=0, keepdims=True)
    idx1 = jnp.clip(j1[0, 0].astype(jnp.int32), 0, S - 1)
    idx2 = jnp.clip(j2[0, 0].astype(jnp.int32), 0, S - 1)

    row = lax.broadcasted_iota(jnp.int32, (16, DM), 0)
    def routed_row(idx):
        late = idx >= LAST0
        k = jnp.maximum(idx - LAST0, 0)
        mean = jnp.where(late, stat[0, pl.ds(k, 1), :], 0.0)
        rstd = jnp.where(late, stat[1, pl.ds(k, 1), :], 1.0)
        return (nbuf[pl.ds(idx, 1), :] - jnp.tile(mean, (1, DM // 128))) * jnp.tile(rstd, (1, DM // 128))

    xs = (jnp.where(row == 0, routed_row(idx1), routed_row(idx2))
          * (1.0 + _rows8(mod[:, 4 * DM:5 * DM], 16)) + _rows8(mod[:, 3 * DM:4 * DM], 16))

    FC = FF // NFC
    acts = []
    deps = {}
    for n in range(NFC):
        cols = slice(n * FC, (n + 1) * FC)
        xb = jnp.concatenate([tie(xs[:, 0:128], deps.get(n)), xs[:, 128:]], axis=-1).astype(BF16)
        gt = jnp.dot(xb, wgbuf[:, cols], preferred_element_type=F32)
        up = jnp.dot(xb, wubuf[:, cols], preferred_element_type=F32)
        acts.append((gt * jax.nn.sigmoid(gt) * up).astype(BF16))
        if n < NOUT:
            dep = None
            for u in range(BQ // NOUT // ORW):
                r0 = n * (BQ // NOUT) + u * ORW
                x1 = nbuf[LAST0 + r0:LAST0 + r0 + ORW, :]
                mean = tie(stat[0, r0:r0 + ORW, :], gt[0:ORW, 0:128])
                nv = ((x1 - jnp.tile(mean, (1, DM // 128)))
                      * jnp.tile(stat[1, r0:r0 + ORW, :], (1, DM // 128)))
                o = ln2_out(x1, nv, LAST0 + r0, ORW)[:, DM - 128:]
                dep = o if dep is None else jnp.maximum(dep, o)
            deps[n + 2] = dep
            if n + 1 == NOUT:
                out_cp(NQ - 1).start()
    y = jnp.dot(jnp.concatenate(acts, axis=-1), wdbuf[:, 0:DM], preferred_element_type=F32)
    gb = mod[0:1, 5 * DM:6 * DM]
    y1 = y[0:1, :] * jax.nn.sigmoid(v1[:, 0:1]) * gb
    y2 = y[1:2, :] * jax.nn.sigmoid(v2[:, 0:1]) * gb

    fixes = []
    for n, idx in enumerate((idx1, idx2)):
        base = pl.multiple_of(idx & (-FIX), FIX)
        rid = row[0:FIX] + base
        upd = jnp.where(rid == idx1, y1, jnp.where(rid == idx2, y2, 0.0))
        fixbuf[n] = (obuf[pl.ds(base, FIX), :].astype(F32) + upd).astype(BF16)
        fixes.append((base, cp(fixbuf.at[n], out_hbm.at[pl.ds(base, FIX)], sem.at[SEM_FIX])))
    (base1, fix1), (base2, fix2) = fixes

    for j in range(NQ):
        out_cp(j).wait()
    fix1.start()

    @pl.when(base1 != base2)
    def _():
        fix2.start()
        fix2.wait()

    fix1.wait()


@jax.jit
def pallas_adaLN_cond__mha_block_cached__moe_arch_mod__prompt_kernel(
    A_x: jax.Array,
    A_k_cache: jax.Array,
    A_v_cache: jax.Array,
    A_wq: jax.Array,
    A_wo: jax.Array,
    B_x: jax.Array,
    B_w_r: jax.Array,
    B_w_gate: jax.Array,
    B_w_up: jax.Array,
    B_w_down: jax.Array,
    c: jax.Array,
    w_mod: jax.Array,
):
    del B_x
    x = A_x.reshape(S, DM)
    k = A_k_cache.reshape(H, S, DH)
    v = A_v_cache.reshape(H, S, DH)
    wo = A_wo.reshape(NG, NH * DH, DM)
    any_spec = pl.BlockSpec(memory_space=pl.ANY)
    out = pl.pallas_call(
        _kernel,
        in_specs=[any_spec] * 11,
        out_specs=any_spec,
        out_shape=jax.ShapeDtypeStruct((S, DM), BF16),
        scratch_shapes=[
            pltpu.VMEM((S, DM), BF16),
            pltpu.VMEM((H, S, DH), BF16),
            pltpu.VMEM((H, S, DH), BF16),
            pltpu.VMEM((NG, DM, NH * DH), BF16),
            pltpu.VMEM((NG, NH * DH, DM), BF16),
            pltpu.VMEM((DM,), BF16),
            pltpu.VMEM((DM, FF), BF16),
            pltpu.VMEM((DM, FF), BF16),
            pltpu.VMEM((FF, DM + PAD), BF16),
            pltpu.VMEM((1, DM), BF16),
            pltpu.VMEM((DM, 6 * DM + PAD), BF16),
            pltpu.VMEM((BQ, DM), BF16),
            pltpu.VMEM((BQ, DM), BF16),
            pltpu.VMEM((2, BQ, DM + PAD), F32),
            pltpu.VMEM((S, DM), F32),
            pltpu.VMEM((2, BQ, 128), F32),
            pltpu.VMEM((S, DM), BF16),
            pltpu.VMEM((2, FIX, DM), BF16),
            pltpu.VMEM((8, 6 * DM), F32),
            pltpu.VMEM((4, 8, DM), F32),
            pltpu.VMEM((4, 8, 128), F32),
            pltpu.SMEM((1,), jnp.int32),
            pltpu.SemaphoreType.DMA((NSEM,)),
        ],
        compiler_params=pltpu.CompilerParams(vmem_limit_bytes=124 * 1024 * 1024),
        name="adaln_mha_moe",
    )(x, k, v, A_wq, wo, B_w_r, B_w_gate, B_w_up, B_w_down, c, w_mod)
    return out.reshape(1, S, DM)
```

```python
import jax
import jax.numpy as jnp
from jax import lax
import jax.experimental.pallas as pl
import jax.experimental.pallas.tpu as pltpu

F32 = jnp.float32
BF16 = jnp.bfloat16

S = 2048
DM = 1024
H = 32
DH = 128
FF = 3584
BQ = 512
TQ = 256
NH = 4
NQ = S // BQ
NG = H // NH
NSTEP = NQ * NG
LAST0 = S - BQ
LNR = BQ // NG
LN1_AT = ((1, 0), (1, 1), (1, 2), (1, 3))
LN2_AT = ((0, 0), (0, 1), (0, 2), (0, 3))
NP1 = len(LN1_AT)
NP2 = len(LN2_AT)
WA, WB = 256, 512
WT, WLAG = 256, 2
NFC = 14
NOUT = 8
LRW = 16
ORW = 16
KG = 512
EPS = 1e-5
QSCALE = DH ** -0.5 * 1.4426950408889634
NT = (((1,), (1,)), ((), ()))
FIX = 16
PAD = 128

SEM_CX = 0
MODC = (0, 512, 896, 1024)
SEM_MOD0 = 1
SEM_A = SEM_MOD0 + len(MODC) - 1
SEM_H0 = SEM_A + 3
GWAIT = (1, 2, 3, 5)
SEM_G = SEM_H0 + NH - 1
SEM_REST = SEM_G + len(GWAIT)
NSEM = SEM_REST + 1
SEM_OUT = SEM_CX
SEM_FIX = SEM_MOD0


def _rows8(v, rows):
    return jnp.tile(v, (rows // 8, 1))


def _normalize(x):
    mean = jnp.sum(x, axis=-1, keepdims=True) * (1.0 / DM)
    xc = x - mean
    var = jnp.sum(xc * xc, axis=-1, keepdims=True) * (1.0 / DM)
    return xc * lax.rsqrt(var + EPS)


def _kernel(x_hbm, k_hbm, v_hbm, wq_hbm, wo_hbm, wr_hbm, wg_hbm, wu_hbm, wd_hbm, c_hbm, wm_hbm,
            out_hbm,
            xbuf, kbuf, vbuf, wqbuf, wobuf, wrbuf, wgbuf, wubuf, wdbuf, cbuf, wmbuf,
            hn, hnext, acc, nbuf, stat, obuf, fixbuf, mod, vec, top, flag, sem):
    cp = pltpu.make_async_copy

    sem_last = SEM_H0 + NH - 2
    c_cp = cp(c_hbm, cbuf, sem.at[SEM_CX])
    wr_cp = cp(wr_hbm, wrbuf, sem.at[SEM_REST])
    x_rng = ((0, BQ, SEM_CX), (BQ, BQ + 2 * LNR, sem_last), (2 * BQ, S, SEM_REST),
             (BQ + 2 * LNR, 2 * BQ, SEM_G + 1))
    x_cp = [cp(x_hbm.at[a:b], xbuf.at[a:b], sem.at[n]) for a, b, n in x_rng]
    mod_cp = [[cp(wm_hbm.at[:, o + MODC[n]:o + MODC[n + 1]], wmbuf.at[:, o + MODC[n]:o + MODC[n + 1]],
                  sem.at[SEM_MOD0 + n]) for o in (0, DM)] for n in range(len(MODC) - 1)]
    modr_cp = cp(wm_hbm.at[:, 2 * DM:], wmbuf.at[:, 2 * DM:6 * DM], sem.at[SEM_REST])

    def head0_cps(h):
        sq, sk, sv = (SEM_A, SEM_A + 1, SEM_A + 2) if h == 0 else (SEM_H0 + h - 1,) * 3
        return [cp(wq_hbm.at[:, h * DH:(h + 1) * DH], wqbuf.at[0, :, h * DH:(h + 1) * DH], sem.at[sq]),
                cp(k_hbm.at[h], kbuf.at[h], sem.at[sk]),
                cp(v_hbm.at[h], vbuf.at[h], sem.at[sv])]

    wo0_cp = cp(wo_hbm.at[0], wobuf.at[0], sem.at[sem_last])

    def group_cps(g):
        sg = sem.at[SEM_G + max(n for n, t in enumerate(GWAIT) if t <= g)]
        heads = slice(g * NH, (g + 1) * NH)
        return [cp(wq_hbm.at[:, g * NH * DH:(g + 1) * NH * DH], wqbuf.at[g], sg),
                cp(k_hbm.at[heads], kbuf.at[heads], sg),
                cp(v_hbm.at[heads], vbuf.at[heads], sg),
                cp(wo_hbm.at[g], wobuf.at[g], sg)]

    ffn_cp = [cp(wg_hbm, wgbuf, sem.at[SEM_REST]), cp(wu_hbm, wubuf, sem.at[SEM_REST]),
              cp(wd_hbm, wdbuf.at[:, 0:DM], sem.at[SEM_REST])]

    def out_cp(j):
        if isinstance(j, int):
            rows = slice(j * BQ, (j + 1) * BQ)
        else:
            rows = pl.ds(pl.multiple_of(j * BQ, BQ), BQ)
        return cp(obuf.at[rows], out_hbm.at[rows], sem.at[SEM_OUT])

    c_cp.start()
    x_cp[0].start()
    for ds in mod_cp:
        for d in ds:
            d.start()
    for h in range(NH):
        for d in head0_cps(h):
            d.start()
    wo0_cp.start()
    x_cp[1].start()
    wr_cp.start()
    for g in range(1, NG):
        for d in group_cps(g):
            d.start()
        if g == 2:
            x_cp[3].start()
    modr_cp.start()
    x_cp[2].start()
    for d in ffn_cp:
        d.start()

    flag[0] = 0
    acc[1, :, 0:DM] = jnp.zeros((BQ, DM), F32)
    mod[:, 2 * DM:] = jnp.zeros((8, 4 * DM), F32)
    vec[...] = jnp.zeros((4, 8, DM), F32)
    top[0] = jnp.full((8, 128), -jnp.inf, F32)
    top[1] = jnp.zeros((8, 128), F32)
    top[2] = jnp.full((8, 128), -jnp.inf, F32)
    top[3] = jnp.zeros((8, 128), F32)

    def silu_c():
        cf = cbuf[...].astype(F32)
        sc = cf * jax.nn.sigmoid(cf)
        return jnp.broadcast_to(sc, (16, DM)).astype(BF16)

    def mod_cols(sc, lo, hi):
        mod[:, lo:hi] = jnp.dot(sc, wmbuf[:, lo:hi], preferred_element_type=F32)[:8]

    def tie(val, dep):
        if dep is None:
            return val
        n = dep.shape[0]
        head = jnp.where(flag[0] != 0, dep, val[:n])
        return head if n == val.shape[0] else jnp.concatenate([head, val[n:]], axis=0)

    def ln1_apply(n, rows, lo=0, hi=DM):
        return n * (1.0 + _rows8(mod[:, DM + lo:DM + hi], rows)) + _rows8(mod[:, lo:hi], rows)

    def load_top():
        return top[0], top[1], top[2], top[3]

    def store_top(st):
        top[0], top[1], top[2], top[3] = st

    def fold_vectors():
        sb, cb1, gb = mod[:, 3 * DM:4 * DM], 1.0 + mod[:, 4 * DM:5 * DM], mod[:, 5 * DM:6 * DM]
        wr = jnp.broadcast_to(wrbuf[...].astype(F32).reshape(1, DM), (8, DM))
        vec[0] = gb * cb1
        vec[1] = gb * sb
        vec[2] = cb1 * wr
        vec[3] = jnp.broadcast_to(jnp.sum(sb * wr, axis=-1, keepdims=True), (8, DM))

    def ln2_out(x1, n, row0, rows):
        out = x1 + n * _rows8(vec[0], rows) + _rows8(vec[1], rows)
        obuf[pl.ds(row0, rows), :] = out.astype(BF16)
        return out

    def ln2(a, row0, rows, valid, st, finish=True):
        rs = pl.ds(row0, rows)
        x1 = xbuf[rs, :].astype(F32) + _rows8(mod[:, 2 * DM:3 * DM], rows) * a
        mean = jnp.sum(x1, axis=-1, keepdims=True) * (1.0 / DM)
        xc = x1 - mean
        var = jnp.sum(xc * xc, axis=-1, keepdims=True) * (1.0 / DM)
        rstd = lax.rsqrt(var + EPS)
        if finish:
            n = xc * rstd
            nbuf[rs, :] = n
            ln2_out(x1, n, row0, rows)
            r = jnp.sum(n * _rows8(vec[2], rows), axis=-1, keepdims=True)
        else:
            nbuf[rs, :] = x1
            stat[0, pl.ds(row0 - LAST0, rows), :] = jnp.broadcast_to(mean, (rows, 128))
            stat[1, pl.ds(row0 - LAST0, rows), :] = jnp.broadcast_to(rstd, (rows, 128))
            r = jnp.sum(xc * _rows8(vec[2], rows), axis=-1, keepdims=True) * rstd
        r = r + _rows8(vec[3, :, 0:128], rows)
        if valid is not None:
            r = jnp.where(valid, r, -jnp.inf)
        m1, i1, m2, i2 = st
        base = (lax.broadcasted_iota(jnp.int32, (8, 128), 0) + row0).astype(F32)
        for u in range(rows // 8):
            ru = r[u * 8:(u + 1) * 8]
            iu = base + float(u * 8)
            gt1 = ru > m1
            gt2 = ru > m2
            m2 = jnp.where(gt1, m1, jnp.where(gt2, ru, m2))
            i2 = jnp.where(gt1, i1, jnp.where(gt2, iu, i2))
            m1 = jnp.where(gt1, ru, m1)
            i1 = jnp.where(gt1, iu, i1)
        return m1, i1, m2, i2

    def qproj(g, c, h):
        q = jnp.dot(hn[c * TQ:(c + 1) * TQ, :], wqbuf[g, :, h * DH:(h + 1) * DH],
                    preferred_element_type=F32)
        return (q * QSCALE).astype(BF16)

    def qk(q, g, h):
        return lax.dot_general(q, kbuf[g * NH + h], NT, preferred_element_type=F32)

    def pv(s, g, h, dep=None, m=None):
        if m is None:
            m = jnp.max(s, axis=-1, keepdims=True)
        lsum = None
        parts = []
        for j in range(S // KG):
            ss = [s[:, j * KG + u * 128:j * KG + (u + 1) * 128] for u in range(KG // 128)]
            if j == 0:
                ss[0] = tie(ss[0], dep)
            ps = [jnp.exp2(z - m) for z in ss]
            t = (ps[0] + ps[1]) + (ps[2] + ps[3])
            lsum = t if lsum is None else lsum + t
            ps[-1] = jnp.minimum(ps[-1], lsum)
            parts += ps
        p = jnp.concatenate(parts, axis=-1).astype(BF16)
        return jnp.dot(p, vbuf[g * NH + h], preferred_element_type=F32), lsum

    def normalize_heads(res):
        gate = jnp.minimum(res[-1][0], 0.0)
        outs = []
        for o, lsum in res:
            l = jnp.sum(jnp.maximum(lsum, gate), axis=-1, keepdims=True)
            r = pl.reciprocal(l, approx=True)
            r = r * (2.0 - l * r)
            outs.append(o * r)
        return outs

    def woproj(slot, g, first, c, outs, lo, hi, dep=None, r0=0, r1=TQ):
        parts = [o[r0:r1] for o in outs]
        oc = jnp.concatenate([tie(parts[0], dep)] + parts[1:], axis=-1).astype(BF16)
        y = jnp.dot(oc, wobuf[g, :, lo:hi], preferred_element_type=F32)
        rows = slice(c * TQ + r0, c * TQ + r1)
        if first is True:
            acc[slot, rows, lo:hi] = y
        elif first is False:
            acc[slot, rows, lo:hi] = acc[slot, rows, lo:hi] + y
        else:
            acc[slot, rows, lo:hi] = jnp.where(first, 0.0, acc[slot, rows, lo:hi]) + y
        return y

    def ln1_piece(i, g, u, gate=None):
        pr = LNR // NP1
        if isinstance(i, int) and isinstance(g, int):
            row0, off = (i + 1) * BQ + g * LNR + u * pr, g * LNR + u * pr
        else:
            row0 = pl.multiple_of(jnp.minimum((i + 1) * BQ + g * LNR, S - LNR) + u * pr, pr)
            off = pl.multiple_of(g * LNR + u * pr, pr)
        xv = xbuf[pl.ds(row0, pr), :].astype(F32)
        if gate is not None:
            xv = jnp.concatenate([tie(xv[:, 0:128], gate[0:pr, 0:128]), xv[:, 128:]], axis=-1)
        hv = ln1_apply(_normalize(xv), pr)
        hnext[pl.ds(off, pr), :] = hv.astype(BF16)
        return hv[:, 0:128]

    def ln2_piece(i, g, u, st):
        pr = LNR // NP2
        for k in range(pr // LRW):
            off = pl.multiple_of(g * LNR + u * pr + k * LRW, LRW)
            row0 = pl.multiple_of(jnp.maximum(i - 1, 0) * BQ + off, LRW)
            st = ln2(acc[(i + 1) & 1, pl.ds(off, LRW), 0:DM], row0, LRW, i > 0, st)
        return st

    def wo_tail(g, slot, first, o0, o1, work):
        pieces = [(0, o0, lo) for lo in range(WB, DM, WT)] + [(1, o1, lo) for lo in range(0, DM, WT)]
        deps = {}
        for n, (c, o, lo) in enumerate(pieces):
            y = woproj(slot, g, first, c, o, lo, lo + WT, deps.get(n))
            if n in work:
                deps[n + WLAG] = work[n](y)

    chains = [(c, h) for c in range(2) for h in range(NH)]

    def attention_step(i, g, g1, slot, first):
        st = [load_top()]

        def ln2_work(u):
            st[0] = ln2_piece(i, g, u, st[0])
            return st[0][3]

        pv_dep, work = {}, {}
        for u, at in enumerate(LN2_AT):
            if isinstance(at, tuple):
                pv_dep[at] = ln2_work(u)
            else:
                work[at] = lambda y, u=u: ln2_work(u)
        for u, at in enumerate(LN1_AT):
            if isinstance(at, tuple):
                pv_dep[at] = ln1_piece(i, g, u)
            else:
                work[at] = lambda y, u=u: ln1_piece(i, g, u, y)
        q = qproj(g, 0, 0)
        res = ([], [])
        o0 = None
        for n, (c, h) in enumerate(chains):
            s = qk(q, g, h)
            if n + 1 < len(chains):
                q = qproj((g, g1)[chains[n + 1][0]], *chains[n + 1])
            if (c, h) == (1, 0):
                o0 = normalize_heads(res[0])
                woproj(slot, g, first, 0, o0, 0, WA)
            if (c, h) == (1, NH - 1):
                woproj(slot, g, first, 0, o0, WA, WB)
            res[c].append(pv(s, g, h, pv_dep.get((c, h))))
        wo_tail(g, slot, first, o0, normalize_heads(res[1]), work)
        store_top(st[0])

    c_cp.wait()
    x_cp[0].wait()
    sc = silu_c()
    acc[0, :, 0:DM] = _normalize(xbuf[0:BQ, :].astype(F32))
    for n in range(len(MODC) - 1):
        lo, hi = MODC[n], MODC[n + 1]
        for d in mod_cp[n]:
            d.wait()
        mod_cols(sc, lo, hi)
        mod_cols(sc, DM + lo, DM + hi)
        hn[:, lo:hi] = ln1_apply(acc[0, :, lo:hi], BQ, lo, hi).astype(BF16)

    wq_cp, k_cp, v_cp = head0_cps(0)
    wq_cp.wait()
    qa = qproj(0, 0, 0)
    qb = qproj(0, 1, 0)
    k_cp.wait()
    sa = qk(qa, 0, 0)
    s = qk(qb, 0, 0)
    ma = jnp.max(sa, axis=-1, keepdims=True)
    v_cp.wait()
    res = ([pv(sa, 0, 0, None, ma)], [pv(s, 0, 0)])
    for h in range(1, NH):
        for d in head0_cps(h):
            d.wait()
        if h + 1 == NH:
            wo0_cp.wait()
            x_cp[1].wait()
        q = qproj(0, 0, h)
        if h > 1:
            res[1].append(pv(s, 0, h - 1))
        s = qk(q, 0, h)
        q = qproj(0, 1, h)
        res[0].append(pv(s, 0, h))
        s = qk(q, 0, h)
    o0 = normalize_heads(res[0])
    woproj(0, 0, True, 0, o0, 0, WB)
    res[1].append(pv(s, 0, NH - 1))
    npt = (2 * DM - WB) // WT - WLAG
    work0 = {}
    for u in range(NP1):
        work0.setdefault(u * npt // NP1, []).append(u)
    wo_tail(0, 0, True, o0, normalize_heads(res[1]),
            {n: (lambda y, us=us: jnp.concatenate([ln1_piece(0, 0, u, y) for u in us], axis=0))
             for n, us in work0.items()})

    def step(t, carry):
        i = lax.shift_right_logical(t, NG.bit_length() - 1)
        g = t & (NG - 1)

        @pl.when(jnp.logical_or(t <= GWAIT[-1], g == 0))
        def _():
            for t0, t1 in zip(GWAIT, GWAIT[1:] + (NG,)):
                @pl.when(t == t0)
                def _():
                    for gg in range(t0, t1):
                        for d in group_cps(gg):
                            d.wait()
                    if t0 == 2:
                        x_cp[3].wait()

            @pl.when(g == 0)
            def _():
                @pl.when(t == NG)
                def _():
                    for d in [modr_cp, x_cp[2], wr_cp] + ffn_cp:
                        d.wait()
                    hn[...] = hnext[...]
                    mod_cols(silu_c(), 2 * DM, 6 * DM)
                    fold_vectors()

                @pl.when(t > NG)
                def _():
                    out_cp(i - 2).start()
                    hn[...] = hnext[...]

        attention_step(i, g, (t + NG) & (NG - 1), i & 1, g == 0)
        return carry

    lax.fori_loop(1, NSTEP, step, 0)

    out_cp(NQ - 2).start()
    last = (NQ - 1) % 2
    st = load_top()
    for u in range(BQ // LNR):
        st = ln2(acc[last, u * LNR:(u + 1) * LNR, 0:DM], LAST0 + u * LNR, LNR, None, st, False)

    m1, i1, m2, i2 = st
    big = float(S)
    v1 = jnp.max(m1, axis=0, keepdims=True)
    j1 = jnp.min(jnp.where(m1 == v1, i1, big), axis=0, keepdims=True)
    taken = i1 == j1
    m1b = jnp.where(taken, m2, m1)
    i1b = jnp.where(taken, i2, i1)
    v2 = jnp.max(m1b, axis=0, keepdims=True)
    j2 = jnp.min(jnp.where(m1b == v2, i1b, big), axis=0, keepdims=True)
    idx1 = jnp.clip(j1[0, 0].astype(jnp.int32), 0, S - 1)
    idx2 = jnp.clip(j2[0, 0].astype(jnp.int32), 0, S - 1)

    row = lax.broadcasted_iota(jnp.int32, (16, DM), 0)
    def routed_row(idx):
        late = idx >= LAST0
        k = jnp.maximum(idx - LAST0, 0)
        mean = jnp.where(late, stat[0, pl.ds(k, 1), :], 0.0)
        rstd = jnp.where(late, stat[1, pl.ds(k, 1), :], 1.0)
        return (nbuf[pl.ds(idx, 1), :] - jnp.tile(mean, (1, DM // 128))) * jnp.tile(rstd, (1, DM // 128))

    xs = (jnp.where(row == 0, routed_row(idx1), routed_row(idx2))
          * (1.0 + _rows8(mod[:, 4 * DM:5 * DM], 16)) + _rows8(mod[:, 3 * DM:4 * DM], 16))

    FC = FF // NFC
    acts = []
    deps = {}
    for n in range(NFC):
        cols = slice(n * FC, (n + 1) * FC)
        xb = jnp.concatenate([tie(xs[:, 0:128], deps.get(n)), xs[:, 128:]], axis=-1).astype(BF16)
        gt = jnp.dot(xb, wgbuf[:, cols], preferred_element_type=F32)
        up = jnp.dot(xb, wubuf[:, cols], preferred_element_type=F32)
        acts.append((gt * jax.nn.sigmoid(gt) * up).astype(BF16))
        if n < NOUT:
            dep = None
            for u in range(BQ // NOUT // ORW):
                r0 = n * (BQ // NOUT) + u * ORW
                x1 = nbuf[LAST0 + r0:LAST0 + r0 + ORW, :]
                mean = tie(stat[0, r0:r0 + ORW, :], gt[0:ORW, 0:128])
                nv = ((x1 - jnp.tile(mean, (1, DM // 128)))
                      * jnp.tile(stat[1, r0:r0 + ORW, :], (1, DM // 128)))
                o = ln2_out(x1, nv, LAST0 + r0, ORW)[:, DM - 128:]
                dep = o if dep is None else jnp.maximum(dep, o)
            deps[n + 2] = dep
            if n + 1 == NOUT:
                out_cp(NQ - 1).start()
    y = jnp.dot(jnp.concatenate(acts, axis=-1), wdbuf[:, 0:DM], preferred_element_type=F32)
    gb = mod[0:1, 5 * DM:6 * DM]
    y1 = y[0:1, :] * jax.nn.sigmoid(v1[:, 0:1]) * gb
    y2 = y[1:2, :] * jax.nn.sigmoid(v2[:, 0:1]) * gb

    fixes = []
    for n, idx in enumerate((idx1, idx2)):
        base = pl.multiple_of(idx & (-FIX), FIX)
        rid = row[0:FIX] + base
        upd = jnp.where(rid == idx1, y1, jnp.where(rid == idx2, y2, 0.0))
        fixbuf[n] = (obuf[pl.ds(base, FIX), :].astype(F32) + upd).astype(BF16)
        fixes.append((base, cp(fixbuf.at[n], out_hbm.at[pl.ds(base, FIX)], sem.at[SEM_FIX])))
    (base1, fix1), (base2, fix2) = fixes

    for j in range(NQ):
        out_cp(j).wait()
    fix1.start()

    @pl.when(base1 != base2)
    def _():
        fix2.start()
        fix2.wait()

    fix1.wait()


@jax.jit
def pallas_adaLN_cond__mha_block_cached__moe_arch_mod__prompt_kernel(
    A_x: jax.Array,
    A_k_cache: jax.Array,
    A_v_cache: jax.Array,
    A_wq: jax.Array,
    A_wo: jax.Array,
    B_x: jax.Array,
    B_w_r: jax.Array,
    B_w_gate: jax.Array,
    B_w_up: jax.Array,
    B_w_down: jax.Array,
    c: jax.Array,
    w_mod: jax.Array,
):
    del B_x
    x = A_x.reshape(S, DM)
    k = A_k_cache.reshape(H, S, DH)
    v = A_v_cache.reshape(H, S, DH)
    wo = A_wo.reshape(NG, NH * DH, DM)
    any_spec = pl.BlockSpec(memory_space=pl.ANY)
    out = pl.pallas_call(
        _kernel,
        in_specs=[any_spec] * 11,
        out_specs=any_spec,
        out_shape=jax.ShapeDtypeStruct((S, DM), BF16),
        scratch_shapes=[
            pltpu.VMEM((S, DM), BF16),
            pltpu.VMEM((H, S, DH), BF16),
            pltpu.VMEM((H, S, DH), BF16),
            pltpu.VMEM((NG, DM, NH * DH), BF16),
            pltpu.VMEM((NG, NH * DH, DM), BF16),
            pltpu.VMEM((DM,), BF16),
            pltpu.VMEM((DM, FF), BF16),
            pltpu.VMEM((DM, FF), BF16),
            pltpu.VMEM((FF, DM + PAD), BF16),
            pltpu.VMEM((1, DM), BF16),
            pltpu.VMEM((DM, 6 * DM + PAD), BF16),
            pltpu.VMEM((BQ, DM), BF16),
            pltpu.VMEM((BQ, DM), BF16),
            pltpu.VMEM((2, BQ, DM + PAD), F32),
            pltpu.VMEM((S, DM), F32),
            pltpu.VMEM((2, BQ, 128), F32),
            pltpu.VMEM((S, DM), BF16),
            pltpu.VMEM((2, FIX, DM), BF16),
            pltpu.VMEM((8, 6 * DM), F32),
            pltpu.VMEM((4, 8, DM), F32),
            pltpu.VMEM((4, 8, 128), F32),
            pltpu.SMEM((1,), jnp.int32),
            pltpu.SemaphoreType.DMA((NSEM,)),
        ],
        compiler_params=pltpu.CompilerParams(vmem_limit_bytes=124 * 1024 * 1024),
        name="adaln_mha_moe",
    )(x, k, v, A_wq, wo, B_w_r, B_w_gate, B_w_up, B_w_down, c, w_mod)
    return out.reshape(1, S, DM)
```

```python
import jax
import jax.numpy as jnp
from jax import lax
import jax.experimental.pallas as pl
import jax.experimental.pallas.tpu as pltpu

F32 = jnp.float32
BF16 = jnp.bfloat16

S = 2048
DM = 1024
H = 32
DH = 128
FF = 3584
BQ = 512
TQ = 256
NH = 4
NQ = S // BQ
NG = H // NH
NSTEP = NQ * NG
LAST0 = S - BQ
LNR = BQ // NG
LN1_AT = ((1, 0), (1, 1), (1, 2), (1, 3))
LN2_AT = ((0, 0), (0, 1), (0, 2), (0, 3))
NP1 = len(LN1_AT)
NP2 = len(LN2_AT)
WA, WB = 256, 512
WT, WLAG = 256, 2
NFC = 14
NOUT = 8
LRW = 16
ORW = 16
KG = 512
EPS = 1e-5
QSCALE = DH ** -0.5 * 1.4426950408889634
NT = (((1,), (1,)), ((), ()))
FIX = 16
PAD = 128

SEM_CX = 0
MODC = (0, 640, 896, 1024)
SEM_MOD0 = 1
SEM_A = SEM_MOD0 + len(MODC) - 1
GWAIT = (1, 2, 3, 5)
SEM_G = SEM_A + 4
SEM_REST = SEM_G + len(GWAIT)
NSEM = SEM_REST + 1
SEM_OUT = SEM_CX
SEM_FIX = SEM_MOD0


def _rows8(v, rows):
    return jnp.tile(v, (rows // 8, 1))


def _normalize(x):
    mean = jnp.sum(x, axis=-1, keepdims=True) * (1.0 / DM)
    xc = x - mean
    var = jnp.sum(xc * xc, axis=-1, keepdims=True) * (1.0 / DM)
    return xc * lax.rsqrt(var + EPS)


def _kernel(x_hbm, k_hbm, v_hbm, wq_hbm, wo_hbm, wr_hbm, wg_hbm, wu_hbm, wd_hbm, c_hbm, wm_hbm,
            out_hbm,
            xbuf, kbuf, vbuf, wqbuf, wobuf, wrbuf, wgbuf, wubuf, wdbuf, cbuf, wmbuf,
            hn, hnext, acc, nbuf, stat, obuf, fixbuf, mod, vec, top, flag, sem):
    cp = pltpu.make_async_copy

    sem_last = SEM_A + 3
    c_cp = cp(c_hbm, cbuf, sem.at[SEM_CX])
    wr_cp = cp(wr_hbm, wrbuf, sem.at[SEM_REST])
    x_rng = ((0, BQ, SEM_CX), (BQ, BQ + 2 * LNR, sem_last), (2 * BQ, S, SEM_REST),
             (BQ + 2 * LNR, 2 * BQ, SEM_G + 1))
    x_cp = [cp(x_hbm.at[a:b], xbuf.at[a:b], sem.at[n]) for a, b, n in x_rng]
    mod_cp = [[cp(wm_hbm.at[:, o + MODC[n]:o + MODC[n + 1]], wmbuf.at[:, o + MODC[n]:o + MODC[n + 1]],
                  sem.at[SEM_MOD0 + n]) for o in (0, DM)] for n in range(len(MODC) - 1)]
    modr_cp = cp(wm_hbm.at[:, 2 * DM:], wmbuf.at[:, 2 * DM:6 * DM], sem.at[SEM_REST])

    def wq0_cp(h0, h1, sm):
        return cp(wq_hbm.at[:, h0 * DH:h1 * DH], wqbuf.at[0, :, h0 * DH:h1 * DH], sem.at[sm])

    def k0_cp(h, sm):
        return cp(k_hbm.at[h], kbuf.at[h], sem.at[sm])

    def v0_cp(h, sm):
        return cp(v_hbm.at[h], vbuf.at[h], sem.at[sm])

    wqe_cp = wq0_cp(0, 2, SEM_MOD0)
    step0_cp = [[k0_cp(0, SEM_A)],
                [v0_cp(0, SEM_A + 1), k0_cp(1, SEM_A + 1)],
                [v0_cp(1, SEM_A + 2), wq0_cp(2, 3, SEM_A + 2), k0_cp(2, SEM_A + 2), v0_cp(2, SEM_A + 2)],
                [wq0_cp(3, 4, sem_last), k0_cp(3, sem_last), v0_cp(3, sem_last),
                 cp(wo_hbm.at[0], wobuf.at[0], sem.at[sem_last]), x_cp[1]]]

    def group_cps(g):
        sg = sem.at[SEM_G + max(n for n, t in enumerate(GWAIT) if t <= g)]
        heads = slice(g * NH, (g + 1) * NH)
        return [cp(wq_hbm.at[:, g * NH * DH:(g + 1) * NH * DH], wqbuf.at[g], sg),
                cp(k_hbm.at[heads], kbuf.at[heads], sg),
                cp(v_hbm.at[heads], vbuf.at[heads], sg),
                cp(wo_hbm.at[g], wobuf.at[g], sg)]

    ffn_cp = [cp(wg_hbm, wgbuf, sem.at[SEM_REST]), cp(wu_hbm, wubuf, sem.at[SEM_REST]),
              cp(wd_hbm, wdbuf.at[:, 0:DM], sem.at[SEM_REST])]

    def out_cp(j):
        if isinstance(j, int):
            rows = slice(j * BQ, (j + 1) * BQ)
        else:
            rows = pl.ds(pl.multiple_of(j * BQ, BQ), BQ)
        return cp(obuf.at[rows], out_hbm.at[rows], sem.at[SEM_OUT])

    c_cp.start()
    x_cp[0].start()
    wqe_cp.start()
    for ds in mod_cp + step0_cp:
        for d in ds:
            d.start()
    for g in range(1, NG):
        for d in group_cps(g):
            d.start()
        if g == 2:
            x_cp[3].start()
    modr_cp.start()
    wr_cp.start()
    x_cp[2].start()
    for d in ffn_cp:
        d.start()

    flag[0] = 0
    acc[1, :, 0:DM] = jnp.zeros((BQ, DM), F32)
    mod[:, 2 * DM:] = jnp.zeros((8, 4 * DM), F32)
    vec[...] = jnp.zeros((4, 8, DM), F32)
    top[0] = jnp.full((8, 128), -jnp.inf, F32)
    top[1] = jnp.zeros((8, 128), F32)
    top[2] = jnp.full((8, 128), -jnp.inf, F32)
    top[3] = jnp.zeros((8, 128), F32)

    def silu_c():
        cf = cbuf[...].astype(F32)
        sc = cf * jax.nn.sigmoid(cf)
        return jnp.broadcast_to(sc, (16, DM)).astype(BF16)

    def mod_cols(sc, lo, hi):
        mod[:, lo:hi] = jnp.dot(sc, wmbuf[:, lo:hi], preferred_element_type=F32)[:8]

    def tie(val, dep):
        if dep is None:
            return val
        n = dep.shape[0]
        head = jnp.where(flag[0] != 0, dep, val[:n])
        return head if n == val.shape[0] else jnp.concatenate([head, val[n:]], axis=0)

    def ln1_apply(n, rows, lo=0, hi=DM):
        return n * (1.0 + _rows8(mod[:, DM + lo:DM + hi], rows)) + _rows8(mod[:, lo:hi], rows)

    def load_top():
        return top[0], top[1], top[2], top[3]

    def store_top(st):
        top[0], top[1], top[2], top[3] = st

    def fold_vectors():
        sb, cb1, gb = mod[:, 3 * DM:4 * DM], 1.0 + mod[:, 4 * DM:5 * DM], mod[:, 5 * DM:6 * DM]
        wr = jnp.broadcast_to(wrbuf[...].astype(F32).reshape(1, DM), (8, DM))
        vec[0] = gb * cb1
        vec[1] = gb * sb
        vec[2] = cb1 * wr
        vec[3] = jnp.broadcast_to(jnp.sum(sb * wr, axis=-1, keepdims=True), (8, DM))

    def ln2_out(x1, n, row0, rows):
        out = x1 + n * _rows8(vec[0], rows) + _rows8(vec[1], rows)
        obuf[pl.ds(row0, rows), :] = out.astype(BF16)
        return out

    def ln2(a, row0, rows, valid, st, finish=True):
        rs = pl.ds(row0, rows)
        x1 = xbuf[rs, :].astype(F32) + _rows8(mod[:, 2 * DM:3 * DM], rows) * a
        mean = jnp.sum(x1, axis=-1, keepdims=True) * (1.0 / DM)
        xc = x1 - mean
        var = jnp.sum(xc * xc, axis=-1, keepdims=True) * (1.0 / DM)
        rstd = lax.rsqrt(var + EPS)
        if finish:
            n = xc * rstd
            nbuf[rs, :] = n
            ln2_out(x1, n, row0, rows)
            r = jnp.sum(n * _rows8(vec[2], rows), axis=-1, keepdims=True)
        else:
            nbuf[rs, :] = x1
            stat[0, pl.ds(row0 - LAST0, rows), :] = jnp.broadcast_to(mean, (rows, 128))
            stat[1, pl.ds(row0 - LAST0, rows), :] = jnp.broadcast_to(rstd, (rows, 128))
            r = jnp.sum(xc * _rows8(vec[2], rows), axis=-1, keepdims=True) * rstd
        r = r + _rows8(vec[3, :, 0:128], rows)
        if valid is not None:
            r = jnp.where(valid, r, -jnp.inf)
        m1, i1, m2, i2 = st
        base = (lax.broadcasted_iota(jnp.int32, (8, 128), 0) + row0).astype(F32)
        for u in range(rows // 8):
            ru = r[u * 8:(u + 1) * 8]
            iu = base + float(u * 8)
            gt1 = ru > m1
            gt2 = ru > m2
            m2 = jnp.where(gt1, m1, jnp.where(gt2, ru, m2))
            i2 = jnp.where(gt1, i1, jnp.where(gt2, iu, i2))
            m1 = jnp.where(gt1, ru, m1)
            i1 = jnp.where(gt1, iu, i1)
        return m1, i1, m2, i2

    def qproj(g, c, h):
        q = jnp.dot(hn[c * TQ:(c + 1) * TQ, :], wqbuf[g, :, h * DH:(h + 1) * DH],
                    preferred_element_type=F32)
        return (q * QSCALE).astype(BF16)

    def qk(q, g, h):
        return lax.dot_general(q, kbuf[g * NH + h], NT, preferred_element_type=F32)

    def pv(s, g, h, dep=None, m=None):
        if m is None:
            m = jnp.max(s, axis=-1, keepdims=True)
        lsum = None
        parts = []
        for j in range(S // KG):
            ss = [s[:, j * KG + u * 128:j * KG + (u + 1) * 128] for u in range(KG // 128)]
            if j == 0:
                ss[0] = tie(ss[0], dep)
            ps = [jnp.exp2(z - m) for z in ss]
            t = (ps[0] + ps[1]) + (ps[2] + ps[3])
            lsum = t if lsum is None else lsum + t
            ps[-1] = jnp.minimum(ps[-1], lsum)
            parts += ps
        p = jnp.concatenate(parts, axis=-1).astype(BF16)
        return jnp.dot(p, vbuf[g * NH + h], preferred_element_type=F32), lsum

    def normalize_heads(res):
        gate = jnp.minimum(res[-1][0], 0.0)
        outs = []
        for o, lsum in res:
            l = jnp.sum(jnp.maximum(lsum, gate), axis=-1, keepdims=True)
            r = pl.reciprocal(l, approx=True)
            r = r * (2.0 - l * r)
            outs.append(o * r)
        return outs

    def woproj(slot, g, first, c, outs, lo, hi, dep=None, r0=0, r1=TQ):
        parts = [o[r0:r1] for o in outs]
        oc = jnp.concatenate([tie(parts[0], dep)] + parts[1:], axis=-1).astype(BF16)
        y = jnp.dot(oc, wobuf[g, :, lo:hi], preferred_element_type=F32)
        rows = slice(c * TQ + r0, c * TQ + r1)
        if first is True:
            acc[slot, rows, lo:hi] = y
        elif first is False:
            acc[slot, rows, lo:hi] = acc[slot, rows, lo:hi] + y
        else:
            acc[slot, rows, lo:hi] = jnp.where(first, 0.0, acc[slot, rows, lo:hi]) + y
        return y

    def ln1_piece(i, g, u, gate=None):
        pr = LNR // NP1
        if isinstance(i, int) and isinstance(g, int):
            row0, off = (i + 1) * BQ + g * LNR + u * pr, g * LNR + u * pr
        else:
            row0 = pl.multiple_of(jnp.minimum((i + 1) * BQ + g * LNR, S - LNR) + u * pr, pr)
            off = pl.multiple_of(g * LNR + u * pr, pr)
        xv = xbuf[pl.ds(row0, pr), :].astype(F32)
        if gate is not None:
            xv = jnp.concatenate([tie(xv[:, 0:128], gate[0:pr, 0:128]), xv[:, 128:]], axis=-1)
        hv = ln1_apply(_normalize(xv), pr)
        hnext[pl.ds(off, pr), :] = hv.astype(BF16)
        return hv[:, 0:128]

    def ln2_piece(i, g, u, st):
        pr = LNR // NP2
        for k in range(pr // LRW):
            off = pl.multiple_of(g * LNR + u * pr + k * LRW, LRW)
            row0 = pl.multiple_of(jnp.maximum(i - 1, 0) * BQ + off, LRW)
            st = ln2(acc[(i + 1) & 1, pl.ds(off, LRW), 0:DM], row0, LRW, i > 0, st)
        return st

    def wo_tail(g, slot, first, o0, o1, work):
        pieces = [(0, o0, lo) for lo in range(WB, DM, WT)] + [(1, o1, lo) for lo in range(0, DM, WT)]
        deps = {}
        for n, (c, o, lo) in enumerate(pieces):
            y = woproj(slot, g, first, c, o, lo, lo + WT, deps.get(n))
            if n in work:
                deps[n + WLAG] = work[n](y)

    chains = [(c, h) for c in range(2) for h in range(NH)]

    def attention_step(i, g, g1, slot, first):
        st = [load_top()]

        def ln2_work(u):
            st[0] = ln2_piece(i, g, u, st[0])
            return st[0][3]

        pv_dep, work = {}, {}
        for u, at in enumerate(LN2_AT):
            if isinstance(at, tuple):
                pv_dep[at] = ln2_work(u)
            else:
                work[at] = lambda y, u=u: ln2_work(u)
        for u, at in enumerate(LN1_AT):
            if isinstance(at, tuple):
                pv_dep[at] = ln1_piece(i, g, u)
            else:
                work[at] = lambda y, u=u: ln1_piece(i, g, u, y)
        q = qproj(g, 0, 0)
        res = ([], [])
        o0 = None
        for n, (c, h) in enumerate(chains):
            s = qk(q, g, h)
            if n + 1 < len(chains):
                q = qproj((g, g1)[chains[n + 1][0]], *chains[n + 1])
            if (c, h) == (1, 0):
                o0 = normalize_heads(res[0])
                woproj(slot, g, first, 0, o0, 0, WA)
            if (c, h) == (1, NH - 1):
                woproj(slot, g, first, 0, o0, WA, WB)
            res[c].append(pv(s, g, h, pv_dep.get((c, h))))
        wo_tail(g, slot, first, o0, normalize_heads(res[1]), work)
        store_top(st[0])

    c_cp.wait()
    x_cp[0].wait()
    sc = silu_c()
    acc[0, :, 0:DM] = _normalize(xbuf[0:BQ, :].astype(F32))
    for n in range(len(MODC) - 1):
        lo, hi = MODC[n], MODC[n + 1]
        if n == 0:
            wqe_cp.wait()
        for d in mod_cp[n]:
            d.wait()
        mod_cols(sc, lo, hi)
        mod_cols(sc, DM + lo, DM + hi)
        hn[:, lo:hi] = ln1_apply(acc[0, :, lo:hi], BQ, lo, hi).astype(BF16)
        for c in range(2):
            rows = slice(c * TQ, (c + 1) * TQ)
            part = jnp.dot(hn[rows, lo:hi], wqbuf[0, lo:hi, 0:2 * DH], preferred_element_type=F32)
            if n > 0:
                part = part + nbuf[rows, 0:2 * DH]
            if hi < DM:
                nbuf[rows, 0:2 * DH] = part
            else:
                hnext[rows, 0:2 * DH] = (part * QSCALE).astype(BF16)

    def wait0(n):
        for d in step0_cp[n]:
            d.wait()

    def qk_pair(h):
        sa, sb = [qk(hnext[c * TQ:(c + 1) * TQ, h * DH:(h + 1) * DH], 0, h) for c in range(2)]
        return sa, jnp.max(sa, axis=-1, keepdims=True), sb

    wait0(0)
    sa, ma, s = qk_pair(0)
    wait0(1)
    res = ([pv(sa, 0, 0, None, ma)], [pv(s, 0, 0)])
    sa, ma, s = qk_pair(1)
    wait0(2)
    res[0].append(pv(sa, 0, 1, None, ma))
    for h in range(2, NH):
        if h == 3:
            wait0(3)
        q = qproj(0, 0, h)
        res[1].append(pv(s, 0, h - 1))
        s = qk(q, 0, h)
        q = qproj(0, 1, h)
        res[0].append(pv(s, 0, h))
        s = qk(q, 0, h)
    o0 = normalize_heads(res[0])
    woproj(0, 0, True, 0, o0, 0, WB)
    res[1].append(pv(s, 0, NH - 1))
    npt = (2 * DM - WB) // WT - WLAG
    work0 = {}
    for u in range(NP1):
        work0.setdefault(u * npt // NP1, []).append(u)
    wo_tail(0, 0, True, o0, normalize_heads(res[1]),
            {n: (lambda y, us=us: jnp.concatenate([ln1_piece(0, 0, u, y) for u in us], axis=0))
             for n, us in work0.items()})

    def step(t, carry):
        i = lax.shift_right_logical(t, NG.bit_length() - 1)
        g = t & (NG - 1)

        @pl.when(jnp.logical_or(t <= GWAIT[-1], g == 0))
        def _():
            for t0, t1 in zip(GWAIT, GWAIT[1:] + (NG,)):
                @pl.when(t == t0)
                def _():
                    for gg in range(t0, t1):
                        for d in group_cps(gg):
                            d.wait()
                    if t0 == 2:
                        x_cp[3].wait()

            @pl.when(g == 0)
            def _():
                @pl.when(t == NG)
                def _():
                    for d in [modr_cp, x_cp[2], wr_cp] + ffn_cp:
                        d.wait()
                    hn[...] = hnext[...]
                    mod_cols(silu_c(), 2 * DM, 6 * DM)
                    fold_vectors()

                @pl.when(t > NG)
                def _():
                    out_cp(i - 2).start()
                    hn[...] = hnext[...]

        attention_step(i, g, (t + NG) & (NG - 1), i & 1, g == 0)
        return carry

    lax.fori_loop(1, NSTEP, step, 0)

    out_cp(NQ - 2).start()
    last = (NQ - 1) % 2
    st = load_top()
    for u in range(BQ // LNR):
        st = ln2(acc[last, u * LNR:(u + 1) * LNR, 0:DM], LAST0 + u * LNR, LNR, None, st, False)

    m1, i1, m2, i2 = st
    big = float(S)
    v1 = jnp.max(m1, axis=0, keepdims=True)
    j1 = jnp.min(jnp.where(m1 == v1, i1, big), axis=0, keepdims=True)
    taken = i1 == j1
    m1b = jnp.where(taken, m2, m1)
    i1b = jnp.where(taken, i2, i1)
    v2 = jnp.max(m1b, axis=0, keepdims=True)
    j2 = jnp.min(jnp.where(m1b == v2, i1b, big), axis=0, keepdims=True)
    idx1 = jnp.clip(j1[0, 0].astype(jnp.int32), 0, S - 1)
    idx2 = jnp.clip(j2[0, 0].astype(jnp.int32), 0, S - 1)

    row = lax.broadcasted_iota(jnp.int32, (16, DM), 0)
    def routed_row(idx):
        late = idx >= LAST0
        k = jnp.maximum(idx - LAST0, 0)
        mean = jnp.where(late, stat[0, pl.ds(k, 1), :], 0.0)
        rstd = jnp.where(late, stat[1, pl.ds(k, 1), :], 1.0)
        return (nbuf[pl.ds(idx, 1), :] - jnp.tile(mean, (1, DM // 128))) * jnp.tile(rstd, (1, DM // 128))

    xs = (jnp.where(row == 0, routed_row(idx1), routed_row(idx2))
          * (1.0 + _rows8(mod[:, 4 * DM:5 * DM], 16)) + _rows8(mod[:, 3 * DM:4 * DM], 16))

    FC = FF // NFC
    acts = []
    deps = {}
    for n in range(NFC):
        cols = slice(n * FC, (n + 1) * FC)
        xb = jnp.concatenate([tie(xs[:, 0:128], deps.get(n)), xs[:, 128:]], axis=-1).astype(BF16)
        gt = jnp.dot(xb, wgbuf[:, cols], preferred_element_type=F32)
        up = jnp.dot(xb, wubuf[:, cols], preferred_element_type=F32)
        acts.append((gt * jax.nn.sigmoid(gt) * up).astype(BF16))
        if n < NOUT:
            dep = None
            for u in range(BQ // NOUT // ORW):
                r0 = n * (BQ // NOUT) + u * ORW
                x1 = nbuf[LAST0 + r0:LAST0 + r0 + ORW, :]
                mean = tie(stat[0, r0:r0 + ORW, :], gt[0:ORW, 0:128])
                nv = ((x1 - jnp.tile(mean, (1, DM // 128)))
                      * jnp.tile(stat[1, r0:r0 + ORW, :], (1, DM // 128)))
                o = ln2_out(x1, nv, LAST0 + r0, ORW)[:, DM - 128:]
                dep = o if dep is None else jnp.maximum(dep, o)
            deps[n + 2] = dep
            if n + 1 == NOUT:
                out_cp(NQ - 1).start()
    y = jnp.dot(jnp.concatenate(acts, axis=-1), wdbuf[:, 0:DM], preferred_element_type=F32)
    gb = mod[0:1, 5 * DM:6 * DM]
    y1 = y[0:1, :] * jax.nn.sigmoid(v1[:, 0:1]) * gb
    y2 = y[1:2, :] * jax.nn.sigmoid(v2[:, 0:1]) * gb

    fixes = []
    for n, idx in enumerate((idx1, idx2)):
        base = pl.multiple_of(idx & (-FIX), FIX)
        rid = row[0:FIX] + base
        upd = jnp.where(rid == idx1, y1, jnp.where(rid == idx2, y2, 0.0))
        fixbuf[n] = (obuf[pl.ds(base, FIX), :].astype(F32) + upd).astype(BF16)
        fixes.append((base, cp(fixbuf.at[n], out_hbm.at[pl.ds(base, FIX)], sem.at[SEM_FIX])))
    (base1, fix1), (base2, fix2) = fixes

    for j in range(NQ):
        out_cp(j).wait()
    fix1.start()

    @pl.when(base1 != base2)
    def _():
        fix2.start()
        fix2.wait()

    fix1.wait()


@jax.jit
def pallas_adaLN_cond__mha_block_cached__moe_arch_mod__prompt_kernel(
    A_x: jax.Array,
    A_k_cache: jax.Array,
    A_v_cache: jax.Array,
    A_wq: jax.Array,
    A_wo: jax.Array,
    B_x: jax.Array,
    B_w_r: jax.Array,
    B_w_gate: jax.Array,
    B_w_up: jax.Array,
    B_w_down: jax.Array,
    c: jax.Array,
    w_mod: jax.Array,
):
    del B_x
    x = A_x.reshape(S, DM)
    k = A_k_cache.reshape(H, S, DH)
    v = A_v_cache.reshape(H, S, DH)
    wo = A_wo.reshape(NG, NH * DH, DM)
    any_spec = pl.BlockSpec(memory_space=pl.ANY)
    out = pl.pallas_call(
        _kernel,
        in_specs=[any_spec] * 11,
        out_specs=any_spec,
        out_shape=jax.ShapeDtypeStruct((S, DM), BF16),
        scratch_shapes=[
            pltpu.VMEM((S, DM), BF16),
            pltpu.VMEM((H, S, DH), BF16),
            pltpu.VMEM((H, S, DH), BF16),
            pltpu.VMEM((NG, DM, NH * DH), BF16),
            pltpu.VMEM((NG, NH * DH, DM), BF16),
            pltpu.VMEM((DM,), BF16),
            pltpu.VMEM((DM, FF), BF16),
            pltpu.VMEM((DM, FF), BF16),
            pltpu.VMEM((FF, DM + PAD), BF16),
            pltpu.VMEM((1, DM), BF16),
            pltpu.VMEM((DM, 6 * DM + PAD), BF16),
            pltpu.VMEM((BQ, DM), BF16),
            pltpu.VMEM((BQ, DM), BF16),
            pltpu.VMEM((2, BQ, DM + PAD), F32),
            pltpu.VMEM((S, DM), F32),
            pltpu.VMEM((2, BQ, 128), F32),
            pltpu.VMEM((S, DM), BF16),
            pltpu.VMEM((2, FIX, DM), BF16),
            pltpu.VMEM((8, 6 * DM), F32),
            pltpu.VMEM((4, 8, DM), F32),
            pltpu.VMEM((4, 8, 128), F32),
            pltpu.SMEM((1,), jnp.int32),
            pltpu.SemaphoreType.DMA((NSEM,)),
        ],
        compiler_params=pltpu.CompilerParams(vmem_limit_bytes=124 * 1024 * 1024),
        name="adaln_mha_moe",
    )(x, k, v, A_wq, wo, B_w_r, B_w_gate, B_w_up, B_w_down, c, w_mod)
    return out.reshape(1, S, DM)
```

```python
import jax
import jax.numpy as jnp
from jax import lax
import jax.experimental.pallas as pl
import jax.experimental.pallas.tpu as pltpu

F32 = jnp.float32
BF16 = jnp.bfloat16

S = 2048
DM = 1024
H = 32
DH = 128
FF = 3584
BQ = 512
TQ = 256
NH = 4
NQ = S // BQ
NG = H // NH
NSTEP = NQ * NG
LAST0 = S - BQ
LNR = BQ // NG
LN1_AT = ((1, 0), (1, 1), (1, 2), (1, 3))
LN2_AT = ((0, 0), (0, 1), (0, 2), (0, 3))
NP1 = len(LN1_AT)
NP2 = len(LN2_AT)
WA, WB = 256, 512
WT, WLAG = 256, 2
DLAG = 3
OUT_SPLIT = (0, 192, 352, 448, BQ)
LRW = 16
ORW = 16
KG = 512
EPS = 1e-5
QSCALE = DH ** -0.5 * 1.4426950408889634
NT = (((1,), (1,)), ((), ()))
FIX = 16
PAD = 128

SEM_CX = 0
MODC = (0, 640, 896, 1024)
SEM_MOD0 = 1
SEM_A = SEM_MOD0 + len(MODC) - 1
GWAIT = (1, 2, 3, 5)
SEM_G = SEM_A + 4
SEM_REST = SEM_G + len(GWAIT)
NSEM = SEM_REST + 1
SEM_OUT = SEM_CX
SEM_FIX = SEM_MOD0


def _rows8(v, rows):
    return jnp.tile(v, (rows // 8, 1))


def _normalize(x):
    mean = jnp.sum(x, axis=-1, keepdims=True) * (1.0 / DM)
    xc = x - mean
    var = jnp.sum(xc * xc, axis=-1, keepdims=True) * (1.0 / DM)
    return xc * lax.rsqrt(var + EPS)


def _kernel(x_hbm, k_hbm, v_hbm, wq_hbm, wo_hbm, wr_hbm, wg_hbm, wu_hbm, wd_hbm, c_hbm, wm_hbm,
            out_hbm,
            xbuf, kbuf, vbuf, wqbuf, wobuf, wrbuf, wgbuf, wubuf, wdbuf, cbuf, scbuf, wmbuf,
            hn, hnext, acc, nbuf, stat, obuf, fixbuf, mod, vec, top, flag, sem):
    cp = pltpu.make_async_copy

    sem_last = SEM_A + 3
    c_cp = cp(c_hbm, cbuf, sem.at[SEM_CX])
    wr_cp = cp(wr_hbm, wrbuf, sem.at[SEM_REST])
    x_rng = ((0, BQ, SEM_CX), (BQ, BQ + 2 * LNR, sem_last), (2 * BQ, S, SEM_REST),
             (BQ + 2 * LNR, 2 * BQ, SEM_G + 1))
    x_cp = [cp(x_hbm.at[a:b], xbuf.at[a:b], sem.at[n]) for a, b, n in x_rng]
    mod_cp = [[cp(wm_hbm.at[:, o + MODC[n]:o + MODC[n + 1]], wmbuf.at[:, o + MODC[n]:o + MODC[n + 1]],
                  sem.at[SEM_MOD0 + n]) for o in (0, DM)] for n in range(len(MODC) - 1)]
    modr_cp = cp(wm_hbm.at[:, 2 * DM:], wmbuf.at[:, 2 * DM:6 * DM], sem.at[SEM_REST])

    def wq0_cp(h0, h1, sm):
        return cp(wq_hbm.at[:, h0 * DH:h1 * DH], wqbuf.at[0, :, h0 * DH:h1 * DH], sem.at[sm])

    def k0_cp(h, sm):
        return cp(k_hbm.at[h], kbuf.at[h], sem.at[sm])

    def v0_cp(h, sm):
        return cp(v_hbm.at[h], vbuf.at[h], sem.at[sm])

    wqe_cp = wq0_cp(0, 2, SEM_MOD0)
    step0_cp = [[k0_cp(0, SEM_A)],
                [v0_cp(0, SEM_A + 1), k0_cp(1, SEM_A + 1)],
                [v0_cp(1, SEM_A + 2), wq0_cp(2, 3, SEM_A + 2), k0_cp(2, SEM_A + 2), v0_cp(2, SEM_A + 2)],
                [wq0_cp(3, 4, sem_last), k0_cp(3, sem_last), v0_cp(3, sem_last),
                 cp(wo_hbm.at[0], wobuf.at[0], sem.at[sem_last]), x_cp[1]]]

    def group_cps(g):
        sg = sem.at[SEM_G + max(n for n, t in enumerate(GWAIT) if t <= g)]
        heads = slice(g * NH, (g + 1) * NH)
        return [cp(wq_hbm.at[:, g * NH * DH:(g + 1) * NH * DH], wqbuf.at[g], sg),
                cp(k_hbm.at[heads], kbuf.at[heads], sg),
                cp(v_hbm.at[heads], vbuf.at[heads], sg),
                cp(wo_hbm.at[g], wobuf.at[g], sg)]

    ffn_cp = [cp(wg_hbm, wgbuf, sem.at[SEM_REST]), cp(wu_hbm, wubuf, sem.at[SEM_REST]),
              cp(wd_hbm, wdbuf.at[:, 0:DM], sem.at[SEM_REST])]

    def out_cp(j):
        if isinstance(j, int):
            rows = slice(j * BQ, (j + 1) * BQ)
        else:
            rows = pl.ds(pl.multiple_of(j * BQ, BQ), BQ)
        return cp(obuf.at[rows], out_hbm.at[rows], sem.at[SEM_OUT])

    last_cp = [cp(obuf.at[LAST0 + a:LAST0 + b], out_hbm.at[LAST0 + a:LAST0 + b], sem.at[SEM_OUT])
               for a, b in zip(OUT_SPLIT[:-1], OUT_SPLIT[1:])]

    c_cp.start()
    x_cp[0].start()
    wqe_cp.start()
    for ds in mod_cp + step0_cp:
        for d in ds:
            d.start()
    for g in range(1, NG):
        for d in group_cps(g):
            d.start()
        if g == 2:
            x_cp[3].start()
    modr_cp.start()
    wr_cp.start()
    x_cp[2].start()
    for d in ffn_cp:
        d.start()

    flag[0] = 0
    acc[1, :, 0:DM] = jnp.zeros((BQ, DM), F32)
    mod[:, 2 * DM:] = jnp.zeros((8, 4 * DM), F32)
    vec[...] = jnp.zeros((4, 8, DM), F32)
    top[0] = jnp.full((8, 128), -jnp.inf, F32)
    top[1] = jnp.zeros((8, 128), F32)
    top[2] = jnp.full((8, 128), -jnp.inf, F32)
    top[3] = jnp.zeros((8, 128), F32)

    def silu_c():
        cf = cbuf[...].astype(F32)
        sc = cf * jax.nn.sigmoid(cf)
        return jnp.broadcast_to(sc, (16, DM)).astype(BF16)

    def mod_cols(sc, lo, hi):
        mod[:, lo:hi] = jnp.dot(sc, wmbuf[:, lo:hi], preferred_element_type=F32)[:8]

    def tie(val, dep):
        if dep is None:
            return val
        n = dep.shape[0]
        head = jnp.where(flag[0] != 0, dep, val[:n])
        return head if n == val.shape[0] else jnp.concatenate([head, val[n:]], axis=0)

    def ln1_apply(n, rows, lo=0, hi=DM):
        return n * (1.0 + _rows8(mod[:, DM + lo:DM + hi], rows)) + _rows8(mod[:, lo:hi], rows)

    def load_top():
        return top[0], top[1], top[2], top[3]

    def store_top(st):
        top[0], top[1], top[2], top[3] = st

    def fold_vectors():
        sb, cb1, gb = mod[:, 3 * DM:4 * DM], 1.0 + mod[:, 4 * DM:5 * DM], mod[:, 5 * DM:6 * DM]
        wr = jnp.broadcast_to(wrbuf[...].astype(F32).reshape(1, DM), (8, DM))
        vec[0] = gb * cb1
        vec[1] = gb * sb
        vec[2] = cb1 * wr
        vec[3] = jnp.broadcast_to(jnp.sum(sb * wr, axis=-1, keepdims=True), (8, DM))

    def ln2_out(x1, n, row0, rows):
        out = x1 + n * _rows8(vec[0], rows) + _rows8(vec[1], rows)
        obuf[pl.ds(row0, rows), :] = out.astype(BF16)
        return out

    def ln2(a, row0, rows, valid, st, finish=True):
        rs = pl.ds(row0, rows)
        x1 = xbuf[rs, :].astype(F32) + _rows8(mod[:, 2 * DM:3 * DM], rows) * a
        mean = jnp.sum(x1, axis=-1, keepdims=True) * (1.0 / DM)
        xc = x1 - mean
        var = jnp.sum(xc * xc, axis=-1, keepdims=True) * (1.0 / DM)
        rstd = lax.rsqrt(var + EPS)
        if finish:
            n = xc * rstd
            nbuf[rs, :] = n
            ln2_out(x1, n, row0, rows)
            r = jnp.sum(n * _rows8(vec[2], rows), axis=-1, keepdims=True)
        else:
            nbuf[rs, :] = x1
            stat[0, pl.ds(row0 - LAST0, rows), :] = jnp.broadcast_to(mean, (rows, 128))
            stat[1, pl.ds(row0 - LAST0, rows), :] = jnp.broadcast_to(rstd, (rows, 128))
            r = jnp.sum(xc * _rows8(vec[2], rows), axis=-1, keepdims=True) * rstd
        r = r + _rows8(vec[3, :, 0:128], rows)
        if valid is not None:
            r = jnp.where(valid, r, -jnp.inf)
        m1, i1, m2, i2 = st
        base = (lax.broadcasted_iota(jnp.int32, (8, 128), 0) + row0).astype(F32)
        for u in range(rows // 8):
            ru = r[u * 8:(u + 1) * 8]
            iu = base + float(u * 8)
            gt1 = ru > m1
            gt2 = ru > m2
            m2 = jnp.where(gt1, m1, jnp.where(gt2, ru, m2))
            i2 = jnp.where(gt1, i1, jnp.where(gt2, iu, i2))
            m1 = jnp.where(gt1, ru, m1)
            i1 = jnp.where(gt1, iu, i1)
        return m1, i1, m2, i2

    def qproj(g, c, h):
        q = jnp.dot(hn[c * TQ:(c + 1) * TQ, :], wqbuf[g, :, h * DH:(h + 1) * DH],
                    preferred_element_type=F32)
        return (q * QSCALE).astype(BF16)

    def qk(q, g, h):
        return lax.dot_general(q, kbuf[g * NH + h], NT, preferred_element_type=F32)

    def pv(s, g, h, dep=None, m=None):
        if m is None:
            m = jnp.max(s, axis=-1, keepdims=True)
        lsum = None
        parts = []
        for j in range(S // KG):
            ss = [s[:, j * KG + u * 128:j * KG + (u + 1) * 128] for u in range(KG // 128)]
            if j == 0:
                ss[0] = tie(ss[0], dep)
            ps = [jnp.exp2(z - m) for z in ss]
            t = (ps[0] + ps[1]) + (ps[2] + ps[3])
            lsum = t if lsum is None else lsum + t
            ps[-1] = jnp.minimum(ps[-1], lsum)
            parts += ps
        p = jnp.concatenate(parts, axis=-1).astype(BF16)
        return jnp.dot(p, vbuf[g * NH + h], preferred_element_type=F32), lsum

    def normalize_heads(res):
        gate = jnp.minimum(res[-1][0], 0.0)
        outs = []
        for o, lsum in res:
            l = jnp.sum(jnp.maximum(lsum, gate), axis=-1, keepdims=True)
            r = pl.reciprocal(l, approx=True)
            r = r * (2.0 - l * r)
            outs.append(o * r)
        return outs

    def woproj(slot, g, first, c, outs, lo, hi, dep=None, r0=0, r1=TQ):
        parts = [o[r0:r1] for o in outs]
        oc = jnp.concatenate([tie(parts[0], dep)] + parts[1:], axis=-1).astype(BF16)
        y = jnp.dot(oc, wobuf[g, :, lo:hi], preferred_element_type=F32)
        rows = slice(c * TQ + r0, c * TQ + r1)
        if first is True:
            acc[slot, rows, lo:hi] = y
        elif first is False:
            acc[slot, rows, lo:hi] = acc[slot, rows, lo:hi] + y
        else:
            acc[slot, rows, lo:hi] = jnp.where(first, 0.0, acc[slot, rows, lo:hi]) + y
        return y

    def ln1_piece(i, g, u, gate=None):
        pr = LNR // NP1
        if isinstance(i, int) and isinstance(g, int):
            row0, off = (i + 1) * BQ + g * LNR + u * pr, g * LNR + u * pr
        else:
            row0 = pl.multiple_of(jnp.minimum((i + 1) * BQ + g * LNR, S - LNR) + u * pr, pr)
            off = pl.multiple_of(g * LNR + u * pr, pr)
        xv = xbuf[pl.ds(row0, pr), :].astype(F32)
        if gate is not None:
            xv = jnp.concatenate([tie(xv[:, 0:128], gate[0:pr, 0:128]), xv[:, 128:]], axis=-1)
        hv = ln1_apply(_normalize(xv), pr)
        hnext[pl.ds(off, pr), :] = hv.astype(BF16)
        return hv[:, 0:128]

    def ln2_piece(i, g, u, st):
        pr = LNR // NP2
        for k in range(pr // LRW):
            off = pl.multiple_of(g * LNR + u * pr + k * LRW, LRW)
            row0 = pl.multiple_of(jnp.maximum(i - 1, 0) * BQ + off, LRW)
            st = ln2(acc[(i + 1) & 1, pl.ds(off, LRW), 0:DM], row0, LRW, i > 0, st)
        return st

    def wo_tail(g, slot, first, o0, o1, work):
        pieces = [(0, o0, lo) for lo in range(WB, DM, WT)] + [(1, o1, lo) for lo in range(0, DM, WT)]
        deps = {}
        for n, (c, o, lo) in enumerate(pieces):
            y = woproj(slot, g, first, c, o, lo, lo + WT, deps.get(n))
            if n in work:
                deps[n + WLAG] = work[n](y)

    chains = [(c, h) for c in range(2) for h in range(NH)]

    def attention_step(i, g, g1, slot, first):
        st = [load_top()]

        def ln2_work(u):
            st[0] = ln2_piece(i, g, u, st[0])
            return st[0][3]

        pv_dep, work = {}, {}
        for u, at in enumerate(LN2_AT):
            if isinstance(at, tuple):
                pv_dep[at] = ln2_work(u)
            else:
                work[at] = lambda y, u=u: ln2_work(u)
        for u, at in enumerate(LN1_AT):
            if isinstance(at, tuple):
                pv_dep[at] = ln1_piece(i, g, u)
            else:
                work[at] = lambda y, u=u: ln1_piece(i, g, u, y)
        q = qproj(g, 0, 0)
        res = ([], [])
        o0 = None
        for n, (c, h) in enumerate(chains):
            s = qk(q, g, h)
            if n + 1 < len(chains):
                q = qproj((g, g1)[chains[n + 1][0]], *chains[n + 1])
            if (c, h) == (1, 0):
                o0 = normalize_heads(res[0])
                woproj(slot, g, first, 0, o0, 0, WA)
            if (c, h) == (1, NH - 1):
                woproj(slot, g, first, 0, o0, WA, WB)
            res[c].append(pv(s, g, h, pv_dep.get((c, h))))
        wo_tail(g, slot, first, o0, normalize_heads(res[1]), work)
        store_top(st[0])

    c_cp.wait()
    x_cp[0].wait()
    sc = silu_c()
    scbuf[...] = sc
    acc[0, :, 0:DM] = _normalize(xbuf[0:BQ, :].astype(F32))
    for n in range(len(MODC) - 1):
        lo, hi = MODC[n], MODC[n + 1]
        if n == 0:
            wqe_cp.wait()
        for d in mod_cp[n]:
            d.wait()
        mod_cols(sc, lo, hi)
        mod_cols(sc, DM + lo, DM + hi)
        hn[:, lo:hi] = ln1_apply(acc[0, :, lo:hi], BQ, lo, hi).astype(BF16)
        for c in range(2):
            rows = slice(c * TQ, (c + 1) * TQ)
            part = jnp.dot(hn[rows, lo:hi], wqbuf[0, lo:hi, 0:2 * DH], preferred_element_type=F32)
            if n > 0:
                part = part + nbuf[rows, 0:2 * DH]
            if hi < DM:
                nbuf[rows, 0:2 * DH] = part
            else:
                hnext[rows, 0:2 * DH] = (part * QSCALE).astype(BF16)

    def wait0(n):
        for d in step0_cp[n]:
            d.wait()

    def qk_pair(h):
        sa, sb = [qk(hnext[c * TQ:(c + 1) * TQ, h * DH:(h + 1) * DH], 0, h) for c in range(2)]
        return sa, jnp.max(sa, axis=-1, keepdims=True), sb

    wait0(0)
    sa, ma, s = qk_pair(0)
    wait0(1)
    res = ([pv(sa, 0, 0, None, ma)], [pv(s, 0, 0)])
    sa, ma, s = qk_pair(1)
    wait0(2)
    res[0].append(pv(sa, 0, 1, None, ma))
    for h in range(2, NH):
        if h == 3:
            wait0(3)
        q = qproj(0, 0, h)
        res[1].append(pv(s, 0, h - 1))
        s = qk(q, 0, h)
        q = qproj(0, 1, h)
        res[0].append(pv(s, 0, h))
        s = qk(q, 0, h)
    o0 = normalize_heads(res[0])
    woproj(0, 0, True, 0, o0, 0, WB)
    res[1].append(pv(s, 0, NH - 1))
    npt = (2 * DM - WB) // WT - WLAG
    work0 = {}
    for u in range(NP1):
        work0.setdefault(u * npt // NP1, []).append(u)
    wo_tail(0, 0, True, o0, normalize_heads(res[1]),
            {n: (lambda y, us=us: jnp.concatenate([ln1_piece(0, 0, u, y) for u in us], axis=0))
             for n, us in work0.items()})

    def step(t, carry):
        i = lax.shift_right_logical(t, NG.bit_length() - 1)
        g = t & (NG - 1)

        @pl.when(jnp.logical_or(t <= GWAIT[-1], g == 0))
        def _():
            for t0, t1 in zip(GWAIT, GWAIT[1:] + (NG,)):
                @pl.when(t == t0)
                def _():
                    for gg in range(t0, t1):
                        for d in group_cps(gg):
                            d.wait()
                    if t0 == 2:
                        x_cp[3].wait()

            @pl.when(g == 0)
            def _():
                @pl.when(t == NG)
                def _():
                    for d in [modr_cp, x_cp[2], wr_cp] + ffn_cp:
                        d.wait()
                    hn[...] = hnext[...]
                    mod_cols(scbuf[...], 2 * DM, 6 * DM)
                    fold_vectors()

                @pl.when(t > NG)
                def _():
                    out_cp(i - 2).start()
                    hn[...] = hnext[...]

        attention_step(i, g, (t + NG) & (NG - 1), i & 1, g == 0)
        return carry

    lax.fori_loop(1, NSTEP, step, 0)

    out_cp(NQ - 2).start()
    last = (NQ - 1) % 2
    st = load_top()
    for u in range(BQ // LNR):
        st = ln2(acc[last, u * LNR:(u + 1) * LNR, 0:DM], LAST0 + u * LNR, LNR, None, st, False)

    m1, i1, m2, i2 = st
    big = float(S)
    v1 = jnp.max(m1, axis=0, keepdims=True)
    j1 = jnp.min(jnp.where(m1 == v1, i1, big), axis=0, keepdims=True)
    taken = i1 == j1
    m1b = jnp.where(taken, m2, m1)
    i1b = jnp.where(taken, i2, i1)
    v2 = jnp.max(m1b, axis=0, keepdims=True)
    j2 = jnp.min(jnp.where(m1b == v2, i1b, big), axis=0, keepdims=True)
    idx1 = jnp.clip(j1[0, 0].astype(jnp.int32), 0, S - 1)
    idx2 = jnp.clip(j2[0, 0].astype(jnp.int32), 0, S - 1)

    row = lax.broadcasted_iota(jnp.int32, (16, DM), 0)
    def routed_row(idx):
        late = idx >= LAST0
        k = jnp.maximum(idx - LAST0, 0)
        mean = jnp.where(late, stat[0, pl.ds(k, 1), :], 0.0)
        rstd = jnp.where(late, stat[1, pl.ds(k, 1), :], 1.0)
        return (nbuf[pl.ds(idx, 1), :] - jnp.tile(mean, (1, DM // 128))) * jnp.tile(rstd, (1, DM // 128))

    xs = (jnp.where(row == 0, routed_row(idx1), routed_row(idx2))
          * (1.0 + _rows8(mod[:, 4 * DM:5 * DM], 16)) + _rows8(mod[:, 3 * DM:4 * DM], 16))

    acts = []
    ys = []

    def tied_bf16(v, dep):
        return jnp.concatenate([tie(v[:, 0:128], dep), v[:, 128:]], axis=-1).astype(BF16)

    def gate_up(n, dep):
        cols = slice(n * 128, (n + 1) * 128)
        xb = tied_bf16(xs, dep)
        gt = jnp.dot(xb, wgbuf[:, cols], preferred_element_type=F32)
        up = jnp.dot(xb, wubuf[:, cols], preferred_element_type=F32)
        acts.append(gt * jax.nn.sigmoid(gt) * up)
        return gt

    def down(n, dep):
        ab = tied_bf16(jnp.concatenate(acts[2 * n:2 * n + 2], axis=-1), dep)
        ys.append(jnp.dot(ab, wdbuf[n * 256:(n + 1) * 256, 0:DM], preferred_element_type=F32))
        return ys[-1]

    slots = []
    for n in range(FF // 128):
        slots.append((gate_up, n))
        if n % 2 == 1 and n >= DLAG:
            slots.append((down, (n - DLAG) // 2))
    slots += [(down, n) for n in range(FF // 256) if (down, n) not in slots]
    deps = {}
    for k, (fn, n) in enumerate(slots):
        gate = fn(n, deps.get(k))
        r0 = k * ORW
        if r0 < BQ:
            x1 = nbuf[LAST0 + r0:LAST0 + r0 + ORW, :]
            mean = tie(stat[0, r0:r0 + ORW, :], gate[0:ORW, 0:128])
            nv = (x1 - jnp.tile(mean, (1, DM // 128))) * jnp.tile(stat[1, r0:r0 + ORW, :], (1, DM // 128))
            deps[k + 2] = ln2_out(x1, nv, LAST0 + r0, ORW)[:, DM - 128:]
            if r0 + ORW in OUT_SPLIT:
                last_cp[OUT_SPLIT.index(r0 + ORW) - 1].start()
    y = sum(ys[1:], ys[0])
    gb = mod[0:1, 5 * DM:6 * DM]
    y1 = y[0:1, :] * jax.nn.sigmoid(v1[:, 0:1]) * gb
    y2 = y[1:2, :] * jax.nn.sigmoid(v2[:, 0:1]) * gb

    fixes = []
    for n, idx in enumerate((idx1, idx2)):
        base = pl.multiple_of(idx & (-FIX), FIX)
        rid = row[0:FIX] + base
        upd = jnp.where(rid == idx1, y1, jnp.where(rid == idx2, y2, 0.0))
        fixbuf[n] = (obuf[pl.ds(base, FIX), :].astype(F32) + upd).astype(BF16)
        fixes.append((base, cp(fixbuf.at[n], out_hbm.at[pl.ds(base, FIX)], sem.at[SEM_FIX])))
    (base1, fix1), (base2, fix2) = fixes

    for d in [out_cp(j) for j in range(NQ - 1)] + last_cp:
        d.wait()
    fix1.start()

    @pl.when(base1 != base2)
    def _():
        fix2.start()
        fix2.wait()

    fix1.wait()


@jax.jit
def pallas_adaLN_cond__mha_block_cached__moe_arch_mod__prompt_kernel(
    A_x: jax.Array,
    A_k_cache: jax.Array,
    A_v_cache: jax.Array,
    A_wq: jax.Array,
    A_wo: jax.Array,
    B_x: jax.Array,
    B_w_r: jax.Array,
    B_w_gate: jax.Array,
    B_w_up: jax.Array,
    B_w_down: jax.Array,
    c: jax.Array,
    w_mod: jax.Array,
):
    del B_x
    x = A_x.reshape(S, DM)
    k = A_k_cache.reshape(H, S, DH)
    v = A_v_cache.reshape(H, S, DH)
    wo = A_wo.reshape(NG, NH * DH, DM)
    any_spec = pl.BlockSpec(memory_space=pl.ANY)
    out = pl.pallas_call(
        _kernel,
        in_specs=[any_spec] * 11,
        out_specs=any_spec,
        out_shape=jax.ShapeDtypeStruct((S, DM), BF16),
        scratch_shapes=[
            pltpu.VMEM((S, DM), BF16),
            pltpu.VMEM((H, S, DH), BF16),
            pltpu.VMEM((H, S, DH), BF16),
            pltpu.VMEM((NG, DM, NH * DH), BF16),
            pltpu.VMEM((NG, NH * DH, DM), BF16),
            pltpu.VMEM((DM,), BF16),
            pltpu.VMEM((DM, FF), BF16),
            pltpu.VMEM((DM, FF), BF16),
            pltpu.VMEM((FF, DM + PAD), BF16),
            pltpu.VMEM((1, DM), BF16),
            pltpu.VMEM((16, DM), BF16),
            pltpu.VMEM((DM, 6 * DM + PAD), BF16),
            pltpu.VMEM((BQ, DM), BF16),
            pltpu.VMEM((BQ, DM), BF16),
            pltpu.VMEM((2, BQ, DM + PAD), F32),
            pltpu.VMEM((S, DM), F32),
            pltpu.VMEM((2, BQ, 128), F32),
            pltpu.VMEM((S, DM), BF16),
            pltpu.VMEM((2, FIX, DM), BF16),
            pltpu.VMEM((8, 6 * DM), F32),
            pltpu.VMEM((4, 8, DM), F32),
            pltpu.VMEM((4, 8, 128), F32),
            pltpu.SMEM((1,), jnp.int32),
            pltpu.SemaphoreType.DMA((NSEM,)),
        ],
        compiler_params=pltpu.CompilerParams(vmem_limit_bytes=124 * 1024 * 1024),
        name="adaln_mha_moe",
    )(x, k, v, A_wq, wo, B_w_r, B_w_gate, B_w_up, B_w_down, c, w_mod)
    return out.reshape(1, S, DM)
```

```python
import jax
import jax.numpy as jnp
from jax import lax
import jax.experimental.pallas as pl
import jax.experimental.pallas.tpu as pltpu

F32 = jnp.float32
BF16 = jnp.bfloat16

S = 2048
DM = 1024
H = 32
DH = 128
FF = 3584
BQ = 512
TQ = 256
NH = 4
NQ = S // BQ
NG = H // NH
NSTEP = NQ * NG
LAST0 = S - BQ
LNR = BQ // NG
LN1_AT = ((1, 0), (1, 1), (1, 2), (1, 3))
LN2_AT = ((0, 0), (0, 1), (0, 2), (0, 3))
NP1 = len(LN1_AT)
NP2 = len(LN2_AT)
WA, WB = 256, 512
WT, WLAG = 256, 2
DLAG = 3
OUT_SPLIT = (0, 192, 352, 448, BQ)
LRW = 16
ORW = 16
KG = 512
EPS = 1e-5
QSCALE = DH ** -0.5 * 1.4426950408889634
NT = (((1,), (1,)), ((), ()))
FIX = 16
PAD = 128

SEM_CX = 0
MODC = (0, 640, 896, 1024)
SEM_MOD0 = 1
SEM_A = SEM_MOD0 + len(MODC) - 1
GWAIT = (1, 2, 3, 5)
SEM_G = SEM_A + 4
SEM_REST = SEM_G + len(GWAIT)
NSEM = SEM_REST + 1
SEM_OUT = SEM_CX
SEM_FIX = SEM_MOD0


def _rows8(v, rows):
    return jnp.tile(v, (rows // 8, 1))


def _normalize(x):
    mean = jnp.sum(x, axis=-1, keepdims=True) * (1.0 / DM)
    xc = x - mean
    var = jnp.sum(xc * xc, axis=-1, keepdims=True) * (1.0 / DM)
    return xc * lax.rsqrt(var + EPS)


def _kernel(x_hbm, k_hbm, v_hbm, wq_hbm, wo_hbm, wr_hbm, wg_hbm, wu_hbm, wd_hbm, c_hbm, wm_hbm,
            out_hbm,
            xbuf, kbuf, vbuf, wqbuf, wobuf, wrbuf, wgbuf, wubuf, wdbuf, cbuf, scbuf, wmbuf,
            hn, hnext, acc, nbuf, stat, obuf, fixbuf, mod, vec, top, flag, sem):
    cp = pltpu.make_async_copy

    sem_last = SEM_A + 3
    c_cp = cp(c_hbm, cbuf, sem.at[SEM_CX])
    wr_cp = cp(wr_hbm, wrbuf, sem.at[SEM_REST])
    x_rng = ((0, BQ, SEM_CX), (BQ, BQ + 2 * LNR, sem_last), (2 * BQ, S, SEM_REST),
             (BQ + 2 * LNR, 2 * BQ, SEM_G + 1))
    x_cp = [cp(x_hbm.at[a:b], xbuf.at[a:b], sem.at[n]) for a, b, n in x_rng]
    mod_cp = [[cp(wm_hbm.at[:, o + MODC[n]:o + MODC[n + 1]], wmbuf.at[:, o + MODC[n]:o + MODC[n + 1]],
                  sem.at[SEM_MOD0 + n]) for o in (0, DM)] for n in range(len(MODC) - 1)]
    modr_cp = cp(wm_hbm.at[:, 2 * DM:], wmbuf.at[:, 2 * DM:6 * DM], sem.at[SEM_REST])

    def wq0_cp(h0, h1, sm):
        return cp(wq_hbm.at[:, h0 * DH:h1 * DH], wqbuf.at[0, :, h0 * DH:h1 * DH], sem.at[sm])

    def k0_cp(h, sm):
        return cp(k_hbm.at[h], kbuf.at[h], sem.at[sm])

    def v0_cp(h, sm):
        return cp(v_hbm.at[h], vbuf.at[h], sem.at[sm])

    wqe_cp = wq0_cp(0, 2, SEM_MOD0)
    step0_cp = [[k0_cp(0, SEM_A)],
                [v0_cp(0, SEM_A + 1), k0_cp(1, SEM_A + 1)],
                [v0_cp(1, SEM_A + 2), wq0_cp(2, 3, SEM_A + 2), k0_cp(2, SEM_A + 2), v0_cp(2, SEM_A + 2)],
                [wq0_cp(3, 4, sem_last), k0_cp(3, sem_last), v0_cp(3, sem_last),
                 cp(wo_hbm.at[0], wobuf.at[0], sem.at[sem_last]), x_cp[1]]]

    def group_cps(g):
        sg = sem.at[SEM_G + max(n for n, t in enumerate(GWAIT) if t <= g)]
        heads = slice(g * NH, (g + 1) * NH)
        return [cp(wq_hbm.at[:, g * NH * DH:(g + 1) * NH * DH], wqbuf.at[g], sg),
                cp(k_hbm.at[heads], kbuf.at[heads], sg),
                cp(v_hbm.at[heads], vbuf.at[heads], sg),
                cp(wo_hbm.at[g], wobuf.at[g], sg)]

    ffn_cp = [cp(wg_hbm, wgbuf, sem.at[SEM_REST]), cp(wu_hbm, wubuf, sem.at[SEM_REST]),
              cp(wd_hbm, wdbuf.at[:, 0:DM], sem.at[SEM_REST])]

    def out_cp(j):
        if isinstance(j, int):
            rows = slice(j * BQ, (j + 1) * BQ)
        else:
            rows = pl.ds(pl.multiple_of(j * BQ, BQ), BQ)
        return cp(obuf.at[rows], out_hbm.at[rows], sem.at[SEM_OUT])

    last_cp = [cp(obuf.at[LAST0 + a:LAST0 + b], out_hbm.at[LAST0 + a:LAST0 + b], sem.at[SEM_OUT])
               for a, b in zip(OUT_SPLIT[:-1], OUT_SPLIT[1:])]

    c_cp.start()
    x_cp[0].start()
    wqe_cp.start()
    for ds in mod_cp + step0_cp:
        for d in ds:
            d.start()
    for g in range(1, NG):
        for d in group_cps(g):
            d.start()
        if g == 2:
            x_cp[3].start()
    modr_cp.start()
    wr_cp.start()
    x_cp[2].start()
    for d in ffn_cp:
        d.start()

    flag[0] = 0
    acc[1, :, 0:DM] = jnp.zeros((BQ, DM), F32)
    mod[:, 2 * DM:] = jnp.zeros((8, 4 * DM), F32)
    vec[...] = jnp.zeros((4, 8, DM), F32)
    top[0] = jnp.full((8, 128), -jnp.inf, F32)
    top[1] = jnp.zeros((8, 128), F32)
    top[2] = jnp.full((8, 128), -jnp.inf, F32)
    top[3] = jnp.zeros((8, 128), F32)

    def silu_c():
        cf = cbuf[...].astype(F32)
        sc = cf * jax.nn.sigmoid(cf)
        return jnp.broadcast_to(sc, (16, DM)).astype(BF16)

    def mod_cols(sc, lo, hi):
        mod[:, lo:hi] = jnp.dot(sc, wmbuf[:, lo:hi], preferred_element_type=F32)[:8]

    def tie(val, dep):
        if dep is None:
            return val
        n = dep.shape[0]
        head = jnp.where(flag[0] != 0, dep, val[:n])
        return head if n == val.shape[0] else jnp.concatenate([head, val[n:]], axis=0)

    def ln1_apply(n, rows, lo=0, hi=DM):
        return n * (1.0 + _rows8(mod[:, DM + lo:DM + hi], rows)) + _rows8(mod[:, lo:hi], rows)

    def load_top():
        return top[0], top[1], top[2], top[3]

    def store_top(st):
        top[0], top[1], top[2], top[3] = st

    def fold_vectors():
        sb, cb1, gb = mod[:, 3 * DM:4 * DM], 1.0 + mod[:, 4 * DM:5 * DM], mod[:, 5 * DM:6 * DM]
        wr = jnp.broadcast_to(wrbuf[...].astype(F32).reshape(1, DM), (8, DM))
        vec[0] = gb * cb1
        vec[1] = gb * sb
        vec[2] = cb1 * wr
        vec[3] = jnp.broadcast_to(jnp.sum(sb * wr, axis=-1, keepdims=True), (8, DM))

    def ln2_out(x1, n, row0, rows):
        out = x1 + n * _rows8(vec[0], rows) + _rows8(vec[1], rows)
        obuf[pl.ds(row0, rows), :] = out.astype(BF16)
        return out

    def ln2(a, row0, rows, valid, st, finish=True):
        rs = pl.ds(row0, rows)
        x1 = xbuf[rs, :].astype(F32) + _rows8(mod[:, 2 * DM:3 * DM], rows) * a
        mean = jnp.sum(x1, axis=-1, keepdims=True) * (1.0 / DM)
        xc = x1 - mean
        var = jnp.sum(xc * xc, axis=-1, keepdims=True) * (1.0 / DM)
        rstd = lax.rsqrt(var + EPS)
        if finish:
            n = xc * rstd
            nbuf[rs, :] = n
            ln2_out(x1, n, row0, rows)
            r = jnp.sum(n * _rows8(vec[2], rows), axis=-1, keepdims=True)
        else:
            nbuf[rs, :] = x1
            stat[0, pl.ds(row0 - LAST0, rows), :] = jnp.broadcast_to(mean, (rows, 128))
            stat[1, pl.ds(row0 - LAST0, rows), :] = jnp.broadcast_to(rstd, (rows, 128))
            r = jnp.sum(xc * _rows8(vec[2], rows), axis=-1, keepdims=True) * rstd
        r = r + _rows8(vec[3, :, 0:128], rows)
        if valid is not None:
            r = jnp.where(valid, r, -jnp.inf)
        m1, i1, m2, i2 = st
        base = (lax.broadcasted_iota(jnp.int32, (8, 128), 0) + row0).astype(F32)
        for u in range(rows // 8):
            ru = r[u * 8:(u + 1) * 8]
            iu = base + float(u * 8)
            gt1 = ru > m1
            gt2 = ru > m2
            m2 = jnp.where(gt1, m1, jnp.where(gt2, ru, m2))
            i2 = jnp.where(gt1, i1, jnp.where(gt2, iu, i2))
            m1 = jnp.where(gt1, ru, m1)
            i1 = jnp.where(gt1, iu, i1)
        return m1, i1, m2, i2

    def qproj(g, c, h):
        q = jnp.dot(hn[c * TQ:(c + 1) * TQ, :], wqbuf[g, :, h * DH:(h + 1) * DH],
                    preferred_element_type=F32)
        return (q * QSCALE).astype(BF16)

    def qk(q, g, h):
        return lax.dot_general(q, kbuf[g * NH + h], NT, preferred_element_type=F32)

    def pv(s, g, h, dep=None, m=None):
        if m is None:
            m = jnp.max(s, axis=-1, keepdims=True)
        lsum = None
        parts = []
        for j in range(S // KG):
            ss = [s[:, j * KG + u * 128:j * KG + (u + 1) * 128] for u in range(KG // 128)]
            if j == 0:
                ss[0] = tie(ss[0], dep)
            ps = [jnp.exp2(z - m) for z in ss]
            t = (ps[0] + ps[1]) + (ps[2] + ps[3])
            lsum = t if lsum is None else lsum + t
            ps[-1] = jnp.minimum(ps[-1], lsum)
            parts += ps
        p = jnp.concatenate(parts, axis=-1).astype(BF16)
        return jnp.dot(p, vbuf[g * NH + h], preferred_element_type=F32), lsum

    def normalize_heads(res):
        gate = jnp.minimum(res[-1][0], 0.0)
        outs = []
        for o, lsum in res:
            l = jnp.sum(jnp.maximum(lsum, gate), axis=-1, keepdims=True)
            r = pl.reciprocal(l, approx=True)
            r = r * (2.0 - l * r)
            outs.append(o * r)
        return outs

    def woproj(slot, g, first, c, outs, lo, hi, dep=None, r0=0, r1=TQ):
        parts = [o[r0:r1] for o in outs]
        oc = jnp.concatenate([tie(parts[0], dep)] + parts[1:], axis=-1).astype(BF16)
        y = jnp.dot(oc, wobuf[g, :, lo:hi], preferred_element_type=F32)
        rows = slice(c * TQ + r0, c * TQ + r1)
        if first is True:
            acc[slot, rows, lo:hi] = y
        elif first is False:
            acc[slot, rows, lo:hi] = acc[slot, rows, lo:hi] + y
        else:
            acc[slot, rows, lo:hi] = jnp.where(first, 0.0, acc[slot, rows, lo:hi]) + y
        return y

    def ln1_piece(i, g, u, gate=None):
        pr = LNR // NP1
        if isinstance(i, int) and isinstance(g, int):
            row0, off = (i + 1) * BQ + g * LNR + u * pr, g * LNR + u * pr
        else:
            row0 = pl.multiple_of(jnp.minimum((i + 1) * BQ + g * LNR, S - LNR) + u * pr, pr)
            off = pl.multiple_of(g * LNR + u * pr, pr)
        xv = xbuf[pl.ds(row0, pr), :].astype(F32)
        if gate is not None:
            xv = jnp.concatenate([tie(xv[:, 0:128], gate[0:pr, 0:128]), xv[:, 128:]], axis=-1)
        hv = ln1_apply(_normalize(xv), pr)
        hnext[pl.ds(off, pr), :] = hv.astype(BF16)
        return hv[:, 0:128]

    def ln2_piece(i, g, u, st):
        pr = LNR // NP2
        for k in range(pr // LRW):
            off = pl.multiple_of(g * LNR + u * pr + k * LRW, LRW)
            row0 = pl.multiple_of(jnp.maximum(i - 1, 0) * BQ + off, LRW)
            st = ln2(acc[(i + 1) & 1, pl.ds(off, LRW), 0:DM], row0, LRW, i > 0, st)
        return st

    def wo_tail(g, slot, first, o0, o1, work):
        pieces = [(0, o0, lo) for lo in range(WB, DM, WT)] + [(1, o1, lo) for lo in range(0, DM, WT)]
        deps = {}
        for n, (c, o, lo) in enumerate(pieces):
            y = woproj(slot, g, first, c, o, lo, lo + WT, deps.get(n))
            if n in work:
                deps[n + WLAG] = work[n](y)

    chains = [(c, h) for c in range(2) for h in range(NH)]

    def attention_step(i, g, g1, slot, first):
        st = [load_top()]

        def ln2_work(u):
            st[0] = ln2_piece(i, g, u, st[0])
            return st[0][3]

        pv_dep, work = {}, {}
        for u, at in enumerate(LN2_AT):
            if isinstance(at, tuple):
                pv_dep[at] = ln2_work(u)
            else:
                work[at] = lambda y, u=u: ln2_work(u)
        for u, at in enumerate(LN1_AT):
            if isinstance(at, tuple):
                pv_dep[at] = ln1_piece(i, g, u)
            else:
                work[at] = lambda y, u=u: ln1_piece(i, g, u, y)
        q = qproj(g, 0, 0)
        res = ([], [])
        o0 = None
        for n, (c, h) in enumerate(chains):
            s = qk(q, g, h)
            if n + 1 < len(chains):
                q = qproj((g, g1)[chains[n + 1][0]], *chains[n + 1])
            if (c, h) == (1, 0):
                o0 = normalize_heads(res[0])
                woproj(slot, g, first, 0, o0, 0, WA)
            if (c, h) == (1, NH - 1):
                woproj(slot, g, first, 0, o0, WA, WB)
            res[c].append(pv(s, g, h, pv_dep.get((c, h))))
        wo_tail(g, slot, first, o0, normalize_heads(res[1]), work)
        store_top(st[0])

    c_cp.wait()
    x_cp[0].wait()
    sc = silu_c()
    scbuf[...] = sc
    acc[0, :, 0:DM] = _normalize(xbuf[0:BQ, :].astype(F32))
    for n in range(len(MODC) - 1):
        lo, hi = MODC[n], MODC[n + 1]
        if n == 0:
            wqe_cp.wait()
        for d in mod_cp[n]:
            d.wait()
        mod_cols(sc, lo, hi)
        mod_cols(sc, DM + lo, DM + hi)
        hn[:, lo:hi] = ln1_apply(acc[0, :, lo:hi], BQ, lo, hi).astype(BF16)
        for c in range(2):
            rows = slice(c * TQ, (c + 1) * TQ)
            part = jnp.dot(hn[rows, lo:hi], wqbuf[0, lo:hi, 0:2 * DH], preferred_element_type=F32)
            if n > 0:
                part = part + nbuf[rows, 0:2 * DH]
            if hi < DM:
                nbuf[rows, 0:2 * DH] = part
            else:
                hnext[rows, 0:2 * DH] = (part * QSCALE).astype(BF16)

    def wait0(n):
        for d in step0_cp[n]:
            d.wait()

    def qk_pair(h):
        sa, sb = [qk(hnext[c * TQ:(c + 1) * TQ, h * DH:(h + 1) * DH], 0, h) for c in range(2)]
        return sa, jnp.max(sa, axis=-1, keepdims=True), sb

    wait0(0)
    sa, ma, s = qk_pair(0)
    wait0(1)
    res = ([pv(sa, 0, 0, None, ma)], [pv(s, 0, 0)])
    sa, ma, s = qk_pair(1)
    wait0(2)
    res[0].append(pv(sa, 0, 1, None, ma))
    for h in range(2, NH):
        if h == 3:
            wait0(3)
        q = qproj(0, 0, h)
        res[1].append(pv(s, 0, h - 1))
        s = qk(q, 0, h)
        q = qproj(0, 1, h)
        res[0].append(pv(s, 0, h))
        s = qk(q, 0, h)
    o0 = normalize_heads(res[0])
    woproj(0, 0, True, 0, o0, 0, WB)
    res[1].append(pv(s, 0, NH - 1))
    npt = (2 * DM - WB) // WT - WLAG
    work0 = {}
    for u in range(NP1):
        work0.setdefault(u * npt // NP1, []).append(u)
    wo_tail(0, 0, True, o0, normalize_heads(res[1]),
            {n: (lambda y, us=us: jnp.concatenate([ln1_piece(0, 0, u, y) for u in us], axis=0))
             for n, us in work0.items()})

    def step(t, carry):
        i = lax.shift_right_logical(t, NG.bit_length() - 1)
        g = t & (NG - 1)

        @pl.when(jnp.logical_or(t <= GWAIT[-1], g == 0))
        def _():
            for t0, t1 in zip(GWAIT, GWAIT[1:] + (NG,)):
                @pl.when(t == t0)
                def _():
                    for gg in range(t0, t1):
                        for d in group_cps(gg):
                            d.wait()
                    if t0 == 2:
                        x_cp[3].wait()

            @pl.when(g == 0)
            def _():
                @pl.when(t == NG)
                def _():
                    for d in [modr_cp, x_cp[2], wr_cp] + ffn_cp:
                        d.wait()
                    hn[...] = hnext[...]
                    mod_cols(scbuf[...], 2 * DM, 6 * DM)
                    fold_vectors()

                @pl.when(t > NG)
                def _():
                    out_cp(i - 2).start()
                    hn[...] = hnext[...]

        attention_step(i, g, (t + NG) & (NG - 1), i & 1, g == 0)
        return carry

    lax.fori_loop(1, NSTEP, step, 0)

    out_cp(NQ - 2).start()
    last = (NQ - 1) % 2
    st = load_top()
    for u in range(BQ // LNR):
        st = ln2(acc[last, u * LNR:(u + 1) * LNR, 0:DM], LAST0 + u * LNR, LNR, None, st, False)

    m1, i1, m2, i2 = st
    big = float(S)
    v1 = jnp.max(m1, axis=0, keepdims=True)
    j1 = jnp.min(jnp.where(m1 == v1, i1, big), axis=0, keepdims=True)
    taken = i1 == j1
    m1b = jnp.where(taken, m2, m1)
    i1b = jnp.where(taken, i2, i1)
    v2 = jnp.max(m1b, axis=0, keepdims=True)
    j2 = jnp.min(jnp.where(m1b == v2, i1b, big), axis=0, keepdims=True)
    idx1 = jnp.clip(j1[0, 0].astype(jnp.int32), 0, S - 1)
    idx2 = jnp.clip(j2[0, 0].astype(jnp.int32), 0, S - 1)

    row = lax.broadcasted_iota(jnp.int32, (16, DM), 0)
    def routed_row(idx):
        late = idx >= LAST0
        k = jnp.clip(idx - LAST0, 0, BQ - 1)
        mean = jnp.where(late, stat[0, pl.ds(k, 1), :], 0.0)
        rstd = jnp.where(late, stat[1, pl.ds(k, 1), :], 1.0)
        return (nbuf[pl.ds(idx, 1), :] - jnp.tile(mean, (1, DM // 128))) * jnp.tile(rstd, (1, DM // 128))

    xs = (jnp.where(row == 0, routed_row(idx1), routed_row(idx2))
          * (1.0 + _rows8(mod[:, 4 * DM:5 * DM], 16)) + _rows8(mod[:, 3 * DM:4 * DM], 16))

    acts = []
    ys = []

    def tied_bf16(v, dep):
        return jnp.concatenate([tie(v[:, 0:128], dep), v[:, 128:]], axis=-1).astype(BF16)

    def gate_up(n, dep):
        cols = slice(n * 128, (n + 1) * 128)
        xb = tied_bf16(xs, dep)
        gt = jnp.dot(xb, wgbuf[:, cols], preferred_element_type=F32)
        up = jnp.dot(xb, wubuf[:, cols], preferred_element_type=F32)
        acts.append(gt * jax.nn.sigmoid(gt) * up)
        return gt

    def down(n, dep):
        ab = tied_bf16(jnp.concatenate(acts[2 * n:2 * n + 2], axis=-1), dep)
        ys.append(jnp.dot(ab, wdbuf[n * 256:(n + 1) * 256, 0:DM], preferred_element_type=F32))
        return ys[-1]

    slots = []
    for n in range(FF // 128):
        slots.append((gate_up, n))
        if n % 2 == 1 and n >= DLAG:
            slots.append((down, (n - DLAG) // 2))
    slots += [(down, n) for n in range(FF // 256) if (down, n) not in slots]
    deps = {}
    for k, (fn, n) in enumerate(slots):
        gate = fn(n, deps.get(k))
        r0 = k * ORW
        if r0 < BQ:
            x1 = nbuf[LAST0 + r0:LAST0 + r0 + ORW, :]
            mean = tie(stat[0, r0:r0 + ORW, :], gate[0:ORW, 0:128])
            nv = (x1 - jnp.tile(mean, (1, DM // 128))) * jnp.tile(stat[1, r0:r0 + ORW, :], (1, DM // 128))
            deps[k + 2] = ln2_out(x1, nv, LAST0 + r0, ORW)[:, DM - 128:]
            if r0 + ORW in OUT_SPLIT:
                last_cp[OUT_SPLIT.index(r0 + ORW) - 1].start()
    y = sum(ys[1:], ys[0])
    gb = mod[0:1, 5 * DM:6 * DM]
    y1 = y[0:1, :] * jax.nn.sigmoid(v1[:, 0:1]) * gb
    y2 = y[1:2, :] * jax.nn.sigmoid(v2[:, 0:1]) * gb

    fixes = []
    for n, idx in enumerate((idx1, idx2)):
        grp = jnp.clip(lax.shift_right_logical(idx, FIX.bit_length() - 1), 0, S // FIX - 1)
        base = pl.multiple_of(grp * FIX, FIX)
        rid = row[0:FIX] + base
        upd = jnp.where(rid == idx1, y1, jnp.where(rid == idx2, y2, 0.0))
        fixbuf[n] = (obuf[pl.ds(base, FIX), :].astype(F32) + upd).astype(BF16)
        fixes.append(cp(fixbuf.at[n], out_hbm.at[pl.ds(base, FIX)], sem.at[SEM_FIX]))

    for d in [out_cp(j) for j in range(NQ - 1)] + last_cp:
        d.wait()
    for d in fixes:
        d.start()
        d.wait()


@jax.jit
def pallas_adaLN_cond__mha_block_cached__moe_arch_mod__prompt_kernel(
    A_x: jax.Array,
    A_k_cache: jax.Array,
    A_v_cache: jax.Array,
    A_wq: jax.Array,
    A_wo: jax.Array,
    B_x: jax.Array,
    B_w_r: jax.Array,
    B_w_gate: jax.Array,
    B_w_up: jax.Array,
    B_w_down: jax.Array,
    c: jax.Array,
    w_mod: jax.Array,
):
    del B_x
    x = A_x.reshape(S, DM)
    k = A_k_cache.reshape(H, S, DH)
    v = A_v_cache.reshape(H, S, DH)
    wo = A_wo.reshape(NG, NH * DH, DM)
    any_spec = pl.BlockSpec(memory_space=pl.ANY)
    out = pl.pallas_call(
        _kernel,
        in_specs=[any_spec] * 11,
        out_specs=any_spec,
        out_shape=jax.ShapeDtypeStruct((S, DM), BF16),
        scratch_shapes=[
            pltpu.VMEM((S, DM), BF16),
            pltpu.VMEM((H, S, DH), BF16),
            pltpu.VMEM((H, S, DH), BF16),
            pltpu.VMEM((NG, DM, NH * DH), BF16),
            pltpu.VMEM((NG, NH * DH, DM), BF16),
            pltpu.VMEM((DM,), BF16),
            pltpu.VMEM((DM, FF), BF16),
            pltpu.VMEM((DM, FF), BF16),
            pltpu.VMEM((FF, DM + PAD), BF16),
            pltpu.VMEM((1, DM), BF16),
            pltpu.VMEM((16, DM), BF16),
            pltpu.VMEM((DM, 6 * DM + PAD), BF16),
            pltpu.VMEM((BQ, DM), BF16),
            pltpu.VMEM((BQ, DM), BF16),
            pltpu.VMEM((2, BQ, DM + PAD), F32),
            pltpu.VMEM((S, DM), F32),
            pltpu.VMEM((2, BQ, 128), F32),
            pltpu.VMEM((S, DM), BF16),
            pltpu.VMEM((2, FIX, DM), BF16),
            pltpu.VMEM((8, 6 * DM), F32),
            pltpu.VMEM((4, 8, DM), F32),
            pltpu.VMEM((4, 8, 128), F32),
            pltpu.SMEM((1,), jnp.int32),
            pltpu.SemaphoreType.DMA((NSEM,)),
        ],
        compiler_params=pltpu.CompilerParams(vmem_limit_bytes=124 * 1024 * 1024,
                                             disable_semaphore_checks=True),
        name="adaln_mha_moe",
    )(x, k, v, A_wq, wo, B_w_r, B_w_gate, B_w_up, B_w_down, c, w_mod)
    return out.reshape(1, S, DM)
```

```python
import jax
import jax.numpy as jnp
from jax import lax
import jax.experimental.pallas as pl
import jax.experimental.pallas.tpu as pltpu

F32 = jnp.float32
BF16 = jnp.bfloat16

S = 2048
DM = 1024
H = 32
DH = 128
FF = 3584
BQ = 512
TQ = 256
NH = 4
NQ = S // BQ
NG = H // NH
NSTEP = NQ * NG
LAST0 = S - BQ
LNR = BQ // NG
LN1_AT = ((1, 0), (1, 1), (1, 2), (1, 3))
LN2_AT = ((0, 0), (0, 1), (0, 2), (0, 3))
NP1 = len(LN1_AT)
NP2 = len(LN2_AT)
WA, WB = 256, 512
WT, WLAG = 256, 2
DLAG = 3
OUT_SPLIT = (0, 192, 352, 448, BQ)
LRW = 16
ORW = 16
KG = 512
EPS = 1e-5
QSCALE = DH ** -0.5 * 1.4426950408889634
NT = (((1,), (1,)), ((), ()))
FIX = 16
PAD = 128

SEM_CX = 0
MODC = (0, 640, 896, 1024)
SEM_MOD0 = 1
SEM_A = SEM_MOD0 + len(MODC) - 1
GWAIT = (1, 2, 3, 5)
SEM_G = SEM_A + 4
SEM_REST = SEM_G + len(GWAIT)
NSEM = SEM_REST + 1
SEM_OUT = SEM_CX
SEM_FIX = SEM_MOD0


def _rows8(v, rows):
    return jnp.tile(v, (rows // 8, 1))


def _normalize(x):
    mean = jnp.sum(x, axis=-1, keepdims=True) * (1.0 / DM)
    xc = x - mean
    var = jnp.sum(xc * xc, axis=-1, keepdims=True) * (1.0 / DM)
    return xc * lax.rsqrt(var + EPS)


def _kernel(x_hbm, k_hbm, v_hbm, wq_hbm, wo_hbm, wr_hbm, wg_hbm, wu_hbm, wd_hbm, c_hbm, wm_hbm,
            out_hbm,
            xbuf, kbuf, vbuf, wqbuf, wobuf, wrbuf, wgbuf, wubuf, wdbuf, cbuf, scbuf, wmbuf,
            hn, hnext, acc, nbuf, stat, obuf, fixbuf, mod, vec, top, flag, sem):
    cp = pltpu.make_async_copy

    sem_last = SEM_A + 3
    c_cp = cp(c_hbm, cbuf, sem.at[SEM_CX])
    wr_cp = cp(wr_hbm, wrbuf, sem.at[SEM_REST])
    x_rng = ((0, BQ, SEM_CX), (BQ, BQ + 2 * LNR, sem_last), (2 * BQ, S, SEM_REST),
             (BQ + 2 * LNR, 2 * BQ, SEM_G + 1))
    x_cp = [cp(x_hbm.at[a:b], xbuf.at[a:b], sem.at[n]) for a, b, n in x_rng]
    mod_cp = [[cp(wm_hbm.at[:, o + MODC[n]:o + MODC[n + 1]], wmbuf.at[:, o + MODC[n]:o + MODC[n + 1]],
                  sem.at[SEM_MOD0 + n]) for o in (0, DM)] for n in range(len(MODC) - 1)]
    modr_cp = cp(wm_hbm.at[:, 2 * DM:], wmbuf.at[:, 2 * DM:6 * DM], sem.at[SEM_REST])

    def wq0_cp(h0, h1, sm):
        return cp(wq_hbm.at[:, h0 * DH:h1 * DH], wqbuf.at[0, :, h0 * DH:h1 * DH], sem.at[sm])

    def k0_cp(h, sm):
        return cp(k_hbm.at[h], kbuf.at[h], sem.at[sm])

    def v0_cp(h, sm):
        return cp(v_hbm.at[h], vbuf.at[h], sem.at[sm])

    wqe_cp = wq0_cp(0, 2, SEM_MOD0)
    step0_cp = [[k0_cp(0, SEM_A)],
                [v0_cp(0, SEM_A + 1), k0_cp(1, SEM_A + 1)],
                [v0_cp(1, SEM_A + 2), wq0_cp(2, 3, SEM_A + 2), k0_cp(2, SEM_A + 2), v0_cp(2, SEM_A + 2)],
                [wq0_cp(3, 4, sem_last), k0_cp(3, sem_last), v0_cp(3, sem_last),
                 cp(wo_hbm.at[0], wobuf.at[0], sem.at[sem_last]), x_cp[1]]]

    def group_cps(g):
        sg = sem.at[SEM_G + max(n for n, t in enumerate(GWAIT) if t <= g)]
        heads = slice(g * NH, (g + 1) * NH)
        return [cp(wq_hbm.at[:, g * NH * DH:(g + 1) * NH * DH], wqbuf.at[g], sg),
                cp(k_hbm.at[heads], kbuf.at[heads], sg),
                cp(v_hbm.at[heads], vbuf.at[heads], sg),
                cp(wo_hbm.at[g], wobuf.at[g], sg)]

    ffn_cp = [cp(wg_hbm, wgbuf, sem.at[SEM_REST]), cp(wu_hbm, wubuf, sem.at[SEM_REST]),
              cp(wd_hbm, wdbuf.at[:, 0:DM], sem.at[SEM_REST])]

    def out_cp(j):
        if isinstance(j, int):
            rows = slice(j * BQ, (j + 1) * BQ)
        else:
            rows = pl.ds(pl.multiple_of(j * BQ, BQ), BQ)
        return cp(obuf.at[rows], out_hbm.at[rows], sem.at[SEM_OUT])

    last_cp = [cp(obuf.at[LAST0 + a:LAST0 + b], out_hbm.at[LAST0 + a:LAST0 + b], sem.at[SEM_OUT])
               for a, b in zip(OUT_SPLIT[:-1], OUT_SPLIT[1:])]

    c_cp.start()
    x_cp[0].start()
    wqe_cp.start()
    for ds in mod_cp + step0_cp:
        for d in ds:
            d.start()
    for g in range(1, NG):
        for d in group_cps(g):
            d.start()
        if g == 2:
            x_cp[3].start()
    modr_cp.start()
    wr_cp.start()
    x_cp[2].start()
    for d in ffn_cp:
        d.start()

    flag[0] = 0
    acc[1, :, 0:DM] = jnp.zeros((BQ, DM), F32)
    mod[:, 2 * DM:] = jnp.zeros((8, 4 * DM), F32)
    vec[...] = jnp.zeros((4, 8, DM), F32)
    top[0] = jnp.full((8, 128), -jnp.inf, F32)
    top[1] = jnp.zeros((8, 128), F32)
    top[2] = jnp.full((8, 128), -jnp.inf, F32)
    top[3] = jnp.zeros((8, 128), F32)

    def silu_c():
        cf = cbuf[...].astype(F32)
        sc = cf * jax.nn.sigmoid(cf)
        return jnp.broadcast_to(sc, (16, DM)).astype(BF16)

    def mod_cols(sc, lo, hi):
        mod[:, lo:hi] = jnp.dot(sc, wmbuf[:, lo:hi], preferred_element_type=F32)[:8]

    def tie(val, dep):
        if dep is None:
            return val
        n = dep.shape[0]
        head = jnp.where(flag[0] != 0, dep, val[:n])
        return head if n == val.shape[0] else jnp.concatenate([head, val[n:]], axis=0)

    def ln1_apply(n, rows, lo=0, hi=DM):
        return n * (1.0 + _rows8(mod[:, DM + lo:DM + hi], rows)) + _rows8(mod[:, lo:hi], rows)

    def load_top():
        return top[0], top[1], top[2], top[3]

    def store_top(st):
        top[0], top[1], top[2], top[3] = st

    def fold_vectors():
        sb, cb1, gb = mod[:, 3 * DM:4 * DM], 1.0 + mod[:, 4 * DM:5 * DM], mod[:, 5 * DM:6 * DM]
        wr = jnp.broadcast_to(wrbuf[...].astype(F32).reshape(1, DM), (8, DM))
        vec[0] = gb * cb1
        vec[1] = gb * sb
        vec[2] = cb1 * wr
        vec[3] = jnp.broadcast_to(jnp.sum(sb * wr, axis=-1, keepdims=True), (8, DM))

    def ln2_out(x1, n, row0, rows):
        out = x1 + n * _rows8(vec[0], rows) + _rows8(vec[1], rows)
        obuf[pl.ds(row0, rows), :] = out.astype(BF16)
        return out

    def ln2(a, row0, rows, valid, st, finish=True):
        rs = pl.ds(row0, rows)
        x1 = xbuf[rs, :].astype(F32) + _rows8(mod[:, 2 * DM:3 * DM], rows) * a
        mean = jnp.sum(x1, axis=-1, keepdims=True) * (1.0 / DM)
        xc = x1 - mean
        var = jnp.sum(xc * xc, axis=-1, keepdims=True) * (1.0 / DM)
        rstd = lax.rsqrt(var + EPS)
        if finish:
            n = xc * rstd
            nbuf[rs, :] = n
            ln2_out(x1, n, row0, rows)
            r = jnp.sum(n * _rows8(vec[2], rows), axis=-1, keepdims=True)
        else:
            nbuf[rs, :] = x1
            stat[0, pl.ds(row0 - LAST0, rows), :] = jnp.broadcast_to(mean, (rows, 128))
            stat[1, pl.ds(row0 - LAST0, rows), :] = jnp.broadcast_to(rstd, (rows, 128))
            r = jnp.sum(xc * _rows8(vec[2], rows), axis=-1, keepdims=True) * rstd
        r = r + _rows8(vec[3, :, 0:128], rows)
        if valid is not None:
            r = jnp.where(valid, r, -jnp.inf)
        m1, i1, m2, i2 = st
        base = (lax.broadcasted_iota(jnp.int32, (8, 128), 0) + row0).astype(F32)
        for u in range(rows // 8):
            ru = r[u * 8:(u + 1) * 8]
            iu = base + float(u * 8)
            gt1 = ru > m1
            gt2 = ru > m2
            m2 = jnp.where(gt1, m1, jnp.where(gt2, ru, m2))
            i2 = jnp.where(gt1, i1, jnp.where(gt2, iu, i2))
            m1 = jnp.where(gt1, ru, m1)
            i1 = jnp.where(gt1, iu, i1)
        return m1, i1, m2, i2

    def qproj(g, c, h):
        q = jnp.dot(hn[c * TQ:(c + 1) * TQ, :], wqbuf[g, :, h * DH:(h + 1) * DH],
                    preferred_element_type=F32)
        return (q * QSCALE).astype(BF16)

    def qk(q, g, h):
        return lax.dot_general(q, kbuf[g * NH + h], NT, preferred_element_type=F32)

    def pv(s, g, h, dep=None, m=None):
        if m is None:
            m = jnp.max(s, axis=-1, keepdims=True)
        lsum = None
        parts = []
        for j in range(S // KG):
            ss = [s[:, j * KG + u * 128:j * KG + (u + 1) * 128] for u in range(KG // 128)]
            if j == 0:
                ss[0] = tie(ss[0], dep)
            ps = [jnp.exp2(z - m) for z in ss]
            t = (ps[0] + ps[1]) + (ps[2] + ps[3])
            lsum = t if lsum is None else lsum + t
            ps[-1] = jnp.minimum(ps[-1], lsum)
            parts += ps
        p = jnp.concatenate(parts, axis=-1).astype(BF16)
        return jnp.dot(p, vbuf[g * NH + h], preferred_element_type=F32), lsum

    def normalize_heads(res):
        gate = jnp.minimum(res[-1][0], 0.0)
        outs = []
        for o, lsum in res:
            l = jnp.sum(jnp.maximum(lsum, gate), axis=-1, keepdims=True)
            r = pl.reciprocal(l, approx=True)
            r = r * (2.0 - l * r)
            outs.append(o * r)
        return outs

    def woproj(slot, g, first, c, outs, lo, hi, dep=None, r0=0, r1=TQ):
        parts = [o[r0:r1] for o in outs]
        oc = jnp.concatenate([tie(parts[0], dep)] + parts[1:], axis=-1).astype(BF16)
        y = jnp.dot(oc, wobuf[g, :, lo:hi], preferred_element_type=F32)
        rows = slice(c * TQ + r0, c * TQ + r1)
        if first is True:
            acc[slot, rows, lo:hi] = y
        elif first is False:
            acc[slot, rows, lo:hi] = acc[slot, rows, lo:hi] + y
        else:
            acc[slot, rows, lo:hi] = jnp.where(first, 0.0, acc[slot, rows, lo:hi]) + y
        return y

    def ln1_piece(i, g, u, gate=None):
        pr = LNR // NP1
        if isinstance(i, int) and isinstance(g, int):
            row0, off = (i + 1) * BQ + g * LNR + u * pr, g * LNR + u * pr
        else:
            row0 = pl.multiple_of(jnp.minimum((i + 1) * BQ + g * LNR, S - LNR) + u * pr, pr)
            off = pl.multiple_of(g * LNR + u * pr, pr)
        xv = xbuf[pl.ds(row0, pr), :].astype(F32)
        if gate is not None:
            xv = jnp.concatenate([tie(xv[:, 0:128], gate[0:pr, 0:128]), xv[:, 128:]], axis=-1)
        hv = ln1_apply(_normalize(xv), pr)
        hnext[pl.ds(off, pr), :] = hv.astype(BF16)
        return hv[:, 0:128]

    def ln2_piece(i, g, u, st):
        pr = LNR // NP2
        for k in range(pr // LRW):
            off = pl.multiple_of(g * LNR + u * pr + k * LRW, LRW)
            row0 = pl.multiple_of(jnp.maximum(i - 1, 0) * BQ + off, LRW)
            st = ln2(acc[(i + 1) & 1, pl.ds(off, LRW), 0:DM], row0, LRW, i > 0, st)
        return st

    def wo_tail(g, slot, first, o0, o1, work):
        pieces = [(0, o0, lo) for lo in range(WB, DM, WT)] + [(1, o1, lo) for lo in range(0, DM, WT)]
        deps = {}
        for n, (c, o, lo) in enumerate(pieces):
            y = woproj(slot, g, first, c, o, lo, lo + WT, deps.get(n))
            if n in work:
                deps[n + WLAG] = work[n](y)

    chains = [(c, h) for c in range(2) for h in range(NH)]

    def attention_step(i, g, g1, slot, first):
        st = [load_top()]

        def ln2_work(u):
            st[0] = ln2_piece(i, g, u, st[0])
            return st[0][3]

        pv_dep, work = {}, {}
        for u, at in enumerate(LN2_AT):
            if isinstance(at, tuple):
                pv_dep[at] = ln2_work(u)
            else:
                work[at] = lambda y, u=u: ln2_work(u)
        for u, at in enumerate(LN1_AT):
            if isinstance(at, tuple):
                pv_dep[at] = ln1_piece(i, g, u)
            else:
                work[at] = lambda y, u=u: ln1_piece(i, g, u, y)
        q = qproj(g, 0, 0)
        res = ([], [])
        o0 = None
        for n, (c, h) in enumerate(chains):
            s = qk(q, g, h)
            if n + 1 < len(chains):
                q = qproj((g, g1)[chains[n + 1][0]], *chains[n + 1])
            if (c, h) == (1, 0):
                o0 = normalize_heads(res[0])
                woproj(slot, g, first, 0, o0, 0, WA)
            if (c, h) == (1, NH - 1):
                woproj(slot, g, first, 0, o0, WA, WB)
            res[c].append(pv(s, g, h, pv_dep.get((c, h))))
        wo_tail(g, slot, first, o0, normalize_heads(res[1]), work)
        store_top(st[0])

    c_cp.wait()
    x_cp[0].wait()
    sc = silu_c()
    scbuf[...] = sc
    acc[0, :, 0:DM] = _normalize(xbuf[0:BQ, :].astype(F32))
    for n in range(len(MODC) - 1):
        lo, hi = MODC[n], MODC[n + 1]
        if n == 0:
            wqe_cp.wait()
        for d in mod_cp[n]:
            d.wait()
        mod_cols(sc, lo, hi)
        mod_cols(sc, DM + lo, DM + hi)
        hn[:, lo:hi] = ln1_apply(acc[0, :, lo:hi], BQ, lo, hi).astype(BF16)
        for c in range(2):
            rows = slice(c * TQ, (c + 1) * TQ)
            part = jnp.dot(hn[rows, lo:hi], wqbuf[0, lo:hi, 0:2 * DH], preferred_element_type=F32)
            if n > 0:
                part = part + nbuf[rows, 0:2 * DH]
            if hi < DM:
                nbuf[rows, 0:2 * DH] = part
            else:
                hnext[rows, 0:2 * DH] = (part * QSCALE).astype(BF16)

    def wait0(n):
        for d in step0_cp[n]:
            d.wait()

    def qk_pair(h):
        sa, sb = [qk(hnext[c * TQ:(c + 1) * TQ, h * DH:(h + 1) * DH], 0, h) for c in range(2)]
        return sa, jnp.max(sa, axis=-1, keepdims=True), sb

    wait0(0)
    sa, ma, s = qk_pair(0)
    wait0(1)
    res = ([pv(sa, 0, 0, None, ma)], [pv(s, 0, 0)])
    sa, ma, s = qk_pair(1)
    wait0(2)
    res[0].append(pv(sa, 0, 1, None, ma))
    for h in range(2, NH):
        if h == 3:
            wait0(3)
        q = qproj(0, 0, h)
        res[1].append(pv(s, 0, h - 1))
        s = qk(q, 0, h)
        q = qproj(0, 1, h)
        res[0].append(pv(s, 0, h))
        s = qk(q, 0, h)
    o0 = normalize_heads(res[0])
    woproj(0, 0, True, 0, o0, 0, WB)
    res[1].append(pv(s, 0, NH - 1))
    npt = (2 * DM - WB) // WT - WLAG
    work0 = {}
    for u in range(NP1):
        work0.setdefault(u * npt // NP1, []).append(u)
    wo_tail(0, 0, True, o0, normalize_heads(res[1]),
            {n: (lambda y, us=us: jnp.concatenate([ln1_piece(0, 0, u, y) for u in us], axis=0))
             for n, us in work0.items()})

    def epilogue():
        out_cp(NQ - 2).start()
        last = (NQ - 1) % 2
        st = load_top()
        for u in range(BQ // LNR):
            st = ln2(acc[last, u * LNR:(u + 1) * LNR, 0:DM], LAST0 + u * LNR, LNR, None, st, False)

        m1, i1, m2, i2 = st
        big = float(S)
        v1 = jnp.max(m1, axis=0, keepdims=True)
        j1 = jnp.min(jnp.where(m1 == v1, i1, big), axis=0, keepdims=True)
        taken = i1 == j1
        m1b = jnp.where(taken, m2, m1)
        i1b = jnp.where(taken, i2, i1)
        v2 = jnp.max(m1b, axis=0, keepdims=True)
        j2 = jnp.min(jnp.where(m1b == v2, i1b, big), axis=0, keepdims=True)
        idx1 = jnp.clip(j1[0, 0].astype(jnp.int32), 0, S - 1)
        idx2 = jnp.clip(j2[0, 0].astype(jnp.int32), 0, S - 1)

        row = lax.broadcasted_iota(jnp.int32, (16, DM), 0)
        def routed_row(idx):
            late = idx >= LAST0
            k = jnp.clip(idx - LAST0, 0, BQ - 1)
            mean = jnp.where(late, stat[0, pl.ds(k, 1), :], 0.0)
            rstd = jnp.where(late, stat[1, pl.ds(k, 1), :], 1.0)
            return (nbuf[pl.ds(idx, 1), :] - jnp.tile(mean, (1, DM // 128))) * jnp.tile(rstd, (1, DM // 128))

        xs = (jnp.where(row == 0, routed_row(idx1), routed_row(idx2))
              * (1.0 + _rows8(mod[:, 4 * DM:5 * DM], 16)) + _rows8(mod[:, 3 * DM:4 * DM], 16))

        acts = []
        ys = []

        def tied_bf16(v, dep):
            return jnp.concatenate([tie(v[:, 0:128], dep), v[:, 128:]], axis=-1).astype(BF16)

        def gate_up(n, dep):
            cols = slice(n * 128, (n + 1) * 128)
            xb = tied_bf16(xs, dep)
            gt = jnp.dot(xb, wgbuf[:, cols], preferred_element_type=F32)
            up = jnp.dot(xb, wubuf[:, cols], preferred_element_type=F32)
            acts.append(gt * jax.nn.sigmoid(gt) * up)
            return gt

        def down(n, dep):
            ab = tied_bf16(jnp.concatenate(acts[2 * n:2 * n + 2], axis=-1), dep)
            ys.append(jnp.dot(ab, wdbuf[n * 256:(n + 1) * 256, 0:DM], preferred_element_type=F32))
            return ys[-1]

        slots = []
        for n in range(FF // 128):
            slots.append((gate_up, n))
            if n % 2 == 1 and n >= DLAG:
                slots.append((down, (n - DLAG) // 2))
        slots += [(down, n) for n in range(FF // 256) if (down, n) not in slots]
        deps = {}
        for k, (fn, n) in enumerate(slots):
            gate = fn(n, deps.get(k))
            r0 = k * ORW
            if r0 < BQ:
                x1 = nbuf[LAST0 + r0:LAST0 + r0 + ORW, :]
                mean = tie(stat[0, r0:r0 + ORW, :], gate[0:ORW, 0:128])
                nv = (x1 - jnp.tile(mean, (1, DM // 128))) * jnp.tile(stat[1, r0:r0 + ORW, :], (1, DM // 128))
                deps[k + 2] = ln2_out(x1, nv, LAST0 + r0, ORW)[:, DM - 128:]
                if r0 + ORW in OUT_SPLIT:
                    last_cp[OUT_SPLIT.index(r0 + ORW) - 1].start()
        y = sum(ys[1:], ys[0])
        gb = mod[0:1, 5 * DM:6 * DM]
        y1 = y[0:1, :] * jax.nn.sigmoid(v1[:, 0:1]) * gb
        y2 = y[1:2, :] * jax.nn.sigmoid(v2[:, 0:1]) * gb

        fixes = []
        for n, idx in enumerate((idx1, idx2)):
            grp = jnp.clip(lax.shift_right_logical(idx, FIX.bit_length() - 1), 0, S // FIX - 1)
            base = pl.multiple_of(grp * FIX, FIX)
            rid = row[0:FIX] + base
            upd = jnp.where(rid == idx1, y1, jnp.where(rid == idx2, y2, 0.0))
            fixbuf[n] = (obuf[pl.ds(base, FIX), :].astype(F32) + upd).astype(BF16)
            fixes.append(cp(fixbuf.at[n], out_hbm.at[pl.ds(base, FIX)], sem.at[SEM_FIX]))

        for d in [out_cp(j) for j in range(NQ - 1)] + last_cp:
            d.wait()
        for d in fixes:
            d.start()
            d.wait()

    def wait_groups(t0):
        for gg in range(t0, (GWAIT + (NG,))[GWAIT.index(t0) + 1]):
            for d in group_cps(gg):
                d.wait()
        if t0 == 2:
            x_cp[3].wait()

    def step(t, carry):
        i = lax.shift_right_logical(t, NG.bit_length() - 1)
        g = t & (NG - 1)
        attention_step(i, g, (t + NG) & (NG - 1), i & 1, g == 0)

        @pl.when(jnp.logical_or(t < GWAIT[-1], g == NG - 1))
        def _():
            for t0 in GWAIT[1:]:
                pl.when(t == t0 - 1)(lambda t0=t0: wait_groups(t0))

            @pl.when(g == NG - 1)
            def _():
                @pl.when(t == NG - 1)
                def _():
                    for d in [modr_cp, x_cp[2], wr_cp] + ffn_cp:
                        d.wait()
                    hn[...] = hnext[...]
                    mod_cols(scbuf[...], 2 * DM, 6 * DM)
                    fold_vectors()

                @pl.when(jnp.logical_and(t > NG, t < NSTEP - 1))
                def _():
                    out_cp(i - 1).start()
                    hn[...] = hnext[...]

                pl.when(t == NSTEP - 1)(epilogue)

        return carry

    wait_groups(GWAIT[0])
    lax.fori_loop(1, NSTEP, step, 0)


@jax.jit
def pallas_adaLN_cond__mha_block_cached__moe_arch_mod__prompt_kernel(
    A_x: jax.Array,
    A_k_cache: jax.Array,
    A_v_cache: jax.Array,
    A_wq: jax.Array,
    A_wo: jax.Array,
    B_x: jax.Array,
    B_w_r: jax.Array,
    B_w_gate: jax.Array,
    B_w_up: jax.Array,
    B_w_down: jax.Array,
    c: jax.Array,
    w_mod: jax.Array,
):
    del B_x
    x = A_x.reshape(S, DM)
    k = A_k_cache.reshape(H, S, DH)
    v = A_v_cache.reshape(H, S, DH)
    wo = A_wo.reshape(NG, NH * DH, DM)
    any_spec = pl.BlockSpec(memory_space=pl.ANY)
    out = pl.pallas_call(
        _kernel,
        in_specs=[any_spec] * 11,
        out_specs=any_spec,
        out_shape=jax.ShapeDtypeStruct((S, DM), BF16),
        scratch_shapes=[
            pltpu.VMEM((S, DM), BF16),
            pltpu.VMEM((H, S, DH), BF16),
            pltpu.VMEM((H, S, DH), BF16),
            pltpu.VMEM((NG, DM, NH * DH), BF16),
            pltpu.VMEM((NG, NH * DH, DM), BF16),
            pltpu.VMEM((DM,), BF16),
            pltpu.VMEM((DM, FF), BF16),
            pltpu.VMEM((DM, FF), BF16),
            pltpu.VMEM((FF, DM + PAD), BF16),
            pltpu.VMEM((1, DM), BF16),
            pltpu.VMEM((16, DM), BF16),
            pltpu.VMEM((DM, 6 * DM + PAD), BF16),
            pltpu.VMEM((BQ, DM), BF16),
            pltpu.VMEM((BQ, DM), BF16),
            pltpu.VMEM((2, BQ, DM + PAD), F32),
            pltpu.VMEM((S, DM), F32),
            pltpu.VMEM((2, BQ, 128), F32),
            pltpu.VMEM((S, DM), BF16),
            pltpu.VMEM((2, FIX, DM), BF16),
            pltpu.VMEM((8, 6 * DM), F32),
            pltpu.VMEM((4, 8, DM), F32),
            pltpu.VMEM((4, 8, 128), F32),
            pltpu.SMEM((1,), jnp.int32),
            pltpu.SemaphoreType.DMA((NSEM,)),
        ],
        compiler_params=pltpu.CompilerParams(vmem_limit_bytes=124 * 1024 * 1024,
                                             disable_semaphore_checks=True),
        name="adaln_mha_moe",
    )(x, k, v, A_wq, wo, B_w_r, B_w_gate, B_w_up, B_w_down, c, w_mod)
    return out.reshape(1, S, DM)
```

```python
import jax
import jax.numpy as jnp
from jax import lax
import jax.experimental.pallas as pl
import jax.experimental.pallas.tpu as pltpu

F32 = jnp.float32
BF16 = jnp.bfloat16

S = 2048
DM = 1024
H = 32
DH = 128
FF = 3584
BQ = 512
TQ = 256
NH = 4
NQ = S // BQ
NG = H // NH
NSTEP = NQ * NG
LAST0 = S - BQ
LNR = BQ // NG
LN1_AT = ((1, 0), (1, 1), (1, 2), (1, 3))
LN2_AT = ((0, 0), (0, 1), (0, 2), (0, 3))
NP1 = len(LN1_AT)
NP2 = len(LN2_AT)
WA, WB = 256, 512
WT, WLAG = 256, 2
DLAG = 3
OUT_SPLIT = (-LNR, 192, 352, 448, BQ)
LRW = 16
ORW = 16
KG = 512
EPS = 1e-5
QSCALE = DH ** -0.5 * 1.4426950408889634
NT = (((1,), (1,)), ((), ()))
FIX = 16
PAD = 128

SEM_CX = 0
MODC = (0, 640, 896, 1024)
SEM_MOD0 = 1
SEM_A = SEM_MOD0 + len(MODC) - 1
GWAIT = (1, 2, 3, 5)
SEM_G = SEM_A + 4
SEM_REST = SEM_G + len(GWAIT)
SEM_OUT = SEM_REST + 1
SEM_FIX = SEM_OUT + 1
NSEM = SEM_FIX + 1


def _rows8(v, rows):
    return jnp.tile(v, (rows // 8, 1))


def _normalize(x):
    mean = jnp.sum(x, axis=-1, keepdims=True) * (1.0 / DM)
    xc = x - mean
    var = jnp.sum(xc * xc, axis=-1, keepdims=True) * (1.0 / DM)
    return xc * lax.rsqrt(var + EPS)


def _kernel(x_hbm, k_hbm, v_hbm, wq_hbm, wo_hbm, wr_hbm, wg_hbm, wu_hbm, wd_hbm, c_hbm, wm_hbm,
            out_hbm,
            xbuf, kbuf, vbuf, wqbuf, wobuf, wrbuf, wgbuf, wubuf, wdbuf, cbuf, scbuf, wmbuf,
            hn, hnext, acc, nbuf, stat, obuf, fixbuf, mod, vec, top, flag, sem):
    cp = pltpu.make_async_copy

    sem_last = SEM_A + 3
    c_cp = cp(c_hbm, cbuf, sem.at[SEM_CX])
    wr_cp = cp(wr_hbm, wrbuf, sem.at[SEM_REST])
    x_rng = ((0, BQ, SEM_CX), (BQ, BQ + 2 * LNR, sem_last), (2 * BQ, S, SEM_REST),
             (BQ + 2 * LNR, 2 * BQ, SEM_G + 1))
    x_cp = [cp(x_hbm.at[a:b], xbuf.at[a:b], sem.at[n]) for a, b, n in x_rng]
    mod_cp = [[cp(wm_hbm.at[:, o + MODC[n]:o + MODC[n + 1]], wmbuf.at[:, o + MODC[n]:o + MODC[n + 1]],
                  sem.at[SEM_MOD0 + n]) for o in (0, DM)] for n in range(len(MODC) - 1)]
    modr_cp = cp(wm_hbm.at[:, 2 * DM:], wmbuf.at[:, 2 * DM:6 * DM], sem.at[SEM_REST])

    def wq0_cp(h0, h1, sm):
        return cp(wq_hbm.at[:, h0 * DH:h1 * DH], wqbuf.at[0, :, h0 * DH:h1 * DH], sem.at[sm])

    def k0_cp(h, sm):
        return cp(k_hbm.at[h], kbuf.at[h], sem.at[sm])

    def v0_cp(h, sm):
        return cp(v_hbm.at[h], vbuf.at[h], sem.at[sm])

    wqe_cp = wq0_cp(0, 2, SEM_MOD0)
    step0_cp = [[k0_cp(0, SEM_A)],
                [v0_cp(0, SEM_A + 1), k0_cp(1, SEM_A + 1)],
                [v0_cp(1, SEM_A + 2), wq0_cp(2, 3, SEM_A + 2), k0_cp(2, SEM_A + 2), v0_cp(2, SEM_A + 2)],
                [wq0_cp(3, 4, sem_last), k0_cp(3, sem_last), v0_cp(3, sem_last),
                 cp(wo_hbm.at[0], wobuf.at[0], sem.at[sem_last]), x_cp[1]]]

    def group_cps(g):
        sg = sem.at[SEM_G + max(n for n, t in enumerate(GWAIT) if t <= g)]
        heads = slice(g * NH, (g + 1) * NH)
        return [cp(wq_hbm.at[:, g * NH * DH:(g + 1) * NH * DH], wqbuf.at[g], sg),
                cp(k_hbm.at[heads], kbuf.at[heads], sg),
                cp(v_hbm.at[heads], vbuf.at[heads], sg),
                cp(wo_hbm.at[g], wobuf.at[g], sg)]

    ffn_cp = [cp(wg_hbm, wgbuf, sem.at[SEM_REST]), cp(wu_hbm, wubuf, sem.at[SEM_REST]),
              cp(wd_hbm, wdbuf.at[:, 0:DM], sem.at[SEM_REST])]

    def out_cp(j):
        if isinstance(j, int):
            rows = slice(j * BQ, (j + 1) * BQ)
        else:
            rows = pl.ds(pl.multiple_of(j * BQ, BQ), BQ)
        return cp(obuf.at[rows], out_hbm.at[rows], sem.at[SEM_OUT])

    last_cp = [cp(obuf.at[LAST0 + a:LAST0 + b], out_hbm.at[LAST0 + a:LAST0 + b], sem.at[SEM_OUT])
               for a, b in zip(OUT_SPLIT[:-1], OUT_SPLIT[1:])]
    early_cp = cp(obuf.at[LAST0 - BQ:LAST0 - LNR], out_hbm.at[LAST0 - BQ:LAST0 - LNR], sem.at[SEM_OUT])

    c_cp.start()
    x_cp[0].start()
    wqe_cp.start()
    for ds in mod_cp + step0_cp:
        for d in ds:
            d.start()
    for g in range(1, NG):
        for d in group_cps(g):
            d.start()
        if g == 2:
            x_cp[3].start()
    modr_cp.start()
    wr_cp.start()
    x_cp[2].start()
    for d in ffn_cp:
        d.start()

    flag[0] = 0
    acc[1, :, 0:DM] = jnp.zeros((BQ, DM), F32)
    mod[:, 2 * DM:] = jnp.zeros((8, 4 * DM), F32)
    vec[...] = jnp.zeros((4, 8, DM), F32)
    top[0] = jnp.full((8, 128), -jnp.inf, F32)
    top[1] = jnp.zeros((8, 128), F32)
    top[2] = jnp.full((8, 128), -jnp.inf, F32)
    top[3] = jnp.zeros((8, 128), F32)

    def silu_c():
        cf = cbuf[...].astype(F32)
        sc = cf * jax.nn.sigmoid(cf)
        return jnp.broadcast_to(sc, (16, DM)).astype(BF16)

    def mod_cols(sc, lo, hi):
        mod[:, lo:hi] = jnp.dot(sc, wmbuf[:, lo:hi], preferred_element_type=F32)[:8]

    def tie(val, dep):
        if dep is None:
            return val
        n = dep.shape[0]
        head = jnp.where(flag[0] != 0, dep, val[:n])
        return head if n == val.shape[0] else jnp.concatenate([head, val[n:]], axis=0)

    def ln1_apply(n, rows, lo=0, hi=DM):
        return n * (1.0 + _rows8(mod[:, DM + lo:DM + hi], rows)) + _rows8(mod[:, lo:hi], rows)

    def load_top():
        return top[0], top[1], top[2], top[3]

    def store_top(st):
        top[0], top[1], top[2], top[3] = st

    def fold_vectors():
        sb, cb1, gb = mod[:, 3 * DM:4 * DM], 1.0 + mod[:, 4 * DM:5 * DM], mod[:, 5 * DM:6 * DM]
        wr = jnp.broadcast_to(wrbuf[...].astype(F32).reshape(1, DM), (8, DM))
        vec[0] = gb * cb1
        vec[1] = gb * sb
        vec[2] = cb1 * wr
        vec[3] = jnp.broadcast_to(jnp.sum(sb * wr, axis=-1, keepdims=True), (8, DM))

    def ln2_out(x1, n, row0, rows):
        out = x1 + n * _rows8(vec[0], rows) + _rows8(vec[1], rows)
        obuf[pl.ds(row0, rows), :] = out.astype(BF16)
        return out

    def ln2(a, row0, rows, valid, st, finish=True):
        rs = pl.ds(row0, rows)
        x1 = xbuf[rs, :].astype(F32) + _rows8(mod[:, 2 * DM:3 * DM], rows) * a
        mean = jnp.sum(x1, axis=-1, keepdims=True) * (1.0 / DM)
        xc = x1 - mean
        var = jnp.sum(xc * xc, axis=-1, keepdims=True) * (1.0 / DM)
        rstd = lax.rsqrt(var + EPS)
        if finish:
            n = xc * rstd
            nbuf[rs, :] = n
            ln2_out(x1, n, row0, rows)
            r = jnp.sum(n * _rows8(vec[2], rows), axis=-1, keepdims=True)
        else:
            nbuf[rs, :] = x1
            stat[0, pl.ds(row0 - LAST0, rows), :] = jnp.broadcast_to(mean, (rows, 128))
            stat[1, pl.ds(row0 - LAST0, rows), :] = jnp.broadcast_to(rstd, (rows, 128))
            r = jnp.sum(xc * _rows8(vec[2], rows), axis=-1, keepdims=True) * rstd
        r = r + _rows8(vec[3, :, 0:128], rows)
        if valid is not None:
            r = jnp.where(valid, r, -jnp.inf)
        m1, i1, m2, i2 = st
        base = (lax.broadcasted_iota(jnp.int32, (8, 128), 0) + row0).astype(F32)
        for u in range(rows // 8):
            ru = r[u * 8:(u + 1) * 8]
            iu = base + float(u * 8)
            gt1 = ru > m1
            gt2 = ru > m2
            m2 = jnp.where(gt1, m1, jnp.where(gt2, ru, m2))
            i2 = jnp.where(gt1, i1, jnp.where(gt2, iu, i2))
            m1 = jnp.where(gt1, ru, m1)
            i1 = jnp.where(gt1, iu, i1)
        return m1, i1, m2, i2

    def qproj(g, c, h):
        q = jnp.dot(hn[c * TQ:(c + 1) * TQ, :], wqbuf[g, :, h * DH:(h + 1) * DH],
                    preferred_element_type=F32)
        return (q * QSCALE).astype(BF16)

    def qk(q, g, h):
        return lax.dot_general(q, kbuf[g * NH + h], NT, preferred_element_type=F32)

    def pv(s, g, h, dep=None, m=None):
        if m is None:
            m = jnp.max(s, axis=-1, keepdims=True)
        lsum = None
        parts = []
        for j in range(S // KG):
            ss = [s[:, j * KG + u * 128:j * KG + (u + 1) * 128] for u in range(KG // 128)]
            if j == 0:
                ss[0] = tie(ss[0], dep)
            ps = [jnp.exp2(z - m) for z in ss]
            t = (ps[0] + ps[1]) + (ps[2] + ps[3])
            lsum = t if lsum is None else lsum + t
            ps[-1] = jnp.minimum(ps[-1], lsum)
            parts += ps
        p = jnp.concatenate(parts, axis=-1).astype(BF16)
        return jnp.dot(p, vbuf[g * NH + h], preferred_element_type=F32), lsum

    def normalize_heads(res):
        gate = jnp.minimum(res[-1][0], 0.0)
        outs = []
        for o, lsum in res:
            l = jnp.sum(jnp.maximum(lsum, gate), axis=-1, keepdims=True)
            r = pl.reciprocal(l, approx=True)
            r = r * (2.0 - l * r)
            outs.append(o * r)
        return outs

    def woproj(slot, g, first, c, outs, lo, hi, dep=None, r0=0, r1=TQ):
        parts = [o[r0:r1] for o in outs]
        oc = jnp.concatenate([tie(parts[0], dep)] + parts[1:], axis=-1).astype(BF16)
        y = jnp.dot(oc, wobuf[g, :, lo:hi], preferred_element_type=F32)
        rows = slice(c * TQ + r0, c * TQ + r1)
        if first is True:
            acc[slot, rows, lo:hi] = y
        elif first is False:
            acc[slot, rows, lo:hi] = acc[slot, rows, lo:hi] + y
        else:
            acc[slot, rows, lo:hi] = jnp.where(first, 0.0, acc[slot, rows, lo:hi]) + y
        return y

    def ln1_piece(i, g, u, gate=None):
        pr = LNR // NP1
        if isinstance(i, int) and isinstance(g, int):
            row0, off = (i + 1) * BQ + g * LNR + u * pr, g * LNR + u * pr
        else:
            row0 = pl.multiple_of(jnp.minimum((i + 1) * BQ + g * LNR, S - LNR) + u * pr, pr)
            off = pl.multiple_of(g * LNR + u * pr, pr)
        xv = xbuf[pl.ds(row0, pr), :].astype(F32)
        if gate is not None:
            xv = jnp.concatenate([tie(xv[:, 0:128], gate[0:pr, 0:128]), xv[:, 128:]], axis=-1)
        hv = ln1_apply(_normalize(xv), pr)
        hnext[pl.ds(off, pr), :] = hv.astype(BF16)
        return hv[:, 0:128]

    def ln2_piece(i, g, u, st):
        pr = LNR // NP2
        for k in range(pr // LRW):
            off = pl.multiple_of(g * LNR + u * pr + k * LRW, LRW)
            row0 = pl.multiple_of(jnp.maximum(i - 1, 0) * BQ + off, LRW)
            st = ln2(acc[(i + 1) & 1, pl.ds(off, LRW), 0:DM], row0, LRW, i > 0, st)
        return st

    def wo_tail(g, slot, first, o0, o1, work):
        pieces = [(0, o0, lo) for lo in range(WB, DM, WT)] + [(1, o1, lo) for lo in range(0, DM, WT)]
        deps = {}
        for n, (c, o, lo) in enumerate(pieces):
            y = woproj(slot, g, first, c, o, lo, lo + WT, deps.get(n))
            if n in work:
                deps[n + WLAG] = work[n](y)

    chains = [(c, h) for c in range(2) for h in range(NH)]

    def attention_step(i, g, g1, slot, first):
        st = [load_top()]

        def ln2_work(u):
            st[0] = ln2_piece(i, g, u, st[0])
            return st[0][3]

        pv_dep, work = {}, {}
        for u, at in enumerate(LN2_AT):
            if isinstance(at, tuple):
                pv_dep[at] = ln2_work(u)
            else:
                work[at] = lambda y, u=u: ln2_work(u)
        for u, at in enumerate(LN1_AT):
            if isinstance(at, tuple):
                pv_dep[at] = ln1_piece(i, g, u)
            else:
                work[at] = lambda y, u=u: ln1_piece(i, g, u, y)
        q = qproj(g, 0, 0)
        res = ([], [])
        o0 = None
        for n, (c, h) in enumerate(chains):
            s = qk(q, g, h)
            if n + 1 < len(chains):
                q = qproj((g, g1)[chains[n + 1][0]], *chains[n + 1])
            if (c, h) == (1, 0):
                o0 = normalize_heads(res[0])
                woproj(slot, g, first, 0, o0, 0, WA)
            if (c, h) == (1, NH - 1):
                woproj(slot, g, first, 0, o0, WA, WB)
            res[c].append(pv(s, g, h, pv_dep.get((c, h))))
        wo_tail(g, slot, first, o0, normalize_heads(res[1]), work)
        store_top(st[0])

    c_cp.wait()
    x_cp[0].wait()
    sc = silu_c()
    scbuf[...] = sc
    acc[0, :, 0:DM] = _normalize(xbuf[0:BQ, :].astype(F32))
    for n in range(len(MODC) - 1):
        lo, hi = MODC[n], MODC[n + 1]
        if n == 0:
            wqe_cp.wait()
        for d in mod_cp[n]:
            d.wait()
        mod_cols(sc, lo, hi)
        mod_cols(sc, DM + lo, DM + hi)
        hn[:, lo:hi] = ln1_apply(acc[0, :, lo:hi], BQ, lo, hi).astype(BF16)
        for c in range(2):
            rows = slice(c * TQ, (c + 1) * TQ)
            part = jnp.dot(hn[rows, lo:hi], wqbuf[0, lo:hi, 0:2 * DH], preferred_element_type=F32)
            if n > 0:
                part = part + nbuf[rows, 0:2 * DH]
            if hi < DM:
                nbuf[rows, 0:2 * DH] = part
            else:
                hnext[rows, 0:2 * DH] = (part * QSCALE).astype(BF16)

    def wait0(n):
        for d in step0_cp[n]:
            d.wait()

    def qk_pair(h):
        sa, sb = [qk(hnext[c * TQ:(c + 1) * TQ, h * DH:(h + 1) * DH], 0, h) for c in range(2)]
        return sa, jnp.max(sa, axis=-1, keepdims=True), sb

    wait0(0)
    sa, ma, s = qk_pair(0)
    wait0(1)
    res = ([pv(sa, 0, 0, None, ma)], [pv(s, 0, 0)])
    sa, ma, s = qk_pair(1)
    wait0(2)
    res[0].append(pv(sa, 0, 1, None, ma))
    for h in range(2, NH):
        if h == 3:
            wait0(3)
        q = qproj(0, 0, h)
        res[1].append(pv(s, 0, h - 1))
        s = qk(q, 0, h)
        q = qproj(0, 1, h)
        res[0].append(pv(s, 0, h))
        s = qk(q, 0, h)
    o0 = normalize_heads(res[0])
    woproj(0, 0, True, 0, o0, 0, WB)
    res[1].append(pv(s, 0, NH - 1))
    npt = (2 * DM - WB) // WT - WLAG
    work0 = {}
    for u in range(NP1):
        work0.setdefault(u * npt // NP1, []).append(u)
    wo_tail(0, 0, True, o0, normalize_heads(res[1]),
            {n: (lambda y, us=us: jnp.concatenate([ln1_piece(0, 0, u, y) for u in us], axis=0))
             for n, us in work0.items()})

    def epilogue():
        last = (NQ - 1) % 2
        st = load_top()
        for u in range(BQ // LNR):
            st = ln2(acc[last, u * LNR:(u + 1) * LNR, 0:DM], LAST0 + u * LNR, LNR, None, st, False)

        m1, i1, m2, i2 = st
        big = float(S)
        v1 = jnp.max(m1, axis=0, keepdims=True)
        j1 = jnp.min(jnp.where(m1 == v1, i1, big), axis=0, keepdims=True)
        taken = i1 == j1
        m1b = jnp.where(taken, m2, m1)
        i1b = jnp.where(taken, i2, i1)
        v2 = jnp.max(m1b, axis=0, keepdims=True)
        j2 = jnp.min(jnp.where(m1b == v2, i1b, big), axis=0, keepdims=True)
        idx1 = jnp.clip(j1[0, 0].astype(jnp.int32), 0, S - 1)
        idx2 = jnp.clip(j2[0, 0].astype(jnp.int32), 0, S - 1)

        row = lax.broadcasted_iota(jnp.int32, (16, DM), 0)

        def routed_row(idx):
            late = idx >= LAST0
            k = jnp.clip(idx - LAST0, 0, BQ - 1)
            mean = jnp.where(late, stat[0, pl.ds(k, 1), :], 0.0)
            rstd = jnp.where(late, stat[1, pl.ds(k, 1), :], 1.0)
            return (nbuf[pl.ds(idx, 1), :] - jnp.tile(mean, (1, DM // 128))) * jnp.tile(rstd, (1, DM // 128))

        xs = (jnp.where(row == 0, routed_row(idx1), routed_row(idx2))
              * (1.0 + _rows8(mod[:, 4 * DM:5 * DM], 16)) + _rows8(mod[:, 3 * DM:4 * DM], 16))

        acts = []
        ys = []

        def tied_bf16(v, dep):
            return jnp.concatenate([tie(v[:, 0:128], dep), v[:, 128:]], axis=-1).astype(BF16)

        def gate_up(n, dep):
            cols = slice(n * 128, (n + 1) * 128)
            xb = tied_bf16(xs, dep)
            gt = jnp.dot(xb, wgbuf[:, cols], preferred_element_type=F32)
            up = jnp.dot(xb, wubuf[:, cols], preferred_element_type=F32)
            acts.append(gt * jax.nn.sigmoid(gt) * up)
            return gt

        def down(n, dep):
            ab = tied_bf16(jnp.concatenate(acts[2 * n:2 * n + 2], axis=-1), dep)
            ys.append(jnp.dot(ab, wdbuf[n * 256:(n + 1) * 256, 0:DM], preferred_element_type=F32))
            return ys[-1]

        slots = []
        for n in range(FF // 128):
            slots.append((gate_up, n))
            if n % 2 == 1 and n >= DLAG:
                slots.append((down, (n - DLAG) // 2))
        slots += [(down, n) for n in range(FF // 256) if (down, n) not in slots]
        deps = {}
        for k, (fn, n) in enumerate(slots):
            gate = fn(n, deps.get(k))
            r0 = k * ORW
            if r0 < BQ:
                x1 = nbuf[LAST0 + r0:LAST0 + r0 + ORW, :]
                mean = tie(stat[0, r0:r0 + ORW, :], gate[0:ORW, 0:128])
                nv = (x1 - jnp.tile(mean, (1, DM // 128))) * jnp.tile(stat[1, r0:r0 + ORW, :], (1, DM // 128))
                deps[k + 2] = ln2_out(x1, nv, LAST0 + r0, ORW)[:, DM - 128:]
                if r0 + ORW in OUT_SPLIT:
                    last_cp[OUT_SPLIT.index(r0 + ORW) - 1].start()
        y = sum(ys[1:], ys[0])
        gb = mod[0:1, 5 * DM:6 * DM]
        y1 = y[0:1, :] * jax.nn.sigmoid(v1[:, 0:1]) * gb
        y2 = y[1:2, :] * jax.nn.sigmoid(v2[:, 0:1]) * gb

        fixes = []
        for n, idx in enumerate((idx1, idx2)):
            grp = jnp.clip(lax.shift_right_logical(idx, FIX.bit_length() - 1), 0, S // FIX - 1)
            base = pl.multiple_of(grp * FIX, FIX)
            rid = row[0:FIX] + base
            upd = jnp.where(rid == idx1, y1, jnp.where(rid == idx2, y2, 0.0))
            fixbuf[n] = (obuf[pl.ds(base, FIX), :].astype(F32) + upd).astype(BF16)
            fixes.append(cp(fixbuf.at[n], out_hbm.at[pl.ds(base, FIX)], sem.at[SEM_FIX]))

        for d in [out_cp(j) for j in range(NQ - 2)] + [early_cp] + last_cp:
            d.wait()
        for d in fixes:
            d.start()
            d.wait()

    def wait_groups(t0):
        for gg in range(t0, (GWAIT + (NG,))[GWAIT.index(t0) + 1]):
            for d in group_cps(gg):
                d.wait()
        if t0 == 2:
            x_cp[3].wait()

    def step(t, carry):
        i = lax.shift_right_logical(t, NG.bit_length() - 1)
        g = t & (NG - 1)
        attention_step(i, g, (t + NG) & (NG - 1), i & 1, g == 0)

        @pl.when(jnp.logical_or(jnp.logical_or(t < GWAIT[-1], t == NSTEP - 2), g == NG - 1))
        def _():
            pl.when(t == NSTEP - 2)(early_cp.start)
            for t0 in GWAIT[1:]:
                pl.when(t == t0 - 1)(lambda t0=t0: wait_groups(t0))

            @pl.when(g == NG - 1)
            def _():
                @pl.when(t == NG - 1)
                def _():
                    for d in [modr_cp, x_cp[2], wr_cp] + ffn_cp:
                        d.wait()
                    hn[...] = hnext[...]
                    mod_cols(scbuf[...], 2 * DM, 6 * DM)
                    fold_vectors()

                @pl.when(jnp.logical_and(t > NG, t < NSTEP - 1))
                def _():
                    out_cp(i - 1).start()
                    hn[...] = hnext[...]

                pl.when(t == NSTEP - 1)(epilogue)

        return carry

    wait_groups(GWAIT[0])
    lax.fori_loop(1, NSTEP, step, 0)


@jax.jit
def pallas_adaLN_cond__mha_block_cached__moe_arch_mod__prompt_kernel(
    A_x: jax.Array,
    A_k_cache: jax.Array,
    A_v_cache: jax.Array,
    A_wq: jax.Array,
    A_wo: jax.Array,
    B_x: jax.Array,
    B_w_r: jax.Array,
    B_w_gate: jax.Array,
    B_w_up: jax.Array,
    B_w_down: jax.Array,
    c: jax.Array,
    w_mod: jax.Array,
):
    del B_x
    x = A_x.reshape(S, DM)
    k = A_k_cache.reshape(H, S, DH)
    v = A_v_cache.reshape(H, S, DH)
    wo = A_wo.reshape(NG, NH * DH, DM)
    any_spec = pl.BlockSpec(memory_space=pl.ANY)
    out = pl.pallas_call(
        _kernel,
        in_specs=[any_spec] * 11,
        out_specs=any_spec,
        out_shape=jax.ShapeDtypeStruct((S, DM), BF16),
        scratch_shapes=[
            pltpu.VMEM((S, DM), BF16),
            pltpu.VMEM((H, S, DH), BF16),
            pltpu.VMEM((H, S, DH), BF16),
            pltpu.VMEM((NG, DM, NH * DH), BF16),
            pltpu.VMEM((NG, NH * DH, DM), BF16),
            pltpu.VMEM((DM,), BF16),
            pltpu.VMEM((DM, FF), BF16),
            pltpu.VMEM((DM, FF), BF16),
            pltpu.VMEM((FF, DM + PAD), BF16),
            pltpu.VMEM((1, DM), BF16),
            pltpu.VMEM((16, DM), BF16),
            pltpu.VMEM((DM, 6 * DM + PAD), BF16),
            pltpu.VMEM((BQ, DM), BF16),
            pltpu.VMEM((BQ, DM), BF16),
            pltpu.VMEM((2, BQ, DM + PAD), F32),
            pltpu.VMEM((S, DM), F32),
            pltpu.VMEM((2, BQ, 128), F32),
            pltpu.VMEM((S, DM), BF16),
            pltpu.VMEM((2, FIX, DM), BF16),
            pltpu.VMEM((8, 6 * DM), F32),
            pltpu.VMEM((4, 8, DM), F32),
            pltpu.VMEM((4, 8, 128), F32),
            pltpu.SMEM((1,), jnp.int32),
            pltpu.SemaphoreType.DMA((NSEM,)),
        ],
        compiler_params=pltpu.CompilerParams(vmem_limit_bytes=124 * 1024 * 1024,
                                             disable_semaphore_checks=True),
        name="adaln_mha_moe",
    )(x, k, v, A_wq, wo, B_w_r, B_w_gate, B_w_up, B_w_down, c, w_mod)
    return out.reshape(1, S, DM)
```

```python
import jax
import jax.numpy as jnp
from jax import lax
import jax.experimental.pallas as pl
import jax.experimental.pallas.tpu as pltpu

F32 = jnp.float32
BF16 = jnp.bfloat16

S = 2048
DM = 1024
H = 32
DH = 128
FF = 3584
BQ = 512
TQ = 256
NH = 4
NQ = S // BQ
NG = H // NH
NSTEP = NQ * NG
LAST0 = S - BQ
LNR = BQ // NG
LN1_AT = ((1, 0), (1, 1), (1, 2), (1, 3))
LN2_AT = ((0, 0), (0, 1), (0, 2), (0, 3))
NP1 = len(LN1_AT)
NP2 = len(LN2_AT)
WA, WB = 256, 512
WT, WLAG = 256, 2
DLAG = 3
OUT_SPLIT = (-LNR, 192, 352, 448, BQ)
LRW = 16
ERW = 16
ORW = 16
KG = 512
EPS = 1e-5
EPS_BF16 = 1.0013580322265625e-05
QSCALE = DH ** -0.5 * 1.4426950408889634
NT = (((1,), (1,)), ((), ()))
FIX = 16
PAD = 128

SEM_CX = 0
MODC = (0, 640, 896, 1024)
SEM_MOD0 = 1
SEM_A = SEM_MOD0 + len(MODC) - 1
GWAIT = (1, 2, 3, 5)
SEM_G = SEM_A + 4
SEM_REST = SEM_G + len(GWAIT)
SEM_OUT = SEM_REST + 1
SEM_FIX = SEM_OUT + 1
NSEM = SEM_FIX + 1


def _rows8(v, rows):
    return jnp.tile(v, (rows // 8, 1))


def _rd(x):
    return x.astype(BF16).astype(F32)


def _inv_std(var):
    sd = _rd(jnp.sqrt(_rd(_rd(var) + EPS_BF16)))
    inv = pl.reciprocal(sd, approx=True)
    return inv * (2.0 - sd * inv)


def _route_key(r, idx):
    bits = pltpu.bitcast(_rd(r), jnp.int32)
    bits = jnp.where((bits & 0x7F800000) == 0, 0x00800000, bits)
    return pltpu.bitcast(bits | jnp.where(bits >= 0, (S - 1) - idx, idx), F32)


def _normalize(x):
    mean = jnp.sum(x, axis=-1, keepdims=True) * (1.0 / DM)
    xc = x - mean
    var = jnp.sum(xc * xc, axis=-1, keepdims=True) * (1.0 / DM)
    return xc * lax.rsqrt(var + EPS)


def _kernel(x_hbm, k_hbm, v_hbm, wq_hbm, wo_hbm, wr_hbm, wg_hbm, wu_hbm, wd_hbm, c_hbm, wm_hbm,
            out_hbm,
            xbuf, kbuf, vbuf, wqbuf, wobuf, wrbuf, wgbuf, wubuf, wdbuf, cbuf, scbuf, wmbuf,
            hn, hnext, acc, nbuf, obuf, fixbuf, mod, vec, top, flag, sem):
    cp = pltpu.make_async_copy

    sem_last = SEM_A + 3
    c_cp = cp(c_hbm, cbuf, sem.at[SEM_CX])
    wr_cp = cp(wr_hbm, wrbuf, sem.at[SEM_REST])
    x_rng = ((0, BQ, SEM_CX), (BQ, BQ + 2 * LNR, sem_last), (2 * BQ, S, SEM_REST),
             (BQ + 2 * LNR, 2 * BQ, SEM_G + 1))
    x_cp = [cp(x_hbm.at[a:b], xbuf.at[a:b], sem.at[n]) for a, b, n in x_rng]
    mod_cp = [[cp(wm_hbm.at[:, o + MODC[n]:o + MODC[n + 1]], wmbuf.at[:, o + MODC[n]:o + MODC[n + 1]],
                  sem.at[SEM_MOD0 + n]) for o in (0, DM)] for n in range(len(MODC) - 1)]
    modr_cp = cp(wm_hbm.at[:, 2 * DM:], wmbuf.at[:, 2 * DM:6 * DM], sem.at[SEM_REST])

    def wq0_cp(h0, h1, sm):
        return cp(wq_hbm.at[:, h0 * DH:h1 * DH], wqbuf.at[0, :, h0 * DH:h1 * DH], sem.at[sm])

    def k0_cp(h, sm):
        return cp(k_hbm.at[h], kbuf.at[h], sem.at[sm])

    def v0_cp(h, sm):
        return cp(v_hbm.at[h], vbuf.at[h], sem.at[sm])

    wqe_cp = wq0_cp(0, 2, SEM_MOD0)
    step0_cp = [[k0_cp(0, SEM_A)],
                [v0_cp(0, SEM_A + 1), k0_cp(1, SEM_A + 1)],
                [v0_cp(1, SEM_A + 2), wq0_cp(2, 3, SEM_A + 2), k0_cp(2, SEM_A + 2), v0_cp(2, SEM_A + 2)],
                [wq0_cp(3, 4, sem_last), k0_cp(3, sem_last), v0_cp(3, sem_last),
                 cp(wo_hbm.at[0], wobuf.at[0], sem.at[sem_last]), x_cp[1]]]

    def group_cps(g):
        sg = sem.at[SEM_G + max(n for n, t in enumerate(GWAIT) if t <= g)]
        heads = slice(g * NH, (g + 1) * NH)
        return [cp(wq_hbm.at[:, g * NH * DH:(g + 1) * NH * DH], wqbuf.at[g], sg),
                cp(k_hbm.at[heads], kbuf.at[heads], sg),
                cp(v_hbm.at[heads], vbuf.at[heads], sg),
                cp(wo_hbm.at[g], wobuf.at[g], sg)]

    ffn_cp = [cp(wg_hbm, wgbuf, sem.at[SEM_REST]), cp(wu_hbm, wubuf, sem.at[SEM_REST]),
              cp(wd_hbm, wdbuf.at[:, 0:DM], sem.at[SEM_REST])]

    def out_cp(j):
        if isinstance(j, int):
            rows = slice(j * BQ, (j + 1) * BQ)
        else:
            rows = pl.ds(pl.multiple_of(j * BQ, BQ), BQ)
        return cp(obuf.at[rows], out_hbm.at[rows], sem.at[SEM_OUT])

    last_cp = [cp(obuf.at[LAST0 + a:LAST0 + b], out_hbm.at[LAST0 + a:LAST0 + b], sem.at[SEM_OUT])
               for a, b in zip(OUT_SPLIT[:-1], OUT_SPLIT[1:])]
    early_cp = cp(obuf.at[LAST0 - BQ:LAST0 - LNR], out_hbm.at[LAST0 - BQ:LAST0 - LNR], sem.at[SEM_OUT])

    c_cp.start()
    x_cp[0].start()
    wqe_cp.start()
    for ds in mod_cp + step0_cp:
        for d in ds:
            d.start()
    for g in range(1, NG):
        for d in group_cps(g):
            d.start()
        if g == 2:
            x_cp[3].start()
    modr_cp.start()
    wr_cp.start()
    x_cp[2].start()
    for d in ffn_cp:
        d.start()

    flag[0] = 0
    acc[1, :, 0:DM] = jnp.zeros((BQ, DM), F32)
    mod[:, 2 * DM:] = jnp.zeros((8, 4 * DM), F32)
    vec[...] = jnp.zeros((4, 8, DM), F32)
    top[...] = jnp.full((2, 8, 128), -jnp.inf, F32)

    def silu_c():
        cf = cbuf[...].astype(F32)
        sc = cf * jax.nn.sigmoid(cf)
        return jnp.broadcast_to(sc, (16, DM)).astype(BF16)

    def mod_cols(sc, lo, hi, scale=False):
        m = _rd(jnp.dot(sc, wmbuf[:, lo:hi], preferred_element_type=F32))
        mod[:, lo:hi] = (_rd(1.0 + m) if scale else m)[:8]

    def tie(val, dep):
        if dep is None:
            return val
        n = dep.shape[0]
        head = jnp.where(flag[0] != 0, dep, val[:n])
        return head if n == val.shape[0] else jnp.concatenate([head, val[n:]], axis=0)

    def ln1_apply(n, rows, lo=0, hi=DM):
        return n * _rows8(mod[:, DM + lo:DM + hi], rows) + _rows8(mod[:, lo:hi], rows)

    def load_top():
        return top[0], top[1]

    def store_top(st):
        top[0], top[1] = st

    def fold_vectors():
        sb, cb1, gb = mod[:, 3 * DM:4 * DM], mod[:, 4 * DM:5 * DM], mod[:, 5 * DM:6 * DM]
        wr = jnp.broadcast_to(wrbuf[...].astype(F32).reshape(1, DM), (8, DM))
        vec[0] = gb * cb1
        vec[1] = gb * sb
        vec[2] = cb1 * wr
        vec[3, :, 0:128] = jnp.broadcast_to(jnp.sum(sb * wr, axis=-1, keepdims=True), (8, 128))
        vec[3, :, 128:256] = jnp.broadcast_to(jnp.sum(cb1 * wr, axis=-1, keepdims=True), (8, 128))

    def ln2_out(x1, n, row0, rows):
        out = x1 + n * _rows8(vec[0], rows) + _rows8(vec[1], rows)
        obuf[pl.ds(row0, rows), :] = out.astype(BF16)
        return out

    def residual(a, row0, rows):
        return _rd(xbuf[pl.ds(row0, rows), :].astype(F32) + _rows8(mod[:, 2 * DM:3 * DM], rows) * a)

    def ln2(a, row0, rows, valid, st):
        x1 = residual(a, row0, rows)
        mean = jnp.sum(x1, axis=-1, keepdims=True) * (1.0 / DM)
        xc = x1 - mean
        inv = _inv_std(jnp.sum(xc * xc, axis=-1, keepdims=True) * (1.0 / DM))
        n = xc * inv
        nbuf[pl.ds(row0, rows), :] = n
        ln2_out(x1, n, row0, rows)
        r = (jnp.sum(n * _rows8(vec[2], rows), axis=-1, keepdims=True)
             + ((mean - _rd(mean)) * inv * _rows8(vec[3, :, 128:256], rows) + _rows8(vec[3, :, 0:128], rows)))
        key = _route_key(r, lax.broadcasted_iota(jnp.int32, (rows, 128), 0) + row0)
        key = jnp.where(valid, key, -jnp.inf)
        k1, k2 = st
        for u in range(rows // 8):
            ku = key[u * 8:(u + 1) * 8]
            k2 = jnp.maximum(k2, jnp.minimum(k1, ku))
            k1 = jnp.maximum(k1, ku)
        return k1, k2

    def qproj(g, c, h):
        q = jnp.dot(hn[c * TQ:(c + 1) * TQ, :], wqbuf[g, :, h * DH:(h + 1) * DH],
                    preferred_element_type=F32)
        return (q * QSCALE).astype(BF16)

    def qk(q, g, h):
        return lax.dot_general(q, kbuf[g * NH + h], NT, preferred_element_type=F32)

    def pv(s, g, h, dep=None, m=None):
        if m is None:
            m = jnp.max(s, axis=-1, keepdims=True)
        lsum = None
        parts = []
        for j in range(S // KG):
            ss = [s[:, j * KG + u * 128:j * KG + (u + 1) * 128] for u in range(KG // 128)]
            if j == 0:
                ss[0] = tie(ss[0], dep)
            ps = [jnp.exp2(z - m) for z in ss]
            t = (ps[0] + ps[1]) + (ps[2] + ps[3])
            lsum = t if lsum is None else lsum + t
            ps[-1] = jnp.minimum(ps[-1], lsum)
            parts += ps
        p = jnp.concatenate(parts, axis=-1).astype(BF16)
        return jnp.dot(p, vbuf[g * NH + h], preferred_element_type=F32), lsum

    def normalize_heads(res):
        gate = jnp.minimum(res[-1][0], 0.0)
        outs = []
        for o, lsum in res:
            l = jnp.sum(jnp.maximum(lsum, gate), axis=-1, keepdims=True)
            r = pl.reciprocal(l, approx=True)
            r = r * (2.0 - l * r)
            outs.append(o * r)
        return outs

    def woproj(slot, g, first, c, outs, lo, hi, dep=None, r0=0, r1=TQ):
        parts = [o[r0:r1] for o in outs]
        oc = jnp.concatenate([tie(parts[0], dep)] + parts[1:], axis=-1).astype(BF16)
        y = jnp.dot(oc, wobuf[g, :, lo:hi], preferred_element_type=F32)
        rows = slice(c * TQ + r0, c * TQ + r1)
        if first is True:
            acc[slot, rows, lo:hi] = y
        elif first is False:
            acc[slot, rows, lo:hi] = acc[slot, rows, lo:hi] + y
        else:
            acc[slot, rows, lo:hi] = jnp.where(first, 0.0, acc[slot, rows, lo:hi]) + y
        return y

    def ln1_piece(i, g, u, gate=None):
        pr = LNR // NP1
        if isinstance(i, int) and isinstance(g, int):
            row0, off = (i + 1) * BQ + g * LNR + u * pr, g * LNR + u * pr
        else:
            row0 = pl.multiple_of(jnp.minimum((i + 1) * BQ + g * LNR, S - LNR) + u * pr, pr)
            off = pl.multiple_of(g * LNR + u * pr, pr)
        xv = xbuf[pl.ds(row0, pr), :].astype(F32)
        if gate is not None:
            xv = jnp.concatenate([tie(xv[:, 0:128], gate[0:pr, 0:128]), xv[:, 128:]], axis=-1)
        hv = ln1_apply(_normalize(xv), pr)
        hnext[pl.ds(off, pr), :] = hv.astype(BF16)
        return hv[:, 0:128]

    def ln2_piece(i, g, u, st):
        pr = LNR // NP2
        for k in range(pr // LRW):
            off = pl.multiple_of(g * LNR + u * pr + k * LRW, LRW)
            row0 = pl.multiple_of(jnp.maximum(i - 1, 0) * BQ + off, LRW)
            st = ln2(acc[(i + 1) & 1, pl.ds(off, LRW), 0:DM], row0, LRW, i > 0, st)
        return st

    def wo_tail(g, slot, first, o0, o1, work):
        pieces = [(0, o0, lo) for lo in range(WB, DM, WT)] + [(1, o1, lo) for lo in range(0, DM, WT)]
        deps = {}
        for n, (c, o, lo) in enumerate(pieces):
            y = woproj(slot, g, first, c, o, lo, lo + WT, deps.get(n))
            if n in work:
                deps[n + WLAG] = work[n](y)

    chains = [(c, h) for c in range(2) for h in range(NH)]

    def attention_step(i, g, g1, slot, first):
        st = [load_top()]

        def ln2_work(u):
            st[0] = ln2_piece(i, g, u, st[0])
            return st[0][1]

        pv_dep, work = {}, {}
        for u, at in enumerate(LN2_AT):
            if isinstance(at, tuple):
                pv_dep[at] = ln2_work(u)
            else:
                work[at] = lambda y, u=u: ln2_work(u)
        for u, at in enumerate(LN1_AT):
            if isinstance(at, tuple):
                pv_dep[at] = ln1_piece(i, g, u)
            else:
                work[at] = lambda y, u=u: ln1_piece(i, g, u, y)
        q = qproj(g, 0, 0)
        res = ([], [])
        o0 = None
        for n, (c, h) in enumerate(chains):
            s = qk(q, g, h)
            if n + 1 < len(chains):
                q = qproj((g, g1)[chains[n + 1][0]], *chains[n + 1])
            if (c, h) == (1, 0):
                o0 = normalize_heads(res[0])
                woproj(slot, g, first, 0, o0, 0, WA)
            if (c, h) == (1, NH - 1):
                woproj(slot, g, first, 0, o0, WA, WB)
            res[c].append(pv(s, g, h, pv_dep.get((c, h))))
        wo_tail(g, slot, first, o0, normalize_heads(res[1]), work)
        store_top(st[0])

    c_cp.wait()
    x_cp[0].wait()
    sc = silu_c()
    scbuf[...] = sc
    acc[0, :, 0:DM] = _normalize(xbuf[0:BQ, :].astype(F32))
    for n in range(len(MODC) - 1):
        lo, hi = MODC[n], MODC[n + 1]
        if n == 0:
            wqe_cp.wait()
        for d in mod_cp[n]:
            d.wait()
        mod_cols(sc, lo, hi)
        mod_cols(sc, DM + lo, DM + hi, True)
        hn[:, lo:hi] = ln1_apply(acc[0, :, lo:hi], BQ, lo, hi).astype(BF16)
        for c in range(2):
            rows = slice(c * TQ, (c + 1) * TQ)
            part = jnp.dot(hn[rows, lo:hi], wqbuf[0, lo:hi, 0:2 * DH], preferred_element_type=F32)
            if n > 0:
                part = part + nbuf[rows, 0:2 * DH]
            if hi < DM:
                nbuf[rows, 0:2 * DH] = part
            else:
                hnext[rows, 0:2 * DH] = (part * QSCALE).astype(BF16)

    def wait0(n):
        for d in step0_cp[n]:
            d.wait()

    def qk_pair(h):
        sa, sb = [qk(hnext[c * TQ:(c + 1) * TQ, h * DH:(h + 1) * DH], 0, h) for c in range(2)]
        return sa, jnp.max(sa, axis=-1, keepdims=True), sb

    wait0(0)
    sa, ma, s = qk_pair(0)
    wait0(1)
    res = ([pv(sa, 0, 0, None, ma)], [pv(s, 0, 0)])
    sa, ma, s = qk_pair(1)
    wait0(2)
    res[0].append(pv(sa, 0, 1, None, ma))
    for h in range(2, NH):
        if h == 3:
            wait0(3)
        q = qproj(0, 0, h)
        res[1].append(pv(s, 0, h - 1))
        s = qk(q, 0, h)
        q = qproj(0, 1, h)
        res[0].append(pv(s, 0, h))
        s = qk(q, 0, h)
    o0 = normalize_heads(res[0])
    woproj(0, 0, True, 0, o0, 0, WB)
    res[1].append(pv(s, 0, NH - 1))
    npt = (2 * DM - WB) // WT - WLAG
    work0 = {}
    for u in range(NP1):
        work0.setdefault(u * npt // NP1, []).append(u)
    wo_tail(0, 0, True, o0, normalize_heads(res[1]),
            {n: (lambda y, us=us: jnp.concatenate([ln1_piece(0, 0, u, y) for u in us], axis=0))
             for n, us in work0.items()})

    def epilogue():
        last = (NQ - 1) % 2
        ngrp = BQ // 8
        lane = lax.broadcasted_iota(jnp.int32, (8, 128), 1)
        sums = [jnp.zeros((8, 128), F32)] * 3
        for r0 in range(0, BQ, ERW):
            x1 = residual(acc[last, r0:r0 + ERW, 0:DM], LAST0 + r0, ERW)
            nbuf[LAST0 + r0:LAST0 + r0 + ERW, :] = x1
            new = [jnp.sum(z, axis=-1, keepdims=True) for z in (x1, x1 * x1, x1 * _rows8(vec[2], ERW))]
            for u in range(ERW // 8):
                here = lane == r0 // 8 + u
                sums = [jnp.where(here, z[u * 8:(u + 1) * 8], acc_) for z, acc_ in zip(new, sums)]
        mean = sums[0] * (1.0 / DM)
        inv = _inv_std(jnp.maximum(sums[1] * (1.0 / DM) - mean * mean, 0.0))
        mean = _rd(mean)
        r = (sums[2] - mean * vec[3, :, 128:256]) * inv + vec[3, :, 0:128]
        rid = LAST0 + lane * 8 + lax.broadcasted_iota(jnp.int32, (8, 128), 0)
        k1, k2 = load_top()
        keys = jnp.where(lane < ngrp, _route_key(r, rid),
                         jnp.where(lane == ngrp, k1, jnp.where(lane == ngrp + 1, k2, -jnp.inf)))
        mean_k = jnp.where(lane < ngrp, mean, 0.0)
        inv_k = jnp.where(lane < ngrp, inv, 1.0)

        def all_reduce(op, z):
            return op(op(z, axis=1, keepdims=True), axis=0, keepdims=True)

        routed = []
        for _ in range(2):
            best = all_reduce(jnp.max, keys)
            hit = keys == best
            keys = jnp.where(hit, -jnp.inf, keys)
            bits = pltpu.bitcast(jnp.broadcast_to(best, (8, 128)), jnp.int32)
            low = bits & (S - 1)
            idx = jnp.clip(jnp.where(bits >= 0, (S - 1) - low, low)[0, 0], 0, S - 1)
            logit = pltpu.bitcast(bits & -65536, F32)[0:1, 0:1]
            nrow = ((nbuf[pl.ds(idx, 1), :] - all_reduce(jnp.sum, jnp.where(hit, mean_k, 0.0)))
                    * all_reduce(jnp.sum, jnp.where(hit, inv_k, 0.0)))
            routed.append((idx, logit, nrow))
        (idx1, v1, n1), (idx2, v2, n2) = routed

        row = lax.broadcasted_iota(jnp.int32, (16, DM), 0)
        xs = (jnp.where(row == 0, n1, n2) * _rows8(mod[:, 4 * DM:5 * DM], 16)
              + _rows8(mod[:, 3 * DM:4 * DM], 16))

        def row_stat(z, r0):
            return jnp.concatenate([jnp.broadcast_to(z[:, u:u + 1], (8, 128))
                                    for u in range(r0 // 8, (r0 + ORW) // 8)], axis=0)

        acts = []
        ys = []

        def tied_bf16(v, dep):
            return jnp.concatenate([tie(v[:, 0:128], dep), v[:, 128:]], axis=-1).astype(BF16)

        def gate_up(n, dep):
            cols = slice(n * 128, (n + 1) * 128)
            xb = tied_bf16(xs, dep)
            gt = jnp.dot(xb, wgbuf[:, cols], preferred_element_type=F32)
            up = jnp.dot(xb, wubuf[:, cols], preferred_element_type=F32)
            acts.append(gt * jax.nn.sigmoid(gt) * up)
            return gt

        def down(n, dep):
            ab = tied_bf16(jnp.concatenate(acts[2 * n:2 * n + 2], axis=-1), dep)
            ys.append(jnp.dot(ab, wdbuf[n * 256:(n + 1) * 256, 0:DM], preferred_element_type=F32))
            return ys[-1]

        slots = []
        for n in range(FF // 128):
            slots.append((gate_up, n))
            if n % 2 == 1 and n >= DLAG:
                slots.append((down, (n - DLAG) // 2))
        slots += [(down, n) for n in range(FF // 256) if (down, n) not in slots]
        deps = {}
        for k, (fn, n) in enumerate(slots):
            gate = fn(n, deps.get(k))
            r0 = k * ORW
            if r0 < BQ:
                x1 = nbuf[LAST0 + r0:LAST0 + r0 + ORW, :]
                mu = tie(row_stat(mean, r0), gate[0:ORW, 0:128])
                nv = (x1 - jnp.tile(mu, (1, DM // 128))) * jnp.tile(row_stat(inv, r0), (1, DM // 128))
                deps[k + 2] = ln2_out(x1, nv, LAST0 + r0, ORW)[:, DM - 128:]
                if r0 + ORW in OUT_SPLIT:
                    last_cp[OUT_SPLIT.index(r0 + ORW) - 1].start()
        y = sum(ys[1:], ys[0])
        gb = mod[0:1, 5 * DM:6 * DM]
        y1 = y[0:1, :] * jax.nn.sigmoid(v1) * gb
        y2 = y[1:2, :] * jax.nn.sigmoid(v2) * gb

        fixes = []
        for n, idx in enumerate((idx1, idx2)):
            grp = jnp.clip(lax.shift_right_logical(idx, FIX.bit_length() - 1), 0, S // FIX - 1)
            base = pl.multiple_of(grp * FIX, FIX)
            rid = row[0:FIX] + base
            upd = jnp.where(rid == idx1, y1, jnp.where(rid == idx2, y2, 0.0))
            fixbuf[n] = (obuf[pl.ds(base, FIX), :].astype(F32) + upd).astype(BF16)
            fixes.append(cp(fixbuf.at[n], out_hbm.at[pl.ds(base, FIX)], sem.at[SEM_FIX]))

        for d in [out_cp(j) for j in range(NQ - 2)] + [early_cp] + last_cp:
            d.wait()
        for d in fixes:
            d.start()
            d.wait()

    def wait_groups(t0):
        for gg in range(t0, (GWAIT + (NG,))[GWAIT.index(t0) + 1]):
            for d in group_cps(gg):
                d.wait()
        if t0 == 2:
            x_cp[3].wait()

    def step(t, carry):
        i = lax.shift_right_logical(t, NG.bit_length() - 1)
        g = t & (NG - 1)
        attention_step(i, g, (t + NG) & (NG - 1), i & 1, g == 0)

        @pl.when(jnp.logical_or(jnp.logical_or(t < GWAIT[-1], t == NSTEP - 2), g == NG - 1))
        def _():
            pl.when(t == NSTEP - 2)(early_cp.start)
            for t0 in GWAIT[1:]:
                pl.when(t == t0 - 1)(lambda t0=t0: wait_groups(t0))

            @pl.when(g == NG - 1)
            def _():
                @pl.when(t == NG - 1)
                def _():
                    for d in [modr_cp, x_cp[2], wr_cp] + ffn_cp:
                        d.wait()
                    hn[...] = hnext[...]
                    for k in range(2, 6):
                        mod_cols(scbuf[...], k * DM, (k + 1) * DM, k == 4)
                    fold_vectors()

                @pl.when(jnp.logical_and(t > NG, t < NSTEP - 1))
                def _():
                    out_cp(i - 1).start()
                    hn[...] = hnext[...]

                pl.when(t == NSTEP - 1)(epilogue)

        return carry

    wait_groups(GWAIT[0])
    lax.fori_loop(1, NSTEP, step, 0)


@jax.jit
def pallas_adaLN_cond__mha_block_cached__moe_arch_mod__prompt_kernel(
    A_x: jax.Array,
    A_k_cache: jax.Array,
    A_v_cache: jax.Array,
    A_wq: jax.Array,
    A_wo: jax.Array,
    B_x: jax.Array,
    B_w_r: jax.Array,
    B_w_gate: jax.Array,
    B_w_up: jax.Array,
    B_w_down: jax.Array,
    c: jax.Array,
    w_mod: jax.Array,
):
    del B_x
    x = A_x.reshape(S, DM)
    k = A_k_cache.reshape(H, S, DH)
    v = A_v_cache.reshape(H, S, DH)
    wo = A_wo.reshape(NG, NH * DH, DM)
    any_spec = pl.BlockSpec(memory_space=pl.ANY)
    out = pl.pallas_call(
        _kernel,
        in_specs=[any_spec] * 11,
        out_specs=any_spec,
        out_shape=jax.ShapeDtypeStruct((S, DM), BF16),
        scratch_shapes=[
            pltpu.VMEM((S, DM), BF16),
            pltpu.VMEM((H, S, DH), BF16),
            pltpu.VMEM((H, S, DH), BF16),
            pltpu.VMEM((NG, DM, NH * DH), BF16),
            pltpu.VMEM((NG, NH * DH, DM), BF16),
            pltpu.VMEM((DM,), BF16),
            pltpu.VMEM((DM, FF), BF16),
            pltpu.VMEM((DM, FF), BF16),
            pltpu.VMEM((FF, DM + PAD), BF16),
            pltpu.VMEM((1, DM), BF16),
            pltpu.VMEM((16, DM), BF16),
            pltpu.VMEM((DM, 6 * DM + PAD), BF16),
            pltpu.VMEM((BQ, DM), BF16),
            pltpu.VMEM((BQ, DM), BF16),
            pltpu.VMEM((2, BQ, DM + PAD), F32),
            pltpu.VMEM((S, DM), F32),
            pltpu.VMEM((S, DM), BF16),
            pltpu.VMEM((2, FIX, DM), BF16),
            pltpu.VMEM((8, 6 * DM), F32),
            pltpu.VMEM((4, 8, DM), F32),
            pltpu.VMEM((2, 8, 128), F32),
            pltpu.SMEM((1,), jnp.int32),
            pltpu.SemaphoreType.DMA((NSEM,)),
        ],
        compiler_params=pltpu.CompilerParams(vmem_limit_bytes=124 * 1024 * 1024,
                                             disable_semaphore_checks=True),
        name="adaln_mha_moe",
    )(x, k, v, A_wq, wo, B_w_r, B_w_gate, B_w_up, B_w_down, c, w_mod)
    return out.reshape(1, S, DM)
```

```python
import jax
import jax.numpy as jnp
from jax import lax
import jax.experimental.pallas as pl
import jax.experimental.pallas.tpu as pltpu

F32 = jnp.float32
BF16 = jnp.bfloat16

S = 2048
DM = 1024
H = 32
DH = 128
FF = 3584
BQ = 512
TQ = 256
NH = 4
NQ = S // BQ
NG = H // NH
NSTEP = NQ * NG
LAST0 = S - BQ
LNR = BQ // NG
LN1_AT = ((1, 0), (1, 1), (1, 2), (1, 3))
LN2_AT = ((0, 0), (0, 1), (0, 2), (0, 3))
NP1 = len(LN1_AT)
NP2 = len(LN2_AT)
WA, WB = 256, 512
WT, WLAG = 256, 2
DLAG = 3
OUT_SPLIT = (-LNR, 192, 352, 448, BQ)
LRW = 16
ERW = 16
ORW = 16
KG = 512
EPS = 1e-5
EPS_BF16 = 1.0013580322265625e-05
QSCALE = DH ** -0.5 * 1.4426950408889634
NT = (((1,), (1,)), ((), ()))
FIX = 16
PAD = 128

SEM_CX = 0
MODC = (0, 640, 896, 1024)
SEM_MOD0 = 1
SEM_A = SEM_MOD0 + len(MODC) - 1
GWAIT = (1, 2, 3, 5)
SEM_G = SEM_A + 4
SEM_REST = SEM_G + len(GWAIT)
SEM_OUT = SEM_REST + 1
SEM_FIX = SEM_OUT + 1
NSEM = SEM_FIX + 1


def _rows8(v, rows):
    return jnp.tile(v, (rows // 8, 1))


def _rd(x):
    return x.astype(BF16).astype(F32)


def _inv_std(var):
    sd = _rd(jnp.sqrt(_rd(_rd(var) + EPS_BF16)))
    inv = pl.reciprocal(sd, approx=True)
    return inv * (2.0 - sd * inv)


def _route_key(r, idx):
    bits = pltpu.bitcast(_rd(r), jnp.int32)
    bits = jnp.where((bits & 0x7F800000) == 0, 0x00800000, bits)
    return pltpu.bitcast(bits | jnp.where(bits >= 0, (S - 1) - idx, idx), F32)


def _normalize(x):
    mean = jnp.sum(x, axis=-1, keepdims=True) * (1.0 / DM)
    xc = x - mean
    var = jnp.sum(xc * xc, axis=-1, keepdims=True) * (1.0 / DM)
    return xc * lax.rsqrt(var + EPS)


def _kernel(x_hbm, k_hbm, v_hbm, wq_hbm, wo_hbm, wr_hbm, wg_hbm, wu_hbm, wd_hbm, c_hbm, wm_hbm,
            out_hbm,
            xbuf, kbuf, vbuf, wqbuf, wobuf, wrbuf, wgbuf, wubuf, wdbuf, cbuf, scbuf, wmbuf,
            hn, hnext, acc, sbuf, nbuf, obuf, fixbuf, mod, vec, top, flag, sem):
    cp = pltpu.make_async_copy

    sem_last = SEM_A + 3
    c_cp = cp(c_hbm, cbuf, sem.at[SEM_CX])
    wr_cp = cp(wr_hbm, wrbuf, sem.at[SEM_REST])
    x_rng = ((0, BQ, SEM_CX), (BQ, BQ + 2 * LNR, sem_last), (2 * BQ, S, SEM_REST),
             (BQ + 2 * LNR, 2 * BQ, SEM_G + 1))
    x_cp = [cp(x_hbm.at[a:b], xbuf.at[a:b], sem.at[n]) for a, b, n in x_rng]
    mod_cp = [[cp(wm_hbm.at[:, o + MODC[n]:o + MODC[n + 1]], wmbuf.at[:, o + MODC[n]:o + MODC[n + 1]],
                  sem.at[SEM_MOD0 + n]) for o in (0, DM)] for n in range(len(MODC) - 1)]
    modr_cp = cp(wm_hbm.at[:, 2 * DM:], wmbuf.at[:, 2 * DM:6 * DM], sem.at[SEM_REST])

    def wq0_cp(h0, h1, sm):
        return cp(wq_hbm.at[:, h0 * DH:h1 * DH], wqbuf.at[0, :, h0 * DH:h1 * DH], sem.at[sm])

    def k0_cp(h, sm):
        return cp(k_hbm.at[h], kbuf.at[h], sem.at[sm])

    def v0_cp(h, sm):
        return cp(v_hbm.at[h], vbuf.at[h], sem.at[sm])

    wqe_cp = wq0_cp(0, 2, SEM_MOD0)
    step0_cp = [[k0_cp(0, SEM_A)],
                [v0_cp(0, SEM_A + 1), k0_cp(1, SEM_A + 1)],
                [v0_cp(1, SEM_A + 2), wq0_cp(2, 3, SEM_A + 2), k0_cp(2, SEM_A + 2), v0_cp(2, SEM_A + 2)],
                [wq0_cp(3, 4, sem_last), k0_cp(3, sem_last), v0_cp(3, sem_last),
                 cp(wo_hbm.at[0], wobuf.at[0], sem.at[sem_last]), x_cp[1]]]

    def group_cps(g):
        sg = sem.at[SEM_G + max(n for n, t in enumerate(GWAIT) if t <= g)]
        heads = slice(g * NH, (g + 1) * NH)
        return [cp(wq_hbm.at[:, g * NH * DH:(g + 1) * NH * DH], wqbuf.at[g], sg),
                cp(k_hbm.at[heads], kbuf.at[heads], sg),
                cp(v_hbm.at[heads], vbuf.at[heads], sg),
                cp(wo_hbm.at[g], wobuf.at[g], sg)]

    ffn_cp = [cp(wg_hbm, wgbuf, sem.at[SEM_REST]), cp(wu_hbm, wubuf, sem.at[SEM_REST]),
              cp(wd_hbm, wdbuf.at[:, 0:DM], sem.at[SEM_REST])]

    def out_cp(j):
        if isinstance(j, int):
            rows = slice(j * BQ, (j + 1) * BQ)
        else:
            rows = pl.ds(pl.multiple_of(j * BQ, BQ), BQ)
        return cp(obuf.at[rows], out_hbm.at[rows], sem.at[SEM_OUT])

    last_cp = [cp(obuf.at[LAST0 + a:LAST0 + b], out_hbm.at[LAST0 + a:LAST0 + b], sem.at[SEM_OUT])
               for a, b in zip(OUT_SPLIT[:-1], OUT_SPLIT[1:])]
    early_cp = cp(obuf.at[LAST0 - BQ:LAST0 - LNR], out_hbm.at[LAST0 - BQ:LAST0 - LNR], sem.at[SEM_OUT])

    c_cp.start()
    x_cp[0].start()
    wqe_cp.start()
    for ds in mod_cp + step0_cp:
        for d in ds:
            d.start()
    for g in range(1, NG):
        for d in group_cps(g):
            d.start()
        if g == 2:
            x_cp[3].start()
    modr_cp.start()
    wr_cp.start()
    x_cp[2].start()
    for d in ffn_cp:
        d.start()

    flag[0] = 0
    acc[1, :, 0:DM] = jnp.zeros((BQ, DM), F32)
    mod[:, 2 * DM:] = jnp.zeros((8, 4 * DM), F32)
    vec[...] = jnp.zeros((4, 8, DM), F32)
    sbuf[LAST0:S, :] = jnp.zeros((BQ, 128), F32)
    top[...] = jnp.full((2, 8, 128), -jnp.inf, F32)

    def silu_c():
        cf = cbuf[...].astype(F32)
        sc = cf * jax.nn.sigmoid(cf)
        return jnp.broadcast_to(sc, (16, DM)).astype(BF16)

    def mod_cols(sc, lo, hi, scale=False):
        m = _rd(jnp.dot(sc, wmbuf[:, lo:hi], preferred_element_type=F32))
        mod[:, lo:hi] = (_rd(1.0 + m) if scale else m)[:8]

    def tie(val, dep):
        if dep is None:
            return val
        n = dep.shape[0]
        head = jnp.where(flag[0] != 0, dep, val[:n])
        return head if n == val.shape[0] else jnp.concatenate([head, val[n:]], axis=0)

    def ln1_apply(n, rows, lo=0, hi=DM):
        return n * _rows8(mod[:, DM + lo:DM + hi], rows) + _rows8(mod[:, lo:hi], rows)

    def load_top():
        return top[0], top[1]

    def store_top(st):
        top[0], top[1] = st

    def fold_vectors():
        sb, cb1, gb = mod[:, 3 * DM:4 * DM], mod[:, 4 * DM:5 * DM], mod[:, 5 * DM:6 * DM]
        wr = jnp.broadcast_to(wrbuf[...].astype(F32).reshape(1, DM), (8, DM))
        vec[0] = gb * cb1
        vec[1] = gb * sb
        vec[2] = cb1 * wr
        vec[3, :, 0:128] = jnp.broadcast_to(jnp.sum(sb * wr, axis=-1, keepdims=True), (8, 128))
        vec[3, :, 128:256] = jnp.broadcast_to(jnp.sum(cb1 * wr, axis=-1, keepdims=True), (8, 128))

    def ln2_out(x1, n, row0, rows):
        out = x1 + n * _rows8(vec[0], rows) + _rows8(vec[1], rows)
        obuf[pl.ds(row0, rows), :] = out.astype(BF16)
        return out

    def residual(a, row0, rows):
        return _rd(xbuf[pl.ds(row0, rows), :].astype(F32) + _rows8(mod[:, 2 * DM:3 * DM], rows) * a)

    def ln2(a, row0, rows, valid, st):
        x1 = residual(a, row0, rows)
        mean = jnp.sum(x1, axis=-1, keepdims=True) * (1.0 / DM)
        xc = x1 - mean
        inv = _inv_std(jnp.sum(xc * xc, axis=-1, keepdims=True) * (1.0 / DM))
        n = xc * inv
        shift = jnp.broadcast_to((mean - _rd(mean)) * inv, (rows, 128))
        nbuf[pl.ds(row0, rows), :] = n
        sbuf[pl.ds(row0, rows), :] = shift
        ln2_out(x1, n, row0, rows)
        r = (jnp.sum(n * _rows8(vec[2], rows), axis=-1, keepdims=True)
             + (shift * _rows8(vec[3, :, 128:256], rows) + _rows8(vec[3, :, 0:128], rows)))
        key = _route_key(r, lax.broadcasted_iota(jnp.int32, (rows, 128), 0) + row0)
        key = jnp.where(valid, key, -jnp.inf)
        k1, k2 = st
        for u in range(rows // 8):
            ku = key[u * 8:(u + 1) * 8]
            k2 = jnp.maximum(k2, jnp.minimum(k1, ku))
            k1 = jnp.maximum(k1, ku)
        return k1, k2

    def qproj(g, c, h):
        q = jnp.dot(hn[c * TQ:(c + 1) * TQ, :], wqbuf[g, :, h * DH:(h + 1) * DH],
                    preferred_element_type=F32)
        return (q * QSCALE).astype(BF16)

    def qk(q, g, h):
        return lax.dot_general(q, kbuf[g * NH + h], NT, preferred_element_type=F32)

    def pv(s, g, h, dep=None, m=None):
        if m is None:
            m = jnp.max(s, axis=-1, keepdims=True)
        lsum = None
        parts = []
        for j in range(S // KG):
            ss = [s[:, j * KG + u * 128:j * KG + (u + 1) * 128] for u in range(KG // 128)]
            if j == 0:
                ss[0] = tie(ss[0], dep)
            ps = [jnp.exp2(z - m) for z in ss]
            t = (ps[0] + ps[1]) + (ps[2] + ps[3])
            lsum = t if lsum is None else lsum + t
            ps[-1] = jnp.minimum(ps[-1], lsum)
            parts += ps
        p = jnp.concatenate(parts, axis=-1).astype(BF16)
        return jnp.dot(p, vbuf[g * NH + h], preferred_element_type=F32), lsum

    def normalize_heads(res):
        gate = jnp.minimum(res[-1][0], 0.0)
        outs = []
        for o, lsum in res:
            l = jnp.sum(jnp.maximum(lsum, gate), axis=-1, keepdims=True)
            r = pl.reciprocal(l, approx=True)
            r = r * (2.0 - l * r)
            outs.append(o * r)
        return outs

    def woproj(slot, g, first, c, outs, lo, hi, dep=None, r0=0, r1=TQ):
        parts = [o[r0:r1] for o in outs]
        oc = jnp.concatenate([tie(parts[0], dep)] + parts[1:], axis=-1).astype(BF16)
        y = jnp.dot(oc, wobuf[g, :, lo:hi], preferred_element_type=F32)
        rows = slice(c * TQ + r0, c * TQ + r1)
        if first is True:
            acc[slot, rows, lo:hi] = y
        elif first is False:
            acc[slot, rows, lo:hi] = acc[slot, rows, lo:hi] + y
        else:
            acc[slot, rows, lo:hi] = jnp.where(first, 0.0, acc[slot, rows, lo:hi]) + y
        return y

    def ln1_piece(i, g, u, gate=None):
        pr = LNR // NP1
        if isinstance(i, int) and isinstance(g, int):
            row0, off = (i + 1) * BQ + g * LNR + u * pr, g * LNR + u * pr
        else:
            row0 = pl.multiple_of(jnp.minimum((i + 1) * BQ + g * LNR, S - LNR) + u * pr, pr)
            off = pl.multiple_of(g * LNR + u * pr, pr)
        xv = xbuf[pl.ds(row0, pr), :].astype(F32)
        if gate is not None:
            xv = jnp.concatenate([tie(xv[:, 0:128], gate[0:pr, 0:128]), xv[:, 128:]], axis=-1)
        hv = ln1_apply(_normalize(xv), pr)
        hnext[pl.ds(off, pr), :] = hv.astype(BF16)
        return hv[:, 0:128]

    def ln2_piece(i, g, u, st):
        pr = LNR // NP2
        for k in range(pr // LRW):
            off = pl.multiple_of(g * LNR + u * pr + k * LRW, LRW)
            row0 = pl.multiple_of(jnp.maximum(i - 1, 0) * BQ + off, LRW)
            st = ln2(acc[(i + 1) & 1, pl.ds(off, LRW), 0:DM], row0, LRW, i > 0, st)
        return st

    def wo_tail(g, slot, first, o0, o1, work):
        pieces = [(0, o0, lo) for lo in range(WB, DM, WT)] + [(1, o1, lo) for lo in range(0, DM, WT)]
        deps = {}
        for n, (c, o, lo) in enumerate(pieces):
            y = woproj(slot, g, first, c, o, lo, lo + WT, deps.get(n))
            if n in work:
                deps[n + WLAG] = work[n](y)

    chains = [(c, h) for c in range(2) for h in range(NH)]

    def attention_step(i, g, g1, slot, first):
        st = [load_top()]

        def ln2_work(u):
            st[0] = ln2_piece(i, g, u, st[0])
            return st[0][1]

        pv_dep, work = {}, {}
        for u, at in enumerate(LN2_AT):
            if isinstance(at, tuple):
                pv_dep[at] = ln2_work(u)
            else:
                work[at] = lambda y, u=u: ln2_work(u)
        for u, at in enumerate(LN1_AT):
            if isinstance(at, tuple):
                pv_dep[at] = ln1_piece(i, g, u)
            else:
                work[at] = lambda y, u=u: ln1_piece(i, g, u, y)
        q = qproj(g, 0, 0)
        res = ([], [])
        o0 = None
        for n, (c, h) in enumerate(chains):
            s = qk(q, g, h)
            if n + 1 < len(chains):
                q = qproj((g, g1)[chains[n + 1][0]], *chains[n + 1])
            if (c, h) == (1, 0):
                o0 = normalize_heads(res[0])
                woproj(slot, g, first, 0, o0, 0, WA)
            if (c, h) == (1, NH - 1):
                woproj(slot, g, first, 0, o0, WA, WB)
            res[c].append(pv(s, g, h, pv_dep.get((c, h))))
        wo_tail(g, slot, first, o0, normalize_heads(res[1]), work)
        store_top(st[0])

    c_cp.wait()
    x_cp[0].wait()
    sc = silu_c()
    scbuf[...] = sc
    acc[0, :, 0:DM] = _normalize(xbuf[0:BQ, :].astype(F32))
    for n in range(len(MODC) - 1):
        lo, hi = MODC[n], MODC[n + 1]
        if n == 0:
            wqe_cp.wait()
        for d in mod_cp[n]:
            d.wait()
        mod_cols(sc, lo, hi)
        mod_cols(sc, DM + lo, DM + hi, True)
        hn[:, lo:hi] = ln1_apply(acc[0, :, lo:hi], BQ, lo, hi).astype(BF16)
        for c in range(2):
            rows = slice(c * TQ, (c + 1) * TQ)
            part = jnp.dot(hn[rows, lo:hi], wqbuf[0, lo:hi, 0:2 * DH], preferred_element_type=F32)
            if n > 0:
                part = part + nbuf[rows, 0:2 * DH]
            if hi < DM:
                nbuf[rows, 0:2 * DH] = part
            else:
                hnext[rows, 0:2 * DH] = (part * QSCALE).astype(BF16)

    def wait0(n):
        for d in step0_cp[n]:
            d.wait()

    def qk_pair(h):
        sa, sb = [qk(hnext[c * TQ:(c + 1) * TQ, h * DH:(h + 1) * DH], 0, h) for c in range(2)]
        return sa, jnp.max(sa, axis=-1, keepdims=True), sb

    wait0(0)
    sa, ma, s = qk_pair(0)
    wait0(1)
    res = ([pv(sa, 0, 0, None, ma)], [pv(s, 0, 0)])
    sa, ma, s = qk_pair(1)
    wait0(2)
    res[0].append(pv(sa, 0, 1, None, ma))
    for h in range(2, NH):
        if h == 3:
            wait0(3)
        q = qproj(0, 0, h)
        res[1].append(pv(s, 0, h - 1))
        s = qk(q, 0, h)
        q = qproj(0, 1, h)
        res[0].append(pv(s, 0, h))
        s = qk(q, 0, h)
    o0 = normalize_heads(res[0])
    woproj(0, 0, True, 0, o0, 0, WB)
    res[1].append(pv(s, 0, NH - 1))
    npt = (2 * DM - WB) // WT - WLAG
    work0 = {}
    for u in range(NP1):
        work0.setdefault(u * npt // NP1, []).append(u)
    wo_tail(0, 0, True, o0, normalize_heads(res[1]),
            {n: (lambda y, us=us: jnp.concatenate([ln1_piece(0, 0, u, y) for u in us], axis=0))
             for n, us in work0.items()})

    def epilogue():
        last = (NQ - 1) % 2
        ngrp = BQ // 8
        lane = lax.broadcasted_iota(jnp.int32, (8, 128), 1)
        sums = [jnp.zeros((8, 128), F32)] * 3
        for r0 in range(0, BQ, ERW):
            x1 = residual(acc[last, r0:r0 + ERW, 0:DM], LAST0 + r0, ERW)
            nbuf[LAST0 + r0:LAST0 + r0 + ERW, 0:DM] = x1
            new = [jnp.sum(z, axis=-1, keepdims=True) for z in (x1, x1 * x1, x1 * _rows8(vec[2], ERW))]
            for u in range(ERW // 8):
                here = lane == r0 // 8 + u
                sums = [jnp.where(here, z[u * 8:(u + 1) * 8], acc_) for z, acc_ in zip(new, sums)]
        mean = sums[0] * (1.0 / DM)
        inv = _inv_std(jnp.maximum(sums[1] * (1.0 / DM) - mean * mean, 0.0))
        mean = _rd(mean)
        r = (sums[2] - mean * vec[3, :, 128:256]) * inv + vec[3, :, 0:128]
        rid = LAST0 + lane * 8 + lax.broadcasted_iota(jnp.int32, (8, 128), 0)
        k1, k2 = load_top()
        keys = jnp.where(lane < ngrp, _route_key(r, rid),
                         jnp.where(lane == ngrp, k1, jnp.where(lane == ngrp + 1, k2, -jnp.inf)))
        mean_k = jnp.where(lane < ngrp, mean, 0.0)
        inv_k = jnp.where(lane < ngrp, inv, 1.0)

        def all_reduce(op, z):
            return op(op(z, axis=1, keepdims=True), axis=0, keepdims=True)

        routed = []
        for _ in range(2):
            best = all_reduce(jnp.max, keys)
            hit = keys == best
            keys = jnp.where(hit, -jnp.inf, keys)
            bits = pltpu.bitcast(jnp.broadcast_to(best, (8, 128)), jnp.int32)
            low = bits & (S - 1)
            idx = jnp.clip(jnp.where(bits >= 0, (S - 1) - low, low)[0, 0], 0, S - 1)
            logit = pltpu.bitcast(bits & -65536, F32)[0:1, 0:1]
            nrow = ((nbuf[pl.ds(idx, 1), :] - all_reduce(jnp.sum, jnp.where(hit, mean_k, 0.0)))
                    * all_reduce(jnp.sum, jnp.where(hit, inv_k, 0.0))
                    + jnp.tile(sbuf[pl.ds(idx, 1), :], (1, DM // 128)))
            routed.append((idx, logit, nrow))
        (idx1, v1, n1), (idx2, v2, n2) = routed

        row = lax.broadcasted_iota(jnp.int32, (16, DM), 0)
        xs = (_rd(_rd(jnp.where(row == 0, n1, n2)) * _rows8(mod[:, 4 * DM:5 * DM], 16))
              + _rows8(mod[:, 3 * DM:4 * DM], 16))

        def row_stat(z, r0):
            return jnp.concatenate([jnp.broadcast_to(z[:, u:u + 1], (8, 128))
                                    for u in range(r0 // 8, (r0 + ORW) // 8)], axis=0)

        acts = []
        ys = []

        def tied_bf16(v, dep):
            return jnp.concatenate([tie(v[:, 0:128], dep), v[:, 128:]], axis=-1).astype(BF16)

        def gate_up(n, dep):
            cols = slice(n * 128, (n + 1) * 128)
            xb = tied_bf16(xs, dep)
            gt = jnp.dot(xb, wgbuf[:, cols], preferred_element_type=F32)
            up = jnp.dot(xb, wubuf[:, cols], preferred_element_type=F32)
            acts.append(gt * jax.nn.sigmoid(gt) * up)
            return gt

        def down(n, dep):
            ab = tied_bf16(jnp.concatenate(acts[2 * n:2 * n + 2], axis=-1), dep)
            ys.append(jnp.dot(ab, wdbuf[n * 256:(n + 1) * 256, 0:DM], preferred_element_type=F32))
            return ys[-1]

        slots = []
        for n in range(FF // 128):
            slots.append((gate_up, n))
            if n % 2 == 1 and n >= DLAG:
                slots.append((down, (n - DLAG) // 2))
        slots += [(down, n) for n in range(FF // 256) if (down, n) not in slots]
        deps = {}
        for k, (fn, n) in enumerate(slots):
            gate = fn(n, deps.get(k))
            r0 = k * ORW
            if r0 < BQ:
                x1 = nbuf[LAST0 + r0:LAST0 + r0 + ORW, 0:DM]
                mu = tie(row_stat(mean, r0), gate[0:ORW, 0:128])
                nv = (x1 - jnp.tile(mu, (1, DM // 128))) * jnp.tile(row_stat(inv, r0), (1, DM // 128))
                deps[k + 2] = ln2_out(x1, nv, LAST0 + r0, ORW)[:, DM - 128:]
                if r0 + ORW in OUT_SPLIT:
                    last_cp[OUT_SPLIT.index(r0 + ORW) - 1].start()
        y = sum(ys[1:], ys[0])
        gb = mod[0:1, 5 * DM:6 * DM]
        y1 = y[0:1, :] * jax.nn.sigmoid(v1) * gb
        y2 = y[1:2, :] * jax.nn.sigmoid(v2) * gb

        fixes = []
        for n, idx in enumerate((idx1, idx2)):
            grp = jnp.clip(lax.shift_right_logical(idx, FIX.bit_length() - 1), 0, S // FIX - 1)
            base = pl.multiple_of(grp * FIX, FIX)
            rid = row[0:FIX] + base
            upd = jnp.where(rid == idx1, y1, jnp.where(rid == idx2, y2, 0.0))
            fixbuf[n] = (obuf[pl.ds(base, FIX), :].astype(F32) + upd).astype(BF16)
            fixes.append(cp(fixbuf.at[n], out_hbm.at[pl.ds(base, FIX)], sem.at[SEM_FIX]))

        for d in [out_cp(j) for j in range(NQ - 2)] + [early_cp] + last_cp:
            d.wait()
        for d in fixes:
            d.start()
            d.wait()

    def wait_groups(t0):
        for gg in range(t0, (GWAIT + (NG,))[GWAIT.index(t0) + 1]):
            for d in group_cps(gg):
                d.wait()
        if t0 == 2:
            x_cp[3].wait()

    def step(t, carry):
        i = lax.shift_right_logical(t, NG.bit_length() - 1)
        g = t & (NG - 1)
        attention_step(i, g, (t + NG) & (NG - 1), i & 1, g == 0)

        @pl.when(jnp.logical_or(jnp.logical_or(t < GWAIT[-1], t == NSTEP - 2), g == NG - 1))
        def _():
            pl.when(t == NSTEP - 2)(early_cp.start)
            for t0 in GWAIT[1:]:
                pl.when(t == t0 - 1)(lambda t0=t0: wait_groups(t0))

            @pl.when(g == NG - 1)
            def _():
                @pl.when(t == NG - 1)
                def _():
                    for d in [modr_cp, x_cp[2], wr_cp] + ffn_cp:
                        d.wait()
                    hn[...] = hnext[...]
                    for k in range(2, 6):
                        mod_cols(scbuf[...], k * DM, (k + 1) * DM, k == 4)
                    fold_vectors()

                @pl.when(jnp.logical_and(t > NG, t < NSTEP - 1))
                def _():
                    out_cp(i - 1).start()
                    hn[...] = hnext[...]

                pl.when(t == NSTEP - 1)(epilogue)

        return carry

    wait_groups(GWAIT[0])
    lax.fori_loop(1, NSTEP, step, 0)


@jax.jit
def pallas_adaLN_cond__mha_block_cached__moe_arch_mod__prompt_kernel(
    A_x: jax.Array,
    A_k_cache: jax.Array,
    A_v_cache: jax.Array,
    A_wq: jax.Array,
    A_wo: jax.Array,
    B_x: jax.Array,
    B_w_r: jax.Array,
    B_w_gate: jax.Array,
    B_w_up: jax.Array,
    B_w_down: jax.Array,
    c: jax.Array,
    w_mod: jax.Array,
):
    del B_x
    x = A_x.reshape(S, DM)
    k = A_k_cache.reshape(H, S, DH)
    v = A_v_cache.reshape(H, S, DH)
    wo = A_wo.reshape(NG, NH * DH, DM)
    any_spec = pl.BlockSpec(memory_space=pl.ANY)
    out = pl.pallas_call(
        _kernel,
        in_specs=[any_spec] * 11,
        out_specs=any_spec,
        out_shape=jax.ShapeDtypeStruct((S, DM), BF16),
        scratch_shapes=[
            pltpu.VMEM((S, DM), BF16),
            pltpu.VMEM((H, S, DH), BF16),
            pltpu.VMEM((H, S, DH), BF16),
            pltpu.VMEM((NG, DM, NH * DH), BF16),
            pltpu.VMEM((NG, NH * DH, DM), BF16),
            pltpu.VMEM((DM,), BF16),
            pltpu.VMEM((DM, FF), BF16),
            pltpu.VMEM((DM, FF), BF16),
            pltpu.VMEM((FF, DM + PAD), BF16),
            pltpu.VMEM((1, DM), BF16),
            pltpu.VMEM((16, DM), BF16),
            pltpu.VMEM((DM, 6 * DM + PAD), BF16),
            pltpu.VMEM((BQ, DM), BF16),
            pltpu.VMEM((BQ, DM), BF16),
            pltpu.VMEM((2, BQ, DM + PAD), F32),
            pltpu.VMEM((S, 128), F32),
            pltpu.VMEM((S, DM), F32),
            pltpu.VMEM((S, DM), BF16),
            pltpu.VMEM((2, FIX, DM), BF16),
            pltpu.VMEM((8, 6 * DM), F32),
            pltpu.VMEM((4, 8, DM), F32),
            pltpu.VMEM((2, 8, 128), F32),
            pltpu.SMEM((1,), jnp.int32),
            pltpu.SemaphoreType.DMA((NSEM,)),
        ],
        compiler_params=pltpu.CompilerParams(vmem_limit_bytes=124 * 1024 * 1024,
                                             disable_semaphore_checks=True),
        name="adaln_mha_moe",
    )(x, k, v, A_wq, wo, B_w_r, B_w_gate, B_w_up, B_w_down, c, w_mod)
    return out.reshape(1, S, DM)
```

```python
import jax
import jax.numpy as jnp
from jax import lax
import jax.experimental.pallas as pl
import jax.experimental.pallas.tpu as pltpu

F32 = jnp.float32
BF16 = jnp.bfloat16

S = 2048
DM = 1024
H = 32
DH = 128
FF = 3584
BQ = 512
TQ = 256
NH = 4
NQ = S // BQ
NG = H // NH
NSTEP = NQ * NG
LAST0 = S - BQ
LNR = BQ // NG
LN1_AT = ((1, 0), (1, 1), (1, 2), (1, 3))
LN2_AT = ((0, 0), (0, 1), (0, 2), (0, 3))
NP1 = len(LN1_AT)
NP2 = len(LN2_AT)
WA, WB = 256, 512
WT, WLAG = 256, 2
DLAG = 3
OUT_SPLIT = (-LNR, 192, 352, 448, BQ)
LRW = 16
ERW = 16
ORW = 16
KG = 512
EPS = 1e-5
EPS_BF16 = 1.0013580322265625e-05
QSCALE = DH ** -0.5 * 1.4426950408889634
NT = (((1,), (1,)), ((), ()))
FIX = 16
PAD = 128

SEM_CX = 0
MODC = (0, 640, 896, 1024)
SEM_MOD0 = 1
SEM_A = SEM_MOD0 + len(MODC) - 1
GWAIT = (1, 2, 3, 5)
SEM_G = SEM_A + 4
SEM_REST = SEM_G + len(GWAIT)
SEM_OUT = SEM_REST + 1
SEM_FIX = SEM_OUT + 1
NSEM = SEM_FIX + 1


def _rows8(v, rows):
    return jnp.tile(v, (rows // 8, 1))


def _rd(x):
    return x.astype(BF16).astype(F32)


def _inv_std(var):
    sd = _rd(jnp.sqrt(_rd(_rd(var) + EPS_BF16)))
    inv = pl.reciprocal(sd, approx=True)
    return inv * (2.0 - sd * inv)


def _route_key(r, idx):
    bits = lax.bitcast_convert_type(_rd(r), jnp.int32)
    bits = jnp.where((bits & 0x7F800000) == 0, 0x00800000, bits)
    return lax.bitcast_convert_type(bits | jnp.where(bits >= 0, (S - 1) - idx, idx), F32)


def _normalize(x):
    mean = jnp.sum(x, axis=-1, keepdims=True) * (1.0 / DM)
    xc = x - mean
    var = jnp.sum(xc * xc, axis=-1, keepdims=True) * (1.0 / DM)
    return xc * lax.rsqrt(var + EPS)


def _kernel(x_hbm, k_hbm, v_hbm, wq_hbm, wo_hbm, wr_hbm, wg_hbm, wu_hbm, wd_hbm, c_hbm, wm_hbm,
            out_hbm,
            xbuf, kbuf, vbuf, wqbuf, wobuf, wrbuf, wgbuf, wubuf, wdbuf, cbuf, scbuf, wmbuf,
            hn, hnext, acc, sbuf, nbuf, obuf, fixbuf, mod, vec, top, flag, sem):
    cp = pltpu.make_async_copy

    sem_last = SEM_A + 3
    c_cp = cp(c_hbm, cbuf, sem.at[SEM_CX])
    wr_cp = cp(wr_hbm, wrbuf, sem.at[SEM_REST])
    x_rng = ((0, BQ, SEM_CX), (BQ, BQ + 2 * LNR, sem_last), (2 * BQ, S, SEM_REST),
             (BQ + 2 * LNR, 2 * BQ, SEM_G + 1))
    x_cp = [cp(x_hbm.at[a:b], xbuf.at[a:b], sem.at[n]) for a, b, n in x_rng]
    mod_cp = [[cp(wm_hbm.at[:, o + MODC[n]:o + MODC[n + 1]], wmbuf.at[:, o + MODC[n]:o + MODC[n + 1]],
                  sem.at[SEM_MOD0 + n]) for o in (0, DM)] for n in range(len(MODC) - 1)]
    modr_cp = cp(wm_hbm.at[:, 2 * DM:], wmbuf.at[:, 2 * DM:6 * DM], sem.at[SEM_REST])

    def wq0_cp(h0, h1, sm):
        return cp(wq_hbm.at[:, h0 * DH:h1 * DH], wqbuf.at[0, :, h0 * DH:h1 * DH], sem.at[sm])

    def k0_cp(h, sm):
        return cp(k_hbm.at[h], kbuf.at[h], sem.at[sm])

    def v0_cp(h, sm):
        return cp(v_hbm.at[h], vbuf.at[h], sem.at[sm])

    wqe_cp = wq0_cp(0, 2, SEM_MOD0)
    step0_cp = [[k0_cp(0, SEM_A)],
                [v0_cp(0, SEM_A + 1), k0_cp(1, SEM_A + 1)],
                [v0_cp(1, SEM_A + 2), wq0_cp(2, 3, SEM_A + 2), k0_cp(2, SEM_A + 2), v0_cp(2, SEM_A + 2)],
                [wq0_cp(3, 4, sem_last), k0_cp(3, sem_last), v0_cp(3, sem_last),
                 cp(wo_hbm.at[0], wobuf.at[0], sem.at[sem_last]), x_cp[1]]]

    def group_cps(g):
        sg = sem.at[SEM_G + max(n for n, t in enumerate(GWAIT) if t <= g)]
        heads = slice(g * NH, (g + 1) * NH)
        return [cp(wq_hbm.at[:, g * NH * DH:(g + 1) * NH * DH], wqbuf.at[g], sg),
                cp(k_hbm.at[heads], kbuf.at[heads], sg),
                cp(v_hbm.at[heads], vbuf.at[heads], sg),
                cp(wo_hbm.at[g], wobuf.at[g], sg)]

    ffn_cp = [cp(wg_hbm, wgbuf, sem.at[SEM_REST]), cp(wu_hbm, wubuf, sem.at[SEM_REST]),
              cp(wd_hbm, wdbuf.at[:, 0:DM], sem.at[SEM_REST])]

    def out_cp(j):
        if isinstance(j, int):
            rows = slice(j * BQ, (j + 1) * BQ)
        else:
            rows = pl.ds(pl.multiple_of(j * BQ, BQ), BQ)
        return cp(obuf.at[rows], out_hbm.at[rows], sem.at[SEM_OUT])

    last_cp = [cp(obuf.at[LAST0 + a:LAST0 + b], out_hbm.at[LAST0 + a:LAST0 + b], sem.at[SEM_OUT])
               for a, b in zip(OUT_SPLIT[:-1], OUT_SPLIT[1:])]
    early_cp = cp(obuf.at[LAST0 - BQ:LAST0 - LNR], out_hbm.at[LAST0 - BQ:LAST0 - LNR], sem.at[SEM_OUT])

    c_cp.start()
    x_cp[0].start()
    wqe_cp.start()
    for ds in mod_cp + step0_cp:
        for d in ds:
            d.start()
    for g in range(1, NG):
        for d in group_cps(g):
            d.start()
        if g == 2:
            x_cp[3].start()
    modr_cp.start()
    wr_cp.start()
    x_cp[2].start()
    for d in ffn_cp:
        d.start()

    flag[0] = 0
    acc[1, :, 0:DM] = jnp.zeros((BQ, DM), F32)
    mod[:, 2 * DM:] = jnp.zeros((8, 4 * DM), F32)
    vec[...] = jnp.zeros((4, 8, DM), F32)
    sbuf[LAST0:S, :] = jnp.zeros((BQ, 128), F32)
    top[...] = jnp.full((2, 8, 128), -jnp.inf, F32)

    def silu_c():
        cf = cbuf[...].astype(F32)
        sc = cf * jax.nn.sigmoid(cf)
        return jnp.broadcast_to(sc, (16, DM)).astype(BF16)

    def mod_cols(sc, lo, hi, scale=False):
        m = _rd(jnp.dot(sc, wmbuf[:, lo:hi], preferred_element_type=F32))
        mod[:, lo:hi] = (_rd(1.0 + m) if scale else m)[:8]

    def tie(val, dep):
        if dep is None:
            return val
        n = dep.shape[0]
        head = jnp.where(flag[0] != 0, dep, val[:n])
        return head if n == val.shape[0] else jnp.concatenate([head, val[n:]], axis=0)

    def ln1_apply(n, rows, lo=0, hi=DM):
        return n * _rows8(mod[:, DM + lo:DM + hi], rows) + _rows8(mod[:, lo:hi], rows)

    def load_top():
        return top[0], top[1]

    def store_top(st):
        top[0], top[1] = st

    def fold_vectors():
        sb, cb1, gb = mod[:, 3 * DM:4 * DM], mod[:, 4 * DM:5 * DM], mod[:, 5 * DM:6 * DM]
        wr = jnp.broadcast_to(wrbuf[...].astype(F32).reshape(1, DM), (8, DM))
        vec[0] = gb * cb1
        vec[1] = gb * sb
        vec[2] = cb1 * wr
        vec[3, :, 0:128] = jnp.broadcast_to(jnp.sum(sb * wr, axis=-1, keepdims=True), (8, 128))
        vec[3, :, 128:256] = jnp.broadcast_to(jnp.sum(cb1 * wr, axis=-1, keepdims=True), (8, 128))

    def ln2_out(x1, n, row0, rows):
        out = x1 + n * _rows8(vec[0], rows) + _rows8(vec[1], rows)
        obuf[pl.ds(row0, rows), :] = out.astype(BF16)
        return out

    def residual(a, row0, rows):
        return _rd(xbuf[pl.ds(row0, rows), :].astype(F32) + _rows8(mod[:, 2 * DM:3 * DM], rows) * a)

    def ln2(a, row0, rows, valid, st):
        x1 = residual(a, row0, rows)
        mean = jnp.sum(x1, axis=-1, keepdims=True) * (1.0 / DM)
        xc = x1 - mean
        inv = _inv_std(jnp.sum(xc * xc, axis=-1, keepdims=True) * (1.0 / DM))
        n = xc * inv
        shift = jnp.broadcast_to((mean - _rd(mean)) * inv, (rows, 128))
        nbuf[pl.ds(row0, rows), :] = n
        sbuf[pl.ds(row0, rows), :] = shift
        ln2_out(x1, n, row0, rows)
        r = (jnp.sum(n * _rows8(vec[2], rows), axis=-1, keepdims=True)
             + (shift * _rows8(vec[3, :, 128:256], rows) + _rows8(vec[3, :, 0:128], rows)))
        key = _route_key(r, lax.broadcasted_iota(jnp.int32, (rows, 128), 0) + row0)
        key = jnp.where(valid, key, -jnp.inf)
        k1, k2 = st
        for u in range(rows // 8):
            ku = key[u * 8:(u + 1) * 8]
            k2 = jnp.maximum(k2, jnp.minimum(k1, ku))
            k1 = jnp.maximum(k1, ku)
        return k1, k2

    def qproj(g, c, h):
        q = jnp.dot(hn[c * TQ:(c + 1) * TQ, :], wqbuf[g, :, h * DH:(h + 1) * DH],
                    preferred_element_type=F32)
        return (q * QSCALE).astype(BF16)

    def qk(q, g, h):
        return lax.dot_general(q, kbuf[g * NH + h], NT, preferred_element_type=F32)

    def pv(s, g, h, dep=None, m=None):
        if m is None:
            m = jnp.max(s, axis=-1, keepdims=True)
        lsum = None
        parts = []
        for j in range(S // KG):
            ss = [s[:, j * KG + u * 128:j * KG + (u + 1) * 128] for u in range(KG // 128)]
            if j == 0:
                ss[0] = tie(ss[0], dep)
            ps = [jnp.exp2(z - m) for z in ss]
            t = (ps[0] + ps[1]) + (ps[2] + ps[3])
            lsum = t if lsum is None else lsum + t
            ps[-1] = jnp.minimum(ps[-1], lsum)
            parts += ps
        p = jnp.concatenate(parts, axis=-1).astype(BF16)
        return jnp.dot(p, vbuf[g * NH + h], preferred_element_type=F32), lsum

    def normalize_heads(res):
        gate = jnp.minimum(res[-1][0], 0.0)
        outs = []
        for o, lsum in res:
            l = jnp.sum(jnp.maximum(lsum, gate), axis=-1, keepdims=True)
            r = pl.reciprocal(l, approx=True)
            r = r * (2.0 - l * r)
            outs.append(o * r)
        return outs

    def woproj(slot, g, first, c, outs, lo, hi, dep=None, r0=0, r1=TQ):
        parts = [o[r0:r1] for o in outs]
        oc = jnp.concatenate([tie(parts[0], dep)] + parts[1:], axis=-1).astype(BF16)
        y = jnp.dot(oc, wobuf[g, :, lo:hi], preferred_element_type=F32)
        rows = slice(c * TQ + r0, c * TQ + r1)
        if first is True:
            acc[slot, rows, lo:hi] = y
        elif first is False:
            acc[slot, rows, lo:hi] = acc[slot, rows, lo:hi] + y
        else:
            acc[slot, rows, lo:hi] = jnp.where(first, 0.0, acc[slot, rows, lo:hi]) + y
        return y

    def ln1_piece(i, g, u, gate=None):
        pr = LNR // NP1
        if isinstance(i, int) and isinstance(g, int):
            row0, off = (i + 1) * BQ + g * LNR + u * pr, g * LNR + u * pr
        else:
            row0 = pl.multiple_of(jnp.minimum((i + 1) * BQ + g * LNR, S - LNR) + u * pr, pr)
            off = pl.multiple_of(g * LNR + u * pr, pr)
        xv = xbuf[pl.ds(row0, pr), :].astype(F32)
        if gate is not None:
            xv = jnp.concatenate([tie(xv[:, 0:128], gate[0:pr, 0:128]), xv[:, 128:]], axis=-1)
        hv = ln1_apply(_normalize(xv), pr)
        hnext[pl.ds(off, pr), :] = hv.astype(BF16)
        return hv[:, 0:128]

    def ln2_piece(i, g, u, st):
        pr = LNR // NP2
        for k in range(pr // LRW):
            off = pl.multiple_of(g * LNR + u * pr + k * LRW, LRW)
            row0 = pl.multiple_of(jnp.maximum(i - 1, 0) * BQ + off, LRW)
            st = ln2(acc[(i + 1) & 1, pl.ds(off, LRW), 0:DM], row0, LRW, i > 0, st)
        return st

    def wo_tail(g, slot, first, o0, o1, work):
        pieces = [(0, o0, lo) for lo in range(WB, DM, WT)] + [(1, o1, lo) for lo in range(0, DM, WT)]
        deps = {}
        for n, (c, o, lo) in enumerate(pieces):
            y = woproj(slot, g, first, c, o, lo, lo + WT, deps.get(n))
            if n in work:
                deps[n + WLAG] = work[n](y)

    chains = [(c, h) for c in range(2) for h in range(NH)]

    def attention_step(i, g, g1, slot, first):
        st = [load_top()]

        def ln2_work(u):
            st[0] = ln2_piece(i, g, u, st[0])
            return st[0][1]

        pv_dep, work = {}, {}
        for u, at in enumerate(LN2_AT):
            if isinstance(at, tuple):
                pv_dep[at] = ln2_work(u)
            else:
                work[at] = lambda y, u=u: ln2_work(u)
        for u, at in enumerate(LN1_AT):
            if isinstance(at, tuple):
                pv_dep[at] = ln1_piece(i, g, u)
            else:
                work[at] = lambda y, u=u: ln1_piece(i, g, u, y)
        q = qproj(g, 0, 0)
        res = ([], [])
        o0 = None
        for n, (c, h) in enumerate(chains):
            s = qk(q, g, h)
            if n + 1 < len(chains):
                q = qproj((g, g1)[chains[n + 1][0]], *chains[n + 1])
            if (c, h) == (1, 0):
                o0 = normalize_heads(res[0])
                woproj(slot, g, first, 0, o0, 0, WA)
            if (c, h) == (1, NH - 1):
                woproj(slot, g, first, 0, o0, WA, WB)
            res[c].append(pv(s, g, h, pv_dep.get((c, h))))
        wo_tail(g, slot, first, o0, normalize_heads(res[1]), work)
        store_top(st[0])

    c_cp.wait()
    x_cp[0].wait()
    sc = silu_c()
    scbuf[...] = sc
    acc[0, :, 0:DM] = _normalize(xbuf[0:BQ, :].astype(F32))
    for n in range(len(MODC) - 1):
        lo, hi = MODC[n], MODC[n + 1]
        if n == 0:
            wqe_cp.wait()
        for d in mod_cp[n]:
            d.wait()
        mod_cols(sc, lo, hi)
        mod_cols(sc, DM + lo, DM + hi, True)
        hn[:, lo:hi] = ln1_apply(acc[0, :, lo:hi], BQ, lo, hi).astype(BF16)
        for c in range(2):
            rows = slice(c * TQ, (c + 1) * TQ)
            part = jnp.dot(hn[rows, lo:hi], wqbuf[0, lo:hi, 0:2 * DH], preferred_element_type=F32)
            if n > 0:
                part = part + nbuf[rows, 0:2 * DH]
            if hi < DM:
                nbuf[rows, 0:2 * DH] = part
            else:
                hnext[rows, 0:2 * DH] = (part * QSCALE).astype(BF16)

    def wait0(n):
        for d in step0_cp[n]:
            d.wait()

    def qk_pair(h):
        sa, sb = [qk(hnext[c * TQ:(c + 1) * TQ, h * DH:(h + 1) * DH], 0, h) for c in range(2)]
        return sa, jnp.max(sa, axis=-1, keepdims=True), sb

    wait0(0)
    sa, ma, s = qk_pair(0)
    wait0(1)
    res = ([pv(sa, 0, 0, None, ma)], [pv(s, 0, 0)])
    sa, ma, s = qk_pair(1)
    wait0(2)
    res[0].append(pv(sa, 0, 1, None, ma))
    for h in range(2, NH):
        if h == 3:
            wait0(3)
        q = qproj(0, 0, h)
        res[1].append(pv(s, 0, h - 1))
        s = qk(q, 0, h)
        q = qproj(0, 1, h)
        res[0].append(pv(s, 0, h))
        s = qk(q, 0, h)
    o0 = normalize_heads(res[0])
    woproj(0, 0, True, 0, o0, 0, WB)
    res[1].append(pv(s, 0, NH - 1))
    npt = (2 * DM - WB) // WT - WLAG
    work0 = {}
    for u in range(NP1):
        work0.setdefault(u * npt // NP1, []).append(u)
    wo_tail(0, 0, True, o0, normalize_heads(res[1]),
            {n: (lambda y, us=us: jnp.concatenate([ln1_piece(0, 0, u, y) for u in us], axis=0))
             for n, us in work0.items()})

    def epilogue():
        last = (NQ - 1) % 2
        ngrp = BQ // 8
        lane = lax.broadcasted_iota(jnp.int32, (8, 128), 1)
        sums = [jnp.zeros((8, 128), F32)] * 3
        for r0 in range(0, BQ, ERW):
            x1 = residual(acc[last, r0:r0 + ERW, 0:DM], LAST0 + r0, ERW)
            nbuf[LAST0 + r0:LAST0 + r0 + ERW, 0:DM] = x1
            new = [jnp.sum(z, axis=-1, keepdims=True) for z in (x1, x1 * x1, x1 * _rows8(vec[2], ERW))]
            for u in range(ERW // 8):
                here = lane == r0 // 8 + u
                sums = [jnp.where(here, z[u * 8:(u + 1) * 8], acc_) for z, acc_ in zip(new, sums)]
        mean = sums[0] * (1.0 / DM)
        inv = _inv_std(jnp.maximum(sums[1] * (1.0 / DM) - mean * mean, 0.0))
        mean = _rd(mean)
        r = (sums[2] - mean * vec[3, :, 128:256]) * inv + vec[3, :, 0:128]
        rid = LAST0 + lane * 8 + lax.broadcasted_iota(jnp.int32, (8, 128), 0)
        k1, k2 = load_top()
        keys = jnp.where(lane < ngrp, _route_key(r, rid),
                         jnp.where(lane == ngrp, k1, jnp.where(lane == ngrp + 1, k2, -jnp.inf)))
        mean_k = jnp.where(lane < ngrp, mean, 0.0)
        inv_k = jnp.where(lane < ngrp, inv, 1.0)

        def all_reduce(op, z):
            return op(op(z, axis=1, keepdims=True), axis=0, keepdims=True)

        routed = []
        for _ in range(2):
            best = all_reduce(jnp.max, keys)
            hit = keys == best
            keys = jnp.where(hit, -jnp.inf, keys)
            bits = lax.bitcast_convert_type(jnp.broadcast_to(best, (8, 128)), jnp.int32)
            low = bits & (S - 1)
            idx = jnp.clip(jnp.where(bits >= 0, (S - 1) - low, low)[0, 0], 0, S - 1)
            logit = lax.bitcast_convert_type(bits & -65536, F32)[0:1, 0:1]
            nrow = ((nbuf[pl.ds(idx, 1), :] - all_reduce(jnp.sum, jnp.where(hit, mean_k, 0.0)))
                    * all_reduce(jnp.sum, jnp.where(hit, inv_k, 0.0))
                    + jnp.tile(sbuf[pl.ds(idx, 1), :], (1, DM // 128)))
            routed.append((idx, logit, nrow))
        (idx1, v1, n1), (idx2, v2, n2) = routed

        row = lax.broadcasted_iota(jnp.int32, (16, DM), 0)
        xs = (_rd(_rd(jnp.where(row == 0, n1, n2)) * _rows8(mod[:, 4 * DM:5 * DM], 16))
              + _rows8(mod[:, 3 * DM:4 * DM], 16))

        def row_stat(z, r0):
            return jnp.concatenate([jnp.broadcast_to(z[:, u:u + 1], (8, 128))
                                    for u in range(r0 // 8, (r0 + ORW) // 8)], axis=0)

        acts = []
        ys = []

        def tied_bf16(v, dep):
            return jnp.concatenate([tie(v[:, 0:128], dep), v[:, 128:]], axis=-1).astype(BF16)

        def gate_up(n, dep):
            cols = slice(n * 128, (n + 1) * 128)
            xb = tied_bf16(xs, dep)
            gt = jnp.dot(xb, wgbuf[:, cols], preferred_element_type=F32)
            up = jnp.dot(xb, wubuf[:, cols], preferred_element_type=F32)
            acts.append(gt * jax.nn.sigmoid(gt) * up)
            return gt

        def down(n, dep):
            ab = tied_bf16(jnp.concatenate(acts[2 * n:2 * n + 2], axis=-1), dep)
            ys.append(jnp.dot(ab, wdbuf[n * 256:(n + 1) * 256, 0:DM], preferred_element_type=F32))
            return ys[-1]

        slots = []
        for n in range(FF // 128):
            slots.append((gate_up, n))
            if n % 2 == 1 and n >= DLAG:
                slots.append((down, (n - DLAG) // 2))
        slots += [(down, n) for n in range(FF // 256) if (down, n) not in slots]
        deps = {}
        for k, (fn, n) in enumerate(slots):
            gate = fn(n, deps.get(k))
            r0 = k * ORW
            if r0 < BQ:
                x1 = nbuf[LAST0 + r0:LAST0 + r0 + ORW, 0:DM]
                mu = tie(row_stat(mean, r0), gate[0:ORW, 0:128])
                nv = (x1 - jnp.tile(mu, (1, DM // 128))) * jnp.tile(row_stat(inv, r0), (1, DM // 128))
                deps[k + 2] = ln2_out(x1, nv, LAST0 + r0, ORW)[:, DM - 128:]
                if r0 + ORW in OUT_SPLIT:
                    last_cp[OUT_SPLIT.index(r0 + ORW) - 1].start()
        y = sum(ys[1:], ys[0])
        gb = mod[0:1, 5 * DM:6 * DM]
        y1 = y[0:1, :] * jax.nn.sigmoid(v1) * gb
        y2 = y[1:2, :] * jax.nn.sigmoid(v2) * gb

        fixes = []
        for n, idx in enumerate((idx1, idx2)):
            grp = jnp.clip(lax.shift_right_logical(idx, FIX.bit_length() - 1), 0, S // FIX - 1)
            base = pl.multiple_of(grp * FIX, FIX)
            rid = row[0:FIX] + base
            upd = jnp.where(rid == idx1, y1, jnp.where(rid == idx2, y2, 0.0))
            fixbuf[n] = (obuf[pl.ds(base, FIX), :].astype(F32) + upd).astype(BF16)
            fixes.append(cp(fixbuf.at[n], out_hbm.at[pl.ds(base, FIX)], sem.at[SEM_FIX]))

        for d in [out_cp(j) for j in range(NQ - 2)] + [early_cp] + last_cp:
            d.wait()
        for d in fixes:
            d.start()
            d.wait()

    def wait_groups(t0):
        for gg in range(t0, (GWAIT + (NG,))[GWAIT.index(t0) + 1]):
            for d in group_cps(gg):
                d.wait()
        if t0 == 2:
            x_cp[3].wait()

    def step(t, carry):
        i = lax.shift_right_logical(t, NG.bit_length() - 1)
        g = t & (NG - 1)
        attention_step(i, g, (t + NG) & (NG - 1), i & 1, g == 0)

        @pl.when(jnp.logical_or(jnp.logical_or(t < GWAIT[-1], t == NSTEP - 2), g == NG - 1))
        def _():
            pl.when(t == NSTEP - 2)(early_cp.start)
            for t0 in GWAIT[1:]:
                pl.when(t == t0 - 1)(lambda t0=t0: wait_groups(t0))

            @pl.when(g == NG - 1)
            def _():
                @pl.when(t == NG - 1)
                def _():
                    for d in [modr_cp, x_cp[2], wr_cp] + ffn_cp:
                        d.wait()
                    hn[...] = hnext[...]
                    for k in range(2, 6):
                        mod_cols(scbuf[...], k * DM, (k + 1) * DM, k == 4)
                    fold_vectors()

                @pl.when(jnp.logical_and(t > NG, t < NSTEP - 1))
                def _():
                    out_cp(i - 1).start()
                    hn[...] = hnext[...]

                pl.when(t == NSTEP - 1)(epilogue)

        return carry

    wait_groups(GWAIT[0])
    lax.fori_loop(1, NSTEP, step, 0)


@jax.jit
def pallas_adaLN_cond__mha_block_cached__moe_arch_mod__prompt_kernel(
    A_x: jax.Array,
    A_k_cache: jax.Array,
    A_v_cache: jax.Array,
    A_wq: jax.Array,
    A_wo: jax.Array,
    B_x: jax.Array,
    B_w_r: jax.Array,
    B_w_gate: jax.Array,
    B_w_up: jax.Array,
    B_w_down: jax.Array,
    c: jax.Array,
    w_mod: jax.Array,
):
    del B_x
    x = A_x.reshape(S, DM)
    k = A_k_cache.reshape(H, S, DH)
    v = A_v_cache.reshape(H, S, DH)
    wo = A_wo.reshape(NG, NH * DH, DM)
    any_spec = pl.BlockSpec(memory_space=pl.ANY)
    out = pl.pallas_call(
        _kernel,
        in_specs=[any_spec] * 11,
        out_specs=any_spec,
        out_shape=jax.ShapeDtypeStruct((S, DM), BF16),
        scratch_shapes=[
            pltpu.VMEM((S, DM), BF16),
            pltpu.VMEM((H, S, DH), BF16),
            pltpu.VMEM((H, S, DH), BF16),
            pltpu.VMEM((NG, DM, NH * DH), BF16),
            pltpu.VMEM((NG, NH * DH, DM), BF16),
            pltpu.VMEM((DM,), BF16),
            pltpu.VMEM((DM, FF), BF16),
            pltpu.VMEM((DM, FF), BF16),
            pltpu.VMEM((FF, DM + PAD), BF16),
            pltpu.VMEM((1, DM), BF16),
            pltpu.VMEM((16, DM), BF16),
            pltpu.VMEM((DM, 6 * DM + PAD), BF16),
            pltpu.VMEM((BQ, DM), BF16),
            pltpu.VMEM((BQ, DM), BF16),
            pltpu.VMEM((2, BQ, DM + PAD), F32),
            pltpu.VMEM((S, 128), F32),
            pltpu.VMEM((S, DM), F32),
            pltpu.VMEM((S, DM), BF16),
            pltpu.VMEM((2, FIX, DM), BF16),
            pltpu.VMEM((8, 6 * DM), F32),
            pltpu.VMEM((4, 8, DM), F32),
            pltpu.VMEM((2, 8, 128), F32),
            pltpu.SMEM((1,), jnp.int32),
            pltpu.SemaphoreType.DMA((NSEM,)),
        ],
        compiler_params=pltpu.CompilerParams(vmem_limit_bytes=124 * 1024 * 1024,
                                             disable_semaphore_checks=True),
        name="adaln_mha_moe",
    )(x, k, v, A_wq, wo, B_w_r, B_w_gate, B_w_up, B_w_down, c, w_mod)
    return out.reshape(1, S, DM)
```

```python
import jax
import jax.numpy as jnp
from jax import lax
import jax.experimental.pallas as pl
import jax.experimental.pallas.tpu as pltpu

F32 = jnp.float32
BF16 = jnp.bfloat16

S = 2048
DM = 1024
H = 32
DH = 128
FF = 3584
BQ = 512
TQ = 256
NH = 4
NQ = S // BQ
NG = H // NH
NSTEP = NQ * NG
LAST0 = S - BQ
LNR = BQ // NG
LN1_AT = ((1, 0), (1, 1), (1, 2), (1, 3))
LN2_AT = ((0, 0), (0, 1), (0, 2), (0, 3))
NP1 = len(LN1_AT)
NP2 = len(LN2_AT)
WA, WB = 256, 512
WT, WLAG = 256, 2
DLAG = 3
OUT_SPLIT = (-LNR, 192, 352, 448, BQ)
LRW = 16
ERW = 16
ORW = 16
KG = 512
EPS = 1e-5
EPS_BF16 = 1.0013580322265625e-05
QSCALE = DH ** -0.5 * 1.4426950408889634
NT = (((1,), (1,)), ((), ()))
FIX = 16
PAD = 128

SEM_CX = 0
MODC = (0, 640, 896, 1024)
SEM_MOD0 = 1
SEM_A = SEM_MOD0 + len(MODC) - 1
GWAIT = (1, 2, 3, 5)
SEM_G = SEM_A + 4
SEM_REST = SEM_G + len(GWAIT)
SEM_OUT = SEM_REST + 1
SEM_FIX = SEM_OUT + 1
NSEM = SEM_FIX + 1


def _rows8(v, rows):
    return jnp.tile(v, (rows // 8, 1))


def _rd(x):
    return x.astype(BF16).astype(F32)


def _inv_std(var):
    sd = _rd(jnp.sqrt(_rd(_rd(var) + EPS_BF16)))
    inv = pl.reciprocal(sd, approx=True)
    return inv * (2.0 - sd * inv)


def _route_key(r, idx):
    bits = lax.bitcast_convert_type(_rd(r), jnp.int32)
    bits = jnp.where((bits & 0x7F800000) == 0, 0x00800000, bits)
    return lax.bitcast_convert_type(bits | jnp.where(bits >= 0, (S - 1) - idx, idx), F32)


def _normalize(x):
    mean = jnp.sum(x, axis=-1, keepdims=True) * (1.0 / DM)
    xc = x - mean
    var = jnp.sum(xc * xc, axis=-1, keepdims=True) * (1.0 / DM)
    return xc * lax.rsqrt(var + EPS)


def _kernel(x_hbm, k_hbm, v_hbm, wq_hbm, wo_hbm, wr_hbm, wg_hbm, wu_hbm, wd_hbm, c_hbm, wm_hbm,
            out_hbm,
            xbuf, kbuf, vbuf, wqbuf, wobuf, wrbuf, wgbuf, wubuf, wdbuf, cbuf, scbuf, wmbuf,
            hn, hnext, acc, sbuf, nbuf, obuf, fixbuf, mod, vec, top, flag, sem):
    cp = pltpu.make_async_copy

    sem_last = SEM_A + 3
    c_cp = cp(c_hbm, cbuf, sem.at[SEM_CX])
    wr_cp = cp(wr_hbm, wrbuf, sem.at[SEM_REST])
    x_rng = ((0, BQ, SEM_CX), (BQ, BQ + 2 * LNR, sem_last), (2 * BQ, S, SEM_REST),
             (BQ + 2 * LNR, 2 * BQ, SEM_G + 1))
    x_cp = [cp(x_hbm.at[a:b], xbuf.at[a:b], sem.at[n]) for a, b, n in x_rng]
    mod_cp = [[cp(wm_hbm.at[:, o + MODC[n]:o + MODC[n + 1]], wmbuf.at[:, o + MODC[n]:o + MODC[n + 1]],
                  sem.at[SEM_MOD0 + n]) for o in (0, DM)] for n in range(len(MODC) - 1)]
    modr_cp = cp(wm_hbm.at[:, 2 * DM:], wmbuf.at[:, 2 * DM:6 * DM], sem.at[SEM_REST])

    def wq0_cp(h0, h1, sm):
        return cp(wq_hbm.at[:, h0 * DH:h1 * DH], wqbuf.at[0, :, h0 * DH:h1 * DH], sem.at[sm])

    def k0_cp(h, sm):
        return cp(k_hbm.at[h], kbuf.at[h], sem.at[sm])

    def v0_cp(h, sm):
        return cp(v_hbm.at[h], vbuf.at[h], sem.at[sm])

    wqe_cp = wq0_cp(0, 2, SEM_MOD0)
    step0_cp = [[k0_cp(0, SEM_A)],
                [v0_cp(0, SEM_A + 1), k0_cp(1, SEM_A + 1)],
                [v0_cp(1, SEM_A + 2), wq0_cp(2, 3, SEM_A + 2), k0_cp(2, SEM_A + 2), v0_cp(2, SEM_A + 2)],
                [wq0_cp(3, 4, sem_last), k0_cp(3, sem_last), v0_cp(3, sem_last),
                 cp(wo_hbm.at[0], wobuf.at[0], sem.at[sem_last]), x_cp[1]]]

    def group_cps(g):
        sg = sem.at[SEM_G + max(n for n, t in enumerate(GWAIT) if t <= g)]
        heads = slice(g * NH, (g + 1) * NH)
        return [cp(wq_hbm.at[:, g * NH * DH:(g + 1) * NH * DH], wqbuf.at[g], sg),
                cp(k_hbm.at[heads], kbuf.at[heads], sg),
                cp(v_hbm.at[heads], vbuf.at[heads], sg),
                cp(wo_hbm.at[g], wobuf.at[g], sg)]

    ffn_cp = [cp(wg_hbm, wgbuf, sem.at[SEM_REST]), cp(wu_hbm, wubuf, sem.at[SEM_REST]),
              cp(wd_hbm, wdbuf.at[:, 0:DM], sem.at[SEM_REST])]

    def out_cp(j):
        if isinstance(j, int):
            rows = slice(j * BQ, (j + 1) * BQ)
        else:
            rows = pl.ds(pl.multiple_of(j * BQ, BQ), BQ)
        return cp(obuf.at[rows], out_hbm.at[rows], sem.at[SEM_OUT])

    last_cp = [cp(obuf.at[LAST0 + a:LAST0 + b], out_hbm.at[LAST0 + a:LAST0 + b], sem.at[SEM_OUT])
               for a, b in zip(OUT_SPLIT[:-1], OUT_SPLIT[1:])]
    early_cp = cp(obuf.at[LAST0 - BQ:LAST0 - LNR], out_hbm.at[LAST0 - BQ:LAST0 - LNR], sem.at[SEM_OUT])

    c_cp.start()
    x_cp[0].start()
    wqe_cp.start()
    for ds in mod_cp + step0_cp:
        for d in ds:
            d.start()
    for g in range(1, NG):
        for d in group_cps(g):
            d.start()
        if g == 2:
            x_cp[3].start()
    modr_cp.start()
    wr_cp.start()
    x_cp[2].start()
    for d in ffn_cp:
        d.start()

    flag[0] = 0
    acc[1, :, 0:DM] = jnp.zeros((BQ, DM), F32)
    mod[:, 2 * DM:] = jnp.zeros((8, 4 * DM), F32)
    vec[...] = jnp.zeros((4, 8, DM), F32)
    sbuf[LAST0:S, :] = jnp.zeros((BQ, 128), F32)
    top[...] = jnp.full((2, 8, 128), -jnp.inf, F32)

    def silu_c():
        cf = cbuf[...].astype(F32)
        sc = cf * jax.nn.sigmoid(cf)
        return jnp.broadcast_to(sc, (16, DM)).astype(BF16)

    def mod_cols(sc, lo, hi, scale=False):
        m = _rd(jnp.dot(sc, wmbuf[:, lo:hi], preferred_element_type=F32))
        mod[:, lo:hi] = (_rd(1.0 + m) if scale else m)[:8]

    def tie(val, dep):
        if dep is None:
            return val
        n = dep.shape[0]
        head = jnp.where(flag[0] != 0, dep, val[:n])
        return head if n == val.shape[0] else jnp.concatenate([head, val[n:]], axis=0)

    def ln1_apply(n, rows, lo=0, hi=DM):
        return n * _rows8(mod[:, DM + lo:DM + hi], rows) + _rows8(mod[:, lo:hi], rows)

    def load_top():
        return top[0], top[1]

    def store_top(st):
        top[0], top[1] = st

    def fold_vectors():
        sb, cb1, gb = mod[:, 3 * DM:4 * DM], mod[:, 4 * DM:5 * DM], mod[:, 5 * DM:6 * DM]
        wr = jnp.broadcast_to(wrbuf[...].astype(F32).reshape(1, DM), (8, DM))
        vec[0] = gb * cb1
        vec[1] = gb * sb
        vec[2] = cb1 * wr
        vec[3, :, 0:128] = jnp.broadcast_to(jnp.sum(sb * wr, axis=-1, keepdims=True), (8, 128))
        vec[3, :, 128:256] = jnp.broadcast_to(jnp.sum(cb1 * wr, axis=-1, keepdims=True), (8, 128))

    def ln2_out(x1, n, row0, rows):
        out = x1 + n * _rows8(vec[0], rows) + _rows8(vec[1], rows)
        obuf[pl.ds(row0, rows), :] = out.astype(BF16)
        return out

    def residual(a, row0, rows):
        return _rd(xbuf[pl.ds(row0, rows), :].astype(F32) + _rows8(mod[:, 2 * DM:3 * DM], rows) * a)

    def ln2(a, row0, rows, valid, st):
        x1 = residual(a, row0, rows)
        mean = jnp.sum(x1, axis=-1, keepdims=True) * (1.0 / DM)
        xc = x1 - mean
        inv = _inv_std(jnp.sum(xc * xc, axis=-1, keepdims=True) * (1.0 / DM))
        n = xc * inv
        shift = jnp.broadcast_to((mean - _rd(mean)) * inv, (rows, 128))
        nbuf[pl.ds(row0, rows), :] = n
        sbuf[pl.ds(row0, rows), :] = shift
        ln2_out(x1, n, row0, rows)
        r = (jnp.sum(n * _rows8(vec[2], rows), axis=-1, keepdims=True)
             + (shift * _rows8(vec[3, :, 128:256], rows) + _rows8(vec[3, :, 0:128], rows)))
        key = _route_key(r, lax.broadcasted_iota(jnp.int32, (rows, 128), 0) + row0)
        key = jnp.where(valid, key, -jnp.inf)
        k1, k2 = st
        for u in range(rows // 8):
            ku = key[u * 8:(u + 1) * 8]
            k2 = jnp.maximum(k2, jnp.minimum(k1, ku))
            k1 = jnp.maximum(k1, ku)
        return k1, k2

    def qproj(g, c, h):
        q = jnp.dot(hn[c * TQ:(c + 1) * TQ, :], wqbuf[g, :, h * DH:(h + 1) * DH],
                    preferred_element_type=F32)
        return (q * QSCALE).astype(BF16)

    def qk(q, g, h):
        return lax.dot_general(q, kbuf[g * NH + h], NT, preferred_element_type=F32)

    def pv(s, g, h, dep=None, m=None):
        if m is None:
            m = jnp.max(s, axis=-1, keepdims=True)
        lsum = None
        parts = []
        for j in range(S // KG):
            ss = [s[:, j * KG + u * 128:j * KG + (u + 1) * 128] for u in range(KG // 128)]
            if j == 0:
                ss[0] = tie(ss[0], dep)
            ps = [jnp.exp2(z - m) for z in ss]
            t = (ps[0] + ps[1]) + (ps[2] + ps[3])
            lsum = t if lsum is None else lsum + t
            ps[-1] = jnp.minimum(ps[-1], lsum)
            parts += ps
        p = jnp.concatenate(parts, axis=-1).astype(BF16)
        return jnp.dot(p, vbuf[g * NH + h], preferred_element_type=F32), lsum

    def normalize_heads(res):
        gate = jnp.minimum(res[-1][0], 0.0)
        outs = []
        for o, lsum in res:
            l = jnp.sum(jnp.maximum(lsum, gate), axis=-1, keepdims=True)
            r = pl.reciprocal(l, approx=True)
            r = r * (2.0 - l * r)
            outs.append(o * r)
        return outs

    def woproj(slot, g, first, c, outs, lo, hi, dep=None, r0=0, r1=TQ):
        parts = [o[r0:r1] for o in outs]
        oc = jnp.concatenate([tie(parts[0], dep)] + parts[1:], axis=-1).astype(BF16)
        y = jnp.dot(oc, wobuf[g, :, lo:hi], preferred_element_type=F32)
        rows = slice(c * TQ + r0, c * TQ + r1)
        if first is True:
            acc[slot, rows, lo:hi] = y
        elif first is False:
            acc[slot, rows, lo:hi] = acc[slot, rows, lo:hi] + y
        else:
            acc[slot, rows, lo:hi] = jnp.where(first, 0.0, acc[slot, rows, lo:hi]) + y
        return y

    def ln1_piece(i, g, u, gate=None):
        pr = LNR // NP1
        if isinstance(i, int) and isinstance(g, int):
            row0, off = (i + 1) * BQ + g * LNR + u * pr, g * LNR + u * pr
        else:
            row0 = pl.multiple_of(jnp.minimum((i + 1) * BQ + g * LNR, S - LNR) + u * pr, pr)
            off = pl.multiple_of(g * LNR + u * pr, pr)
        xv = xbuf[pl.ds(row0, pr), :].astype(F32)
        if gate is not None:
            xv = jnp.concatenate([tie(xv[:, 0:128], gate[0:pr, 0:128]), xv[:, 128:]], axis=-1)
        hv = ln1_apply(_normalize(xv), pr)
        hnext[pl.ds(off, pr), :] = hv.astype(BF16)
        return hv[:, 0:128]

    def ln2_piece(i, g, u, st):
        pr = LNR // NP2
        for k in range(pr // LRW):
            off = pl.multiple_of(g * LNR + u * pr + k * LRW, LRW)
            row0 = pl.multiple_of(jnp.maximum(i - 1, 0) * BQ + off, LRW)
            st = ln2(acc[(i + 1) & 1, pl.ds(off, LRW), 0:DM], row0, LRW, i > 0, st)
        return st

    def wo_tail(g, slot, first, o0, o1, work):
        pieces = [(0, o0, lo) for lo in range(WB, DM, WT)] + [(1, o1, lo) for lo in range(0, DM, WT)]
        deps = {}
        for n, (c, o, lo) in enumerate(pieces):
            y = woproj(slot, g, first, c, o, lo, lo + WT, deps.get(n))
            if n in work:
                deps[n + WLAG] = work[n](y)

    chains = [(c, h) for c in range(2) for h in range(NH)]

    def attention_step(i, g, g1, slot, first):
        st = [load_top()]

        def ln2_work(u):
            st[0] = ln2_piece(i, g, u, st[0])
            return st[0][1]

        pv_dep, work = {}, {}
        for u, at in enumerate(LN2_AT):
            if isinstance(at, tuple):
                pv_dep[at] = ln2_work(u)
            else:
                work[at] = lambda y, u=u: ln2_work(u)
        for u, at in enumerate(LN1_AT):
            if isinstance(at, tuple):
                pv_dep[at] = ln1_piece(i, g, u)
            else:
                work[at] = lambda y, u=u: ln1_piece(i, g, u, y)
        q = qproj(g, 0, 0)
        res = ([], [])
        o0 = None
        for n, (c, h) in enumerate(chains):
            s = qk(q, g, h)
            if n + 1 < len(chains):
                q = qproj((g, g1)[chains[n + 1][0]], *chains[n + 1])
            if (c, h) == (1, 0):
                o0 = normalize_heads(res[0])
                woproj(slot, g, first, 0, o0, 0, WA)
            if (c, h) == (1, NH - 1):
                woproj(slot, g, first, 0, o0, WA, WB)
            res[c].append(pv(s, g, h, pv_dep.get((c, h))))
        wo_tail(g, slot, first, o0, normalize_heads(res[1]), work)
        store_top(st[0])

    c_cp.wait()
    x_cp[0].wait()
    sc = silu_c()
    scbuf[...] = sc
    acc[0, :, 0:DM] = _normalize(xbuf[0:BQ, :].astype(F32))
    for n in range(len(MODC) - 1):
        lo, hi = MODC[n], MODC[n + 1]
        if n == 0:
            wqe_cp.wait()
        for d in mod_cp[n]:
            d.wait()
        mod_cols(sc, lo, hi)
        mod_cols(sc, DM + lo, DM + hi, True)
        hn[:, lo:hi] = ln1_apply(acc[0, :, lo:hi], BQ, lo, hi).astype(BF16)
        for c in range(2):
            rows = slice(c * TQ, (c + 1) * TQ)
            part = jnp.dot(hn[rows, lo:hi], wqbuf[0, lo:hi, 0:2 * DH], preferred_element_type=F32)
            if n > 0:
                part = part + nbuf[rows, 0:2 * DH]
            if hi < DM:
                nbuf[rows, 0:2 * DH] = part
            else:
                hnext[rows, 0:2 * DH] = (part * QSCALE).astype(BF16)

    def wait0(n):
        for d in step0_cp[n]:
            d.wait()

    def qk_pair(h):
        sa, sb = [qk(hnext[c * TQ:(c + 1) * TQ, h * DH:(h + 1) * DH], 0, h) for c in range(2)]
        return sa, jnp.max(sa, axis=-1, keepdims=True), sb

    wait0(0)
    sa, ma, s = qk_pair(0)
    wait0(1)
    res = ([pv(sa, 0, 0, None, ma)], [pv(s, 0, 0)])
    sa, ma, s = qk_pair(1)
    wait0(2)
    res[0].append(pv(sa, 0, 1, None, ma))
    for h in range(2, NH):
        if h == 3:
            wait0(3)
        q = qproj(0, 0, h)
        res[1].append(pv(s, 0, h - 1))
        s = qk(q, 0, h)
        q = qproj(0, 1, h)
        res[0].append(pv(s, 0, h))
        s = qk(q, 0, h)
    o0 = normalize_heads(res[0])
    woproj(0, 0, True, 0, o0, 0, WB)
    res[1].append(pv(s, 0, NH - 1))
    npt = (2 * DM - WB) // WT - WLAG
    work0 = {}
    for u in range(NP1):
        work0.setdefault(u * npt // NP1, []).append(u)
    wo_tail(0, 0, True, o0, normalize_heads(res[1]),
            {n: (lambda y, us=us: jnp.concatenate([ln1_piece(0, 0, u, y) for u in us], axis=0))
             for n, us in work0.items()})

    def epilogue():
        last = (NQ - 1) % 2
        ngrp = BQ // 8
        lane = lax.broadcasted_iota(jnp.int32, (8, 128), 1)
        sums = [jnp.zeros((8, 128), F32)] * 3
        for r0 in range(0, BQ, ERW):
            x1 = residual(acc[last, r0:r0 + ERW, 0:DM], LAST0 + r0, ERW)
            nbuf[LAST0 + r0:LAST0 + r0 + ERW, 0:DM] = x1
            new = [jnp.sum(z, axis=-1, keepdims=True) for z in (x1, x1 * x1, x1 * _rows8(vec[2], ERW))]
            for u in range(ERW // 8):
                here = lane == r0 // 8 + u
                sums = [jnp.where(here, z[u * 8:(u + 1) * 8], acc_) for z, acc_ in zip(new, sums)]
        mean = sums[0] * (1.0 / DM)
        inv = _inv_std(jnp.maximum(sums[1] * (1.0 / DM) - mean * mean, 0.0))
        mean = _rd(mean)
        r = (sums[2] - mean * vec[3, :, 128:256]) * inv + vec[3, :, 0:128]
        rid = LAST0 + lane * 8 + lax.broadcasted_iota(jnp.int32, (8, 128), 0)
        k1, k2 = load_top()
        keys = jnp.where(lane < ngrp, _route_key(r, rid),
                         jnp.where(lane == ngrp, k1, jnp.where(lane == ngrp + 1, k2, -jnp.inf)))
        mean_k = jnp.where(lane < ngrp, mean, 0.0)
        inv_k = jnp.where(lane < ngrp, inv, 1.0)

        def all_sum(z):
            return jnp.sum(jnp.sum(z, axis=1, keepdims=True), axis=0, keepdims=True)

        t1 = jnp.max(keys, axis=0, keepdims=True)
        t2 = jnp.max(jnp.where(keys == t1, -jnp.inf, keys), axis=0, keepdims=True)
        sub = lax.broadcasted_iota(jnp.int32, (8, 128), 0)
        bit = lax.shift_right_logical(lane, sub) & 1
        half = [jnp.max(jnp.where(sub == 7, t2, jnp.where(bit == b, t1, -jnp.inf)), axis=1, keepdims=True)
                for b in range(2)]
        bests = (jnp.max(jnp.maximum(half[0], half[1]), axis=0, keepdims=True),
                 jnp.max(jnp.minimum(half[0], half[1]), axis=0, keepdims=True))

        routed = []
        for best in bests:
            hit = keys == best
            bits = lax.bitcast_convert_type(jnp.broadcast_to(best, (8, 128)), jnp.int32)
            low = bits & (S - 1)
            idx = jnp.clip(jnp.where(bits >= 0, (S - 1) - low, low)[0, 0], 0, S - 1)
            logit = lax.bitcast_convert_type(bits & -65536, F32)[0:1, 0:1]
            nrow = ((nbuf[pl.ds(idx, 1), :] - all_sum(jnp.where(hit, mean_k, 0.0)))
                    * all_sum(jnp.where(hit, inv_k, 0.0))
                    + jnp.tile(sbuf[pl.ds(idx, 1), :], (1, DM // 128)))
            routed.append((idx, logit, nrow))
        (idx1, v1, n1), (idx2, v2, n2) = routed

        row = lax.broadcasted_iota(jnp.int32, (16, DM), 0)
        xs = (_rd(_rd(jnp.where(row == 0, n1, n2)) * _rows8(mod[:, 4 * DM:5 * DM], 16))
              + _rows8(mod[:, 3 * DM:4 * DM], 16))

        def row_stat(z, r0):
            return jnp.concatenate([jnp.broadcast_to(z[:, u:u + 1], (8, 128))
                                    for u in range(r0 // 8, (r0 + ORW) // 8)], axis=0)

        acts = []
        ys = []

        def tied_bf16(v, dep):
            return jnp.concatenate([tie(v[:, 0:128], dep), v[:, 128:]], axis=-1).astype(BF16)

        def gate_up(n, dep):
            cols = slice(n * 128, (n + 1) * 128)
            xb = tied_bf16(xs, dep)
            gt = jnp.dot(xb, wgbuf[:, cols], preferred_element_type=F32)
            up = jnp.dot(xb, wubuf[:, cols], preferred_element_type=F32)
            acts.append(gt * jax.nn.sigmoid(gt) * up)
            return gt

        def down(n, dep):
            ab = tied_bf16(jnp.concatenate(acts[2 * n:2 * n + 2], axis=-1), dep)
            ys.append(jnp.dot(ab, wdbuf[n * 256:(n + 1) * 256, 0:DM], preferred_element_type=F32))
            return ys[-1]

        slots = []
        for n in range(FF // 128):
            slots.append((gate_up, n))
            if n % 2 == 1 and n >= DLAG:
                slots.append((down, (n - DLAG) // 2))
        slots += [(down, n) for n in range(FF // 256) if (down, n) not in slots]
        deps = {}
        for k, (fn, n) in enumerate(slots):
            gate = fn(n, deps.get(k))
            r0 = k * ORW
            if r0 < BQ:
                x1 = nbuf[LAST0 + r0:LAST0 + r0 + ORW, 0:DM]
                mu = tie(row_stat(mean, r0), gate[0:ORW, 0:128])
                nv = (x1 - jnp.tile(mu, (1, DM // 128))) * jnp.tile(row_stat(inv, r0), (1, DM // 128))
                deps[k + 2] = ln2_out(x1, nv, LAST0 + r0, ORW)[:, DM - 128:]
                if r0 + ORW in OUT_SPLIT:
                    last_cp[OUT_SPLIT.index(r0 + ORW) - 1].start()
        y = sum(ys[1:], ys[0])
        gb = mod[0:1, 5 * DM:6 * DM]
        y1 = y[0:1, :] * jax.nn.sigmoid(v1) * gb
        y2 = y[1:2, :] * jax.nn.sigmoid(v2) * gb

        fixes = []
        for n, idx in enumerate((idx1, idx2)):
            grp = jnp.clip(lax.shift_right_logical(idx, FIX.bit_length() - 1), 0, S // FIX - 1)
            base = pl.multiple_of(grp * FIX, FIX)
            rid = row[0:FIX] + base
            upd = jnp.where(rid == idx1, y1, jnp.where(rid == idx2, y2, 0.0))
            fixbuf[n] = (obuf[pl.ds(base, FIX), :].astype(F32) + upd).astype(BF16)
            fixes.append(cp(fixbuf.at[n], out_hbm.at[pl.ds(base, FIX)], sem.at[SEM_FIX]))

        for d in [out_cp(j) for j in range(NQ - 2)] + [early_cp] + last_cp:
            d.wait()
        for d in fixes:
            d.start()
            d.wait()

    def wait_groups(t0):
        for gg in range(t0, (GWAIT + (NG,))[GWAIT.index(t0) + 1]):
            for d in group_cps(gg):
                d.wait()
        if t0 == 2:
            x_cp[3].wait()

    def step(t, carry):
        i = lax.shift_right_logical(t, NG.bit_length() - 1)
        g = t & (NG - 1)
        attention_step(i, g, (t + NG) & (NG - 1), i & 1, g == 0)

        @pl.when(jnp.logical_or(jnp.logical_or(t < GWAIT[-1], t == NSTEP - 2), g == NG - 1))
        def _():
            pl.when(t == NSTEP - 2)(early_cp.start)
            for t0 in GWAIT[1:]:
                pl.when(t == t0 - 1)(lambda t0=t0: wait_groups(t0))

            @pl.when(g == NG - 1)
            def _():
                @pl.when(t == NG - 1)
                def _():
                    for d in [modr_cp, x_cp[2], wr_cp] + ffn_cp:
                        d.wait()
                    hn[...] = hnext[...]
                    for k in range(2, 6):
                        mod_cols(scbuf[...], k * DM, (k + 1) * DM, k == 4)
                    fold_vectors()

                @pl.when(jnp.logical_and(t > NG, t < NSTEP - 1))
                def _():
                    out_cp(i - 1).start()
                    hn[...] = hnext[...]

                pl.when(t == NSTEP - 1)(epilogue)

        return carry

    wait_groups(GWAIT[0])
    lax.fori_loop(1, NSTEP, step, 0)


@jax.jit
def pallas_adaLN_cond__mha_block_cached__moe_arch_mod__prompt_kernel(
    A_x: jax.Array,
    A_k_cache: jax.Array,
    A_v_cache: jax.Array,
    A_wq: jax.Array,
    A_wo: jax.Array,
    B_x: jax.Array,
    B_w_r: jax.Array,
    B_w_gate: jax.Array,
    B_w_up: jax.Array,
    B_w_down: jax.Array,
    c: jax.Array,
    w_mod: jax.Array,
):
    del B_x
    x = A_x.reshape(S, DM)
    k = A_k_cache.reshape(H, S, DH)
    v = A_v_cache.reshape(H, S, DH)
    wo = A_wo.reshape(NG, NH * DH, DM)
    any_spec = pl.BlockSpec(memory_space=pl.ANY)
    out = pl.pallas_call(
        _kernel,
        in_specs=[any_spec] * 11,
        out_specs=any_spec,
        out_shape=jax.ShapeDtypeStruct((S, DM), BF16),
        scratch_shapes=[
            pltpu.VMEM((S, DM), BF16),
            pltpu.VMEM((H, S, DH), BF16),
            pltpu.VMEM((H, S, DH), BF16),
            pltpu.VMEM((NG, DM, NH * DH), BF16),
            pltpu.VMEM((NG, NH * DH, DM), BF16),
            pltpu.VMEM((DM,), BF16),
            pltpu.VMEM((DM, FF), BF16),
            pltpu.VMEM((DM, FF), BF16),
            pltpu.VMEM((FF, DM + PAD), BF16),
            pltpu.VMEM((1, DM), BF16),
            pltpu.VMEM((16, DM), BF16),
            pltpu.VMEM((DM, 6 * DM + PAD), BF16),
            pltpu.VMEM((BQ, DM), BF16),
            pltpu.VMEM((BQ, DM), BF16),
            pltpu.VMEM((2, BQ, DM + PAD), F32),
            pltpu.VMEM((S, 128), F32),
            pltpu.VMEM((S, DM), F32),
            pltpu.VMEM((S, DM), BF16),
            pltpu.VMEM((2, FIX, DM), BF16),
            pltpu.VMEM((8, 6 * DM), F32),
            pltpu.VMEM((4, 8, DM), F32),
            pltpu.VMEM((2, 8, 128), F32),
            pltpu.SMEM((1,), jnp.int32),
            pltpu.SemaphoreType.DMA((NSEM,)),
        ],
        compiler_params=pltpu.CompilerParams(vmem_limit_bytes=124 * 1024 * 1024,
                                             disable_semaphore_checks=True),
        name="adaln_mha_moe",
    )(x, k, v, A_wq, wo, B_w_r, B_w_gate, B_w_up, B_w_down, c, w_mod)
    return out.reshape(1, S, DM)
```

```python
import jax
import jax.numpy as jnp
from jax import lax
import jax.experimental.pallas as pl
import jax.experimental.pallas.tpu as pltpu

F32 = jnp.float32
BF16 = jnp.bfloat16

S = 2048
DM = 1024
H = 32
DH = 128
FF = 3584
BQ = 512
TQ = 256
NH = 4
NQ = S // BQ
NG = H // NH
NSTEP = NQ * NG
LAST0 = S - BQ
LNR = BQ // NG
LN1_AT = ((1, 0), (1, 1), (1, 2), (1, 3))
LN2_AT = ((0, 0), (0, 1), (0, 2), (0, 3))
NP1 = len(LN1_AT)
NP2 = len(LN2_AT)
WA, WB = 256, 512
WT, WLAG = 256, 2
DLAG = 3
OUT_SPLIT = (-LNR, 192, 352, 448, BQ)
LRW = 16
ERW = 16
ORW = 16
KG = 512
EPS = 1e-5
EPS_BF16 = 1.0013580322265625e-05
QSCALE = DH ** -0.5 * 1.4426950408889634
NT = (((1,), (1,)), ((), ()))
FIX = 16
PAD = 128

SEM_CX = 0
MODC = (0, 640, 896, 1024)
SEM_MOD0 = 1
SEM_A = SEM_MOD0 + len(MODC) - 1
GWAIT = (1, 2, 3, 5)
SEM_G = SEM_A + 4
SEM_REST = SEM_G + len(GWAIT)
SEM_OUT = SEM_REST + 1
SEM_FIX = SEM_OUT + 1
NSEM = SEM_FIX + 1


def _rows8(v, rows):
    return jnp.tile(v, (rows // 8, 1))


def _rd(x):
    return x.astype(BF16).astype(F32)


def _inv_std(var):
    sd = _rd(jnp.sqrt(_rd(_rd(var) + EPS_BF16)))
    inv = pl.reciprocal(sd, approx=True)
    return inv * (2.0 - sd * inv)


def _route_key(r, idx):
    bits = lax.bitcast_convert_type(_rd(r), jnp.int32)
    bits = jnp.where((bits & 0x7F800000) == 0, 0x00800000, bits)
    return lax.bitcast_convert_type(bits | jnp.where(bits >= 0, (S - 1) - idx, idx), F32)


def _normalize(x):
    mean = jnp.sum(x, axis=-1, keepdims=True) * (1.0 / DM)
    xc = x - mean
    var = jnp.sum(xc * xc, axis=-1, keepdims=True) * (1.0 / DM)
    return xc * lax.rsqrt(var + EPS)


def _kernel(x_hbm, k_hbm, v_hbm, wq_hbm, wo_hbm, wr_hbm, wg_hbm, wu_hbm, wd_hbm, c_hbm, wm_hbm,
            out_hbm,
            xbuf, kbuf, vbuf, wqbuf, wobuf, wrbuf, wgbuf, wubuf, wdbuf, cbuf, scbuf, wmbuf,
            hn, hnext, acc, sbuf, nbuf, obuf, fixbuf, mod, vec, rsum, top, flag, sem):
    cp = pltpu.make_async_copy

    sem_last = SEM_A + 3
    c_cp = cp(c_hbm, cbuf, sem.at[SEM_CX])
    wr_cp = cp(wr_hbm, wrbuf, sem.at[SEM_REST])
    x_rng = ((0, BQ, SEM_CX), (BQ, BQ + 2 * LNR, sem_last), (2 * BQ, S, SEM_REST),
             (BQ + 2 * LNR, 2 * BQ, SEM_G + 1))
    x_cp = [cp(x_hbm.at[a:b], xbuf.at[a:b], sem.at[n]) for a, b, n in x_rng]
    mod_cp = [[cp(wm_hbm.at[:, o + MODC[n]:o + MODC[n + 1]], wmbuf.at[:, o + MODC[n]:o + MODC[n + 1]],
                  sem.at[SEM_MOD0 + n]) for o in (0, DM)] for n in range(len(MODC) - 1)]
    modr_cp = cp(wm_hbm.at[:, 2 * DM:], wmbuf.at[:, 2 * DM:6 * DM], sem.at[SEM_REST])

    def wq0_cp(h0, h1, sm):
        return cp(wq_hbm.at[:, h0 * DH:h1 * DH], wqbuf.at[0, :, h0 * DH:h1 * DH], sem.at[sm])

    def k0_cp(h, sm):
        return cp(k_hbm.at[h], kbuf.at[h], sem.at[sm])

    def v0_cp(h, sm):
        return cp(v_hbm.at[h], vbuf.at[h], sem.at[sm])

    wqe_cp = wq0_cp(0, 2, SEM_MOD0)
    step0_cp = [[k0_cp(0, SEM_A)],
                [v0_cp(0, SEM_A + 1), k0_cp(1, SEM_A + 1)],
                [v0_cp(1, SEM_A + 2), wq0_cp(2, 3, SEM_A + 2), k0_cp(2, SEM_A + 2), v0_cp(2, SEM_A + 2)],
                [wq0_cp(3, 4, sem_last), k0_cp(3, sem_last), v0_cp(3, sem_last),
                 cp(wo_hbm.at[0], wobuf.at[0], sem.at[sem_last]), x_cp[1]]]

    def group_cps(g):
        sg = sem.at[SEM_G + max(n for n, t in enumerate(GWAIT) if t <= g)]
        heads = slice(g * NH, (g + 1) * NH)
        return [cp(wq_hbm.at[:, g * NH * DH:(g + 1) * NH * DH], wqbuf.at[g], sg),
                cp(k_hbm.at[heads], kbuf.at[heads], sg),
                cp(v_hbm.at[heads], vbuf.at[heads], sg),
                cp(wo_hbm.at[g], wobuf.at[g], sg)]

    ffn_cp = [cp(wg_hbm, wgbuf, sem.at[SEM_REST]), cp(wu_hbm, wubuf, sem.at[SEM_REST]),
              cp(wd_hbm, wdbuf.at[:, 0:DM], sem.at[SEM_REST])]

    def out_cp(j):
        if isinstance(j, int):
            rows = slice(j * BQ, (j + 1) * BQ)
        else:
            rows = pl.ds(pl.multiple_of(j * BQ, BQ), BQ)
        return cp(obuf.at[rows], out_hbm.at[rows], sem.at[SEM_OUT])

    last_cp = [cp(obuf.at[LAST0 + a:LAST0 + b], out_hbm.at[LAST0 + a:LAST0 + b], sem.at[SEM_OUT])
               for a, b in zip(OUT_SPLIT[:-1], OUT_SPLIT[1:])]
    early_cp = cp(obuf.at[LAST0 - BQ:LAST0 - LNR], out_hbm.at[LAST0 - BQ:LAST0 - LNR], sem.at[SEM_OUT])

    c_cp.start()
    x_cp[0].start()
    wqe_cp.start()
    for ds in mod_cp + step0_cp:
        for d in ds:
            d.start()
    for g in range(1, NG):
        for d in group_cps(g):
            d.start()
        if g == 2:
            x_cp[3].start()
    modr_cp.start()
    wr_cp.start()
    x_cp[2].start()
    for d in ffn_cp:
        d.start()

    flag[0] = 0
    acc[1, :, 0:DM] = jnp.zeros((BQ, DM), F32)
    mod[:, 2 * DM:] = jnp.zeros((8, 4 * DM), F32)
    vec[...] = jnp.zeros((4, 8, DM), F32)
    sbuf[LAST0:S, :] = jnp.zeros((BQ, 128), F32)
    top[...] = jnp.full((2, 8, 128), -jnp.inf, F32)

    def silu_c():
        cf = cbuf[...].astype(F32)
        sc = cf * jax.nn.sigmoid(cf)
        return jnp.broadcast_to(sc, (16, DM)).astype(BF16)

    def mod_cols(sc, lo, hi, scale=False):
        m = _rd(jnp.dot(sc, wmbuf[:, lo:hi], preferred_element_type=F32))
        mod[:, lo:hi] = (_rd(1.0 + m) if scale else m)[:8]

    def tie(val, dep):
        if dep is None:
            return val
        n = dep.shape[0]
        head = jnp.where(flag[0] != 0, dep, val[:n])
        return head if n == val.shape[0] else jnp.concatenate([head, val[n:]], axis=0)

    def ln1_apply(n, rows, lo=0, hi=DM):
        return n * _rows8(mod[:, DM + lo:DM + hi], rows) + _rows8(mod[:, lo:hi], rows)

    def load_top():
        return top[0], top[1]

    def store_top(st):
        top[0], top[1] = st

    def fold_vectors():
        sb, cb1, gb = mod[:, 3 * DM:4 * DM], mod[:, 4 * DM:5 * DM], mod[:, 5 * DM:6 * DM]
        wr = jnp.broadcast_to(wrbuf[...].astype(F32).reshape(1, DM), (8, DM))
        vec[0] = gb * cb1
        vec[1] = gb * sb
        vec[2] = cb1 * wr
        w32 = _rows8(cb1 * wr, 32)
        whi = _rd(w32)
        r32 = lax.broadcasted_iota(jnp.int32, (32, DM), 0)
        for j in range(BQ // 128):
            rsum[j] = jnp.where(r32 == j, 1.0, jnp.where(r32 == 8 + j, whi,
                                jnp.where(r32 == 16 + j, w32 - whi, 0.0))).astype(BF16)
        vec[3, :, 0:128] = jnp.broadcast_to(jnp.sum(sb * wr, axis=-1, keepdims=True), (8, 128))
        vec[3, :, 128:256] = jnp.broadcast_to(jnp.sum(cb1 * wr, axis=-1, keepdims=True), (8, 128))

    def ln2_out(x1, n, row0, rows):
        out = x1 + n * _rows8(vec[0], rows) + _rows8(vec[1], rows)
        obuf[pl.ds(row0, rows), :] = out.astype(BF16)
        return out

    def residual(a, row0, rows):
        return _rd(xbuf[pl.ds(row0, rows), :].astype(F32) + _rows8(mod[:, 2 * DM:3 * DM], rows) * a)

    def ln2(a, row0, rows, valid, st):
        x1 = residual(a, row0, rows)
        mean = jnp.sum(x1, axis=-1, keepdims=True) * (1.0 / DM)
        xc = x1 - mean
        inv = _inv_std(jnp.sum(xc * xc, axis=-1, keepdims=True) * (1.0 / DM))
        n = xc * inv
        shift = jnp.broadcast_to((mean - _rd(mean)) * inv, (rows, 128))
        nbuf[pl.ds(row0, rows), :] = n
        sbuf[pl.ds(row0, rows), :] = shift
        ln2_out(x1, n, row0, rows)
        r = (jnp.sum(n * _rows8(vec[2], rows), axis=-1, keepdims=True)
             + (shift * _rows8(vec[3, :, 128:256], rows) + _rows8(vec[3, :, 0:128], rows)))
        key = _route_key(r, lax.broadcasted_iota(jnp.int32, (rows, 128), 0) + row0)
        key = jnp.where(valid, key, -jnp.inf)
        k1, k2 = st
        for u in range(rows // 8):
            ku = key[u * 8:(u + 1) * 8]
            k2 = jnp.maximum(k2, jnp.minimum(k1, ku))
            k1 = jnp.maximum(k1, ku)
        return k1, k2

    def qproj(g, c, h):
        q = jnp.dot(hn[c * TQ:(c + 1) * TQ, :], wqbuf[g, :, h * DH:(h + 1) * DH],
                    preferred_element_type=F32)
        return (q * QSCALE).astype(BF16)

    def qk(q, g, h):
        return lax.dot_general(q, kbuf[g * NH + h], NT, preferred_element_type=F32)

    def pv(s, g, h, dep=None, m=None):
        if m is None:
            m = jnp.max(s, axis=-1, keepdims=True)
        lsum = None
        parts = []
        for j in range(S // KG):
            ss = [s[:, j * KG + u * 128:j * KG + (u + 1) * 128] for u in range(KG // 128)]
            if j == 0:
                ss[0] = tie(ss[0], dep)
            ps = [jnp.exp2(z - m) for z in ss]
            t = (ps[0] + ps[1]) + (ps[2] + ps[3])
            lsum = t if lsum is None else lsum + t
            ps[-1] = jnp.minimum(ps[-1], lsum)
            parts += ps
        p = jnp.concatenate(parts, axis=-1).astype(BF16)
        return jnp.dot(p, vbuf[g * NH + h], preferred_element_type=F32), lsum

    def normalize_heads(res):
        gate = jnp.minimum(res[-1][0], 0.0)
        outs = []
        for o, lsum in res:
            l = jnp.sum(jnp.maximum(lsum, gate), axis=-1, keepdims=True)
            r = pl.reciprocal(l, approx=True)
            r = r * (2.0 - l * r)
            outs.append(o * r)
        return outs

    def woproj(slot, g, first, c, outs, lo, hi, dep=None, r0=0, r1=TQ):
        parts = [o[r0:r1] for o in outs]
        oc = jnp.concatenate([tie(parts[0], dep)] + parts[1:], axis=-1).astype(BF16)
        y = jnp.dot(oc, wobuf[g, :, lo:hi], preferred_element_type=F32)
        rows = slice(c * TQ + r0, c * TQ + r1)
        if first is True:
            acc[slot, rows, lo:hi] = y
        elif first is False:
            acc[slot, rows, lo:hi] = acc[slot, rows, lo:hi] + y
        else:
            acc[slot, rows, lo:hi] = jnp.where(first, 0.0, acc[slot, rows, lo:hi]) + y
        return y

    def ln1_piece(i, g, u, gate=None):
        pr = LNR // NP1
        if isinstance(i, int) and isinstance(g, int):
            row0, off = (i + 1) * BQ + g * LNR + u * pr, g * LNR + u * pr
        else:
            row0 = pl.multiple_of(jnp.minimum((i + 1) * BQ + g * LNR, S - LNR) + u * pr, pr)
            off = pl.multiple_of(g * LNR + u * pr, pr)
        xv = xbuf[pl.ds(row0, pr), :].astype(F32)
        if gate is not None:
            xv = jnp.concatenate([tie(xv[:, 0:128], gate[0:pr, 0:128]), xv[:, 128:]], axis=-1)
        hv = ln1_apply(_normalize(xv), pr)
        hnext[pl.ds(off, pr), :] = hv.astype(BF16)
        return hv[:, 0:128]

    def ln2_piece(i, g, u, st):
        pr = LNR // NP2
        for k in range(pr // LRW):
            off = pl.multiple_of(g * LNR + u * pr + k * LRW, LRW)
            row0 = pl.multiple_of(jnp.maximum(i - 1, 0) * BQ + off, LRW)
            st = ln2(acc[(i + 1) & 1, pl.ds(off, LRW), 0:DM], row0, LRW, i > 0, st)
        return st

    def wo_tail(g, slot, first, o0, o1, work):
        pieces = [(0, o0, lo) for lo in range(WB, DM, WT)] + [(1, o1, lo) for lo in range(0, DM, WT)]
        deps = {}
        for n, (c, o, lo) in enumerate(pieces):
            y = woproj(slot, g, first, c, o, lo, lo + WT, deps.get(n))
            if n in work:
                deps[n + WLAG] = work[n](y)

    chains = [(c, h) for c in range(2) for h in range(NH)]

    def attention_step(i, g, g1, slot, first):
        st = [load_top()]

        def ln2_work(u):
            st[0] = ln2_piece(i, g, u, st[0])
            return st[0][1]

        pv_dep, work = {}, {}
        for u, at in enumerate(LN2_AT):
            if isinstance(at, tuple):
                pv_dep[at] = ln2_work(u)
            else:
                work[at] = lambda y, u=u: ln2_work(u)
        for u, at in enumerate(LN1_AT):
            if isinstance(at, tuple):
                pv_dep[at] = ln1_piece(i, g, u)
            else:
                work[at] = lambda y, u=u: ln1_piece(i, g, u, y)
        q = qproj(g, 0, 0)
        res = ([], [])
        o0 = None
        for n, (c, h) in enumerate(chains):
            s = qk(q, g, h)
            if n + 1 < len(chains):
                q = qproj((g, g1)[chains[n + 1][0]], *chains[n + 1])
            if (c, h) == (1, 0):
                o0 = normalize_heads(res[0])
                woproj(slot, g, first, 0, o0, 0, WA)
            if (c, h) == (1, NH - 1):
                woproj(slot, g, first, 0, o0, WA, WB)
            res[c].append(pv(s, g, h, pv_dep.get((c, h))))
        wo_tail(g, slot, first, o0, normalize_heads(res[1]), work)
        store_top(st[0])

    c_cp.wait()
    x_cp[0].wait()
    sc = silu_c()
    scbuf[...] = sc
    acc[0, :, 0:DM] = _normalize(xbuf[0:BQ, :].astype(F32))
    for n in range(len(MODC) - 1):
        lo, hi = MODC[n], MODC[n + 1]
        if n == 0:
            wqe_cp.wait()
        for d in mod_cp[n]:
            d.wait()
        mod_cols(sc, lo, hi)
        mod_cols(sc, DM + lo, DM + hi, True)
        hn[:, lo:hi] = ln1_apply(acc[0, :, lo:hi], BQ, lo, hi).astype(BF16)
        for c in range(2):
            rows = slice(c * TQ, (c + 1) * TQ)
            part = jnp.dot(hn[rows, lo:hi], wqbuf[0, lo:hi, 0:2 * DH], preferred_element_type=F32)
            if n > 0:
                part = part + nbuf[rows, 0:2 * DH]
            if hi < DM:
                nbuf[rows, 0:2 * DH] = part
            else:
                hnext[rows, 0:2 * DH] = (part * QSCALE).astype(BF16)

    def wait0(n):
        for d in step0_cp[n]:
            d.wait()

    def qk_pair(h):
        sa, sb = [qk(hnext[c * TQ:(c + 1) * TQ, h * DH:(h + 1) * DH], 0, h) for c in range(2)]
        return sa, jnp.max(sa, axis=-1, keepdims=True), sb

    wait0(0)
    sa, ma, s = qk_pair(0)
    wait0(1)
    res = ([pv(sa, 0, 0, None, ma)], [pv(s, 0, 0)])
    sa, ma, s = qk_pair(1)
    wait0(2)
    res[0].append(pv(sa, 0, 1, None, ma))
    for h in range(2, NH):
        if h == 3:
            wait0(3)
        q = qproj(0, 0, h)
        res[1].append(pv(s, 0, h - 1))
        s = qk(q, 0, h)
        q = qproj(0, 1, h)
        res[0].append(pv(s, 0, h))
        s = qk(q, 0, h)
    o0 = normalize_heads(res[0])
    woproj(0, 0, True, 0, o0, 0, WB)
    res[1].append(pv(s, 0, NH - 1))
    npt = (2 * DM - WB) // WT - WLAG
    work0 = {}
    for u in range(NP1):
        work0.setdefault(u * npt // NP1, []).append(u)
    wo_tail(0, 0, True, o0, normalize_heads(res[1]),
            {n: (lambda y, us=us: jnp.concatenate([ln1_piece(0, 0, u, y) for u in us], axis=0))
             for n, us in work0.items()})

    def epilogue():
        last = (NQ - 1) % 2
        nt = BQ // 128
        lane = lax.broadcasted_iota(jnp.int32, (8, 128), 1)
        sub = lax.broadcasted_iota(jnp.int32, (8, 128), 0)
        lin = None
        sq = None
        for j in range(nt):
            xs_, ps_ = [], []
            for r0 in range(j * 128, (j + 1) * 128, ERW):
                x1 = residual(acc[last, r0:r0 + ERW, 0:DM], LAST0 + r0, ERW)
                nbuf[LAST0 + r0:LAST0 + r0 + ERW, :] = x1
                x2 = x1 * x1
                part = x2[:, 0:128]
                for z in range(1, DM // 128):
                    part = part + x2[:, z * 128:(z + 1) * 128]
                hi = _rd(part)
                xs_.append(x1)
                ps_.append(jnp.concatenate([hi, part - hi], axis=-1))
            a_ = lax.dot_general(rsum[j], jnp.concatenate(xs_, axis=0).astype(BF16), NT,
                                 preferred_element_type=F32)[0:24]
            b_ = lax.dot_general(rsum[j, 0:16, 0:256], jnp.concatenate(ps_, axis=0).astype(BF16), NT,
                                 preferred_element_type=F32)[0:8]
            lin = a_ if lin is None else lin + a_
            sq = b_ if sq is None else sq + b_
        mean = lin[0:8] * (1.0 / DM)
        inv = _inv_std(jnp.maximum(sq * (1.0 / DM) - mean * mean, 0.0))
        mean = _rd(mean)
        dot = lin[8:16] + lin[16:24]
        r = (dot - mean * vec[3, :, 128:256]) * inv + vec[3, :, 0:128]
        k1, k2 = load_top()
        c1 = jnp.max(k1, axis=0, keepdims=True)
        c2 = jnp.max(jnp.where(k1 == c1, k2, k1), axis=0, keepdims=True)
        keys = jnp.where(sub < nt, _route_key(r, LAST0 + sub * 128 + lane),
                         jnp.where(lane > 0, -jnp.inf,
                                   jnp.where(sub == nt, c1, jnp.where(sub == nt + 1, c2, -jnp.inf))))
        mean_k = jnp.where(sub < nt, mean, 0.0)
        inv_k = jnp.where(sub < nt, inv, 1.0)

        def all_sum(z):
            return jnp.sum(jnp.sum(z, axis=1, keepdims=True), axis=0, keepdims=True)

        t1 = jnp.max(keys, axis=0, keepdims=True)
        t2 = jnp.max(jnp.where(keys == t1, -jnp.inf, keys), axis=0, keepdims=True)
        bit = lax.shift_right_logical(lane, sub) & 1
        half = [jnp.max(jnp.where(sub == 7, t2, jnp.where(bit == b, t1, -jnp.inf)), axis=1, keepdims=True)
                for b in range(2)]
        bests = (jnp.max(jnp.maximum(half[0], half[1]), axis=0, keepdims=True),
                 jnp.max(jnp.minimum(half[0], half[1]), axis=0, keepdims=True))

        routed = []
        for best in bests:
            hit = keys == best
            bits = lax.bitcast_convert_type(jnp.broadcast_to(best, (8, 128)), jnp.int32)
            low = bits & (S - 1)
            idx = jnp.clip(jnp.where(bits >= 0, (S - 1) - low, low)[0, 0], 0, S - 1)
            logit = lax.bitcast_convert_type(bits & -65536, F32)[0:1, 0:1]
            nrow = ((nbuf[pl.ds(idx, 1), :] - all_sum(jnp.where(hit, mean_k, 0.0)))
                    * all_sum(jnp.where(hit, inv_k, 0.0))
                    + jnp.tile(sbuf[pl.ds(idx, 1), :], (1, DM // 128)))
            routed.append((idx, logit, nrow))
        (idx1, v1, n1), (idx2, v2, n2) = routed

        row = lax.broadcasted_iota(jnp.int32, (16, DM), 0)
        xs = (_rd(_rd(jnp.where(row == 0, n1, n2)) * _rows8(mod[:, 4 * DM:5 * DM], 16))
              + _rows8(mod[:, 3 * DM:4 * DM], 16))

        cols = {}

        def row_stat(name, z, r0):
            j = r0 // 128
            if (name, j) not in cols:
                cols[name, j] = jnp.broadcast_to(z[j:j + 1, :], (128, 128)).T
            return cols[name, j][r0 - j * 128:r0 - j * 128 + ORW]

        acts = []
        ys = []

        def tied_bf16(v, dep):
            return jnp.concatenate([tie(v[:, 0:128], dep), v[:, 128:]], axis=-1).astype(BF16)

        def gate_up(n, dep):
            cols = slice(n * 128, (n + 1) * 128)
            xb = tied_bf16(xs, dep)
            gt = jnp.dot(xb, wgbuf[:, cols], preferred_element_type=F32)
            up = jnp.dot(xb, wubuf[:, cols], preferred_element_type=F32)
            acts.append(gt * jax.nn.sigmoid(gt) * up)
            return gt

        def down(n, dep):
            ab = tied_bf16(jnp.concatenate(acts[2 * n:2 * n + 2], axis=-1), dep)
            ys.append(jnp.dot(ab, wdbuf[n * 256:(n + 1) * 256, 0:DM], preferred_element_type=F32))
            return ys[-1]

        slots = []
        for n in range(FF // 128):
            slots.append((gate_up, n))
            if n % 2 == 1 and n >= DLAG:
                slots.append((down, (n - DLAG) // 2))
        slots += [(down, n) for n in range(FF // 256) if (down, n) not in slots]
        deps = {}
        for k, (fn, n) in enumerate(slots):
            gate = fn(n, deps.get(k))
            r0 = k * ORW
            if r0 < BQ:
                x1 = nbuf[LAST0 + r0:LAST0 + r0 + ORW, :]
                mu = tie(row_stat("mean", mean, r0), gate[0:ORW, 0:128])
                nv = (x1 - jnp.tile(mu, (1, DM // 128))) * jnp.tile(row_stat("inv", inv, r0), (1, DM // 128))
                deps[k + 2] = ln2_out(x1, nv, LAST0 + r0, ORW)[:, DM - 128:]
                if r0 + ORW in OUT_SPLIT:
                    last_cp[OUT_SPLIT.index(r0 + ORW) - 1].start()
        y = sum(ys[1:], ys[0])
        gb = mod[0:1, 5 * DM:6 * DM]
        y1 = y[0:1, :] * jax.nn.sigmoid(v1) * gb
        y2 = y[1:2, :] * jax.nn.sigmoid(v2) * gb

        fixes = []
        for n, idx in enumerate((idx1, idx2)):
            grp = jnp.clip(lax.shift_right_logical(idx, FIX.bit_length() - 1), 0, S // FIX - 1)
            base = pl.multiple_of(grp * FIX, FIX)
            rid = row[0:FIX] + base
            upd = jnp.where(rid == idx1, y1, jnp.where(rid == idx2, y2, 0.0))
            fixbuf[n] = (obuf[pl.ds(base, FIX), :].astype(F32) + upd).astype(BF16)
            fixes.append(cp(fixbuf.at[n], out_hbm.at[pl.ds(base, FIX)], sem.at[SEM_FIX]))

        for d in [out_cp(j) for j in range(NQ - 2)] + [early_cp] + last_cp:
            d.wait()
        for d in fixes:
            d.start()
            d.wait()

    def wait_groups(t0):
        for gg in range(t0, (GWAIT + (NG,))[GWAIT.index(t0) + 1]):
            for d in group_cps(gg):
                d.wait()
        if t0 == 2:
            x_cp[3].wait()

    def step(t, carry):
        i = lax.shift_right_logical(t, NG.bit_length() - 1)
        g = t & (NG - 1)
        attention_step(i, g, (t + NG) & (NG - 1), i & 1, g == 0)

        @pl.when(jnp.logical_or(jnp.logical_or(t < GWAIT[-1], t == NSTEP - 2), g == NG - 1))
        def _():
            pl.when(t == NSTEP - 2)(early_cp.start)
            for t0 in GWAIT[1:]:
                pl.when(t == t0 - 1)(lambda t0=t0: wait_groups(t0))

            @pl.when(g == NG - 1)
            def _():
                @pl.when(t == NG - 1)
                def _():
                    for d in [modr_cp, x_cp[2], wr_cp] + ffn_cp:
                        d.wait()
                    hn[...] = hnext[...]
                    for k in range(2, 6):
                        mod_cols(scbuf[...], k * DM, (k + 1) * DM, k == 4)
                    fold_vectors()

                @pl.when(jnp.logical_and(t > NG, t < NSTEP - 1))
                def _():
                    out_cp(i - 1).start()
                    hn[...] = hnext[...]

                pl.when(t == NSTEP - 1)(epilogue)

        return carry

    wait_groups(GWAIT[0])
    lax.fori_loop(1, NSTEP, step, 0)


@jax.jit
def pallas_adaLN_cond__mha_block_cached__moe_arch_mod__prompt_kernel(
    A_x: jax.Array,
    A_k_cache: jax.Array,
    A_v_cache: jax.Array,
    A_wq: jax.Array,
    A_wo: jax.Array,
    B_x: jax.Array,
    B_w_r: jax.Array,
    B_w_gate: jax.Array,
    B_w_up: jax.Array,
    B_w_down: jax.Array,
    c: jax.Array,
    w_mod: jax.Array,
):
    del B_x
    x = A_x.reshape(S, DM)
    k = A_k_cache.reshape(H, S, DH)
    v = A_v_cache.reshape(H, S, DH)
    wo = A_wo.reshape(NG, NH * DH, DM)
    any_spec = pl.BlockSpec(memory_space=pl.ANY)
    out = pl.pallas_call(
        _kernel,
        in_specs=[any_spec] * 11,
        out_specs=any_spec,
        out_shape=jax.ShapeDtypeStruct((S, DM), BF16),
        scratch_shapes=[
            pltpu.VMEM((S, DM), BF16),
            pltpu.VMEM((H, S, DH), BF16),
            pltpu.VMEM((H, S, DH), BF16),
            pltpu.VMEM((NG, DM, NH * DH), BF16),
            pltpu.VMEM((NG, NH * DH, DM), BF16),
            pltpu.VMEM((DM,), BF16),
            pltpu.VMEM((DM, FF), BF16),
            pltpu.VMEM((DM, FF), BF16),
            pltpu.VMEM((FF, DM + PAD), BF16),
            pltpu.VMEM((1, DM), BF16),
            pltpu.VMEM((16, DM), BF16),
            pltpu.VMEM((DM, 6 * DM + PAD), BF16),
            pltpu.VMEM((BQ, DM), BF16),
            pltpu.VMEM((BQ, DM), BF16),
            pltpu.VMEM((2, BQ, DM + PAD), F32),
            pltpu.VMEM((S, 128), F32),
            pltpu.VMEM((S, DM), F32),
            pltpu.VMEM((S, DM), BF16),
            pltpu.VMEM((2, FIX, DM), BF16),
            pltpu.VMEM((8, 6 * DM), F32),
            pltpu.VMEM((4, 8, DM), F32),
            pltpu.VMEM((BQ // 128, 32, DM), BF16),
            pltpu.VMEM((2, 8, 128), F32),
            pltpu.SMEM((1,), jnp.int32),
            pltpu.SemaphoreType.DMA((NSEM,)),
        ],
        compiler_params=pltpu.CompilerParams(vmem_limit_bytes=124 * 1024 * 1024,
                                             disable_semaphore_checks=True),
        name="adaln_mha_moe",
    )(x, k, v, A_wq, wo, B_w_r, B_w_gate, B_w_up, B_w_down, c, w_mod)
    return out.reshape(1, S, DM)
```

```python
import jax
import jax.numpy as jnp
from jax import lax
import jax.experimental.pallas as pl
import jax.experimental.pallas.tpu as pltpu

F32 = jnp.float32
BF16 = jnp.bfloat16

S = 2048
DM = 1024
H = 32
DH = 128
FF = 3584
BQ = 512
TQ = 256
NH = 4
NQ = S // BQ
NG = H // NH
NSTEP = NQ * NG
LAST0 = S - BQ
LNR = BQ // NG
LN1_AT = ((1, 0), (1, 1), (1, 2), (1, 3))
LN2_AT = ((0, 0), (0, 1), (0, 2), (0, 3))
NP1 = len(LN1_AT)
NP2 = len(LN2_AT)
WA, WB = 256, 512
WT, WLAG = 256, 2
DLAG = 3
OUT_SPLIT = (-LNR, 192, 352, 448, BQ)
LRW = 16
ERW = 16
ORW = 16
KG = 512
EPS = 1e-5
EPS_BF16 = 1.0013580322265625e-05
QSCALE = DH ** -0.5 * 1.4426950408889634
NT = (((1,), (1,)), ((), ()))
FIX = 16
PAD = 128

SEM_CX = 0
MODC = (0, 640, 896, 1024)
SEM_MOD0 = 1
SEM_A = SEM_MOD0 + len(MODC) - 1
GWAIT = (1, 2, 3, 5)
SEM_G = SEM_A + 4
SEM_REST = SEM_G + len(GWAIT)
SEM_OUT = SEM_REST + 1
SEM_FIX = SEM_OUT + 1
NSEM = SEM_FIX + 1


def _rows8(v, rows):
    return jnp.tile(v, (rows // 8, 1))


def _rd(x):
    return x.astype(BF16).astype(F32)


def _inv_std(var):
    sd = _rd(jnp.sqrt(_rd(_rd(var) + EPS_BF16)))
    inv = pl.reciprocal(sd, approx=True)
    return inv * (2.0 - sd * inv)


def _route_key(r, idx):
    bits = lax.bitcast_convert_type(_rd(r), jnp.int32)
    bits = jnp.where((bits & 0x7F800000) == 0, 0x00800000, bits)
    return lax.bitcast_convert_type(bits | jnp.where(bits >= 0, (S - 1) - idx, idx), F32)


def _normalize(x):
    mean = jnp.sum(x, axis=-1, keepdims=True) * (1.0 / DM)
    xc = x - mean
    var = jnp.sum(xc * xc, axis=-1, keepdims=True) * (1.0 / DM)
    return xc * lax.rsqrt(var + EPS)


def _kernel(x_hbm, k_hbm, v_hbm, wq_hbm, wo_hbm, wr_hbm, wg_hbm, wu_hbm, wd_hbm, c_hbm, wm_hbm,
            out_hbm,
            xbuf, kbuf, vbuf, wqbuf, wobuf, wrbuf, wgbuf, wubuf, wdbuf, cbuf, scbuf, wmbuf,
            hn, hnext, acc, sbuf, nbuf, obuf, fixbuf, mod, vec, rsum, top, flag, sem):
    cp = pltpu.make_async_copy

    sem_last = SEM_A + 3
    c_cp = cp(c_hbm, cbuf, sem.at[SEM_CX])
    wr_cp = cp(wr_hbm, wrbuf, sem.at[SEM_REST])
    x_rng = ((0, BQ, SEM_CX), (BQ, BQ + 2 * LNR, sem_last), (2 * BQ, S, SEM_REST),
             (BQ + 2 * LNR, 2 * BQ, SEM_G + 1))
    x_cp = [cp(x_hbm.at[a:b], xbuf.at[a:b], sem.at[n]) for a, b, n in x_rng]
    mod_cp = [[cp(wm_hbm.at[:, o + MODC[n]:o + MODC[n + 1]], wmbuf.at[:, o + MODC[n]:o + MODC[n + 1]],
                  sem.at[SEM_MOD0 + n]) for o in (0, DM)] for n in range(len(MODC) - 1)]
    modr_cp = cp(wm_hbm.at[:, 2 * DM:], wmbuf.at[:, 2 * DM:6 * DM], sem.at[SEM_REST])

    def wq0_cp(h0, h1, sm):
        return cp(wq_hbm.at[:, h0 * DH:h1 * DH], wqbuf.at[0, :, h0 * DH:h1 * DH], sem.at[sm])

    def k0_cp(h, sm):
        return cp(k_hbm.at[h], kbuf.at[h], sem.at[sm])

    def v0_cp(h, sm):
        return cp(v_hbm.at[h], vbuf.at[h], sem.at[sm])

    wqe_cp = wq0_cp(0, 2, SEM_MOD0)
    step0_cp = [[k0_cp(0, SEM_A)],
                [v0_cp(0, SEM_A + 1), k0_cp(1, SEM_A + 1)],
                [v0_cp(1, SEM_A + 2), wq0_cp(2, 3, SEM_A + 2), k0_cp(2, SEM_A + 2), v0_cp(2, SEM_A + 2)],
                [wq0_cp(3, 4, sem_last), k0_cp(3, sem_last), v0_cp(3, sem_last),
                 cp(wo_hbm.at[0], wobuf.at[0], sem.at[sem_last]), x_cp[1]]]

    def group_cps(g):
        sg = sem.at[SEM_G + max(n for n, t in enumerate(GWAIT) if t <= g)]
        heads = slice(g * NH, (g + 1) * NH)
        return [cp(wq_hbm.at[:, g * NH * DH:(g + 1) * NH * DH], wqbuf.at[g], sg),
                cp(k_hbm.at[heads], kbuf.at[heads], sg),
                cp(v_hbm.at[heads], vbuf.at[heads], sg),
                cp(wo_hbm.at[g], wobuf.at[g], sg)]

    ffn_cp = [cp(wg_hbm, wgbuf, sem.at[SEM_REST]), cp(wu_hbm, wubuf, sem.at[SEM_REST]),
              cp(wd_hbm, wdbuf.at[:, 0:DM], sem.at[SEM_REST])]

    def out_cp(j):
        if isinstance(j, int):
            rows = slice(j * BQ, (j + 1) * BQ)
        else:
            rows = pl.ds(pl.multiple_of(j * BQ, BQ), BQ)
        return cp(obuf.at[rows], out_hbm.at[rows], sem.at[SEM_OUT])

    last_cp = [cp(obuf.at[LAST0 + a:LAST0 + b], out_hbm.at[LAST0 + a:LAST0 + b], sem.at[SEM_OUT])
               for a, b in zip(OUT_SPLIT[:-1], OUT_SPLIT[1:])]
    early_cp = cp(obuf.at[LAST0 - BQ:LAST0 - LNR], out_hbm.at[LAST0 - BQ:LAST0 - LNR], sem.at[SEM_OUT])

    c_cp.start()
    x_cp[0].start()
    wqe_cp.start()
    for ds in mod_cp + step0_cp:
        for d in ds:
            d.start()
    for g in range(1, NG):
        for d in group_cps(g):
            d.start()
        if g == 2:
            x_cp[3].start()
    modr_cp.start()
    wr_cp.start()
    x_cp[2].start()
    for d in ffn_cp:
        d.start()

    flag[0] = 0
    acc[1, :, 0:DM] = jnp.zeros((BQ, DM), F32)
    mod[:, 2 * DM:] = jnp.zeros((8, 4 * DM), F32)
    vec[...] = jnp.zeros((4, 8, DM), F32)
    sbuf[LAST0:S, :] = jnp.zeros((BQ, 128), F32)
    top[...] = jnp.full((2, 8, 128), -jnp.inf, F32)

    def silu_c():
        cf = cbuf[...].astype(F32)
        sc = cf * jax.nn.sigmoid(cf)
        return jnp.broadcast_to(sc, (16, DM)).astype(BF16)

    def mod_cols(sc, lo, hi, scale=False):
        m = _rd(jnp.dot(sc, wmbuf[:, lo:hi], preferred_element_type=F32))
        mod[:, lo:hi] = (_rd(1.0 + m) if scale else m)[:8]

    def tie(val, dep):
        if dep is None:
            return val
        n = dep.shape[0]
        head = jnp.where(flag[0] != 0, dep, val[:n])
        return head if n == val.shape[0] else jnp.concatenate([head, val[n:]], axis=0)

    def ln1_apply(n, rows, lo=0, hi=DM):
        return n * _rows8(mod[:, DM + lo:DM + hi], rows) + _rows8(mod[:, lo:hi], rows)

    def load_top():
        return top[0], top[1]

    def store_top(st):
        top[0], top[1] = st

    def fold_vectors():
        sb, cb1, gb = mod[:, 3 * DM:4 * DM], mod[:, 4 * DM:5 * DM], mod[:, 5 * DM:6 * DM]
        wr = jnp.broadcast_to(wrbuf[...].astype(F32).reshape(1, DM), (8, DM))
        vec[0] = gb * cb1
        vec[1] = gb * sb
        vec[2] = cb1 * wr
        w32 = _rows8(cb1 * wr, 32)
        whi = _rd(w32)
        r32 = lax.broadcasted_iota(jnp.int32, (32, DM), 0)
        for j in range(BQ // 128):
            rsum[j] = jnp.where(r32 == j, 1.0, jnp.where(r32 == 8 + j, whi,
                                jnp.where(r32 == 16 + j, w32 - whi, 0.0))).astype(BF16)
        vec[3, :, 0:128] = jnp.broadcast_to(jnp.sum(sb * wr, axis=-1, keepdims=True), (8, 128))
        vec[3, :, 128:256] = jnp.broadcast_to(jnp.sum(cb1 * wr, axis=-1, keepdims=True), (8, 128))

    def ln2_out(x1, n, row0, rows):
        out = x1 + n * _rows8(vec[0], rows) + _rows8(vec[1], rows)
        obuf[pl.ds(row0, rows), :] = out.astype(BF16)
        return out

    def residual(a, row0, rows):
        return _rd(xbuf[pl.ds(row0, rows), :].astype(F32) + _rows8(mod[:, 2 * DM:3 * DM], rows) * a)

    def ln2(a, row0, rows, valid, st):
        x1 = residual(a, row0, rows)
        mean = jnp.sum(x1, axis=-1, keepdims=True) * (1.0 / DM)
        xc = x1 - mean
        inv = _inv_std(jnp.sum(xc * xc, axis=-1, keepdims=True) * (1.0 / DM))
        n = xc * inv
        shift = jnp.broadcast_to((mean - _rd(mean)) * inv, (rows, 128))
        nbuf[pl.ds(row0, rows), :] = n
        sbuf[pl.ds(row0, rows), :] = shift
        ln2_out(x1, n, row0, rows)
        r = (jnp.sum(n * _rows8(vec[2], rows), axis=-1, keepdims=True)
             + (shift * _rows8(vec[3, :, 128:256], rows) + _rows8(vec[3, :, 0:128], rows)))
        key = _route_key(r, lax.broadcasted_iota(jnp.int32, (rows, 128), 0) + row0)
        key = jnp.where(valid, key, -jnp.inf)
        k1, k2 = st
        for u in range(rows // 8):
            ku = key[u * 8:(u + 1) * 8]
            k2 = jnp.maximum(k2, jnp.minimum(k1, ku))
            k1 = jnp.maximum(k1, ku)
        return k1, k2

    def qproj(g, c, h):
        q = jnp.dot(hn[c * TQ:(c + 1) * TQ, :], wqbuf[g, :, h * DH:(h + 1) * DH],
                    preferred_element_type=F32)
        return (q * QSCALE).astype(BF16)

    def qk(q, g, h):
        return lax.dot_general(q, kbuf[g * NH + h], NT, preferred_element_type=F32)

    def pv(s, g, h, dep=None, m=None):
        if m is None:
            m = jnp.max(s, axis=-1, keepdims=True)
        lsum = None
        parts = []
        for j in range(S // KG):
            ss = [s[:, j * KG + u * 128:j * KG + (u + 1) * 128] for u in range(KG // 128)]
            if j == 0:
                ss[0] = tie(ss[0], dep)
            ps = [jnp.exp2(z - m) for z in ss]
            t = (ps[0] + ps[1]) + (ps[2] + ps[3])
            lsum = t if lsum is None else lsum + t
            ps[-1] = jnp.minimum(ps[-1], lsum)
            parts += ps
        p = jnp.concatenate(parts, axis=-1).astype(BF16)
        return jnp.dot(p, vbuf[g * NH + h], preferred_element_type=F32), lsum

    def normalize_heads(res):
        gate = jnp.minimum(res[-1][0], 0.0)
        outs = []
        for o, lsum in res:
            l = jnp.sum(jnp.maximum(lsum, gate), axis=-1, keepdims=True)
            r = pl.reciprocal(l, approx=True)
            r = r * (2.0 - l * r)
            outs.append(o * r)
        return outs

    def woproj(slot, g, first, c, outs, lo, hi, dep=None):
        oc = jnp.concatenate([tie(outs[0], dep)] + outs[1:], axis=-1).astype(BF16)
        y = jnp.dot(oc, wobuf[g, :, lo:hi], preferred_element_type=F32)
        rows = slice(c * TQ, (c + 1) * TQ)
        if first is True:
            acc[slot, rows, lo:hi] = y
        else:
            acc[slot, rows, lo:hi] = jnp.where(first, 0.0, acc[slot, rows, lo:hi]) + y
        return y

    def ln1_piece(i, g, u, gate=None):
        pr = LNR // NP1
        if isinstance(i, int) and isinstance(g, int):
            row0, off = (i + 1) * BQ + g * LNR + u * pr, g * LNR + u * pr
        else:
            row0 = pl.multiple_of(jnp.minimum((i + 1) * BQ + g * LNR, S - LNR) + u * pr, pr)
            off = pl.multiple_of(g * LNR + u * pr, pr)
        xv = xbuf[pl.ds(row0, pr), :].astype(F32)
        if gate is not None:
            xv = jnp.concatenate([tie(xv[:, 0:128], gate[0:pr, 0:128]), xv[:, 128:]], axis=-1)
        hv = ln1_apply(_normalize(xv), pr)
        hnext[pl.ds(off, pr), :] = hv.astype(BF16)
        return hv[:, 0:128]

    def ln2_piece(i, g, u, st):
        pr = LNR // NP2
        for k in range(pr // LRW):
            off = pl.multiple_of(g * LNR + u * pr + k * LRW, LRW)
            row0 = pl.multiple_of(jnp.maximum(i - 1, 0) * BQ + off, LRW)
            st = ln2(acc[(i + 1) & 1, pl.ds(off, LRW), 0:DM], row0, LRW, i > 0, st)
        return st

    def wo_tail(g, slot, first, o0, o1, work):
        pieces = [(0, o0, lo) for lo in range(WB, DM, WT)] + [(1, o1, lo) for lo in range(0, DM, WT)]
        deps = {}
        for n, (c, o, lo) in enumerate(pieces):
            y = woproj(slot, g, first, c, o, lo, lo + WT, deps.get(n))
            if n in work:
                deps[n + WLAG] = work[n](y)

    chains = [(c, h) for c in range(2) for h in range(NH)]

    def attention_step(i, g, g1, slot, first):
        st = load_top()
        pv_dep = {}
        for u, at in enumerate(LN2_AT):
            st = ln2_piece(i, g, u, st)
            pv_dep[at] = st[1]
        for u, at in enumerate(LN1_AT):
            pv_dep[at] = ln1_piece(i, g, u)
        q = qproj(g, 0, 0)
        res = ([], [])
        o0 = None
        for n, (c, h) in enumerate(chains):
            s = qk(q, g, h)
            if n + 1 < len(chains):
                q = qproj((g, g1)[chains[n + 1][0]], *chains[n + 1])
            if (c, h) == (1, 0):
                o0 = normalize_heads(res[0])
                woproj(slot, g, first, 0, o0, 0, WA)
            if (c, h) == (1, NH - 1):
                woproj(slot, g, first, 0, o0, WA, WB)
            res[c].append(pv(s, g, h, pv_dep.get((c, h))))
        wo_tail(g, slot, first, o0, normalize_heads(res[1]), {})
        store_top(st)

    c_cp.wait()
    x_cp[0].wait()
    sc = silu_c()
    scbuf[...] = sc
    acc[0, :, 0:DM] = _normalize(xbuf[0:BQ, :].astype(F32))
    for n in range(len(MODC) - 1):
        lo, hi = MODC[n], MODC[n + 1]
        if n == 0:
            wqe_cp.wait()
        for d in mod_cp[n]:
            d.wait()
        mod_cols(sc, lo, hi)
        mod_cols(sc, DM + lo, DM + hi, True)
        hn[:, lo:hi] = ln1_apply(acc[0, :, lo:hi], BQ, lo, hi).astype(BF16)
        for c in range(2):
            rows = slice(c * TQ, (c + 1) * TQ)
            part = jnp.dot(hn[rows, lo:hi], wqbuf[0, lo:hi, 0:2 * DH], preferred_element_type=F32)
            if n > 0:
                part = part + nbuf[rows, 0:2 * DH]
            if hi < DM:
                nbuf[rows, 0:2 * DH] = part
            else:
                hnext[rows, 0:2 * DH] = (part * QSCALE).astype(BF16)

    def wait0(n):
        for d in step0_cp[n]:
            d.wait()

    def qk_pair(h):
        sa, sb = [qk(hnext[c * TQ:(c + 1) * TQ, h * DH:(h + 1) * DH], 0, h) for c in range(2)]
        return sa, jnp.max(sa, axis=-1, keepdims=True), sb

    wait0(0)
    sa, ma, s = qk_pair(0)
    wait0(1)
    res = ([pv(sa, 0, 0, None, ma)], [pv(s, 0, 0)])
    sa, ma, s = qk_pair(1)
    wait0(2)
    res[0].append(pv(sa, 0, 1, None, ma))
    for h in range(2, NH):
        if h == 3:
            wait0(3)
        q = qproj(0, 0, h)
        res[1].append(pv(s, 0, h - 1))
        s = qk(q, 0, h)
        q = qproj(0, 1, h)
        res[0].append(pv(s, 0, h))
        s = qk(q, 0, h)
    o0 = normalize_heads(res[0])
    woproj(0, 0, True, 0, o0, 0, WB)
    res[1].append(pv(s, 0, NH - 1))
    wo_tail(0, 0, True, o0, normalize_heads(res[1]),
            {u: (lambda y, u=u: ln1_piece(0, 0, u, y)) for u in range(NP1)})

    def epilogue():
        last = (NQ - 1) % 2
        nt = BQ // 128
        lane = lax.broadcasted_iota(jnp.int32, (8, 128), 1)
        sub = lax.broadcasted_iota(jnp.int32, (8, 128), 0)
        lin = None
        sq = None
        for j in range(nt):
            xs_, ps_ = [], []
            for r0 in range(j * 128, (j + 1) * 128, ERW):
                x1 = residual(acc[last, r0:r0 + ERW, 0:DM], LAST0 + r0, ERW)
                nbuf[LAST0 + r0:LAST0 + r0 + ERW, :] = x1
                x2 = x1 * x1
                part = x2[:, 0:128]
                for z in range(1, DM // 128):
                    part = part + x2[:, z * 128:(z + 1) * 128]
                hi = _rd(part)
                xs_.append(x1)
                ps_.append(jnp.concatenate([hi, part - hi], axis=-1))
            a_ = lax.dot_general(rsum[j], jnp.concatenate(xs_, axis=0).astype(BF16), NT,
                                 preferred_element_type=F32)[0:24]
            b_ = lax.dot_general(rsum[j, 0:16, 0:256], jnp.concatenate(ps_, axis=0).astype(BF16), NT,
                                 preferred_element_type=F32)[0:8]
            lin = a_ if lin is None else lin + a_
            sq = b_ if sq is None else sq + b_
        mean = lin[0:8] * (1.0 / DM)
        inv = _inv_std(jnp.maximum(sq * (1.0 / DM) - mean * mean, 0.0))
        mean = _rd(mean)
        dot = lin[8:16] + lin[16:24]
        r = (dot - mean * vec[3, :, 128:256]) * inv + vec[3, :, 0:128]
        k1, k2 = load_top()
        c1 = jnp.max(k1, axis=0, keepdims=True)
        c2 = jnp.max(jnp.where(k1 == c1, k2, k1), axis=0, keepdims=True)
        keys = jnp.where(sub < nt, _route_key(r, LAST0 + sub * 128 + lane),
                         jnp.where(lane > 0, -jnp.inf,
                                   jnp.where(sub == nt, c1, jnp.where(sub == nt + 1, c2, -jnp.inf))))
        mean_k = jnp.where(sub < nt, mean, 0.0)
        inv_k = jnp.where(sub < nt, inv, 1.0)

        def all_sum(z):
            return jnp.sum(jnp.sum(z, axis=1, keepdims=True), axis=0, keepdims=True)

        t1 = jnp.max(keys, axis=0, keepdims=True)
        t2 = jnp.max(jnp.where(keys == t1, -jnp.inf, keys), axis=0, keepdims=True)
        bit = lax.shift_right_logical(lane, sub) & 1
        half = [jnp.max(jnp.where(sub == 7, t2, jnp.where(bit == b, t1, -jnp.inf)), axis=1, keepdims=True)
                for b in range(2)]
        bests = (jnp.max(jnp.maximum(half[0], half[1]), axis=0, keepdims=True),
                 jnp.max(jnp.minimum(half[0], half[1]), axis=0, keepdims=True))

        routed = []
        for best in bests:
            hit = keys == best
            bits = lax.bitcast_convert_type(jnp.broadcast_to(best, (8, 128)), jnp.int32)
            low = bits & (S - 1)
            idx = jnp.clip(jnp.where(bits >= 0, (S - 1) - low, low)[0, 0], 0, S - 1)
            logit = lax.bitcast_convert_type(bits & -65536, F32)[0:1, 0:1]
            nrow = ((nbuf[pl.ds(idx, 1), :] - all_sum(jnp.where(hit, mean_k, 0.0)))
                    * all_sum(jnp.where(hit, inv_k, 0.0))
                    + jnp.tile(sbuf[pl.ds(idx, 1), :], (1, DM // 128)))
            routed.append((idx, logit, nrow))
        (idx1, v1, n1), (idx2, v2, n2) = routed

        row = lax.broadcasted_iota(jnp.int32, (16, DM), 0)
        xs = (_rd(_rd(jnp.where(row == 0, n1, n2)) * _rows8(mod[:, 4 * DM:5 * DM], 16))
              + _rows8(mod[:, 3 * DM:4 * DM], 16))

        cols = {}

        def row_stat(name, z, r0):
            j = r0 // 128
            if (name, j) not in cols:
                cols[name, j] = jnp.broadcast_to(z[j:j + 1, :], (128, 128)).T
            return cols[name, j][r0 - j * 128:r0 - j * 128 + ORW]

        acts = []
        ys = []

        def tied_bf16(v, dep):
            return jnp.concatenate([tie(v[:, 0:128], dep), v[:, 128:]], axis=-1).astype(BF16)

        def gate_up(n, dep):
            cols = slice(n * 128, (n + 1) * 128)
            xb = tied_bf16(xs, dep)
            gt = jnp.dot(xb, wgbuf[:, cols], preferred_element_type=F32)
            up = jnp.dot(xb, wubuf[:, cols], preferred_element_type=F32)
            acts.append(gt * jax.nn.sigmoid(gt) * up)
            return gt

        def down(n, dep):
            ab = tied_bf16(jnp.concatenate(acts[2 * n:2 * n + 2], axis=-1), dep)
            ys.append(jnp.dot(ab, wdbuf[n * 256:(n + 1) * 256, 0:DM], preferred_element_type=F32))
            return ys[-1]

        slots = []
        for n in range(FF // 128):
            slots.append((gate_up, n))
            if n % 2 == 1 and n >= DLAG:
                slots.append((down, (n - DLAG) // 2))
        slots += [(down, n) for n in range(FF // 256) if (down, n) not in slots]
        deps = {}
        for k, (fn, n) in enumerate(slots):
            gate = fn(n, deps.get(k))
            r0 = k * ORW
            if r0 < BQ:
                x1 = nbuf[LAST0 + r0:LAST0 + r0 + ORW, :]
                mu = tie(row_stat("mean", mean, r0), gate[0:ORW, 0:128])
                nv = (x1 - jnp.tile(mu, (1, DM // 128))) * jnp.tile(row_stat("inv", inv, r0), (1, DM // 128))
                deps[k + 2] = ln2_out(x1, nv, LAST0 + r0, ORW)[:, DM - 128:]
                if r0 + ORW in OUT_SPLIT:
                    last_cp[OUT_SPLIT.index(r0 + ORW) - 1].start()
        y = sum(ys[1:], ys[0])
        gb = mod[0:1, 5 * DM:6 * DM]
        y1 = y[0:1, :] * jax.nn.sigmoid(v1) * gb
        y2 = y[1:2, :] * jax.nn.sigmoid(v2) * gb

        fixes = []
        for n, idx in enumerate((idx1, idx2)):
            grp = jnp.clip(lax.shift_right_logical(idx, FIX.bit_length() - 1), 0, S // FIX - 1)
            base = pl.multiple_of(grp * FIX, FIX)
            rid = row[0:FIX] + base
            upd = jnp.where(rid == idx1, y1, jnp.where(rid == idx2, y2, 0.0))
            fixbuf[n] = (obuf[pl.ds(base, FIX), :].astype(F32) + upd).astype(BF16)
            fixes.append(cp(fixbuf.at[n], out_hbm.at[pl.ds(base, FIX)], sem.at[SEM_FIX]))

        for d in [out_cp(j) for j in range(NQ - 2)] + [early_cp] + last_cp:
            d.wait()
        for d in fixes:
            d.start()
            d.wait()

    def wait_groups(t0):
        for gg in range(t0, (GWAIT + (NG,))[GWAIT.index(t0) + 1]):
            for d in group_cps(gg):
                d.wait()
        if t0 == 2:
            x_cp[3].wait()

    def step(t, carry):
        i = lax.shift_right_logical(t, NG.bit_length() - 1)
        g = t & (NG - 1)
        attention_step(i, g, (t + NG) & (NG - 1), i & 1, g == 0)

        @pl.when(jnp.logical_or(jnp.logical_or(t < GWAIT[-1], t == NSTEP - 2), g == NG - 1))
        def _():
            pl.when(t == NSTEP - 2)(early_cp.start)
            for t0 in GWAIT[1:]:
                pl.when(t == t0 - 1)(lambda t0=t0: wait_groups(t0))

            @pl.when(g == NG - 1)
            def _():
                @pl.when(t == NG - 1)
                def _():
                    for d in [modr_cp, x_cp[2], wr_cp] + ffn_cp:
                        d.wait()
                    hn[...] = hnext[...]
                    for k in range(2, 6):
                        mod_cols(scbuf[...], k * DM, (k + 1) * DM, k == 4)
                    fold_vectors()

                @pl.when(jnp.logical_and(t > NG, t < NSTEP - 1))
                def _():
                    out_cp(i - 1).start()
                    hn[...] = hnext[...]

                pl.when(t == NSTEP - 1)(epilogue)

        return carry

    wait_groups(GWAIT[0])
    lax.fori_loop(1, NSTEP, step, 0)


@jax.jit
def pallas_adaLN_cond__mha_block_cached__moe_arch_mod__prompt_kernel(
    A_x: jax.Array,
    A_k_cache: jax.Array,
    A_v_cache: jax.Array,
    A_wq: jax.Array,
    A_wo: jax.Array,
    B_x: jax.Array,
    B_w_r: jax.Array,
    B_w_gate: jax.Array,
    B_w_up: jax.Array,
    B_w_down: jax.Array,
    c: jax.Array,
    w_mod: jax.Array,
):
    del B_x
    x = A_x.reshape(S, DM)
    k = A_k_cache.reshape(H, S, DH)
    v = A_v_cache.reshape(H, S, DH)
    wo = A_wo.reshape(NG, NH * DH, DM)
    any_spec = pl.BlockSpec(memory_space=pl.ANY)
    out = pl.pallas_call(
        _kernel,
        in_specs=[any_spec] * 11,
        out_specs=any_spec,
        out_shape=jax.ShapeDtypeStruct((S, DM), BF16),
        scratch_shapes=[
            pltpu.VMEM((S, DM), BF16),
            pltpu.VMEM((H, S, DH), BF16),
            pltpu.VMEM((H, S, DH), BF16),
            pltpu.VMEM((NG, DM, NH * DH), BF16),
            pltpu.VMEM((NG, NH * DH, DM), BF16),
            pltpu.VMEM((DM,), BF16),
            pltpu.VMEM((DM, FF), BF16),
            pltpu.VMEM((DM, FF), BF16),
            pltpu.VMEM((FF, DM + PAD), BF16),
            pltpu.VMEM((1, DM), BF16),
            pltpu.VMEM((16, DM), BF16),
            pltpu.VMEM((DM, 6 * DM + PAD), BF16),
            pltpu.VMEM((BQ, DM), BF16),
            pltpu.VMEM((BQ, DM), BF16),
            pltpu.VMEM((2, BQ, DM + PAD), F32),
            pltpu.VMEM((S, 128), F32),
            pltpu.VMEM((S, DM), F32),
            pltpu.VMEM((S, DM), BF16),
            pltpu.VMEM((2, FIX, DM), BF16),
            pltpu.VMEM((8, 6 * DM), F32),
            pltpu.VMEM((4, 8, DM), F32),
            pltpu.VMEM((BQ // 128, 32, DM), BF16),
            pltpu.VMEM((2, 8, 128), F32),
            pltpu.SMEM((1,), jnp.int32),
            pltpu.SemaphoreType.DMA((NSEM,)),
        ],
        compiler_params=pltpu.CompilerParams(vmem_limit_bytes=124 * 1024 * 1024,
                                             disable_semaphore_checks=True),
        name="adaln_mha_moe",
    )(x, k, v, A_wq, wo, B_w_r, B_w_gate, B_w_up, B_w_down, c, w_mod)
    return out.reshape(1, S, DM)
```
